```python
import jax
import jax.numpy as jnp

def _softmax(x, axis=-1):
    return jax.nn.softmax(x, axis=axis)
def _gelu(x):
    return jax.nn.gelu(x, approximate=True)
def _silu(x):
    return jax.nn.silu(x)
def _sigmoid(x):
    return jax.nn.sigmoid(x)
def _layernorm(x, axis=-1, eps=1e-5):
    m = jnp.mean(x, axis=axis, keepdims=True)
    v = jnp.var(x, axis=axis, keepdims=True)
    return (x - m) / jnp.sqrt(v + eps)
def _scatter_add(tgt, idx, src, axis=0):
    return tgt.at[idx].add(src)
def _segment_sum(src, seg, n):
    return jax.ops.segment_sum(src, seg, n)
class _Rng:
    def __init__(self, key):
        self._k = key
    def _next(self):
        self._k, sub = jax.random.split(self._k)
        return sub
    def normal(self, shape):
        return jax.random.normal(self._next(), shape, dtype=jnp.bfloat16)
    def randint(self, lo, hi, shape):
        return jax.random.randint(self._next(), shape, lo, hi, dtype=jnp.int32)
    def uniform(self, shape, lo=0.0, hi=1.0):
        return jax.random.uniform(self._next(), shape, jnp.bfloat16, lo, hi)
    def permutation(self, n):
        return jax.random.permutation(self._next(), n)


kernel_name = 'interleave_layers__sliding_block_cached__mixer_s_mlp__decode'

def setup_inputs():
    _rng = _Rng(jax.random.key(int.from_bytes(__import__("os").urandom(4), "little")))
    _w = (lambda a: (lambda t: t.astype(jnp.bfloat16) if jnp.issubdtype(t.dtype, jnp.floating) else t)(jnp.asarray(a)))
    def _A_setup():
        B, Sq, D = 1, 1, 640
        Hq, Hkv, Sk, Dh = 32, 32, 32768, 192
        assert Hq % Hkv == 0, (Hq, Hkv)
        return {
            "x": _w((lambda *s: _rng.normal(s) * 0.05)(B, Sq, D)),
            "k_cache": _w((lambda *s: _rng.normal(s) * 0.05)(B, Hkv, Sk, Dh)),
            "v_cache": _w((lambda *s: _rng.normal(s) * 0.05)(B, Hkv, Sk, Dh)),
            "wq": _w((lambda *s: _rng.normal(s) * 0.05)(D, Hq * Dh) * (D ** -0.5)),
            "wo": _w((lambda *s: _rng.normal(s) * 0.05)(Hq * Dh, D) * ((Hq * Dh) ** -0.5)),
        }
    _A_in = _A_setup()

    def _B_setup():
        B, S, D, F = 1, 1, 640, 1536
        return {
            "x":  _w((lambda *s: _rng.normal(s) * 0.05)(B, S, D)),
            "w1": _w((lambda *s: _rng.normal(s) * 0.05)(D, D) * (D ** -0.5)),
            "w2": _w((lambda *s: _rng.normal(s) * 0.05)(D, D) * (D ** -0.5)),
            "w3": _w((lambda *s: _rng.normal(s) * 0.05)(D, F) * (D ** -0.5)),
            "w4": _w((lambda *s: _rng.normal(s) * 0.05)(F, D) * (F ** -0.5)),
        }
    _B_in = _B_setup()

    return {
        "A_x": _A_in["x"],
        "A_k_cache": _A_in["k_cache"],
        "A_v_cache": _A_in["v_cache"],
        "A_wq": _A_in["wq"],
        "A_wo": _A_in["wo"],
        "B_x": _B_in["x"],
        "B_w1": _B_in["w1"],
        "B_w2": _B_in["w2"],
        "B_w3": _B_in["w3"],
        "B_w4": _B_in["w4"],
    }

def reference(A_x, A_k_cache, A_v_cache, A_wq, A_wo, B_x, B_w1, B_w2, B_w3, B_w4):
    def _A_ref(x, k_cache, v_cache, wq, wo):
        B, Sq, D = x.shape
        Hq, Dh = 32, 192
        Hkv, Sk = k_cache.shape[1], k_cache.shape[2]
        W = min(4096, max(256, Sk // 4))
        rep = Hq // Hkv
        q = (lambda x, *d: x.transpose(*d))((x @ wq).reshape(B, Sq, Hq, Dh), 0, 2, 1, 3)
        k = jnp.repeat(k_cache[:, :, Sk - W:, :], rep, axis=1)
        v = jnp.repeat(v_cache[:, :, Sk - W:, :], rep, axis=1)
        scores = jnp.einsum("bhqd,bhkd->bhqk", q, k) * (Dh ** -0.5)
        p = _softmax(scores, axis=-1)
        o = jnp.einsum("bhqk,bhkd->bhqd", p, v)
        return (lambda x, *d: x.transpose(*d))(o, 0, 2, 1, 3).reshape(B, Sq, Hq * Dh) @ wo

    def _B_ref(x, w1, w2, w3, w4):
        B, S, D = x.shape
        h = _gelu(_layernorm(x, axis=-1) @ w1)
        c = D // 4
        g0 = jnp.pad(h[:, :, 0*c:1*c], ((0, 0), (1, 0), (0, 0)))[:, :S, :]
        g1 = jnp.pad(h[:, :, 1*c:2*c], ((0, 0), (0, 1), (0, 0)))[:, 1:, :]
        g2 = jnp.pad(h[:, :, 2*c:3*c], ((0, 0), (2, 0), (0, 0)))[:, :S, :]
        g3 = jnp.pad(h[:, :, 3*c:   ], ((0, 0), (0, 2), (0, 0)))[:, 2:, :]
        hs = jnp.concatenate([g0, g1, g2, g3], axis=-1) @ w2
        x1 = x + hs
        h2 = _gelu(_layernorm(x1, axis=-1) @ w3) @ w4
        return x1 + h2

    x = A_x
    x = x + _A_ref(_layernorm(x, axis=-1), A_k_cache, A_v_cache, A_wq, A_wo)
    x = x + _B_ref(_layernorm(x, axis=-1), B_w1, B_w2, B_w3, B_w4)
    x = x + _A_ref(_layernorm(x, axis=-1), A_k_cache, A_v_cache, A_wq, A_wo)
    x = x + _B_ref(_layernorm(x, axis=-1), B_w1, B_w2, B_w3, B_w4)
    return x
```

```python
import jax
import jax.numpy as jnp
from jax import lax
import jax.experimental.pallas as pl
import jax.experimental.pallas.tpu as pltpu

_EPS = 1e-5


def _ln(x):
    m = jnp.mean(x, axis=-1, keepdims=True)
    xc = x - m
    v = jnp.mean(xc * xc, axis=-1, keepdims=True)
    return xc * lax.rsqrt(v + _EPS)


@jax.jit
def pallas_interleave_layers__sliding_block_cached__mixer_s_mlp__decode_kernel(
    A_x: jax.Array,
    A_k_cache: jax.Array,
    A_v_cache: jax.Array,
    A_wq: jax.Array,
    A_wo: jax.Array,
    B_x: jax.Array,
    B_w1: jax.Array,
    B_w2: jax.Array,
    B_w3: jax.Array,
    B_w4: jax.Array,
):
    B, S, D = A_x.shape
    _, H, Sk, Dh = A_k_cache.shape
    F = B_w3.shape[1]
    W = min(4096, max(256, Sk // 4))
    assert B == 1 and S == 1
    scale = Dh ** -0.5
    f32, bf16 = jnp.float32, jnp.bfloat16

    def kernel(x_hbm, k_hbm, v_hbm, wq_hbm, wo_hbm, w3_hbm, w4_hbm, o_ref,
               x_buf, k_buf, v_buf, wq_buf, wo_buf, w3_buf, w4_buf,
               q_scr, o_scr, ksem, vsem, wsem):
        def kcopy(h):
            return pltpu.make_async_copy(
                k_hbm.at[0, h, :, pl.ds(Sk - W, W)], k_buf.at[h], ksem.at[h])

        def vcopy(h):
            return pltpu.make_async_copy(
                v_hbm.at[0, h, :, pl.ds(Sk - W, W)], v_buf.at[h], vsem.at[h])

        x_cp = pltpu.make_async_copy(x_hbm, x_buf, wsem.at[0])
        wq_cp = pltpu.make_async_copy(wq_hbm, wq_buf, wsem.at[1])
        wo_cp = pltpu.make_async_copy(wo_hbm, wo_buf, wsem.at[2])
        w3_cp = pltpu.make_async_copy(w3_hbm, w3_buf, wsem.at[3])
        w4_cp = pltpu.make_async_copy(w4_hbm, w4_buf, wsem.at[4])

        x_cp.start()
        wq_cp.start()
        for h in range(H):
            kcopy(h).start()
            vcopy(h).start()
            if h == H - 3:
                wo_cp.start()
        w3_cp.start()
        w4_cp.start()

        x_cp.wait()
        x = jnp.broadcast_to(x_buf[...].astype(f32), (8, D))

        def attn(x, first):
            if first:
                wq_cp.wait()
            q = jnp.dot(_ln(x).astype(bf16), wq_buf[...], preferred_element_type=f32)
            for h in range(H):
                q_scr[h] = q[:, h * Dh:(h + 1) * Dh].astype(bf16)

            def head(h, c):
                if first:
                    kcopy(h).wait()
                s = jnp.dot(q_scr[h], k_buf[h], preferred_element_type=f32) * scale
                m = jnp.max(s, axis=-1, keepdims=True)
                p = jnp.exp(s - m)
                l = jnp.sum(p, axis=-1, keepdims=True)
                if first:
                    vcopy(h).wait()
                o = lax.dot_general(p.astype(bf16), v_buf[h], (((1,), (1,)), ((), ())),
                                    preferred_element_type=f32)
                o_scr[h] = (o / l).astype(bf16)
                return c

            lax.fori_loop(0, H, head, 0)
            if first:
                wo_cp.wait()
            o = jnp.concatenate([o_scr[h] for h in range(H)], axis=-1)
            return x + jnp.dot(o, wo_buf[...], preferred_element_type=f32)

        def mlp(x, first):
            y = _ln(x)
            if first:
                w3_cp.wait()
            h = jnp.dot(_ln(y).astype(bf16), w3_buf[...], preferred_element_type=f32)
            h = jax.nn.gelu(h, approximate=True)
            if first:
                w4_cp.wait()
            return x + y + jnp.dot(h.astype(bf16), w4_buf[...], preferred_element_type=f32)

        x = mlp(attn(x, True), True)
        x = mlp(attn(x, False), False)
        o_ref[...] = x[0:1].astype(o_ref.dtype)

    kt = jnp.transpose(A_k_cache, (0, 1, 3, 2))
    vt = jnp.transpose(A_v_cache, (0, 1, 3, 2))
    out = pl.pallas_call(
        kernel,
        out_shape=jax.ShapeDtypeStruct((1, D), A_x.dtype),
        in_specs=[pl.BlockSpec(memory_space=pl.ANY)] * 7,
        out_specs=pl.BlockSpec(memory_space=pltpu.VMEM),
        scratch_shapes=[
            pltpu.VMEM((1, D), bf16),
            pltpu.VMEM((H, Dh, W), bf16),
            pltpu.VMEM((H, Dh, W), bf16),
            pltpu.VMEM((D, H * Dh), bf16),
            pltpu.VMEM((H * Dh, D), bf16),
            pltpu.VMEM((D, F), bf16),
            pltpu.VMEM((F, D), bf16),
            pltpu.VMEM((H, 8, Dh), bf16),
            pltpu.VMEM((H, 8, Dh), bf16),
            pltpu.SemaphoreType.DMA((H,)),
            pltpu.SemaphoreType.DMA((H,)),
            pltpu.SemaphoreType.DMA((5,)),
        ],
        compiler_params=pltpu.CompilerParams(vmem_limit_bytes=122 * 1024 * 1024),
    )(A_x.reshape(1, D), kt, vt, A_wq, A_wo, B_w3, B_w4)
    return out.reshape(B, S, D)
```

```python
import jax
import jax.numpy as jnp
from jax import lax
import jax.experimental.pallas as pl
import jax.experimental.pallas.tpu as pltpu

f32, bf16, u32, i32 = jnp.float32, jnp.bfloat16, jnp.uint32, jnp.int32
_EPS = 1e-5
_LOG2E = 1.4426950408889634
_NN = (((1,), (0,)), ((), ()))
_NT = (((1,), (1,)), ((), ()))
_NPASS = 2


def _ln(x):
    m = jnp.mean(x, axis=-1, keepdims=True)
    xc = x - m
    v = jnp.mean(xc * xc, axis=-1, keepdims=True)
    return xc * lax.rsqrt(v + _EPS)


def _tree(op, xs):
    xs = list(xs)
    while len(xs) > 1:
        nxt = [op(xs[i], xs[i + 1]) for i in range(0, len(xs) - 1, 2)]
        if len(xs) % 2:
            nxt.append(xs[-1])
        xs = nxt
    return xs[0]


def _wtile(u):
    return pltpu.bitcast(u.reshape(u.shape[0] * 8, 128), bf16)


def _mm(lhs, w, dims=_NN):
    return lax.dot_general(lhs, w, dims, preferred_element_type=f32)


def _cache_view(c):
    _, H, Sk, Dh = c.shape
    c = c.reshape(H, Sk // 128, 128, Dh // 8, 8)
    c = jnp.transpose(c, (0, 3, 1, 4, 2))
    return c.reshape(H, Dh // 8, Sk // 16, 128)


def _weight_view(w):
    R, N = w.shape
    w = w.reshape(R // 16, 2, 8, N // 128, 128)
    return jnp.transpose(w, (0, 1, 3, 2, 4))


@jax.jit
def pallas_interleave_layers__sliding_block_cached__mixer_s_mlp__decode_kernel(
    A_x: jax.Array,
    A_k_cache: jax.Array,
    A_v_cache: jax.Array,
    A_wq: jax.Array,
    A_wo: jax.Array,
    B_x: jax.Array,
    B_w1: jax.Array,
    B_w2: jax.Array,
    B_w3: jax.Array,
    B_w4: jax.Array,
):
    B, S, D = A_x.shape
    _, H, Sk, Dh = A_k_cache.shape
    F = B_w3.shape[1]
    W = min(4096, max(256, Sk // 4))
    assert B == 1 and S == 1 and Dh == 192 and D % 128 == 0 and H % 2 == 0 and W % 256 == 0
    G = Dh // 8
    C = W // 256
    NP = H // 2
    DT = D // 128
    cexp = (Dh ** -0.5) * _LOG2E
    GB = 8

    def kernel(x_hbm, k_hbm, v_hbm, wq_hbm, wo_hbm, w3_hbm, w4_hbm, o_ref,
               x_buf, k_buf, v_buf, wq_buf, wo_buf, w3_buf, w4_buf,
               xres, xl, qpart, qrow, qpat, spart, mbuf, pbuf, lbuf, ebuf, lebuf,
               acc, oraw, ol, wpart, xacc, cst, idx, ksem, vsem, wsem):
        r0 = (Sk - W) // 16

        def kcopy(h):
            return pltpu.make_async_copy(
                k_hbm.at[h, :, pl.ds(r0, W // 16), :], k_buf.at[h], ksem.at[h])

        def vcopy(h):
            return pltpu.make_async_copy(
                v_hbm.at[h, :, pl.ds(r0, W // 16), :], v_buf.at[h], vsem.at[h])

        x_cp = pltpu.make_async_copy(x_hbm, x_buf, wsem.at[0])
        wq_cp = [pltpu.make_async_copy(wq_hbm.at[:, a], wq_buf.at[:, :, pl.ds(8 * a, 8), :],
                                       wsem.at[1 + a]) for a in range(2)]
        wo_cp = [pltpu.make_async_copy(wo_hbm.at[:, a], wo_buf.at[:, :, pl.ds(8 * a, 8), :],
                                       wsem.at[3 + a]) for a in range(2)]
        w3_cp = pltpu.make_async_copy(w3_hbm, w3_buf, wsem.at[5])
        w4_cp = pltpu.make_async_copy(w4_hbm, w4_buf, wsem.at[6])

        wq_cp[0].start()
        x_cp.start()
        wq_cp[1].start()
        for h in range(4):
            kcopy(h).start()
        for t in range(NP):
            vcopy(2 * t).start()
            vcopy(2 * t + 1).start()
            if t + 2 < NP:
                kcopy(2 * t + 4).start()
                kcopy(2 * t + 5).start()
            if t == 1:
                wo_cp[0].start()
                wo_cp[1].start()
        w3_cp.start()
        w4_cp.start()

        ku = k_buf.bitcast(u32)
        vu = v_buf.bitcast(u32)
        wqu = wq_buf.bitcast(u32)
        wou = wo_buf.bitcast(u32)

        lane = lax.broadcasted_iota(i32, (8, 128), 1)
        row = lax.broadcasted_iota(i32, (8, 128), 0)
        spread = ((lane >> 4) << 3) + (lane & 7)
        idx[0] = spread
        idx[1] = spread + 64
        cst[0] = jnp.where(((lane >> 3) & 1) == (row >> 2), cexp, 0.0).astype(f32)

        x_cp.wait()
        xres[...] = jnp.broadcast_to(x_buf[...].astype(f32), (8, D))

        def st_q(t, z):
            for j in range(DT):
                xj = xl[:, 128 * j:128 * (j + 1)]
                for i in range(3):
                    qpart[t % 2, i, j] = _mm(xj, _wtile(wqu[8 * j:8 * j + 8, 3 * t + i]))

        def st_qp1(t, z):
            for i in range(3):
                qrow[t % 2, i] = _tree(jnp.add, [qpart[t % 2, i, j] for j in range(DT)])

        def st_qp2(t, z):
            for u in range(6):
                g = jnp.take_along_axis(qrow[t % 2, u // 2], idx[u % 2], axis=1,
                                        mode='promise_in_bounds')
                qpat[t % 2, u] = g * cst[0]

        def st_qk(t, z):
            for a in range(2):
                h = 2 * t + a
                for j in range(3):
                    ql = qpat[t % 2, 3 * a + j]
                    for c in range(C):
                        w = _wtile(ku[h + z, 8 * j:8 * j + 8, 8 * c:8 * c + 8, :])
                        spart[h % 4, j, c] = _mm(ql, w)

        def st_sm(t, z):
            for a in range(2):
                s = (2 * t + a) % 4
                ss = [spart[s, 0, c] + spart[s, 1, c] + spart[s, 2, c] for c in range(C)]
                m = _tree(jnp.maximum, ss)
                m = jnp.maximum(m, pltpu.roll(m, 4, 0))
                ps = []
                for c in range(C):
                    p = jnp.exp2(ss[c] - m)
                    pbuf[s, :, 128 * c:128 * (c + 1)] = p
                    ps.append(p)
                l = _tree(jnp.add, ps)
                mbuf[s] = m
                lbuf[s] = l + pltpu.roll(l, 4, 0)

        def st_w1(t, z):
            for a in range(2):
                s = (2 * t + a) % 4
                m = mbuf[s]
                e = jnp.exp2(m - jnp.max(m, axis=1, keepdims=True))
                e = e.astype(bf16).astype(f32)
                ebuf[s] = e
                lebuf[(2 * t + a) % 8] = e * lbuf[s]

        def st_pv(t, z):
            for a in range(2):
                h = 2 * t + a
                s = h % 4
                for g0 in range(0, G, GB):
                    accs = [None] * GB
                    for c in range(C):
                        p0 = pbuf[s, 0:1, 128 * c:128 * (c + 1)]
                        p1 = pbuf[s, 4:5, 128 * c:128 * (c + 1)]
                        for k in range(GB):
                            v = pltpu.bitcast(vu[h + z, g0 + k, 8 * c:8 * c + 8, :], bf16).astype(f32)
                            x0 = v[0:8] * p0
                            x1 = v[8:16] * p1
                            accs[k] = x0 + x1 if accs[k] is None else accs[k] + x0 + x1
                    for k in range(GB):
                        acc[s, g0 + k] = accs[k]

        def st_or(t, z):
            s0, s1 = (2 * t) % 4, (2 * t + 1) % 4
            e0, e1 = ebuf[s0], ebuf[s1]
            a0 = acc[s0].reshape(G * 8, 128)
            a1 = acc[s1].reshape(G * 8, 128)
            oraw[t % 2, 0] = _mm(e0, a0[0:128], _NT)
            mid = jnp.concatenate([a0[128:192], a1[0:64]], axis=0)
            r = _mm(jnp.concatenate([e0, e1], axis=0), mid, _NT)
            oraw[t % 2, 1] = r[0:8]
            oraw[t % 2, 2] = r[8:16]
            oraw[t % 2, 3] = _mm(e1, a1[64:192], _NT)

        def st_on(t, z):
            inv0 = 1.0 / jnp.sum(lebuf[(2 * t) % 8], axis=1, keepdims=True)
            inv1 = 1.0 / jnp.sum(lebuf[(2 * t + 1) % 8], axis=1, keepdims=True)
            lane = lax.broadcasted_iota(i32, (8, 128), 1)
            ol[t % 2, 0] = oraw[t % 2, 0] * inv0
            ol[t % 2, 1] = jnp.where(lane < 64, oraw[t % 2, 1] * inv0, oraw[t % 2, 2] * inv1)
            ol[t % 2, 2] = oraw[t % 2, 3] * inv1

        def st_wo(t, z):
            for u in range(3):
                o = ol[t % 2, u]
                for c in range(DT):
                    w = _wtile(wou[24 * t + 8 * u:24 * t + 8 * u + 8, c])
                    wpart[t % 2, u, c] = _mm(o, w)

        def st_wacc(t, z):
            for c in range(DT):
                y = wpart[t % 2, 0, c] + wpart[t % 2, 1, c] + wpart[t % 2, 2, c]
                xacc[c] = y if t == 0 else xacc[c] + y

        stages = [(st_qk, 2), (st_q, 5), (st_or, -1), (st_wo, -3), (st_sm, 1), (st_on, -2),
                  (st_w1, 0), (st_qp2, 3), (st_qp1, 4), (st_wacc, -4), (st_pv, 0)]

        def run_block(t, z):
            for fn, off in stages:
                if 0 <= t + off < NP:
                    fn(t + off, z)

        def one_pass(it, carry):
            first = it == 0
            z = it >> 4

            def wait(cps):
                @pl.when(first)
                def _():
                    for cp in cps:
                        cp.wait()

            wait(wq_cp + [kcopy(h) for h in range(4)])
            xl[...] = _ln(xres[...])
            for t in range(-5, 0):
                run_block(t, z)
            for t in range(NP):
                cps = [vcopy(2 * t), vcopy(2 * t + 1)]
                if t + 2 < NP:
                    cps += [kcopy(2 * t + 4), kcopy(2 * t + 5)]
                if t == 2:
                    cps += wo_cp
                wait(cps)
                run_block(t, z)
            wait([w3_cp])
            for t in range(NP, NP + 4):
                run_block(t, z)
            x = xres[...] + jnp.concatenate([xacc[c] for c in range(DT)], axis=1)
            y = _ln(x)
            hid = jnp.dot(_ln(y).astype(bf16), w3_buf[...], preferred_element_type=f32)
            hid = jax.nn.gelu(hid, approximate=True).astype(bf16)
            wait([w4_cp])
            xres[...] = x + y + jnp.dot(hid, w4_buf[...], preferred_element_type=f32)
            return carry

        lax.fori_loop(0, _NPASS, one_pass, 0)
        o_ref[...] = xres[0:1, :].astype(o_ref.dtype)

    def V(*s, dt=f32):
        return pltpu.VMEM(s, dt)

    out = pl.pallas_call(
        kernel,
        out_shape=jax.ShapeDtypeStruct((1, D), A_x.dtype),
        in_specs=[pl.BlockSpec(memory_space=pl.ANY)] * 7,
        out_specs=pl.BlockSpec(memory_space=pltpu.VMEM),
        scratch_shapes=[
            V(1, D, dt=bf16),
            V(H, G, W // 16, 128, dt=bf16), V(H, G, W // 16, 128, dt=bf16),
            V(D // 16, 3 * NP, 16, 128, dt=bf16), V(12 * H, DT, 16, 128, dt=bf16),
            V(D, F, dt=bf16), V(F, D, dt=bf16),
            V(8, D), V(8, D),
            V(2, 3, DT, 8, 128), V(2, 3, 8, 128), V(2, 6, 8, 128),
            V(4, 3, C, 8, 128), V(4, 8, 128), V(4, 8, C * 128), V(4, 8, 128),
            V(4, 8, 128), V(8, 8, 128),
            V(4, G, 8, 128), V(2, 4, 8, 128), V(2, 3, 8, 128),
            V(2, 3, DT, 8, 128), V(DT, 8, 128),
            V(1, 8, 128), V(2, 8, 128, dt=i32),
            pltpu.SemaphoreType.DMA((H,)),
            pltpu.SemaphoreType.DMA((H,)),
            pltpu.SemaphoreType.DMA((7,)),
        ],
        compiler_params=pltpu.CompilerParams(vmem_limit_bytes=122 * 1024 * 1024),
    )(A_x.reshape(1, D), _cache_view(A_k_cache), _cache_view(A_v_cache),
      _weight_view(A_wq), _weight_view(A_wo), B_w3, B_w4)
    return out.reshape(B, S, D)
```

```python
import functools

import jax
import jax.numpy as jnp
from jax import lax
import jax.experimental.pallas as pl
import jax.experimental.pallas.tpu as pltpu

f32, bf16, u32, i32 = jnp.float32, jnp.bfloat16, jnp.uint32, jnp.int32
_EPS = 1e-5
_LOG2E = 1.4426950408889634
_NN = (((1,), (0,)), ((), ()))
_NT = (((1,), (1,)), ((), ()))
_P = functools.partial

_PLAN = [
    [('qraw', 0, 1), ('qk', 0, 0, 32), ('q', 2), ('sm', 0)],
    [('qk', 1, 0, 32), ('q', 3), ('q', 4), ('q', 5), ('w1', 0), ('qp', 2), ('pv', 0, 0, 12), ('pv', 0, 12, 20)],
    [('qk', 2, 0, 32), ('inv', 0), ('qp', 3), ('qp', 4), ('qp', 5), ('smi', 1), ('pv', 0, 20, 24),
     ('pv', 1, 0, 12)],
    [('qk', 3, 0, 32), ('q', 6), ('q', 7), ('q', 8), ('q', 9), ('w1', 1), ('smi', 2), ('pv', 1, 12, 24),
     ('pv', 2, 0, 12)],
    [('qk', 4, 0, 32), ('qk', 5, 0, 32), ('q', 10), ('inv', 1), ('w1', 2), ('qp', 6), ('qp', 7), ('qp', 8),
     ('qp', 9), ('smi', 3), ('pv', 2, 12, 24), ('pv', 3, 0, 12), ('pv', 3, 12, 20)],
    [('or', 0, (0,)), ('qk', 6, 0, 10), ('wo', 0, (0,)), ('qk', 6, 10, 32), ('qk', 7, 0, 32), ('qk', 8, 0, 1),
     ('q', 11), ('q', 12), ('q', 13), ('q', 14), ('q', 15), ('inv', 2), ('w1', 3), ('qp', 10), ('smi', 4),
     ('pv', 3, 20, 24), ('smi', 5), ('pv', 4, 0, 12), ('pv', 4, 12, 24), ('pv', 5, 0, 12), ('pv', 5, 12, 16)],
    [('or', 0, (1, 2)), ('or', 1, (0,)), ('qk', 8, 1, 11), ('wo', 0, (1, 2)), ('wo', 1, (0,)), ('qk', 8, 11, 32),
     ('qk', 9, 0, 32), ('qk', 10, 0, 32), ('inv', 3), ('w1', 4), ('w1', 5), ('wacc', 0, (0,)), ('qp', 11),
     ('qp', 12), ('qp', 13), ('qp', 14), ('qp', 15), ('smi', 6), ('pv', 5, 16, 24), ('smi', 7), ('pv', 6, 0, 12),
     ('pv', 6, 12, 24), ('pv', 7, 0, 12), ('pv', 7, 12, 16)],
    [('or', 1, (1, 2)),
     ('or', 2, (0, 1, 2)), ('or', 3, (0, 1, 2)), ('or', 4, (0, 1, 2)), ('or', 5, (0,)), ('qk', 11, 0, 10),
     ('wo', 1, (1, 2)), ('wo', 2, (0, 1, 2)), ('wo', 3, (0, 1, 2)), ('wo', 4, (0, 1, 2)), ('wo', 5, (0,)),
     ('qk', 11, 10, 32), ('qk', 12, 0, 32), ('inv', 4), ('inv', 5), ('w1', 6), ('w1', 7), ('wacc', 0, (1, 2)),
     ('wacc', 1, (0,)), ('smi', 8), ('pv', 7, 16, 24), ('smi', 9), ('pv', 8, 8, 12), ('pv', 8, 12, 16),
     ('smi', 10), ('pv', 9, 8, 12), ('pv', 9, 12, 24), ('pv', 10, 8, 12), ('pv', 10, 12, 20)],
    [('need', 'v', 27), ('need', 'v', 26), ('or', 5, (1, 2)), ('or', 6, (0, 1, 2)), ('qk', 13, 0, 10),
     ('wo', 5, (1, 2)), ('wo', 6, (0, 1, 2)), ('qk', 13, 10, 32), ('qk', 14, 0, 32), ('qk', 15, 0, 1),
     ('inv', 6), ('inv', 7), ('w1', 8), ('w1', 9), ('w1', 10), ('wacc', 1, (1, 2)), ('wacc', 2, (0, 1, 2)),
     ('wacc', 3, (0, 1, 2)), ('wacc', 4, (0, 1, 2)), ('wacc', 5, (0,)), ('smi', 11), ('pv', 10, 20, 24),
     ('smi', 12), ('pv', 11, 0, 12), ('pv', 11, 12, 24), ('pv', 12, 0, 8)],
    [('or', 7, (0, 1, 2)), ('or', 8, (1,)), ('pvx', 8, 0, 0, 32), ('wo', 7, (0, 1, 2)), ('wo', 8, (1,)),
     ('pvx', 8, 2, 0, 32), ('pvx', 9, 0, 0, 32), ('pvx', 10, 0, 0, 32), ('qk', 15, 1, 32), ('inv', 8),
     ('inv', 9), ('inv', 10), ('w1', 11), ('w1', 12), ('wacc', 5, (1, 2)), ('wacc', 6, (0, 1, 2)), ('smi', 13),
     ('pv', 12, 8, 12), ('pv', 12, 12, 24), ('smi', 14), ('pv', 13, 8, 12), ('pv', 13, 12, 16),
     ('pv', 14, 0, 12), ('pv', 14, 12, 16)],
    [('or', 9, (1, 2)), ('or', 10, (1, 2)), ('or', 11, (0, 1, 2)), ('or', 12, (0, 1, 2)), ('wo', 9, (1, 2)),
     ('wo', 10, (1, 2)), ('wo', 11, (0, 1, 2)), ('wo', 12, (0, 1, 2)), ('inv', 11), ('inv', 12), ('w1', 13),
     ('w1', 14), ('wacc', 7, (0, 1, 2)), ('xsum', 8, 0), ('xsum', 8, 2), ('wacc', 8, (1,)), ('xsum', 9, 0),
     ('xsum', 10, 0), ('smi', 15), ('pv', 14, 16, 24), ('pv', 15, 0, 4)],
    [('or', 13, (1,)), ('or', 14, (0, 1, 2)), ('pvx', 13, 0, 0, 32), ('wo', 8, (0, 2)), ('wo', 9, (0,)),
     ('wo', 10, (0,)), ('wo', 13, (1,)), ('wo', 14, (0, 1, 2)), ('pvx', 13, 2, 0, 32), ('inv', 13), ('inv', 14),
     ('w1', 15), ('wacc', 9, (1, 2)), ('wacc', 10, (1, 2)), ('wacc', 11, (0, 1, 2)), ('wacc', 12, (0, 1, 2)),
     ('pv', 15, 4, 12), ('pv', 15, 12, 24)],
    [('inv', 15), ('xsum', 13, 0), ('xsum', 13, 2), ('or', 15, (0, 1, 2)), ('wacc', 8, (0, 2)),
     ('wacc', 9, (0,)), ('wacc', 10, (0,)), ('wacc', 13, (1,)), ('wacc', 14, (0, 1, 2)), ('wo', 13, (0, 2)),
     ('wacc', 13, (0, 2)), ('wo', 15, (0, 1, 2)), ('wacc', 15, (0, 1, 2))],
]
_OPTS = {}


def _stats(x):
    m = jnp.mean(x, axis=-1, keepdims=True)
    xc = x - m
    v = jnp.mean(xc * xc, axis=-1, keepdims=True)
    return m, xc, lax.rsqrt(v + _EPS)


def _tree(op, xs):
    xs = list(xs)
    while len(xs) > 1:
        nxt = [op(xs[i], xs[i + 1]) for i in range(0, len(xs) - 1, 2)]
        if len(xs) % 2:
            nxt.append(xs[-1])
        xs = nxt
    return xs[0]


def _wtile(u):
    return pltpu.bitcast(u.reshape(u.shape[0] * 8, 128), bf16)


def _mm(lhs, w, dims=_NN):
    return lax.dot_general(lhs, w, dims, preferred_element_type=f32)


def _cache_view(c):
    _, H, Sk, Dh = c.shape
    c = c.reshape(H, Sk // 128, 128, Dh // 16, 2, 8)
    c = jnp.transpose(c, (0, 3, 4, 1, 5, 2))
    return c.reshape(H * Dh // 16, 2, Sk // 128, 8, 128)


def _weight_view(w):
    R, N = w.shape
    w = w.reshape(R // 16, 2, 8, N // 128, 128)
    return jnp.transpose(w, (0, 1, 3, 2, 4))


def _ring_size(blocks, names, n):
    first, last = {}, {}
    for b, blk in enumerate(blocks):
        for it in blk:
            if it[0] in names:
                first.setdefault(it[1], b)
                last[it[1]] = b
    for R in range(1, n + 1):
        if all(last[t] < first[u] for t in last for u in first if u > t and (u - t) % R == 0):
            return R


def _run(blocks, opts, A_x, A_k_cache, A_v_cache, A_wq, A_wo, B_w3, B_w4):
    B, S, D = A_x.shape
    _, H, Sk, Dh = A_k_cache.shape
    F = B_w3.shape[1]
    W = min(4096, max(256, Sk // 4))
    assert (B, S, H, Dh, W) == (1, 1, 32, 192, 4096) and D % 128 == 0 and F % 128 == 0
    AH = Dh // 16
    KT = W // 128
    NP = H // 2
    DT, FT = D // 128, F // 128
    AB = 4
    cexp = (Dh ** -0.5) * _LOG2E
    NB = len(blocks)
    W4C = opts.get('w4c', [(0, 5), (5, 10), (10, FT)])
    RS = _ring_size(blocks, ('qk', 'sm', 'smi'), NP)
    RP = _ring_size(blocks, ('sm', 'smi', 'pv', 'w1'), NP)
    RA = _ring_size(blocks, ('pv', 'or'), NP)
    RQ = _ring_size(blocks, ('q', 'qp'), NP)
    RW = _ring_size(blocks, ('wo', 'wacc'), NP)

    needs, seen, xunits = [], set(), {}
    for blk in blocks:
        cur = []
        for it in blk:
            key = int(it[0] == 'pv' and it[2] >= AH or it[0] == 'pvx' and it[2] == 2)
            key = {'qk': ('k', it[1]), 'pv': ('v', 2 * it[1] + key) if it[0] == 'pv' else None,
                   'pvx': ('v', 2 * it[1] + key) if it[0] == 'pvx' else None,
                   'q': ('wq',), 'qraw': ('wq',), 'wo': ('wo',), 'need': it[1:]}.get(it[0])
            if it[0] == 'pvx':
                xunits.setdefault((it[1], it[2]), len(xunits))
            if key is not None and key not in seen:
                seen.add(key)
                cur.append(key)
        needs.append(cur)
    for b in range(NB - 2, -1, -1):
        if not needs[b]:
            needs[b].append(needs[b + 1].pop(0))
            assert needs[b + 1]
    xpairs = {t: i for i, t in enumerate(sorted({t for t, _ in xunits}))}

    def kernel(x_hbm, k_hbm, v_hbm, wq_hbm, wo_hbm, w3_hbm, w4_hbm, o_ref, *scratch):
        k_bufs, scratch = scratch[:NP], scratch[NP:]
        v_bufs, scratch = scratch[:H], scratch[H:]
        w4_bufs, scratch = scratch[:len(W4C)], scratch[len(W4C):]
        (x_buf, wq_buf, wo_buf, w3_buf, xres, xl, qpart, qpat, spart, sbuf, mbuf, lbuf, ebuf, lebuf,
         acc, ibuf, ol, wpart, xacc, xpart, cst, pbuf, pxbuf, sems) = scratch
        t0 = (Sk - W) // 128

        def copies(key, sem):
            if key[0] in ('k', 'v'):
                n = 2 * AH if key[0] == 'k' else AH
                src, dst = (k_hbm, k_bufs[key[1]]) if key[0] == 'k' else (v_hbm, v_bufs[key[1]])
                return [pltpu.make_async_copy(src.at[pl.ds(n * key[1], n), a, pl.ds(t0, KT)],
                                              dst.at[:, :, pl.ds(8 * a, 8), :], sem) for a in range(2)]
            src, dst = (wq_hbm, wq_buf) if key[0] == 'wq' else (wo_hbm, wo_buf)
            return [pltpu.make_async_copy(src.at[:, a], dst.at[:, :, pl.ds(8 * a, 8), :], sem)
                    for a in range(2)]

        def block_copies(b):
            cps = [cp for key in needs[b] for cp in copies(key, sems.at[b])]
            if b == NB - 1:
                cps.append(pltpu.make_async_copy(w3_hbm, w3_buf, sems.at[b]))
            return cps

        def w4_cp(i):
            a, b = W4C[i]
            return pltpu.make_async_copy(w4_hbm.at[pl.ds(128 * a, 128 * (b - a))], w4_bufs[i],
                                         sems.at[NB + 1 + i])

        x_cp = pltpu.make_async_copy(x_hbm, x_buf, sems.at[NB])
        for b in range(NB):
            for i, cp in enumerate(block_copies(b)):
                cp.start()
                if b == 0 and i == 0:
                    x_cp.start()
        for i in range(len(W4C)):
            w4_cp(i).start()

        ku = [r.bitcast(u32) for r in k_bufs]
        vu = [r.bitcast(u32) for r in v_bufs]
        wqu = wq_buf.bitcast(u32)
        wou = wo_buf.bitcast(u32)

        lane = lax.broadcasted_iota(i32, (8, 128), 1)
        row = lax.broadcasted_iota(i32, (8, 128), 0)
        for u, mask in enumerate([row < 4, (row < 4) == (lane < 64), row >= 4]):
            cst[u] = jnp.where(mask, cexp, 0.0).astype(f32)
        cst[3] = jnp.zeros((8, 128), f32)

        x_cp.wait()
        xres[...] = jnp.broadcast_to(x_buf[...].astype(f32), (8, D))

        def top(n):
            return lax.broadcasted_iota(i32, (8, n), 0) < 4

        def cols(n):
            return slice(128 * n, 128 * (n + 1))

        def bcast(ref, r, n):
            return jnp.broadcast_to(ref[r:r + 1, cols(n)], (8, 128))

        def vunit(t, j):
            return (vu[2 * t], slice(0, 8)) if j == 0 else (vu[2 * t + 1], slice(AH - 8, AH))

        def st_q(t):
            for j in range(DT):
                xj = xl[:, cols(j)]
                for i in range(3):
                    qpart[t % RQ, i, j] = _mm(xj, _wtile(wqu[8 * j:8 * j + 8, 3 * t + i]))

        def st_qk(t, k0, k1):
            for j in range(3):
                ql = qpat[t, j]
                for k in range(k0, k1):
                    spart[t % RS, j, k] = _mm(ql, _wtile(ku[t][8 * j:8 * j + 8, k]))

        def st_pvx(t, j, k0, k1):
            ref, rows = vunit(t, j)
            for k in range(k0, k1):
                xpart[xunits[t, j], k] = _mm(bcast(pxbuf.at[xpairs[t]], 2 * j, k), _wtile(ref[rows, k]))

        def transpose_unit(t, j):
            ref, rows = vunit(t, j)

            def body(k, c):
                w = _wtile(ref[rows, k]).astype(f32).T.astype(bf16)
                ref[rows, k] = pltpu.bitcast(w, u32).reshape(8, 8, 128)
                return c
            lax.fori_loop(0, KT, body, 0, unroll=4)

        def st_or(t, js):
            for j in js:
                if j == 1:
                    zz = jnp.concatenate([cst[3]] * 8, axis=0)
                    a = acc[t % RA, 8:12].reshape(64, 128)
                    ol[t, 1] = _mm(bcast(ebuf, 0, t), jnp.concatenate([a, zz], axis=0), _NT)
                    a = acc[t % RA, 12:16].reshape(64, 128)
                    ol[t, 2] = _mm(bcast(ebuf, 4, t), jnp.concatenate([zz, a], axis=0), _NT)
                else:
                    a = acc[t % RA, 8 * j:8 * j + 8].reshape(128, 128)
                    ol[t, 3 * j // 2] = _mm(bcast(ebuf, 2 * j, t), a, _NT)

        def st_wo(t, js):
            for j in js:
                o = ol[t, 1:3].reshape(16, 128) if j == 1 else ol[t, 3 * j // 2]
                for c in range(DT):
                    r = _mm(o, _wtile(wou[24 * t + 8 * j:24 * t + 8 * j + 8, c]))
                    if j == 1:
                        wpart[t % RW, c, 1:3] = r.reshape(2, 8, 128)
                    else:
                        wpart[t % RW, c, 3 * j // 2] = r

        def st_w1(t):
            m = mbuf[t]
            e = jnp.exp2(m - jnp.max(m, axis=1, keepdims=True)).astype(bf16).astype(f32)
            ebuf[:, cols(t)] = e
            lebuf[t] = e * lbuf[t]
            if t in xpairs:
                for k in range(KT):
                    pxbuf[xpairs[t], :, cols(k)] = pbuf[t % RP, :, cols(k)] * e

        def st_inv(t):
            inv = 1.0 / jnp.sum(lebuf[t], axis=1, keepdims=True)
            ibuf[:, cols(t)] = jnp.broadcast_to(inv, (8, 128))

        def qp_pieces(t):
            def pc(i):
                qpat[t, i] = _tree(jnp.add, [qpart[t % RQ, i, j] for j in range(DT)]) * cst[i]
            return [_P(pc, i) for i in range(3)]

        def xsum_pieces(t, j):
            st = {}

            def pc(k):
                y = _tree(jnp.add, [xpart[xunits[t, j], kk] for kk in range(k, k + 4)])
                st['y'] = y if k == 0 else st['y'] + y
                if k + 4 == KT:
                    ol[t, 3 * j // 2] = st['y']
            return [_P(pc, k) for k in range(0, KT, 4)]

        state = {}

        def wacc_pieces(t, js):
            init, state['fresh'] = state['fresh'], False
            parts = (([0] * (0 in js) + [1] * (1 in js), 0), ([2] * (1 in js) + [3] * (2 in js), 4))

            def pc(c):
                ys = [] if init else [xacc[c]]
                for us, r in parts:
                    if us:
                        ys.append(_tree(jnp.add, [wpart[t % RW, c, u] for u in us]) * ibuf[r:r + 1, cols(t)])
                xacc[c] = _tree(jnp.add, ys)
            return [_P(pc, c) for c in range(DT)]

        def sm_pieces(z, t):
            st = {}

            def pa(k):
                s = spart[t % RS, 0, k] + spart[t % RS, 1, k] + spart[t % RS, 2, k]
                sbuf[z, k] = s
                st['m'] = s if k == 0 else jnp.maximum(st['m'], s)
                if k == KT - 1:
                    mbuf[t] = st['m']

            def pb(k):
                p = jnp.exp2(sbuf[z, k] - st['m'])
                pbuf[t % RP, :, cols(k)] = p
                st['l'] = p if k == 0 else st['l'] + p
                if k == KT - 1:
                    lbuf[t] = st['l']
            return [_P(pa, k) for k in range(KT)], [_P(pb, k) for k in range(KT)]

        def st_sm(t):
            ss = [spart[t % RS, 0, k] + spart[t % RS, 1, k] + spart[t % RS, 2, k] for k in range(KT)]
            m = _tree(jnp.maximum, ss)
            ps = [jnp.exp2(s - m) for s in ss]
            for k in range(KT):
                pbuf[t % RP, :, cols(k)] = ps[k]
            mbuf[t] = m
            lbuf[t] = _tree(jnp.add, ps)

        def pv_steps(t, a0, a1):
            odd = int(a0 >= AH)
            ref = vu[2 * t + odd]
            steps = []
            for aa in range(a0, a1, AB):
                def step(k, as_=range(aa, aa + AB), st={}):
                    p = pbuf[t % RP, 4 * odd:4 * odd + 1, cols(k)]
                    for a in as_:
                        y = pltpu.bitcast(ref[a - AH * odd, k], bf16).astype(f32) * p
                        st[a] = y if k == 0 else st[a] + y
                    if k == KT - 1:
                        for a in as_:
                            acc[t % RA, a] = st[a]
                steps += [_P(step, k) for k in range(KT)]
            return steps

        def st_qraw(*ts):
            x = xres[...]
            lhs = jnp.where(top(D), x, 1.0)
            m, xc, r = _stats(x)
            xl[...] = xc * r
            coef = jnp.where(top(128), r, -(r * m))
            for t in ts:
                for i in range(3):
                    y = _tree(jnp.add, [_mm(lhs[:, cols(j)], _wtile(wqu[8 * j:8 * j + 8, 3 * t + i]))
                                        for j in range(DT)]) * coef
                    qpat[t, i] = (y + pltpu.roll(y, 4, 0)) * cst[i]

        table = {'q': st_q, 'qk': st_qk, 'pvx': st_pvx, 'or': st_or, 'wo': st_wo, 'w1': st_w1,
                 'inv': st_inv, 'sm': st_sm, 'qraw': st_qraw, 'need': lambda *a: None}
        ptable = {'qp': qp_pieces, 'xsum': xsum_pieces, 'wacc': wacc_pieces}

        def run_block(z, blk):
            has_pv = any(it[0] == 'pv' for it in blk)
            small, seq = [], []
            i = 0
            while i < len(blk):
                it = blk[i]
                i += 1
                if it[0] == 'smi':
                    steps = []
                    while i < len(blk) and blk[i][0] == 'pv' and blk[i][1] != it[1]:
                        steps += pv_steps(*blk[i][1:])
                        i += 1
                    pa, pb = sm_pieces(z, it[1])
                    pre = [[] for _ in steps]
                    hi = len(steps) - 2
                    nb = min(KT, (hi - 1) // 2)
                    for k in range(KT):
                        pre[1 + (k * (hi - nb - 1)) // KT].append(pa[k])
                    for k in range(KT):
                        pre[hi - nb + (k * nb) // KT].append(pb[k])
                    seq += list(zip(steps, pre))
                elif it[0] == 'pv':
                    seq += [(stp, []) for stp in pv_steps(*it[1:])]
                elif it[0] in ptable and has_pv:
                    small += ptable[it[0]](*it[1:])
                elif it[0] in ptable:
                    for pc in ptable[it[0]](*it[1:]):
                        pc()
                else:
                    table[it[0]](*it[1:])
            for k, pc in enumerate(small):
                seq[3 + (k * min(len(seq) - 6, 3 * len(small))) // len(small)][1].append(pc)
            for stp, pre in seq:
                for pc in pre:
                    pc()
                stp()

        def mlp(waits):
            x = xres[...] + jnp.concatenate([xacc[c] for c in range(DT)], axis=1)
            lhs = jnp.where(top(D), x, 1.0)
            m1, xc, r1 = _stats(x)
            y = xc * r1
            m2 = jnp.mean(y, axis=-1, keepdims=True)
            r2 = lax.rsqrt(jnp.mean(y * y, axis=-1, keepdims=True) - m2 * m2 + _EPS)
            coef = jnp.where(top(128), r1 * r2, -(r2 * (r1 * m1 + m2)))
            hs = []
            for n in range(FT):
                u = _tree(jnp.add, [_mm(lhs[:, cols(j)], w3_buf[cols(j), cols(n)]) for j in range(DT)]) * coef
                hs.append(jax.nn.gelu(u + pltpu.roll(u, 4, 0), approximate=True))
            out = [None] * DT
            for ci, (a0, a1) in enumerate(W4C):
                if waits:
                    w4_cp(ci).wait()
                for n in range(a0, a1):
                    for c in range(DT):
                        r = _mm(hs[n], w4_bufs[ci][cols(n - a0), cols(c)])
                        out[c] = r if out[c] is None else out[c] + r
            xres[...] = x + y + jnp.concatenate(out, axis=1)

        def layer(it, carry):
            z = it >> 4
            state['fresh'] = True
            for b, blk in enumerate(blocks[:-1]):
                @pl.when(it == 0)
                def _():
                    for cp in block_copies(b):
                        cp.wait()

                run_block(z, blk)
                todo = [u for u in xunits if ('v', 2 * u[0] + u[1] // 2) in needs[b]]
                if todo:
                    assert not any(x[0] == 'pvx' and x[1:3] in todo for x in blk)

                    @pl.when(it < 1)
                    def _():
                        for t, j in todo:
                            transpose_unit(t, j)

            @pl.when(it == 0)
            def _():
                run_block(z, blocks[-1])
                for cp in block_copies(NB - 1):
                    cp.wait()
                mlp(True)

            @pl.when(it > 0)
            def _():
                run_block(z, blocks[-1])
                mlp(False)
            return carry

        lax.fori_loop(0, opts.get('npass', 2), layer, 0)
        o_ref[...] = xres[0:1, :].astype(o_ref.dtype)

    def V(*s, dt=f32):
        return pltpu.VMEM(s, dt)

    out = pl.pallas_call(
        kernel,
        out_shape=jax.ShapeDtypeStruct((1, D), A_x.dtype),
        in_specs=[pl.BlockSpec(memory_space=pl.ANY)] * 7,
        out_specs=pl.BlockSpec(memory_space=pltpu.VMEM),
        scratch_shapes=(
            [V(2 * AH, KT, 16, 128, dt=bf16)] * NP + [V(AH, KT, 16, 128, dt=bf16)] * H
            + [V(128 * (b - a), D, dt=bf16) for a, b in W4C]
            + [V(1, D, dt=bf16), V(D // 16, 3 * NP, 16, 128, dt=bf16), V(AH * H, DT, 16, 128, dt=bf16),
               V(D, F, dt=bf16),
               V(8, D), V(8, D),
               V(RQ, 3, DT, 8, 128), V(NP, 3, 8, 128),
               V(RS, 3, KT, 8, 128), V(2, KT, 8, 128),
               V(NP, 8, 128), V(NP, 8, 128), V(8, NP * 128), V(NP, 8, 128),
               V(RA, 2 * AH, 16, 128), V(8, NP * 128), V(NP, 4, 8, 128),
               V(RW, DT, 4, 8, 128), V(DT, 8, 128),
               V(len(xunits), KT, 8, 128), V(4, 8, 128),
               V(RP, 8, KT * 128), V(len(xpairs), 8, KT * 128),
               pltpu.SemaphoreType.DMA((NB + 1 + len(W4C),))]),
        compiler_params=pltpu.CompilerParams(
            vmem_limit_bytes=124 * 1024 * 1024,
            disable_semaphore_checks=True, disable_bounds_checks=True),
        name='kexp',
    )(A_x.reshape(1, D), _cache_view(A_k_cache), _cache_view(A_v_cache),
      _weight_view(A_wq), _weight_view(A_wo), B_w3, B_w4)
    return out.reshape(B, S, D)


@jax.jit
def pallas_interleave_layers__sliding_block_cached__mixer_s_mlp__decode_kernel(
    A_x: jax.Array,
    A_k_cache: jax.Array,
    A_v_cache: jax.Array,
    A_wq: jax.Array,
    A_wo: jax.Array,
    B_x: jax.Array,
    B_w1: jax.Array,
    B_w2: jax.Array,
    B_w3: jax.Array,
    B_w4: jax.Array,
):
    return _run(_PLAN, _OPTS, A_x, A_k_cache, A_v_cache, A_wq, A_wo, B_w3, B_w4)
```

```python
import jax
import jax.numpy as jnp
from jax import lax
import jax.experimental.pallas as pl
import jax.experimental.pallas.tpu as pltpu

f32, bf16, u32, i32 = jnp.float32, jnp.bfloat16, jnp.uint32, jnp.int32
_EPS = 1e-5
_LOG2E = 1.4426950408889634
_NN = (((1,), (0,)), ((), ()))
_NT = (((1,), (1,)), ((), ()))

_OPTS = dict(xunits=[(7, 0), (9, 0), (10, 2), (12, 0), (13, 0), (14, 0)], qlead=1.5, keep=20)


def _stats(x):
    m = jnp.mean(x, axis=-1, keepdims=True)
    xc = x - m
    v = jnp.mean(xc * xc, axis=-1, keepdims=True)
    return m, xc, lax.rsqrt(v + _EPS)


def _tree(op, xs):
    xs = list(xs)
    while len(xs) > 1:
        nxt = [op(xs[i], xs[i + 1]) for i in range(0, len(xs) - 1, 2)]
        if len(xs) % 2:
            nxt.append(xs[-1])
        xs = nxt
    return xs[0]


def _wtile(u):
    return pltpu.bitcast(u.reshape(u.shape[0] * 8, 128), bf16)


def _mm(lhs, w, dims=_NN):
    return lax.dot_general(lhs, w, dims, preferred_element_type=f32)


def _cache_view(c):
    _, H, Sk, Dh = c.shape
    c = c.reshape(H, Sk // 128, 128, Dh // 16, 2, 8)
    c = jnp.transpose(c, (0, 3, 4, 1, 5, 2))
    return c.reshape(H * Dh // 16, 2, Sk // 128, 8, 128)


def _weight_view(w):
    R, N = w.shape
    w = w.reshape(R // 16, 2, 8, N // 128, 128)
    return jnp.transpose(w, (0, 1, 3, 2, 4))


def _schedule(NP, KT, DT, AP, AB, SG, xunits, qlead, keep, LAT=205, LEAD=32, WD=750, AD=160, OL=60,
              vcost=5.95, pstride=2, nraw=3, **_):
    xs = list(xunits)
    steps = [(t, a, k) for t in range(NP) for a in range(0, AP, AB) if (t, a // 8) not in xs for k in range(KT)]
    first_step = {}
    for i, s in enumerate(steps):
        first_step.setdefault(s[0], i)
    main = [('qraw', t, i) for t in range(nraw) for i in range(3)]
    for t in range(NP):
        main += [('qk', t, j, k) for j in range(3) for k in range(KT)]
        if nraw <= t + 2 < NP:
            main += [('q', t + 2, i, j) for j in range(DT) for i in range(3)]
    done = {('q', t): 3 for t in range(nraw)}
    or_left = [(t, j) for t in range(NP) for j in range(3) if (t, j) not in xs]
    wo_left = [(t, j) for t in range(NP) for j in range(3)]
    px_left = list(xs)
    ev, pend, wait, cur = [], [], [], []
    s = dict(tm=0.0, tv=0.0, i=0, mi=0, qk=0)

    def sm(t):
        return ([(('sma', t, k), 3 * SG, None, 0) for k in range(0, KT, SG)]
                + [(('smb', t, k), 3 * SG, ('p', t), SG) for k in range(0, KT, SG)])

    def g_wo(n):
        wo = tuple(u for u in wo_left if done.get(('o',) + u, 0) >= 1)[:4]
        if len(wo) < n:
            return None
        for u in wo:
            wo_left.remove(u)
        g = [(('wo', wo, n, c), 8, []) for n in range(len(wo)) for c in range(DT)]
        g[-1] = (g[-1][0], 8, [(('wacc', wo, c), len(wo), None, 0) for c in range(DT)])
        return g

    def g_or(n, last):
        rd = [u for u in or_left if done.get(('acc',) + u, 0) >= 8 // AB and done.get(('w', u[0]), 0)
              and (last or done[('acct',) + u] + AD <= s['tv'])][:4]
        if len(rd) < n:
            return None
        for u in rd:
            or_left.remove(u)
        return [(('or',) + u, 16, [(('ofin',) + u, 1, ('o',) + u, 1)]) for u in rd]

    def g_px():
        rd = [u for u in px_left if done.get(('w', u[0]), 0)]
        if not rd:
            return None
        px_left.remove(rd[0])
        g = [(('pvx',) + rd[0] + (k,), 8, []) for k in range(KT)]
        g[-1] = (g[-1][0], 8, [(('xsum',) + rd[0] + (k,), 4, ('o',) + rd[0], 4 / KT) for k in range(0, KT, 4)])
        return g

    def pick():
        last, endgame, nxt = s['i'] >= len(steps), s['mi'] >= len(main), s['qk']
        if last:
            return g_or(1, True) or g_px() or g_wo(1)
        if endgame:
            return g_or(4, False) or g_px() or g_wo(4) or g_or(1, False) or g_wo(1)
        rem = sum(8 for m in main[s['mi']:s['mi'] + 200] if m[0] != 'qk' or m[1] == nxt)
        if (first_step[nxt] - s['i']) * vcost - rem > qlead * 500:
            g = (g_wo(4) if len(wo_left) > keep else None) or g_or(4, False) or g_px()
            if g:
                return g
        m = main[s['mi']]
        if m[0] == 'qk' and done.get(('q', m[1]), 0) < 3:
            return None
        s['mi'] += 1
        pcs = []
        if m[0] == 'q' and m[2:] == (2, DT - 1):
            pcs = [(('qfin', m[1], i), DT, ('q', m[1]), 1) for i in range(3)]
        if m[:3] == ('qk', 0, 2) and m[3] % SG == SG - 1:
            pcs = [sm(0)[m[3] // SG]] + (sm(0)[KT // SG:] if m[3] == KT - 1 else [])
        elif m[0] == 'qk' and m[2:] == (2, KT - 1):
            pcs = sm(m[1])
        return [(m, 8 * DT if m[0] == 'qraw' else 8, pcs)]

    def later(t, pcs):
        wait.append((t, pcs))
        wait.sort(key=lambda w: w[0])

    def piece():
        a, cv, e, inc = pend.pop(0)
        ev.append(('piece',) + a)
        s['tv'] += cv / 4
        if e is not None:
            done[e] = done.get(e, 0) + inc
        if a[0] == 'smb' and a[2] == KT - SG:
            later(s['tv'] + WD, [(('w', a[1]), 24, ('w', a[1]), 1)])

    def urgent(p):
        return p[2] is not None and p[2][0] != 'p'

    while True:
        while wait and wait[0][0] <= s['tv']:
            pcs = wait.pop(0)[1]
            pend[:] = [p for p in pcs if urgent(p)] + pend + [p for p in pcs if not urgent(p)]
        i = s['i']
        more = i < len(steps)
        blocked = not more or done.get(('p', steps[i][0]), 0) < min(KT, steps[i][2] + 3)
        if not cur and (s['tm'] + LEAD <= s['tv'] or blocked):
            cur = pick() or []
        if not more and not pend and not wait and not cur:
            break
        if cur and (s['tm'] + LEAD <= s['tv']
                    or (blocked and not pend and (not wait or s['tm'] + LEAD <= wait[0][0]))):
            a, cm, pcs = cur.pop(0)
            ev.append(('tile',) + a)
            s['tm'] = max(s['tm'], s['tv'] - LEAD - 8) + cm
            s['tv'] += 0.25 * (a[0] == 'pvx')
            s['qk'] += a[0] == 'qk' and a[2:] == (2, KT - 1)
            if pcs:
                later(s['tm'] + LAT + (OL if a[0] == 'or' and more else 0), pcs)
        elif blocked and pend:
            piece()
        elif blocked:
            s['tv'] = max(s['tv'], wait[0][0])
        else:
            if pend and (i % pstride == 0 or urgent(pend[0])):
                piece()
            t, a, k = steps[i]
            ev.append(('step', t, a, k))
            if k == KT - 1:
                done['acc', t, a // 8] = done.get(('acc', t, a // 8), 0) + 1
                done['acct', t, a // 8] = s['tv']
            s['tv'] += vcost
            s['i'] += 1
    assert not or_left and not wo_left and not px_left

    out, cur, cnt = [], [], 0
    for e in ev + [None]:
        if e is None or (e[0] == 'tile' and cnt % 4 == 0):
            if any(x[0] == 'step' for x in cur) and len(cur) < 24:
                cur = cur[:1] + [x for x in cur[1:] if x[0] == 'piece'] + [x for x in cur[1:] if x[0] != 'piece']
            out += cur
            cur = []
        if e is not None:
            cur.append(e)
            cnt += (DT if e[1] == 'qraw' else 1) * (e[0] == 'tile')
    return out


def _ring(events, names, key=lambda e: e[2]):
    first, last = {}, {}
    for n, e in enumerate(events):
        if (e[1] if e[0] != 'step' else 'step') in names:
            t = key(e) if e[0] != 'step' else e[1]
            first.setdefault(t, n)
            last[t] = n
    return min(R for R in range(1, 99)
               if all(last[t] < first[u] or last[u] < first[t]
                      for t in last for u in last if u > t and (u - t) % R == 0))


def _run(opts, A_x, A_k_cache, A_v_cache, A_wq, A_wo, B_w3, B_w4):
    B, S, D = A_x.shape
    _, H, Sk, Dh = A_k_cache.shape
    F = B_w3.shape[1]
    W = min(4096, max(256, Sk // 4))
    assert (B, S, H, Dh, W) == (1, 1, 32, 192, 4096) and D % 128 == 0 and F % 128 == 0
    AP = Dh // 8
    KT = W // 128
    NP = H // 2
    DT, FT = D // 128, F // 128
    AB, SG, FD = 4, 2, opts.get('fd', 5)
    cexp = (Dh ** -0.5) * _LOG2E
    W4C = opts.get('w4c', [(0, 6), (6, FT - 1), (FT - 1, FT)])
    xunits = list(opts['xunits'])
    events = _schedule(NP, KT, DT, AP, AB, SG, **opts)
    wo_groups = []
    for e in events:
        if e[1] == 'wo' and e[2] not in wo_groups:
            wo_groups.append(e[2])
    RP = max(6, _ring(events, ('sma', 'smb', 'step', 'pvx')))
    RS = _ring(events, ('qk', 'sma'))
    RQ = _ring(events, ('q', 'qfin'))
    RX = _ring(events, ('pvx', 'xsum'), lambda e: xunits.index(e[2:4]))
    RM = _ring(events, ('wo', 'wacc'), lambda e: wo_groups.index(e[2]))
    assert _ring(events, ('sma', 'smb')) == 1
    sizes = [NP * 2 * AP, 3 * NP, DT, 2 * NP, DT, 3 * NP, NP, NP]
    ACC, QP, XL, WB, XA, OB, MB, LB, NBIG = [sum(sizes[:n]) for n in range(len(sizes) + 1)]
    sizes = [RP * KT, 3 * RS * KT, RX * KT, 3 * DT * RQ, 4 * DT * RM, 4 * NP]
    _, SP, XP, QR, WR, OR, NPB = [sum(sizes[:n]) for n in range(len(sizes) + 1)]
    order1 = sorted(range(NP), key=lambda t: all(u[0] != t for u in xunits))

    def kernel(x_hbm, k_hbm, v_hbm, wq_hbm, wo_hbm, w3_hbm, w4_hbm, o_ref, *scratch):
        k_bufs, v_bufs, scratch = scratch[:NP], scratch[NP:2 * NP], scratch[2 * NP:]
        w4_bufs, scratch = scratch[:len(W4C)], scratch[len(W4C):]
        x_buf, wq_buf, wo_buf, w3_buf, xres, hlast, pbuf, cst, big, sems = scratch
        t0 = (Sk - W) // 128

        def kv_cp(kind, t):
            src, dst = (k_hbm, k_bufs[t]) if kind == 0 else (v_hbm, v_bufs[t])
            return [pltpu.make_async_copy(src.at[pl.ds(AP * t, AP), a, pl.ds(t0, KT)],
                                          dst.at[:, :, pl.ds(8 * a, 8), :], sems.at[2 * t + kind])
                    for a in range(2)]

        def w_cp(src, dst, n, sem):
            rows = src.shape[0] // n
            return [pltpu.make_async_copy(src.at[pl.ds(i * rows, rows), a],
                                          dst.at[pl.ds(i * rows, rows), :, pl.ds(8 * a, 8), :], sem)
                    for i in range(n) for a in range(2)]

        def wq_cp():
            cps = w_cp(wq_hbm, wq_buf, 1, sems.at[2 * NP])
            return cps[:1] + [pltpu.make_async_copy(x_hbm, x_buf, sems.at[2 * NP])] + cps[1:]

        def wo_cp():
            return w_cp(wo_hbm, wo_buf, 8, sems.at[2 * NP + 1])

        def w3_cp():
            return [pltpu.make_async_copy(w3_hbm, w3_buf, sems.at[2 * NP + 2])]

        def w4_cp(i):
            a, b = W4C[i]
            return [pltpu.make_async_copy(w4_hbm.at[pl.ds(128 * a, 128 * (b - a))], w4_bufs[i],
                                          sems.at[2 * NP + 3 + i])]

        def wait(cps):
            for cp in cps:
                cp.wait()

        cps = wq_cp()
        for t in order1:
            cps += kv_cp(0, t) + kv_cp(1, t) + (wo_cp() if t == order1[0] else [])
        for cp in cps + w3_cp() + [cp for i in range(len(W4C)) for cp in w4_cp(i)]:
            cp.start()

        ku = [r.bitcast(u32) for r in k_bufs]
        vu = [r.bitcast(u32) for r in v_bufs]
        wqu = wq_buf.bitcast(u32)
        wou = wo_buf.bitcast(u32)

        def top(n):
            return lax.broadcasted_iota(i32, (8, n), 0) < 4

        def left():
            return lax.broadcasted_iota(i32, (8, 128), 1) < 64

        def cols(n):
            return slice(128 * n, 128 * (n + 1))

        def rows(j):
            return slice(8 * j, 8 * j + 8)

        def masks():
            return [top(128), top(128) == left(), jnp.logical_not(top(128))]

        def mlp_hidden(x):
            lhs = jnp.where(top(D), x, 1.0)
            m1, xc, r1 = _stats(x)
            y = xc * r1
            m2 = jnp.mean(y, axis=-1, keepdims=True)
            r2 = lax.rsqrt(jnp.mean(y * y, axis=-1, keepdims=True) - m2 * m2 + _EPS)
            coef = jnp.where(top(128), r1 * r2, -(r2 * (r1 * m1 + m2)))
            hs = []
            for n in range(FT):
                u = _tree(jnp.add, [_mm(lhs[:, cols(j)], w3_buf[cols(j), cols(n)]) for j in range(DT)]) * coef
                hs.append(jax.nn.gelu(u + pltpu.roll(u, 4, 0), approximate=True))
            return y, hs

        def mlp_out(hs, ci, out):
            a0, a1 = W4C[ci]
            for n in range(a0, a1):
                out = [out[c] + _mm(hs[n], w4_bufs[ci][cols(n - a0), cols(c)]) for c in range(DT)]
            return out

        def layer1():
            for u, mask in enumerate(masks()):
                cst[u] = jnp.where(mask, cexp, 0.0).astype(f32)
            wait(wq_cp())
            x = jnp.broadcast_to(x_buf[...].astype(f32), (8, D))
            _, xc, r = _stats(x)
            xn = xc * r

            def q_body(t, c):
                for i in range(3):
                    q = _tree(jnp.add, [_mm(xn[:, cols(j)], _wtile(wqu[rows(j), 3 * t + i])) for j in range(DT)])
                    big[QP + 3 * t + i] = q * cst[i]
                return c
            lax.fori_loop(0, NP, q_body, 0)

            att = [jnp.zeros((8, 128), f32)] * DT
            for t in order1:
                def s_body(k, c, t=t, q=[big[QP + 3 * t + j] for j in range(3)]):
                    big[ACC + k] = _tree(jnp.add, [_mm(q[j], _wtile(ku[t][rows(j), k])) for j in range(3)])
                    return c

                def o_body(k, o, t=t):
                    return [o[j] + _mm(big[ACC + k], _wtile(vu[t][rows(j), k]), _NT) for j in range(3)]

                wait(kv_cp(0, t))
                lax.fori_loop(0, KT, s_body, 0, unroll=8)
                sc = big[ACC:ACC + KT]
                p = jnp.exp2(sc - jnp.max(jnp.max(sc, axis=0), axis=1, keepdims=True))
                big[ACC:ACC + KT] = p
                inv = 1.0 / jnp.sum(jnp.sum(p, axis=0), axis=1, keepdims=True)
                wait(kv_cp(1, t) + (wo_cp() if t == order1[0] else []))
                o = lax.fori_loop(0, KT, o_body, [jnp.zeros((8, 128), f32)] * 3, unroll=8)
                o = [jnp.where(mask, o[j] * inv, 0.0) for j, mask in enumerate(masks())]
                att = [att[c] + _tree(jnp.add, [_mm(o[j], _wtile(wou[rows(3 * t + j), c])) for j in range(3)])
                       for c in range(DT)]
                for j in [j for tt, j in xunits if tt == t]:
                    def t_body(k, c, t=t, j=j):
                        w = _wtile(vu[t][rows(j), k]).astype(f32).T.astype(bf16)
                        vu[t][rows(j), k] = pltpu.bitcast(w, u32).reshape(8, 8, 128)
                        return c
                    lax.fori_loop(0, KT, t_body, 0, unroll=4)
            att = jnp.concatenate(att, axis=1)
            x = x + (att + pltpu.roll(att, 4, 0))
            wait(w3_cp())
            y, hs = mlp_hidden(x)
            out = [(x + y)[:, cols(c)] for c in range(DT)]
            for ci in range(len(W4C) - 1):
                wait(w4_cp(ci))
                out = mlp_out(hs, ci, out)
            xres[...] = jnp.concatenate(out, axis=1)
            for n in range(*W4C[-1]):
                hlast[n - W4C[-1][0]] = hs[n]

        def layer2(z):
            wait(w4_cp(len(W4C) - 1))
            hs = {n: hlast[n - W4C[-1][0]] for n in range(*W4C[-1])}
            x = jnp.concatenate(mlp_out(hs, len(W4C) - 1, [xres[:, cols(c)] for c in range(DT)]), axis=1)
            xres[...] = x
            m, xc, r = _stats(x)
            for j in range(DT):
                big[XL + j] = (xc * r)[:, cols(j)]
            xraw, coef = jnp.where(top(D), x, 1.0), jnp.where(top(128), r, -(r * m))
            acc, val, fwd = {}, {}, []
            st = dict(pin=False, dirty=False, cnt=0, started=False, left=sum(e[0] == 'step' for e in events))

            def lhs(n):
                if st['pin']:
                    st['pin'] = False
                    return big[n + z]
                if n not in val:
                    val[n] = big[n]
                return val[n]

            def checkpoint():
                for (t, a), y in acc.items():
                    big[ACC + 2 * (t * AP + a):ACC + 2 * (t * AP + a) + 2] = y.reshape(2, 8, 128)

            def put(n, r):
                fwd.append((st['cnt'], n, r))

            def flush(upto, pin=False):
                while fwd and fwd[0][0] <= upto:
                    _, n, r = fwd.pop(0)
                    pbuf[z if pin else 0, :, cols(n)] = r
                    pin = False

            def get(n):
                flush(max([c for c, m, _ in fwd if m == n], default=-1))
                return pbuf[0, :, cols(n)]

            def prow(t, odd, k):
                return pbuf[0, 4 * odd:4 * odd + 1, cols((t % RP) * KT + k)]

            def t_qraw(t, i):
                y = _tree(jnp.add, [_mm(xraw[:, cols(j)], _wtile(wqu[rows(j), 3 * t + i])) for j in range(DT)]) * coef
                big[QP + 3 * t + i] = (y + pltpu.roll(y, 4, 0)) * cst[i]
                st['cnt'] += DT - 1

            def t_q(t, i, j):
                put(QR + ((t % RQ) * 3 + i) * DT + j, _mm(lhs(XL + j), _wtile(wqu[rows(j), 3 * t + i])))

            def t_qk(t, j, k):
                put(SP + (3 * (t % RS) + j) * KT + k, _mm(lhs(QP + 3 * t + j), _wtile(ku[t][rows(j), k])))

            def t_or(t, j):
                a0 = ACC + 2 * t * AP + 16 * j
                a = big[a0:a0 + 16].reshape(128, 128)
                if j == 1:
                    r = _mm(jnp.concatenate([lhs(WB + 2 * t), lhs(WB + 2 * t + 1)], axis=0), a, _NT)
                    put(OR + 4 * t + 3, r[8:16])
                else:
                    r = _mm(lhs(WB + 2 * t + j // 2), a, _NT)
                put(OR + 4 * t + j, r[0:8])

            def t_pvx(t, j, k):
                p = prow(t, j // 2, k) * lhs(WB + 2 * t + j // 2)
                put(XP + (xunits.index((t, j)) % RX) * KT + k, _mm(p, _wtile(vu[t][rows(j), k])))

            def t_wo(units, n, c):
                t, j = units[n]
                put(WR + ((wo_groups.index(units) % RM) * 4 + n) * DT + c,
                    _mm(lhs(OB + 3 * t + j), _wtile(wou[rows(3 * t + j), c])))

            def p_qfin(t, i):
                n = QR + ((t % RQ) * 3 + i) * DT
                big[QP + 3 * t + i] = _tree(jnp.add, [get(n + j) for j in range(DT)]) * cst[i]

            def p_sma(t, k0):
                n = SP + 3 * (t % RS) * KT
                ss = []
                for k in range(k0, k0 + SG):
                    ss.append(get(n + k) + get(n + KT + k) + get(n + 2 * KT + k))
                    pbuf[0, :, cols((t % RP) * KT + k)] = ss[-1]
                big[MB + t] = val['m'] = _tree(jnp.maximum, ss + ([val['m']] if k0 else []))

            def p_smb(t, k0):
                ps = []
                for k in range(k0, k0 + SG):
                    ps.append(jnp.exp2(pbuf[0, :, cols((t % RP) * KT + k)] - val['m']))
                    pbuf[0, :, cols((t % RP) * KT + k)] = ps[-1]
                big[LB + t] = val['l'] = _tree(jnp.add, ps + ([val['l']] if k0 else []))

            def p_w(t):
                m = big[MB + t]
                e = jnp.exp2(m - jnp.max(m, axis=1, keepdims=True))
                w = e / jnp.sum(e * big[LB + t], axis=1, keepdims=True)
                for h in range(2):
                    big[WB + 2 * t + h] = jnp.broadcast_to(w[4 * h:4 * h + 1], (8, 128))

            def p_ofin(t, j):
                r = get(OR + 4 * t + j)
                big[OB + 3 * t + j] = jnp.where(left(), r, get(OR + 4 * t + 3)) if j == 1 else r

            def p_xsum(t, j, k0):
                n = XP + (xunits.index((t, j)) % RX) * KT + k0
                ys = [get(n + u) for u in range(4)] + ([val['y', t, j]] if k0 else [])
                big[OB + 3 * t + j] = val['y', t, j] = _tree(jnp.add, ys)

            def p_wacc(units, c):
                g = wo_groups.index(units)
                rs = [get(WR + ((g % RM) * 4 + n) * DT + c) for n in range(len(units))]
                big[XA + c] = _tree(jnp.add, rs + ([big[XA + c]] if g else []))

            fns = {'qraw': t_qraw, 'q': t_q, 'qk': t_qk, 'or': t_or, 'pvx': t_pvx, 'wo': t_wo, 'qfin': p_qfin,
                   'sma': p_sma, 'smb': p_smb, 'w': p_w, 'ofin': p_ofin, 'xsum': p_xsum, 'wacc': p_wacc}
            for e in events:
                if e[0] == 'step':
                    _, t, a0, k = e
                    p = prow(t, int(a0 >= AP // 2), k)
                    for a in range(a0, a0 + AB):
                        y = pltpu.bitcast(vu[t][a, k], bf16).astype(f32) * p
                        acc[t, a] = y if k == 0 else acc[t, a] + y
                    st.update(dirty=True, started=True, left=st['left'] - 1)
                    if k == KT - 1:
                        checkpoint()
                        acc.clear()
                elif e[0] == 'piece':
                    fns[e[1]](*e[2:])
                else:
                    pinned = st['cnt'] % 4 == 0 and st['left'] > 0
                    if pinned and st['dirty']:
                        checkpoint()
                    st.update(pin=pinned and st['started'], dirty=st['dirty'] and not pinned)
                    fns[e[1]](*e[2:])
                    st['pin'] = False
                    if pinned:
                        flush(st['cnt'] - 4 * FD + 3, pin=st['started'])
                    st['cnt'] += 1
            assert not fwd
            x = xres[...] + jnp.concatenate([big[XA + c] for c in range(DT)], axis=1)
            y, hs = mlp_hidden(x)
            out = [(x + y)[:, cols(c)] for c in range(DT)]
            for ci in range(len(W4C)):
                out = mlp_out(hs, ci, out)
            o_ref[...] = jnp.concatenate(out, axis=1)[0:1].astype(o_ref.dtype)

        def body(it, carry):
            pl.when(it == 0)(layer1)
            pl.when(it == 1)(lambda: layer2(it >> 4))
            return carry

        lax.fori_loop(0, 2, body, 0)

    def V(*s, dt=f32):
        return pltpu.VMEM(s, dt)

    out = pl.pallas_call(
        kernel,
        out_shape=jax.ShapeDtypeStruct((1, D), A_x.dtype),
        in_specs=[pl.BlockSpec(memory_space=pl.ANY)] * 7,
        out_specs=pl.BlockSpec(memory_space=pltpu.VMEM),
        scratch_shapes=(
            [V(AP, KT, 16, 128, dt=bf16)] * (2 * NP)
            + [V(128 * (b - a), D, dt=bf16) for a, b in W4C]
            + [V(1, D, dt=bf16), V(D // 16, 3 * NP, 16, 128, dt=bf16), V(AP * NP, DT, 16, 128, dt=bf16),
               V(D, F, dt=bf16), V(8, D), V(W4C[-1][1] - W4C[-1][0], 8, 128),
               V(1, 8, NPB * 128), V(3, 8, 128), V(NBIG, 8, 128),
               pltpu.SemaphoreType.DMA((2 * NP + 3 + len(W4C),))]),
        compiler_params=pltpu.CompilerParams(
            vmem_limit_bytes=124 * 1024 * 1024,
            disable_semaphore_checks=True, disable_bounds_checks=True),
        name='fused_decode_layers',
    )(A_x.reshape(1, D), _cache_view(A_k_cache), _cache_view(A_v_cache),
      _weight_view(A_wq), _weight_view(A_wo), B_w3, B_w4)
    return out.reshape(B, S, D)


@jax.jit
def pallas_interleave_layers__sliding_block_cached__mixer_s_mlp__decode_kernel(
    A_x: jax.Array,
    A_k_cache: jax.Array,
    A_v_cache: jax.Array,
    A_wq: jax.Array,
    A_wo: jax.Array,
    B_x: jax.Array,
    B_w1: jax.Array,
    B_w2: jax.Array,
    B_w3: jax.Array,
    B_w4: jax.Array,
):
    return _run(_OPTS, A_x, A_k_cache, A_v_cache, A_wq, A_wo, B_w3, B_w4)
```

```python
import jax
import jax.numpy as jnp
from jax import lax
import jax.experimental.pallas as pl
import jax.experimental.pallas.tpu as pltpu

f32, bf16, u32, i32 = jnp.float32, jnp.bfloat16, jnp.uint32, jnp.int32
_EPS = 1e-5
_LOG2E = 1.4426950408889634
_NN = (((1,), (0,)), ((), ()))
_NT = (((1,), (1,)), ((), ()))

_OPTS = dict(xunits=[(7, 0), (9, 0), (10, 2), (12, 0), (13, 0), (14, 0)], qlead=1.5, keep=20)


def _stats(x):
    m = jnp.mean(x, axis=-1, keepdims=True)
    xc = x - m
    v = jnp.mean(xc * xc, axis=-1, keepdims=True)
    return m, xc, lax.rsqrt(v + _EPS)


def _tree(op, xs):
    xs = list(xs)
    while len(xs) > 1:
        nxt = [op(xs[i], xs[i + 1]) for i in range(0, len(xs) - 1, 2)]
        if len(xs) % 2:
            nxt.append(xs[-1])
        xs = nxt
    return xs[0]


def _wtile(u):
    return pltpu.bitcast(u.reshape(u.shape[0] * 8, 128), bf16)


def _mm(lhs, w, dims=_NN):
    return lax.dot_general(lhs, w, dims, preferred_element_type=f32)


def _cache_view(c):
    _, H, Sk, Dh = c.shape
    c = c.reshape(H, Sk // 128, 128, Dh // 16, 2, 8)
    c = jnp.transpose(c, (0, 3, 4, 1, 5, 2))
    return c.reshape(H * Dh // 16, 2, Sk // 128, 8, 128)


def _weight_view(w):
    R, N = w.shape
    w = w.reshape(R // 16, 2, 8, N // 128, 128)
    return jnp.transpose(w, (0, 1, 3, 2, 4))


def _schedule(NP, KT, DT, AP, AB, SG, xunits, qlead, keep, LAT=205, LEAD=32, WD=60, WL=400, AD=160,
              vcost=5.95, pstride=2, n1=2, q2at=40, ph=2, wide=(), **_):
    xs = list(xunits)
    grp = [(t, a) for t in range(NP) for a in range(0, AP, AB) if (t, a // 8) not in xs]
    grp[-2:] = grp[:-3:-1]
    steps = [(t, a, k) for t, a in grp for k in range(KT)]
    first_step = {}
    for i, s in enumerate(steps):
        first_step.setdefault(s[0], i)
    raw = [('qraw', t, i) for t in range(2) for i in range(3)]
    main = raw[:3 + n1]
    for t in range(NP):
        qk = [('qk', t, j, k) for j in range(3) for k in range(KT)]
        q = [('q', t + 1, i, j) for j in range(DT) for i in range(3)] if t + 1 < NP else []
        main += qk[:2 * KT] + raw[3 + n1:] + qk[2 * KT:] if t == 0 else qk[:q2at] + q + qk[q2at:]
    done = {('q', 0): 3, ('q', 1): 3}
    or_left = [(t, j) for t in range(NP) for j in range(3) if (t, j) not in xs]
    wo_left = [(t, j) for t in range(NP) for j in range(3)]
    px_left = list(xs)
    ev, pend, wait, cur = [], [], [], []
    s = dict(tm=0.0, tv=0.0, i=0, mi=0, qk=0)

    def sm(t):
        return ([(('sma', t, k), 3 * SG, None, 0) for k in range(0, KT, SG)]
                + [(('smb', t, k), 3 * SG, ('p', t), SG) for k in range(0, KT, SG)])

    def g_wo(n):
        wo = tuple(u for u in wo_left if done.get(('o',) + u, 0) >= 1)[:4]
        if len(wo) < n:
            return None
        for u in wo:
            wo_left.remove(u)
        g = [(('wo', wo, n, c), 8, []) for n in range(len(wo)) for c in range(DT)]
        g[-1] = (g[-1][0], 8, [(('wacc', wo, c), len(wo), None, 0) for c in range(DT)])
        return g

    def g_or(n, last):
        rd = [u for u in or_left if done.get(('acc',) + u, 0) >= 8 // AB and done.get(('w', u[0]), 0)
              and (last or done[('acct',) + u] + AD <= s['tv'])][:4]
        if len(rd) < n:
            return None
        for u in rd:
            or_left.remove(u)
        return [(('gap',), 8 * len(rd), [])] + [(('or',) + u, 8, [(('ofin',) + u, 1, ('o',) + u, 1)]) for u in rd]

    def g_px():
        rd = [u for u in px_left if done.get(('w', u[0]), 0)]
        if not rd:
            return None
        px_left.remove(rd[0])
        g = [(('pvx',) + rd[0] + (k,), 8, []) for k in range(KT)]
        g[-1] = (g[-1][0], 8, [(('xsum',) + rd[0] + (k,), 4, ('o',) + rd[0], 4 / KT) for k in range(0, KT, 4)])
        return g

    def pick():
        last, endgame, nxt = s['i'] >= len(steps), s['mi'] >= len(main), s['qk']
        if last:
            return g_or(1, True) or g_px() or g_wo(1)
        if endgame:
            return g_or(4, False) or g_px() or g_wo(4) or g_or(1, False) or g_wo(1)
        rem = sum(8 for m in main[s['mi']:s['mi'] + 200] if m[0] != 'qk' or m[1] == nxt)
        if (first_step[nxt] - s['i']) * vcost - rem > qlead * 500:
            g = (g_wo(4) if len(wo_left) > keep else None) or g_or(4, False) or g_px()
            if g:
                return g
        m = main[s['mi']]
        if m[0] == 'qk' and done.get(('q', m[1]), 0) < 3:
            return None
        s['mi'] += 1
        pcs = []
        if m[0] == 'q' and m[2:] == (2, DT - 1):
            pcs = [(('qfin', m[1], i), DT, ('q', m[1]), 1) for i in range(3)]
        if m[0] == 'qk' and (m[2] == 2 or m[1:3] == (0, 1)) and m[3] % SG == SG - 1:
            t = m[1] if m[2] == 2 else -1
            pcs = [sm(t)[m[3] // SG]] + (sm(t)[KT // SG:] if m[3] == KT - 1 else [])
        return [(m, 8 * DT if m[0] == 'qraw' else 8, pcs)]

    def later(t, pcs):
        wait.append((t, pcs))
        wait.sort(key=lambda w: w[0])

    def piece():
        a, cv, e, inc = pend.pop(0)
        ev.append(('piece',) + a)
        s['tv'] += cv / 4
        if e is not None:
            done[e] = done.get(e, 0) + inc
        if a[0] == 'smb' and a[2] == KT - SG and a[1] >= 0:
            later(s['tv'] + WD, [(('wld', a[1]), 0, ('wld', a[1]), 1)])
            later(s['tv'] + WD + WL, [(('w', a[1]), 24, ('w', a[1]), 1)])

    def urgent(p):
        return p[2] is not None and p[2][0] != 'p'

    while True:
        while wait and wait[0][0] <= s['tv']:
            pcs = wait.pop(0)[1]
            pend[:] = [p for p in pcs if urgent(p)] + pend + [p for p in pcs if not urgent(p)]
        i = s['i']
        more = i < len(steps)
        blocked = not more or done.get(('p', steps[i][0] - (i < AP // 2 // AB * KT)), 0) < min(KT, steps[i][2] + 3)
        if not cur and (s['tm'] + LEAD <= s['tv'] or blocked):
            cur = pick() or []
        if not more and not pend and not wait and not cur:
            break
        if cur and (s['tm'] + LEAD <= s['tv']
                    or (blocked and not pend and (not wait or s['tm'] + LEAD <= wait[0][0]))):
            a, cm, pcs = cur.pop(0)
            ev.append(('tile',) + a)
            s['tm'] = max(s['tm'], s['tv'] - LEAD - 8) + cm
            s['tv'] += 0.25 * (a[0] == 'pvx')
            s['qk'] += a[0] == 'qk' and a[2:] == (2, KT - 1)
            if pcs:
                later(s['tm'] + LAT, pcs)
        elif blocked and pend:
            piece()
        elif blocked:
            s['tv'] = max(s['tv'], wait[0][0])
        else:
            if pend and (i % pstride == 0 or urgent(pend[0])):
                piece()
            t, a, k = steps[i]
            ev.append(('step', t, a, k))
            if k == KT - 1:
                done['acc', t, a // 8] = done.get(('acc', t, a // 8), 0) + 1
                done['acct', t, a // 8] = s['tv']
            s['tv'] += vcost - 0.5 * sum((t, b) in wide for b in range(a, a + AB))
            s['i'] += 1
    assert not or_left and not wo_left and not px_left

    out, cur, cnt = [], [], 0
    for e in ev + [None]:
        if e is None or (e[0] == 'tile' and e[1] != 'gap' and cnt % 4 == ph):
            if any(x[0] == 'step' for x in cur) and len(cur) < 32:
                cur = cur[:1] + [x for x in cur[1:] if x[0] == 'piece'] + [x for x in cur[1:] if x[0] != 'piece']
            out += cur
            cur = []
        if e is not None:
            cur.append(e)
            cnt += {'qraw': DT, 'gap': 4}.get(e[1], 1) * (e[0] == 'tile')
    return out


def _ring(events, names, key=lambda e: e[2]):
    first, last = {}, {}
    for n, e in enumerate(events):
        if (e[1] if e[0] != 'step' else 'step') in names:
            t = key(e) if e[0] != 'step' else e[1]
            first.setdefault(t, n)
            last[t] = n
    return min(R for R in range(1, 99)
               if all(last[t] < first[u] or last[u] < first[t]
                      for t in last for u in last if u > t and (u - t) % R == 0))


def _run(opts, A_x, A_k_cache, A_v_cache, A_wq, A_wo, B_w3, B_w4):
    B, S, D = A_x.shape
    _, H, Sk, Dh = A_k_cache.shape
    F = B_w3.shape[1]
    W = min(4096, max(256, Sk // 4))
    assert (B, S, H, Dh, W) == (1, 1, 32, 192, 4096) and D % 128 == 0 and F % 128 == 0
    AP = Dh // 8
    KT = W // 128
    NP = H // 2
    DT, FT = D // 128, F // 128
    AB, SG, FD = 4, 2, opts.get('fd', 5)
    cexp = (Dh ** -0.5) * _LOG2E
    W4C = opts.get('w4c', [(0, 6), (6, FT - 1), (FT - 1, FT)])
    xunits = list(opts['xunits'])
    cand = [(t, a) for t in opts.get('wpairs', range(1, NP - 1)) for a in range(0, AP, opts.get('wstep', 2))
            if (t, a // 8) not in xunits]
    wide = cand[:opts.get('nwide', 0)]
    events = _schedule(NP, KT, DT, AP, AB, SG, wide=wide, **opts)
    wo_groups = []
    for e in events:
        if e[1] == 'wo' and e[2] not in wo_groups:
            wo_groups.append(e[2])
    ev0 = [e for e in events if e[1:3] not in (('sma', -1), ('smb', -1))]
    RP = max(opts.get('rp', 6), _ring(ev0, ('sma', 'smb', 'step', 'pvx')))
    RS = _ring(ev0, ('qk', 'sma'))
    RQ = _ring(events, ('q', 'qfin'))
    RX = _ring(events, ('pvx', 'xsum'), lambda e: xunits.index(e[2:4]))
    RM = _ring(events, ('wo', 'wacc'), lambda e: wo_groups.index(e[2]))
    assert _ring(events, ('sma', 'smb')) == 1
    sizes = [NP * 2 * AP, 3 * NP, DT, 2 * NP, DT, 3 * NP, 1]
    ACC, QP, XL, WB, XA, OB, MB, NBIG = [sum(sizes[:n]) for n in range(len(sizes) + 1)]
    sizes = [(RP + 1) * KT, 3 * RS * KT, RX * KT, 3 * DT * RQ, 4 * DT * RM, 4 * NP, 2 * NP]
    _, SP, XP, QR, WR, OR, ML, NPB = [sum(sizes[:n]) for n in range(len(sizes) + 1)]
    order1 = sorted(range(NP), key=lambda t: all(u[0] != t for u in xunits))

    def kernel(x_hbm, k_hbm, v_hbm, wq_hbm, wo_hbm, w3_hbm, w4_hbm, o_ref, *scratch):
        k_bufs, v_bufs, scratch = scratch[:NP], scratch[NP:2 * NP], scratch[2 * NP:]
        w4_bufs, scratch = scratch[:len(W4C)], scratch[len(W4C):]
        x_buf, wq_buf, wo_buf, w3_buf, xres, hlast, pbuf, cst, big, vwide, sems = scratch
        t0 = (Sk - W) // 128

        def kv_cp(kind, t):
            src, dst = (k_hbm, k_bufs[t]) if kind == 0 else (v_hbm, v_bufs[t])
            return [pltpu.make_async_copy(src.at[pl.ds(AP * t, AP), a, pl.ds(t0, KT)],
                                          dst.at[:, :, pl.ds(8 * a, 8), :], sems.at[2 * t + kind])
                    for a in range(2)]

        def w_cp(src, dst, n, sem):
            rows = src.shape[0] // n
            return [pltpu.make_async_copy(src.at[pl.ds(i * rows, rows), a],
                                          dst.at[pl.ds(i * rows, rows), :, pl.ds(8 * a, 8), :], sem)
                    for i in range(n) for a in range(2)]

        def wq_cp():
            cps = w_cp(wq_hbm, wq_buf, 1, sems.at[2 * NP])
            return cps[:1] + [pltpu.make_async_copy(x_hbm, x_buf, sems.at[2 * NP])] + cps[1:]

        def wo_cp():
            return w_cp(wo_hbm, wo_buf, 8, sems.at[2 * NP + 1])

        def w3_cp():
            return [pltpu.make_async_copy(w3_hbm, w3_buf, sems.at[2 * NP + 2])]

        def w4_cp(i):
            a, b = W4C[i]
            return [pltpu.make_async_copy(w4_hbm.at[pl.ds(128 * a, 128 * (b - a))], w4_bufs[i],
                                          sems.at[2 * NP + 3 + i])]

        def wait(cps):
            for cp in cps:
                cp.wait()

        cps = wq_cp()
        for t in order1:
            cps += kv_cp(0, t) + kv_cp(1, t) + (wo_cp() if t == order1[0] else [])
        for cp in cps + w3_cp() + [cp for i in range(len(W4C)) for cp in w4_cp(i)]:
            cp.start()

        ku = [r.bitcast(u32) for r in k_bufs]
        vu = [r.bitcast(u32) for r in v_bufs]
        wqu = wq_buf.bitcast(u32)
        wou = wo_buf.bitcast(u32)

        def top(n):
            return lax.broadcasted_iota(i32, (8, n), 0) < 4

        def left():
            return lax.broadcasted_iota(i32, (8, 128), 1) < 64

        def cols(n):
            return slice(128 * n, 128 * (n + 1))

        def rows(j):
            return slice(8 * j, 8 * j + 8)

        def masks():
            return [top(128), top(128) == left(), jnp.logical_not(top(128))]

        def mlp_hidden(x):
            lhs = jnp.where(top(D), x, 1.0)
            m1, xc, r1 = _stats(x)
            y = xc * r1
            m2 = jnp.mean(y, axis=-1, keepdims=True)
            r2 = lax.rsqrt(jnp.mean(y * y, axis=-1, keepdims=True) - m2 * m2 + _EPS)
            coef = jnp.where(top(128), r1 * r2, -(r2 * (r1 * m1 + m2)))
            hs = []
            for n in range(FT):
                u = _tree(jnp.add, [_mm(lhs[:, cols(j)], w3_buf[cols(j), cols(n)]) for j in range(DT)]) * coef
                hs.append(jax.nn.gelu(u + pltpu.roll(u, 4, 0), approximate=True))
            return y, hs

        def mlp_out(hs, ci, out):
            a0, a1 = W4C[ci]
            for n in range(a0, a1):
                out = [out[c] + _mm(hs[n], w4_bufs[ci][cols(n - a0), cols(c)]) for c in range(DT)]
            return out

        def layer1():
            for u, mask in enumerate(masks()):
                cst[u] = jnp.where(mask, cexp, 0.0).astype(f32)
            wait(wq_cp())
            x = jnp.broadcast_to(x_buf[...].astype(f32), (8, D))
            _, xc, r = _stats(x)
            xn = xc * r

            def q_body(t, c):
                for i in range(3):
                    q = _tree(jnp.add, [_mm(xn[:, cols(j)], _wtile(wqu[rows(j), 3 * t + i])) for j in range(DT)])
                    big[QP + 3 * t + i] = q * cst[i]
                return c
            lax.fori_loop(0, NP, q_body, 0)

            att = [jnp.zeros((8, 128), f32)] * DT
            for t in order1:
                def s_body(k, c, t=t, q=[big[QP + 3 * t + j] for j in range(3)]):
                    big[ACC + k] = _tree(jnp.add, [_mm(q[j], _wtile(ku[t][rows(j), k])) for j in range(3)])
                    return c

                def o_body(k, o, t=t):
                    return [o[j] + _mm(big[ACC + k], _wtile(vu[t][rows(j), k]), _NT) for j in range(3)]

                wait(kv_cp(0, t))
                lax.fori_loop(0, KT, s_body, 0, unroll=8)
                sc = big[ACC:ACC + KT]
                p = jnp.exp2(sc - jnp.max(jnp.max(sc, axis=0), axis=1, keepdims=True))
                big[ACC:ACC + KT] = p
                inv = 1.0 / jnp.sum(jnp.sum(p, axis=0), axis=1, keepdims=True)
                wait(kv_cp(1, t) + (wo_cp() if t == order1[0] else []))
                o = lax.fori_loop(0, KT, o_body, [jnp.zeros((8, 128), f32)] * 3, unroll=8)
                o = [jnp.where(mask, o[j] * inv, 0.0) for j, mask in enumerate(masks())]
                att = [att[c] + _tree(jnp.add, [_mm(o[j], _wtile(wou[rows(3 * t + j), c])) for j in range(3)])
                       for c in range(DT)]
                for j in [j for tt, j in xunits if tt == t]:
                    def t_body(k, c, t=t, j=j):
                        w = _wtile(vu[t][rows(j), k]).astype(f32).T.astype(bf16)
                        vu[t][rows(j), k] = pltpu.bitcast(w, u32).reshape(8, 8, 128)
                        return c
                    lax.fori_loop(0, KT, t_body, 0, unroll=4)
                for n, a in [(n, a) for n, (tt, a) in enumerate(wide) if tt == t]:
                    vwide[n] = _wtile(vu[t][a]).astype(f32).reshape(KT, 16, 128)
            att = jnp.concatenate(att, axis=1)
            x = x + (att + pltpu.roll(att, 4, 0))
            wait(w3_cp())
            y, hs = mlp_hidden(x)
            out = [(x + y)[:, cols(c)] for c in range(DT)]
            for ci in range(len(W4C) - 1):
                wait(w4_cp(ci))
                out = mlp_out(hs, ci, out)
            xres[...] = jnp.concatenate(out, axis=1)
            for n in range(*W4C[-1]):
                hlast[n - W4C[-1][0]] = hs[n]

        def layer2(z):
            wait(w4_cp(len(W4C) - 1))
            hs = {n: hlast[n - W4C[-1][0]] for n in range(*W4C[-1])}
            x = jnp.concatenate(mlp_out(hs, len(W4C) - 1, [xres[:, cols(c)] for c in range(DT)]), axis=1)
            xres[...] = x
            m, xc, r = _stats(x)
            for j in range(DT):
                big[XL + j] = (xc * r)[:, cols(j)]
            xraw, coef0 = jnp.where(top(D), x, 1.0), jnp.where(top(128), 1.0, -m)
            coef = coef0 * r
            acc, val, fwd = {}, {}, []
            st = dict(pin=False, dirty=False, cnt=0, started=False, left=sum(e[0] == 'step' for e in events))

            def lhs(n):
                if st['pin']:
                    st['pin'] = False
                    return big[n + z]
                if n not in val:
                    val[n] = big[n]
                return val[n]

            def checkpoint():
                for (t, a), y in acc.items():
                    big[ACC + 2 * (t * AP + a):ACC + 2 * (t * AP + a) + 2] = y.reshape(2, 8, 128)

            def put(n, r):
                fwd.append((st['cnt'], n, r))

            def flush(upto, pin=False):
                while fwd and fwd[0][0] <= upto:
                    _, n, r = fwd.pop(0)
                    pbuf[z if pin else 0, :, cols(n)] = r
                    if pin and st['left'] <= opts.get('vpin', 72):
                        vu[NP - 1][z, 0] = pltpu.bitcast(r, u32)
                    pin = False

            def get(n):
                flush(max([c for c, m, _ in fwd if m == n], default=-1))
                return pbuf[0, :, cols(n)]

            def ptile(t, k):
                return cols((t % RP if t >= 0 else RP) * KT + k)

            def prow(t, odd, k):
                return pbuf[0, 4 * odd:4 * odd + 1, ptile(t - (t + odd == 0), k)]

            def t_qraw(t, i):
                y = _tree(jnp.add, [_mm(xraw[:, cols(j)], _wtile(wqu[rows(j), 3 * t + i])) for j in range(DT)])
                y = y * (coef if t else coef0)
                big[QP + 3 * t + i] = (y + pltpu.roll(y, 4, 0)) * cst[i]
                st['cnt'] += DT - 1

            def t_q(t, i, j):
                put(QR + ((t % RQ) * 3 + i) * DT + j, _mm(lhs(XL + j), _wtile(wqu[rows(j), 3 * t + i])))

            def t_qk(t, j, k):
                put(SP + (3 * (t % RS) + j) * KT + k, _mm(lhs(QP + 3 * t + j), _wtile(ku[t][rows(j), k])))

            def t_or(t, j):
                a0 = ACC + 2 * t * AP + 16 * j
                a = big[a0:a0 + 16].reshape(128, 128)
                if j == 1:
                    r = _mm(jnp.concatenate([lhs(WB + 2 * t), lhs(WB + 2 * t + 1)], axis=0), a, _NT)
                    put(OR + 4 * t + 3, r[8:16])
                else:
                    r = _mm(lhs(WB + 2 * t + j // 2), a, _NT)
                put(OR + 4 * t + j, r[0:8])

            def t_pvx(t, j, k):
                p = prow(t, j // 2, k) * lhs(WB + 2 * t + j // 2)
                put(XP + (xunits.index((t, j)) % RX) * KT + k, _mm(p, _wtile(vu[t][rows(j), k])))

            def t_wo(units, n, c):
                t, j = units[n]
                put(WR + ((wo_groups.index(units) % RM) * 4 + n) * DT + c,
                    _mm(lhs(OB + 3 * t + j), _wtile(wou[rows(3 * t + j), c])))

            def p_qfin(t, i):
                n = QR + ((t % RQ) * 3 + i) * DT
                big[QP + 3 * t + i] = _tree(jnp.add, [get(n + j) for j in range(DT)]) * cst[i]

            def p_sma(t, k0):
                n = SP + 3 * (max(t, 0) % RS) * KT
                ss = []
                for k in range(k0, k0 + SG):
                    sc = get(n + k) + get(n + KT + k)
                    sc = sc + get(n + 2 * KT + k) if t >= 0 else sc
                    ss.append(sc * r if t <= 0 else sc)
                    pbuf[0, :, ptile(t, k)] = ss[-1]
                big[MB] = val['m'] = _tree(jnp.maximum, ss + ([val['m']] if k0 else []))

            def p_smb(t, k0):
                ps = []
                for k in range(k0, k0 + SG):
                    ps.append(jnp.exp2(pbuf[0, :, ptile(t, k)] - val['m']))
                    pbuf[0, :, ptile(t, k)] = ps[-1]
                if t >= 0:
                    big[MB] = val['l'] = _tree(jnp.add, ps + ([val['l']] if k0 else []))
                if t >= 0 and k0 + SG == KT:
                    pbuf[0, :, cols(ML + 2 * t)] = val['m']
                    pbuf[0, :, cols(ML + 2 * t + 1)] = val['l']

            def p_wld(t):
                val['ml', t] = pbuf[0, :, cols(ML + 2 * t)], pbuf[0, :, cols(ML + 2 * t + 1)]

            def p_w(t):
                m, l = val['ml', t]
                e = jnp.exp2(m - jnp.max(m, axis=1, keepdims=True))
                w = e / jnp.sum(e * l, axis=1, keepdims=True)
                for h in range(2):
                    big[WB + 2 * t + h] = jnp.broadcast_to(w[4 * h:4 * h + 1], (8, 128))

            def p_ofin(t, j):
                r = get(OR + 4 * t + j)
                big[OB + 3 * t + j] = jnp.where(left(), r, get(OR + 4 * t + 3)) if j == 1 else r

            def p_xsum(t, j, k0):
                n = XP + (xunits.index((t, j)) % RX) * KT + k0
                ys = [get(n + u) for u in range(4)] + ([val['y', t, j]] if k0 else [])
                big[OB + 3 * t + j] = val['y', t, j] = _tree(jnp.add, ys)

            def p_wacc(units, c):
                g = wo_groups.index(units)
                rs = [get(WR + ((g % RM) * 4 + n) * DT + c) for n in range(len(units))]
                big[XA + c] = _tree(jnp.add, rs + ([big[XA + c]] if g else []))

            fns = {'qraw': t_qraw, 'q': t_q, 'qk': t_qk, 'or': t_or, 'pvx': t_pvx, 'wo': t_wo, 'qfin': p_qfin,
                   'sma': p_sma, 'smb': p_smb, 'wld': p_wld, 'w': p_w, 'ofin': p_ofin, 'xsum': p_xsum, 'wacc': p_wacc}
            for e in events:
                if e[0] == 'step':
                    _, t, a0, k = e
                    p = prow(t, int(a0 >= AP // 2), k)
                    for a in range(a0, a0 + AB):
                        y = (vwide[wide.index((t, a)), k] if (t, a) in wide
                             else pltpu.bitcast(vu[t][a, k], bf16).astype(f32)) * p
                        acc[t, a] = y if k == 0 else acc[t, a] + y
                    st.update(dirty=True, started=True, left=st['left'] - 1)
                    if k == KT - 1:
                        checkpoint()
                        acc.clear()
                elif e[0] == 'piece':
                    fns[e[1]](*e[2:])
                elif e[1] == 'gap':
                    st['cnt'] += 4
                else:
                    pinned = st['cnt'] % 4 == opts.get('ph', 2) and st['left'] > 0
                    if pinned and st['dirty']:
                        checkpoint()
                    st.update(pin=pinned and st['started'], dirty=st['dirty'] and not pinned)
                    fns[e[1]](*e[2:])
                    st['pin'] = False
                    if pinned:
                        flush(st['cnt'] - 4 * FD + 3, pin=st['started'])
                    st['cnt'] += 1
            assert not fwd
            x = xres[...] + jnp.concatenate([big[XA + c] for c in range(DT)], axis=1)
            y, hs = mlp_hidden(x)
            out = [(x + y)[:, cols(c)] for c in range(DT)]
            for ci in range(len(W4C)):
                out = mlp_out(hs, ci, out)
            o_ref[...] = jnp.concatenate(out, axis=1)[0:1].astype(o_ref.dtype)

        def body(it, carry):
            pl.when(it == 0)(layer1 if not opts.get('skip1') else lambda: None)
            pl.when(it == 1)(lambda: layer2(it >> 4))
            return carry

        lax.fori_loop(0, 2, body, 0)

    def V(*s, dt=f32):
        return pltpu.VMEM(s, dt)

    out = pl.pallas_call(
        kernel,
        out_shape=jax.ShapeDtypeStruct((1, D), A_x.dtype),
        in_specs=[pl.BlockSpec(memory_space=pl.ANY)] * 7,
        out_specs=pl.BlockSpec(memory_space=pltpu.VMEM),
        scratch_shapes=(
            [V(AP, KT, 16, 128, dt=bf16)] * (2 * NP)
            + [V(128 * (b - a), D, dt=bf16) for a, b in W4C]
            + [V(1, D, dt=bf16), V(D // 16, 3 * NP, 16, 128, dt=bf16), V(AP * NP, DT, 16, 128, dt=bf16),
               V(D, F, dt=bf16), V(8, D), V(W4C[-1][1] - W4C[-1][0], 8, 128),
               V(1, 8, NPB * 128), V(3, 8, 128), V(NBIG, 8, 128), V(max(1, len(wide)), KT, 16, 128),
               pltpu.SemaphoreType.DMA((2 * NP + 3 + len(W4C),))]),
        compiler_params=pltpu.CompilerParams(
            vmem_limit_bytes=int(opts.get('vmem', 124) * 1024 * 1024),
            disable_semaphore_checks=True, disable_bounds_checks=True),
        name='fused_decode_layers',
    )(A_x.reshape(1, D), _cache_view(A_k_cache), _cache_view(A_v_cache),
      _weight_view(A_wq), _weight_view(A_wo), B_w3, B_w4)
    return out.reshape(B, S, D)


@jax.jit
def pallas_interleave_layers__sliding_block_cached__mixer_s_mlp__decode_kernel(
    A_x: jax.Array,
    A_k_cache: jax.Array,
    A_v_cache: jax.Array,
    A_wq: jax.Array,
    A_wo: jax.Array,
    B_x: jax.Array,
    B_w1: jax.Array,
    B_w2: jax.Array,
    B_w3: jax.Array,
    B_w4: jax.Array,
):
    return _run(_OPTS, A_x, A_k_cache, A_v_cache, A_wq, A_wo, B_w3, B_w4)
```

```python
import jax
import jax.numpy as jnp
from jax import lax
import jax.experimental.pallas as pl
import jax.experimental.pallas.tpu as pltpu

f32, bf16, u32, i32 = jnp.float32, jnp.bfloat16, jnp.uint32, jnp.int32
_EPS = 1e-5
_LOG2E = 1.4426950408889634
_NN = (((1,), (0,)), ((), ()))
_NT = (((1,), (1,)), ((), ()))

_OPTS = dict(xunits=[(9, 2, 32), (11, 0, 32), (12, 2, 32), (14, 2, 20)], nwide=78, qlead=2.0, keep=8,
             AD=100, LAT=220, LAT0=220, q2at=20, vpin=80)


def _stats(x):
    m = jnp.mean(x, axis=-1, keepdims=True)
    xc = x - m
    v = jnp.mean(xc * xc, axis=-1, keepdims=True)
    return m, xc, lax.rsqrt(v + _EPS)


def _tree(op, xs):
    xs = list(xs)
    while len(xs) > 1:
        nxt = [op(xs[i], xs[i + 1]) for i in range(0, len(xs) - 1, 2)]
        if len(xs) % 2:
            nxt.append(xs[-1])
        xs = nxt
    return xs[0]


def _wtile(u):
    return pltpu.bitcast(u.reshape(u.shape[0] * 8, 128), bf16)


def _mm(lhs, w, dims=_NN):
    return lax.dot_general(lhs, w, dims, preferred_element_type=f32)


def _cache_view(c):
    _, H, Sk, Dh = c.shape
    c = c.reshape(H, Sk // 128, 128, Dh // 16, 2, 8)
    c = jnp.transpose(c, (0, 3, 4, 1, 5, 2))
    return c.reshape(H * Dh // 16, 2, Sk // 128, 8, 128)


def _weight_view(w):
    R, N = w.shape
    w = w.reshape(R // 16, 2, 8, N // 128, 128)
    return jnp.transpose(w, (0, 1, 3, 2, 4))


def _schedule(NP, KT, DT, AP, AB, SG, xunits, qlead, keep, LAT=205, LAT0=165, LEAD=32, WD=60, WL=400, AD=160,
              vcost=5.95, pstride=2, n1=2, q2at=40, ph=2, wide=(), part=None, **_):
    xs = {u[:2]: u[2] for u in xunits}
    grp = [(t, a) for t in range(NP) for a in range(0, AP, AB)]
    grp[-2:] = grp[:-3:-1]
    steps = [(t, a, k) for t, a in grp for k in range(xs.get((t, a // 8), 0), KT)]
    first_step = {}
    for i, s in enumerate(steps):
        first_step.setdefault(s[0], i)
    raw = [('qraw', t, i) for t in range(2) for i in range(3)]
    main = raw[:3 + n1]
    for t in range(NP):
        qk = [('qk', t, j, k) for j in range(3) for k in range(KT)]
        q = [('q', t + 1, i, j) for j in range(DT) for i in range(3)] if t + 1 < NP else []
        main += qk[:2 * KT] + raw[3 + n1:] + qk[2 * KT:] if t == 0 else qk[:q2at] + q + qk[q2at:]
    done = {('q', 0): 3, ('q', 1): 3}
    or_left = [(t, j) for t in range(NP) for j in range(3) if xs.get((t, j), 0) < KT]
    wo_left = [(t, j) for t in range(NP) for j in range(3)]
    px_left = list(xs)
    ev, pend, wait, cur = [], [], [], []
    s = dict(tm=0.0, tv=0.0, i=0, mi=0, qk=0)

    def sm(t):
        return ([(('sma', t, k), 3 * SG, None, 0) for k in range(0, KT, SG)]
                + [(('smb', t, k), 3 * SG, ('p', t), SG) for k in range(0, KT, SG)])

    def g_wo(n):
        wo = tuple(u for u in wo_left if done.get(('o',) + u, 0) >= 1)[:4]
        if len(wo) < n:
            return None
        for u in wo:
            wo_left.remove(u)
        g = [(('wo', wo, n, c), 8, []) for n in range(len(wo)) for c in range(DT)]
        g[-1] = (g[-1][0], 8, [(('wacc', wo, c), len(wo), None, 0) for c in range(DT)])
        return g

    def g_or(n, last):
        rd = [u for u in or_left if done.get(('acc',) + u, 0) >= 8 // AB and done.get(('w', u[0]), 0)
              and (last or done[('acct',) + u] + AD <= s['tv'])
              and done.get(('y',) + u, 0) >= xs.get(u, 0)][:4]
        if len(rd) < n:
            return None
        for u in rd:
            or_left.remove(u)
        return [(('gap',), 8 * len(rd), [])] + [(('or',) + u, 8, [(('ofin',) + u, 1, ('o',) + u, 1)]) for u in rd]

    def g_px():
        rd = [u for u in px_left if done.get(('w', u[0]), 0)]
        if not rd:
            return None
        px_left.remove(rd[0])
        n = xs[rd[0]]
        g = [(('pvx',) + rd[0] + (k,), 8, []) for k in range(n)]
        e, inc = (('o',) + rd[0], 4 / KT) if n == KT else (('y',) + rd[0], 4)
        g[-1] = (g[-1][0], 8, [(('xsum',) + rd[0] + (k,), 4, e, inc) for k in range(0, n, 4)])
        return g

    def pick():
        last, endgame, nxt = s['i'] >= len(steps), s['mi'] >= len(main), s['qk']
        if last:
            return g_or(1, True) or g_px() or g_wo(1)
        if endgame:
            return g_or(4, False) or g_px() or g_wo(4) or g_wo(1)
        rem = sum(8 for m in main[s['mi']:s['mi'] + 200] if m[0] != 'qk' or m[1] == nxt)
        if (first_step[nxt] - s['i']) * vcost - rem > qlead * 500:
            g = (g_wo(4) if len(wo_left) > keep else None) or g_or(4, False) or g_px()
            if g:
                return g
        m = main[s['mi']]
        if m[0] == 'qk' and done.get(('q', m[1]), 0) < 3:
            return None
        s['mi'] += 1
        pcs = []
        if m[0] == 'q' and m[2:] == (2, DT - 1):
            pcs = [(('qfin', m[1], i), DT, ('q', m[1]), 1) for i in range(3)]
        if m[0] == 'qk' and (m[2] == 2 or m[1:3] == (0, 1)) and m[3] % SG == SG - 1:
            t = m[1] if m[2] == 2 else -1
            pcs = [sm(t)[m[3] // SG]] + (sm(t)[KT // SG:] if m[3] == KT - 1 else [])
        return [(m, 8 * DT if m[0] == 'qraw' else 8, pcs)]

    def later(t, pcs):
        wait.append((t, pcs))
        wait.sort(key=lambda w: w[0])

    def piece():
        a, cv, e, inc = pend.pop(0)
        ev.append(('piece',) + a)
        s['tv'] += cv / 4
        if e is not None:
            done[e] = done.get(e, 0) + inc
        if a[0] == 'smb' and a[2] == KT - SG and a[1] >= 0:
            later(s['tv'] + WD, [(('wld', a[1]), 0, ('wld', a[1]), 1)])
            later(s['tv'] + WD + WL, [(('w', a[1]), 24, ('w', a[1]), 1)])

    def urgent(p):
        return p[2] is not None and p[2][0] != 'p'

    while True:
        while wait and wait[0][0] <= s['tv']:
            pcs = wait.pop(0)[1]
            pend[:] = [p for p in pcs if urgent(p)] + pend + [p for p in pcs if not urgent(p)]
        i = s['i']
        more = i < len(steps)
        blocked = not more or done.get(('p', steps[i][0] - (i < AP // 2 // AB * KT)), 0) < min(KT, steps[i][2] + 3)
        if not cur and (s['tm'] + LEAD <= s['tv'] or blocked):
            cur = pick() or []
        if not more and not pend and not wait and not cur:
            break
        if cur and (s['tm'] + LEAD <= s['tv']
                    or (blocked and not pend and (not wait or s['tm'] + LEAD <= wait[0][0]))):
            a, cm, pcs = cur.pop(0)
            ev.append(('tile',) + a)
            s['tm'] = max(s['tm'], s['tv'] - LEAD - 8) + cm
            s['tv'] += 0.25 * (a[0] == 'pvx')
            s['qk'] += a[0] == 'qk' and a[2:] == (2, KT - 1)
            if pcs:
                later(s['tm'] + (LAT if 0 < i < len(steps) else LAT0), pcs)
        elif blocked and pend:
            piece()
        elif blocked:
            s['tv'] = max(s['tv'], wait[0][0])
        else:
            if pend and (i % pstride == 0 or urgent(pend[0])):
                piece()
            t, a, k = steps[i]
            ev.append(('step', t, a, k))
            if k == KT - 1:
                done['acc', t, a // 8] = done.get(('acc', t, a // 8), 0) + 1
                done['acct', t, a // 8] = s['tv']
            s['tv'] += vcost - 0.5 * sum((t, b) in wide for b in range(a, a + AB))
            s['i'] += 1
    assert not or_left and not wo_left and not px_left

    out, cur, cnt = [], [], 0
    for e in ev + [None]:
        if e is None or (e[0] == 'tile' and e[1] != 'gap' and cnt % 4 == ph):
            if any(x[0] == 'step' for x in cur) and len(cur) < 32:
                cur = cur[:1] + [x for x in cur[1:] if x[0] == 'piece'] + [x for x in cur[1:] if x[0] != 'piece']
            out += cur
            cur = []
        if e is not None:
            cur.append(e)
            cnt += {'qraw': DT, 'gap': 4}.get(e[1], 1) * (e[0] == 'tile')
    return out


def _slots(events, key):
    first, last = {}, {}
    for n, e in enumerate(events):
        k = key(e)
        if k is not None:
            first.setdefault(k, n)
            last[k] = n
    slot, busy = {}, []
    for k in first:
        free = [i for i, u in enumerate(busy) if u < first[k]]
        slot[k] = free[0] if free else len(busy)
        busy[slot[k]:slot[k] + 1] = [last[k]]
    return slot, len(busy)


def _run(opts, A_x, A_k_cache, A_v_cache, A_wq, A_wo, B_w3, B_w4):
    B, S, D = A_x.shape
    _, H, Sk, Dh = A_k_cache.shape
    F = B_w3.shape[1]
    W = min(4096, max(256, Sk // 4))
    assert (B, S, H, Dh, W) == (1, 1, 32, 192, 4096) and D % 128 == 0 and F % 128 == 0
    AP = Dh // 8
    KT = W // 128
    NP = H // 2
    DT, FT = D // 128, F // 128
    AB, SG, FD = 4, 2, opts.get('fd', 5)
    cexp = (Dh ** -0.5) * _LOG2E
    W4C = opts.get('w4c', [(0, 6), (6, FT - 1), (FT - 1, FT)])
    nx = {u[:2]: u[2] for u in opts['xunits']}
    xunits = list(nx)
    cand = [(t, a) for b in range(AB) for t in range(NP - 1, opts.get('w0', 0) - 1, -1) for a in range(b, AP, AB)
            if (t, a // 8) not in xunits + [(NP - 1, 2)]]
    wide = cand[:opts['nwide']]
    events = _schedule(NP, KT, DT, AP, AB, SG, wide=wide, **opts)
    sp, RP = _slots(events, lambda e: e[1] - (e[1] == 0 and e[2] < AP // 2) if e[0] == 'step'
                    else e[2] if e[1] in ('sma', 'smb', 'pvx') else None)
    ss, RS = _slots(events, lambda e: max(e[2], 0) if e[1] in ('qk', 'sma') else None)
    sq, RQ = _slots(events, lambda e: e[2] if e[1] in ('q', 'qfin') else None)
    sx, RX = _slots(events, lambda e: e[2:4] if e[1] in ('pvx', 'xsum') else None)
    sw, RM = _slots(events, lambda e: e[2] if e[1] in ('wo', 'wacc') else None)
    so, RO = _slots(events, lambda e: e[2:4] if e[1] in ('or', 'ofin') else None)
    sl, RL = _slots(events, lambda e: e[2] if e[1] in ('smb', 'wld') else None)
    assert _slots(events, lambda e: e[2] if e[1] in ('sma', 'smb') else None)[1] == 1
    sizes = [2 * AB, 2 * AP, 3 * NP, DT, 2 * NP, DT, 3 * NP, 1]
    ACC, AL, QP, XL, WB, XA, OB, MB, NBIG = [sum(sizes[:n]) for n in range(len(sizes) + 1)]
    sizes = [RP * KT, 3 * RS * KT, RX * KT, 3 * DT * RQ, 4 * DT * RM, 2 * RO, 2 * RL]
    _, SP, XP, QR, WR, OR, ML, NPB = [sum(sizes[:n]) for n in range(len(sizes) + 1)]
    if opts.get('verbose'):
        print('RP RS RQ RX RM', RP, RS, RQ, RX, RM, 'free tiles', (int(13.25 * 256) - NBIG - NPB - KT * len(wide)))
    order1 = sorted(range(NP), key=lambda t: all(u[0] != t for u in xunits))

    def kernel(x_hbm, k_hbm, v_hbm, wq_hbm, wo_hbm, w3_hbm, w4_hbm, o_ref, *scratch):
        k_bufs, v_bufs, scratch = scratch[:NP], scratch[NP:2 * NP], scratch[2 * NP:]
        w4_bufs, scratch = scratch[:len(W4C)], scratch[len(W4C):]
        x_buf, wq_buf, wo_buf, w3_buf, xres, hlast, pbuf, cst, big, vwide, sems = scratch
        t0 = (Sk - W) // 128

        def kv_cp(kind, t):
            src, dst = (k_hbm, k_bufs[t]) if kind == 0 else (v_hbm, v_bufs[t])
            return [pltpu.make_async_copy(src.at[pl.ds(AP * t, AP), a, pl.ds(t0, KT)],
                                          dst.at[:, :, pl.ds(8 * a, 8), :], sems.at[2 * t + kind])
                    for a in range(2)]

        def w_cp(src, dst, n, sem):
            rows = src.shape[0] // n
            return [pltpu.make_async_copy(src.at[pl.ds(i * rows, rows), a],
                                          dst.at[pl.ds(i * rows, rows), :, pl.ds(8 * a, 8), :], sem)
                    for i in range(n) for a in range(2)]

        def wq_cp():
            cps = w_cp(wq_hbm, wq_buf, 1, sems.at[2 * NP])
            return cps[:1] + [pltpu.make_async_copy(x_hbm, x_buf, sems.at[2 * NP])] + cps[1:]

        def wo_cp():
            return w_cp(wo_hbm, wo_buf, 8, sems.at[2 * NP + 1])

        def w3_cp():
            return [pltpu.make_async_copy(w3_hbm, w3_buf, sems.at[2 * NP + 2])]

        def w4_cp(i):
            a, b = W4C[i]
            return [pltpu.make_async_copy(w4_hbm.at[pl.ds(128 * a, 128 * (b - a))], w4_bufs[i],
                                          sems.at[2 * NP + 3 + i])]

        def wait(cps):
            for cp in cps:
                cp.wait()

        cps = wq_cp()
        for t in order1:
            cps += kv_cp(0, t) + kv_cp(1, t) + (wo_cp() if t == order1[0] else [])
        for cp in cps + w3_cp() + [cp for i in range(len(W4C)) for cp in w4_cp(i)]:
            cp.start()

        ku = [r.bitcast(u32) for r in k_bufs]
        vu = [r.bitcast(u32) for r in v_bufs]
        wqu = wq_buf.bitcast(u32)
        wou = wo_buf.bitcast(u32)

        def top(n):
            return lax.broadcasted_iota(i32, (8, n), 0) < 4

        def left():
            return lax.broadcasted_iota(i32, (8, 128), 1) < 64

        def cols(n):
            return slice(128 * n, 128 * (n + 1))

        def rows(j):
            return slice(8 * j, 8 * j + 8)

        def masks():
            return [top(128), top(128) == left(), jnp.logical_not(top(128))]

        def mlp_hidden(x):
            lhs = jnp.where(top(D), x, 1.0)
            m1, xc, r1 = _stats(x)
            y = xc * r1
            m2 = jnp.mean(y, axis=-1, keepdims=True)
            r2 = lax.rsqrt(jnp.mean(y * y, axis=-1, keepdims=True) - m2 * m2 + _EPS)
            coef = jnp.where(top(128), r1 * r2, -(r2 * (r1 * m1 + m2)))
            hs = []
            for n in range(FT):
                u = _tree(jnp.add, [_mm(lhs[:, cols(j)], w3_buf[cols(j), cols(n)]) for j in range(DT)]) * coef
                hs.append(jax.nn.gelu(u + pltpu.roll(u, 4, 0), approximate=True))
            return y, hs

        def mlp_out(hs, ci, out):
            a0, a1 = W4C[ci]
            for n in range(a0, a1):
                out = [out[c] + _mm(hs[n], w4_bufs[ci][cols(n - a0), cols(c)]) for c in range(DT)]
            return out

        def layer1():
            for u, mask in enumerate(masks()):
                cst[u] = jnp.where(mask, cexp, 0.0).astype(f32)
            wait(wq_cp())
            x = jnp.broadcast_to(x_buf[...].astype(f32), (8, D))
            _, xc, r = _stats(x)
            xn = xc * r

            def q_body(t, c):
                for i in range(3):
                    q = _tree(jnp.add, [_mm(xn[:, cols(j)], _wtile(wqu[rows(j), 3 * t + i])) for j in range(DT)])
                    big[QP + 3 * t + i] = q * cst[i]
                return c
            lax.fori_loop(0, NP, q_body, 0)

            att = [jnp.zeros((8, 128), f32)] * DT
            for t in order1:
                def s_body(k, c, t=t, q=[big[QP + 3 * t + j] for j in range(3)]):
                    big[AL + k] = _tree(jnp.add, [_mm(q[j], _wtile(ku[t][rows(j), k])) for j in range(3)])
                    return c

                def o_body(k, o, t=t):
                    return [o[j] + _mm(big[AL + k], _wtile(vu[t][rows(j), k]), _NT) for j in range(3)]

                wait(kv_cp(0, t))
                lax.fori_loop(0, KT, s_body, 0, unroll=8)
                sc = big[AL:AL + KT]
                p = jnp.exp2(sc - jnp.max(jnp.max(sc, axis=0), axis=1, keepdims=True))
                big[AL:AL + KT] = p
                inv = 1.0 / jnp.sum(jnp.sum(p, axis=0), axis=1, keepdims=True)
                wait(kv_cp(1, t) + (wo_cp() if t == order1[0] else []))
                o = lax.fori_loop(0, KT, o_body, [jnp.zeros((8, 128), f32)] * 3, unroll=8)
                o = [jnp.where(mask, o[j] * inv, 0.0) for j, mask in enumerate(masks())]
                att = [att[c] + _tree(jnp.add, [_mm(o[j], _wtile(wou[rows(3 * t + j), c])) for j in range(3)])
                       for c in range(DT)]
                for j in [j for tt, j in xunits if tt == t]:
                    def t_body(k, c, t=t, j=j):
                        w = _wtile(vu[t][rows(j), k]).astype(f32).T.astype(bf16)
                        vu[t][rows(j), k] = pltpu.bitcast(w, u32).reshape(8, 8, 128)
                        return c
                    lax.fori_loop(0, nx[t, j], t_body, 0, unroll=4)
                for n, a in [(n, a) for n, (tt, a) in enumerate(wide) if tt == t]:
                    y = _wtile(vu[t][a]).astype(f32).reshape(KT, 16, 128)
                    vwide[n] = y[:, 8:16]
                    vu[t][a] = pltpu.bitcast(y[:, 0:8], u32)
            att = jnp.concatenate(att, axis=1)
            x = x + (att + pltpu.roll(att, 4, 0))
            wait(w3_cp())
            y, hs = mlp_hidden(x)
            out = [(x + y)[:, cols(c)] for c in range(DT)]
            for ci in range(len(W4C) - 1):
                wait(w4_cp(ci))
                out = mlp_out(hs, ci, out)
            xres[...] = jnp.concatenate(out, axis=1)
            for n in range(*W4C[-1]):
                hlast[n - W4C[-1][0]] = hs[n]

        def layer2(z):
            wait(w4_cp(len(W4C) - 1))
            hs = {n: hlast[n - W4C[-1][0]] for n in range(*W4C[-1])}
            x = jnp.concatenate(mlp_out(hs, len(W4C) - 1, [xres[:, cols(c)] for c in range(DT)]), axis=1)
            xres[...] = x
            m, xc, r = _stats(x)
            for j in range(DT):
                big[XL + j] = (xc * r)[:, cols(j)]
            xraw, coef0 = jnp.where(top(D), x, 1.0), jnp.where(top(128), 1.0, -m)
            coef = coef0 * r
            acc, val, fwd = {}, {}, []
            st = dict(pin=False, dirty=False, cnt=0, started=False, left=sum(e[0] == 'step' for e in events))

            def lhs(n):
                if st['pin']:
                    st['pin'] = False
                    return big[n + z]
                if n not in val:
                    val[n] = big[n]
                return val[n]

            def checkpoint():
                for n, y in enumerate(acc.values()):
                    big[ACC + 2 * n:ACC + 2 * n + 2] = y.reshape(2, 8, 128)

            def put(n, r):
                fwd.append((st['cnt'], n, r))

            def flush(upto, pin=False):
                while fwd and fwd[0][0] <= upto:
                    _, n, r = fwd.pop(0)
                    pbuf[z if pin else 0, :, cols(n)] = r
                    if pin and st['left'] <= opts.get('vpin', 72):
                        vu[NP - 1][z, 2] = pltpu.bitcast(r, u32)
                    pin = False

            def get(n):
                flush(max([c for c, m, _ in fwd if m == n], default=-1))
                return pbuf[0, :, cols(n)]

            def ptile(t, k):
                return cols(sp[t] * KT + k)

            def prow(t, odd, k):
                return pbuf[0, 4 * odd:4 * odd + 1, ptile(t - (t + odd == 0), k)]

            def t_qraw(t, i):
                y = _tree(jnp.add, [_mm(xraw[:, cols(j)], _wtile(wqu[rows(j), 3 * t + i])) for j in range(DT)])
                y = y * (coef if t else coef0)
                big[QP + 3 * t + i] = (y + pltpu.roll(y, 4, 0)) * cst[i]
                st['cnt'] += DT - 1

            def t_q(t, i, j):
                put(QR + (sq[t] * 3 + i) * DT + j, _mm(lhs(XL + j), _wtile(wqu[rows(j), 3 * t + i])))

            def t_qk(t, j, k):
                put(SP + (3 * ss[t] + j) * KT + k, _mm(lhs(QP + 3 * t + j), _wtile(ku[t][rows(j), k])))

            def t_or(t, j):
                if t < NP - 1:
                    a = pltpu.bitcast(vu[t][rows(j), KT - 4:KT - 2].reshape(128, 128), f32)
                else:
                    a = big[AL + 16 * j:AL + 16 * j + 16].reshape(128, 128)
                if j == 1:
                    r = _mm(jnp.concatenate([lhs(WB + 2 * t), lhs(WB + 2 * t + 1)], axis=0), a, _NT)
                    put(OR + 2 * so[t, j] + 1, r[8:16])
                else:
                    r = _mm(lhs(WB + 2 * t + j // 2), a, _NT)
                put(OR + 2 * so[t, j], r[0:8])

            def t_pvx(t, j, k):
                p = prow(t, j // 2, k) * lhs(WB + 2 * t + j // 2)
                put(XP + sx[t, j] * KT + k, _mm(p, _wtile(vu[t][rows(j), k])))

            def t_wo(units, n, c):
                t, j = units[n]
                put(WR + (sw[units] * 4 + n) * DT + c, _mm(lhs(OB + 3 * t + j), _wtile(wou[rows(3 * t + j), c])))

            def p_qfin(t, i):
                n = QR + (sq[t] * 3 + i) * DT
                big[QP + 3 * t + i] = _tree(jnp.add, [get(n + j) for j in range(DT)]) * cst[i]

            def p_sma(t, k0):
                n = SP + 3 * ss[max(t, 0)] * KT
                sv = []
                for k in range(k0, k0 + SG):
                    sc = get(n + k) + get(n + KT + k)
                    sc = sc + get(n + 2 * KT + k) if t >= 0 else sc
                    sv.append(sc * r if t <= 0 else sc)
                    pbuf[0, :, ptile(t, k)] = sv[-1]
                big[MB] = val['m'] = _tree(jnp.maximum, sv + ([val['m']] if k0 else []))

            def p_smb(t, k0):
                ps = []
                for k in range(k0, k0 + SG):
                    ps.append(jnp.exp2(pbuf[0, :, ptile(t, k)] - val['m']))
                    pbuf[0, :, ptile(t, k)] = ps[-1]
                if t >= 0:
                    big[MB] = val['l'] = _tree(jnp.add, ps + ([val['l']] if k0 else []))
                if t >= 0 and k0 + SG == KT:
                    pbuf[0, :, cols(ML + 2 * sl[t])] = val['m']
                    pbuf[0, :, cols(ML + 2 * sl[t] + 1)] = val['l']

            def p_wld(t):
                val['ml', t] = pbuf[0, :, cols(ML + 2 * sl[t])], pbuf[0, :, cols(ML + 2 * sl[t] + 1)]

            def p_w(t):
                m, l = val['ml', t]
                e = jnp.exp2(m - jnp.max(m, axis=1, keepdims=True))
                w = e / jnp.sum(e * l, axis=1, keepdims=True)
                for h in range(2):
                    big[WB + 2 * t + h] = jnp.broadcast_to(w[4 * h:4 * h + 1], (8, 128))

            def p_ofin(t, j):
                r = get(OR + 2 * so[t, j])
                r = jnp.where(left(), r, get(OR + 2 * so[t, j] + 1)) if j == 1 else r
                big[OB + 3 * t + j] = r + big[OB + 3 * t + j] if (t, j) in nx else r

            def p_xsum(t, j, k0):
                n = XP + sx[t, j] * KT + k0
                ys = [get(n + u) for u in range(4)] + ([val['y', t, j]] if k0 else [])
                big[OB + 3 * t + j] = val['y', t, j] = _tree(jnp.add, ys)

            def p_wacc(units, c):
                rs = [get(WR + (sw[units] * 4 + n) * DT + c) for n in range(len(units))]
                big[XA + c] = _tree(jnp.add, rs + ([big[XA + c]] if units != next(iter(sw)) else []))

            fns = {'qraw': t_qraw, 'q': t_q, 'qk': t_qk, 'or': t_or, 'pvx': t_pvx, 'wo': t_wo, 'qfin': p_qfin,
                   'sma': p_sma, 'smb': p_smb, 'wld': p_wld, 'w': p_w, 'ofin': p_ofin, 'xsum': p_xsum, 'wacc': p_wacc}
            for e in events:
                if e[0] == 'step':
                    _, t, a0, k = e
                    p = prow(t, int(a0 >= AP // 2), k)
                    for a in range(a0, a0 + AB):
                        if (t, a) in wide:
                            y = jnp.concatenate([pltpu.bitcast(vu[t][a, k], f32), vwide[wide.index((t, a)), k]])
                        else:
                            y = pltpu.bitcast(vu[t][a, k], bf16).astype(f32)
                        y = y * p
                        acc[t, a] = acc[t, a] + y if (t, a) in acc else y
                    st.update(dirty=True, started=True, left=st['left'] - 1)
                    if k == KT - 1:
                        if t < NP - 1:
                            checkpoint()
                        for a in range(a0, a0 + AB):
                            if t < NP - 1:
                                vu[t][a, KT - 4:KT - 2] = pltpu.bitcast(acc.pop((t, a)), u32).reshape(2, 8, 128)
                            else:
                                big[AL + 2 * a:AL + 2 * a + 2] = acc.pop((t, a)).reshape(2, 8, 128)
                elif e[0] == 'piece':
                    fns[e[1]](*e[2:])
                elif e[1] == 'gap':
                    st['cnt'] += 4
                else:
                    pinned = st['cnt'] % 4 == opts.get('ph', 2) and st['left'] > 0
                    if pinned and st['dirty']:
                        checkpoint()
                    st.update(pin=pinned and st['started'], dirty=st['dirty'] and not pinned)
                    fns[e[1]](*e[2:])
                    st['pin'] = False
                    if pinned:
                        flush(st['cnt'] - 4 * FD + 3, pin=st['started'])
                    st['cnt'] += 1
            assert not fwd
            x = xres[...] + jnp.concatenate([big[XA + c] for c in range(DT)], axis=1)
            y, hs = mlp_hidden(x)
            out = [(x + y)[:, cols(c)] for c in range(DT)]
            for ci in range(len(W4C)):
                out = mlp_out(hs, ci, out)
            o_ref[...] = jnp.concatenate(out, axis=1)[0:1].astype(o_ref.dtype)

        def body(it, carry):
            pl.when(it == 0)(layer1 if not opts.get('skip1') else lambda: None)
            pl.when(it == 1)(lambda: layer2(it >> 4))
            return carry

        lax.fori_loop(0, 2, body, 0)

    def V(*s, dt=f32):
        return pltpu.VMEM(s, dt)

    out = pl.pallas_call(
        kernel,
        out_shape=jax.ShapeDtypeStruct((1, D), A_x.dtype),
        in_specs=[pl.BlockSpec(memory_space=pl.ANY)] * 7,
        out_specs=pl.BlockSpec(memory_space=pltpu.VMEM),
        scratch_shapes=(
            [V(AP, KT, 16, 128, dt=bf16)] * (2 * NP)
            + [V(128 * (b - a), D, dt=bf16) for a, b in W4C]
            + [V(1, D, dt=bf16), V(D // 16, 3 * NP, 16, 128, dt=bf16), V(AP * NP, DT, 16, 128, dt=bf16),
               V(D, F, dt=bf16), V(8, D), V(W4C[-1][1] - W4C[-1][0], 8, 128),
               V(1, 8, NPB * 128), V(3, 8, 128), V(NBIG, 8, 128), V(len(wide), KT, 8, 128),
               pltpu.SemaphoreType.DMA((2 * NP + 3 + len(W4C),))]),
        compiler_params=pltpu.CompilerParams(
            vmem_limit_bytes=int(opts.get('vmem', 128) * 1024 * 1024),
            disable_semaphore_checks=True, disable_bounds_checks=True),
        name='fused_decode_layers',
    )(A_x.reshape(1, D), _cache_view(A_k_cache), _cache_view(A_v_cache),
      _weight_view(A_wq), _weight_view(A_wo), B_w3, B_w4)
    return out.reshape(B, S, D)


@jax.jit
def pallas_interleave_layers__sliding_block_cached__mixer_s_mlp__decode_kernel(
    A_x: jax.Array,
    A_k_cache: jax.Array,
    A_v_cache: jax.Array,
    A_wq: jax.Array,
    A_wo: jax.Array,
    B_x: jax.Array,
    B_w1: jax.Array,
    B_w2: jax.Array,
    B_w3: jax.Array,
    B_w4: jax.Array,
):
    return _run(_OPTS, A_x, A_k_cache, A_v_cache, A_wq, A_wo, B_w3, B_w4)
```

```python
import jax
import jax.numpy as jnp
from jax import lax
import jax.experimental.pallas as pl
import jax.experimental.pallas.tpu as pltpu

f32, bf16, u32, i32 = jnp.float32, jnp.bfloat16, jnp.uint32, jnp.int32
_EPS = 1e-5
_LOG2E = 1.4426950408889634
_NN = (((1,), (0,)), ((), ()))
_NT = (((1,), (1,)), ((), ()))

_OPTS = dict(xunits=[(9, 2, 32), (11, 0, 32), (12, 2, 32), (14, 2, 20)], nwide=78, qlead=2.0, keep=8,
             AD=100, LAT=205, LAT0=205, q2at=20, vpin=80)


def _stats(x):
    m = jnp.mean(x, axis=-1, keepdims=True)
    xc = x - m
    v = jnp.mean(xc * xc, axis=-1, keepdims=True)
    return m, xc, lax.rsqrt(v + _EPS)


def _tree(op, xs):
    xs = list(xs)
    while len(xs) > 1:
        nxt = [op(xs[i], xs[i + 1]) for i in range(0, len(xs) - 1, 2)]
        if len(xs) % 2:
            nxt.append(xs[-1])
        xs = nxt
    return xs[0]


def _wtile(u):
    return pltpu.bitcast(u.reshape(u.shape[0] * 8, 128), bf16)


def _mm(lhs, w, dims=_NN):
    return lax.dot_general(lhs, w, dims, preferred_element_type=f32)


def _cache_view(c):
    _, H, Sk, Dh = c.shape
    c = c.reshape(H, Sk // 128, 128, Dh // 16, 2, 8)
    c = jnp.transpose(c, (0, 3, 4, 1, 5, 2))
    return c.reshape(H * Dh // 16, 2, Sk // 128, 8, 128)


def _weight_view(w):
    R, N = w.shape
    w = w.reshape(R // 16, 2, 8, N // 128, 128)
    return jnp.transpose(w, (0, 1, 3, 2, 4))


def _schedule(NP, KT, DT, AP, AB, SG, xunits, qlead, keep, LAT=205, LAT0=165, LEAD=32, WD=60, WL=400, AD=160,
              vcost=5.95, pstride=2, n1=2, q2at=40, ph=2, wide=(), part=None, **_):
    xs = {u[:2]: u[2] for u in xunits}
    grp = [(t, a) for t in range(NP) for a in range(0, AP, AB)]
    grp[-2:] = grp[:-3:-1]
    steps = [(t, a, k) for t, a in grp for k in range(xs.get((t, a // 8), 0), KT)]
    first_step = {}
    for i, s in enumerate(steps):
        first_step.setdefault(s[0], i)
    raw = [('qraw', t, i) for t in range(2) for i in range(3)]
    main = raw[:3 + n1]
    for t in range(NP):
        qk = [('qk', t, j, k) for j in range(3) for k in range(KT)]
        q = [('q', t + 1, i, j) for j in range(DT) for i in range(3)] if t + 1 < NP else []
        main += qk[:2 * KT] + raw[3 + n1:] + qk[2 * KT:] if t == 0 else qk[:q2at] + q + qk[q2at:]
    done = {('q', 0): 3, ('q', 1): 3}
    or_left = [(t, j) for t in range(NP) for j in range(3) if xs.get((t, j), 0) < KT]
    wo_left = [(t, j) for t in range(NP) for j in range(3)]
    px_left = list(xs)
    ev, pend, wait, cur = [], [], [], []
    s = dict(tm=0.0, tv=0.0, i=0, mi=0, qk=0)

    def sm(t):
        return ([(('sma', t, k), 3 * SG, None, 0) for k in range(0, KT, SG)]
                + [(('smb', t, k), 3 * SG, ('p', t), SG) for k in range(0, KT, SG)])

    def g_wo(n):
        wo = tuple(u for u in wo_left if done.get(('o',) + u, 0) >= 1)[:4]
        if len(wo) < n:
            return None
        for u in wo:
            wo_left.remove(u)
        g = [(('wo', wo, n, c), 8, []) for n in range(len(wo)) for c in range(DT)]
        g[-1] = (g[-1][0], 8, [(('wacc', wo, c), len(wo), None, 0) for c in range(DT)])
        return g

    def g_or(n, last):
        rd = [u for u in or_left if done.get(('acc',) + u, 0) >= 8 // AB and done.get(('w', u[0]), 0)
              and (last or done[('acct',) + u] + AD <= s['tv'])
              and done.get(('y',) + u, 0) >= xs.get(u, 0)][:4]
        if len(rd) < n:
            return None
        for u in rd:
            or_left.remove(u)
        return [(('gap',), 8 * len(rd), [])] + [(('or',) + u, 8, [(('ofin',) + u, 1, ('o',) + u, 1)]) for u in rd]

    def g_px():
        rd = [u for u in px_left if done.get(('w', u[0]), 0)]
        if not rd:
            return None
        px_left.remove(rd[0])
        n = xs[rd[0]]
        g = [(('pvx',) + rd[0] + (k,), 8, []) for k in range(n)]
        e, inc = (('o',) + rd[0], 4 / KT) if n == KT else (('y',) + rd[0], 4)
        g[-1] = (g[-1][0], 8, [(('xsum',) + rd[0] + (k,), 4, e, inc) for k in range(0, n, 4)])
        return g

    def pick():
        last, endgame, nxt = s['i'] >= len(steps), s['mi'] >= len(main), s['qk']
        if last:
            return g_or(1, True) or g_px() or g_wo(1)
        if endgame:
            return g_or(4, False) or g_px() or g_wo(4) or g_wo(1)
        rem = sum(8 for m in main[s['mi']:s['mi'] + 200] if m[0] != 'qk' or m[1] == nxt)
        if (first_step[nxt] - s['i']) * vcost - rem > qlead * 500:
            g = (g_wo(4) if len(wo_left) > keep else None) or g_or(4, False) or g_px()
            if g:
                return g
        m = main[s['mi']]
        if m[0] == 'qk' and done.get(('q', m[1]), 0) < 3:
            return None
        s['mi'] += 1
        pcs = []
        if m[0] == 'q' and m[2:] == (2, DT - 1):
            pcs = [(('qfin', m[1], i), DT, ('q', m[1]), 1) for i in range(3)]
        if m[0] == 'qk' and (m[2] == 2 or m[1:3] == (0, 1)) and m[3] % SG == SG - 1:
            t = m[1] if m[2] == 2 else -1
            pcs = [sm(t)[m[3] // SG]] + (sm(t)[KT // SG:] if m[3] == KT - 1 else [])
        return [(m, 8 * DT if m[0] == 'qraw' else 8, pcs)]

    def later(t, pcs):
        wait.append((t, pcs))
        wait.sort(key=lambda w: w[0])

    def piece():
        a, cv, e, inc = pend.pop(0)
        ev.append(('piece',) + a)
        s['tv'] += cv / 4
        if e is not None:
            done[e] = done.get(e, 0) + inc
        if a[0] == 'smb' and a[2] == KT - SG and a[1] >= 0:
            later(s['tv'] + WD, [(('wld', a[1]), 0, ('wld', a[1]), 1)])
            later(s['tv'] + WD + WL, [(('w', a[1]), 24, ('w', a[1]), 1)])

    def urgent(p):
        return p[2] is not None and p[2][0] != 'p'

    while True:
        while wait and wait[0][0] <= s['tv']:
            pcs = wait.pop(0)[1]
            pend[:] = [p for p in pcs if urgent(p)] + pend + [p for p in pcs if not urgent(p)]
        i = s['i']
        more = i < len(steps)
        blocked = not more or done.get(('p', steps[i][0] - (i < AP // 2 // AB * KT)), 0) < min(KT, steps[i][2] + 6)
        if not cur and (s['tm'] + LEAD <= s['tv'] or blocked):
            cur = pick() or []
        if not more and not pend and not wait and not cur:
            break
        if cur and (s['tm'] + LEAD <= s['tv']
                    or (blocked and not pend and (not wait or s['tm'] + LEAD <= wait[0][0]))):
            a, cm, pcs = cur.pop(0)
            ev.append(('tile',) + a)
            s['tm'] = max(s['tm'], s['tv'] - LEAD - 8) + cm
            s['tv'] += 0.25 * (a[0] == 'pvx')
            s['qk'] += a[0] == 'qk' and a[2:] == (2, KT - 1)
            if pcs:
                later(s['tm'] + (LAT if 0 < i < len(steps) else LAT0), pcs)
        elif blocked and pend:
            piece()
        elif blocked:
            s['tv'] = max(s['tv'], wait[0][0])
        else:
            if pend and (i % pstride == 0 or urgent(pend[0])):
                piece()
            t, a, k = steps[i]
            ev.append(('step', t, a, k))
            if k == KT - 1:
                done['acc', t, a // 8] = done.get(('acc', t, a // 8), 0) + 1
                done['acct', t, a // 8] = s['tv']
            s['tv'] += vcost - 0.5 * sum((t, b) in wide for b in range(a, a + AB))
            s['i'] += 1
    assert not or_left and not wo_left and not px_left

    out, cur, cnt = [], [], 0
    for e in ev + [None]:
        if e is None or (e[0] == 'tile' and e[1] != 'gap' and cnt % 4 == ph):
            if any(x[0] == 'step' for x in cur) and len(cur) < 32:
                cur = cur[:1] + [x for x in cur[1:] if x[0] == 'piece'] + [x for x in cur[1:] if x[0] != 'piece']
            out += cur
            cur = []
        if e is not None:
            cur.append(e)
            cnt += {'qraw': DT, 'gap': 4}.get(e[1], 1) * (e[0] == 'tile')
    return out


def _slots(events, key):
    first, last = {}, {}
    for n, e in enumerate(events):
        k = key(e)
        if k is not None:
            first.setdefault(k, n)
            last[k] = n
    slot, busy = {}, []
    for k in first:
        free = [i for i, u in enumerate(busy) if u < first[k]]
        slot[k] = free[0] if free else len(busy)
        busy[slot[k]:slot[k] + 1] = [last[k]]
    return slot, len(busy)


def _run(opts, A_x, A_k_cache, A_v_cache, A_wq, A_wo, B_w3, B_w4):
    B, S, D = A_x.shape
    _, H, Sk, Dh = A_k_cache.shape
    F = B_w3.shape[1]
    W = min(4096, max(256, Sk // 4))
    assert (B, S, H, Dh, W) == (1, 1, 32, 192, 4096) and D % 128 == 0 and F % 128 == 0
    AP = Dh // 8
    KT = W // 128
    NP = H // 2
    DT, FT = D // 128, F // 128
    AB, SG, FD = 4, 2, opts.get('fd', 5)
    SKEW = opts.get('skew', 1)
    cexp = (Dh ** -0.5) * _LOG2E
    W4C = opts.get('w4c', [(0, FT - 5), (FT - 5, FT - 2), (FT - 2, FT - 1), (FT - 1, FT)])
    nx = {u[:2]: u[2] for u in opts['xunits']}
    xunits = list(nx)
    wide = [(t, a) for t in range(NP) for a in range(0, AP, AB) if (t, a // 8) not in xunits + [(NP - 1, 2)]]
    drop = [g for n, g in enumerate(wide) if n % 3][:max(0, len(wide) - opts['nwide'])]
    wide = [g for g in wide if g not in drop] + [(t, a + 2) for t, a in wide[::-1]][:max(0, opts['nwide'] - len(wide))]
    events = _schedule(NP, KT, DT, AP, AB, SG, wide=wide, **opts)
    sp, RP = _slots(events, lambda e: e[1] - (e[1] == 0 and e[2] < AP // 2) if e[0] == 'step'
                    else e[2] if e[1] in ('sma', 'smb', 'pvx') else None)
    ss, RS = _slots(events, lambda e: max(e[2], 0) if e[1] in ('qk', 'sma') else None)
    sq, RQ = _slots(events, lambda e: e[2] if e[1] in ('q', 'qfin') else None)
    sx, RX = _slots(events, lambda e: e[2:4] if e[1] in ('pvx', 'xsum') else None)
    sw, RM = _slots(events, lambda e: e[2] if e[1] in ('wo', 'wacc') else None)
    so, RO = _slots(events, lambda e: e[2:4] if e[1] in ('or', 'ofin') else None)
    sl, RL = _slots(events, lambda e: e[2] if e[1] in ('smb', 'wld') else None)
    assert _slots(events, lambda e: e[2] if e[1] in ('sma', 'smb') else None)[1] == 1
    sizes = [3 * NP, 2 * NP, 3 * NP, DT, DT, 2 * NP + 2 + opts.get('woff', 2), KT, KT * len(wide)]
    QP, WB, OB, XL, XA, MB, AL, WD, NBIG = [sum(sizes[:n]) for n in range(len(sizes) + 1)]
    free, acc_at = [AL, AL + 16], {}
    for e in events:
        if e[0] == 'step' and (e[1], e[2] // 8) not in acc_at:
            acc_at[e[1], e[2] // 8] = free.pop(0)
        if e[0] == 'step' and e[3] == KT - 1:
            free += [WD + KT * wide.index((e[1], a)) + n for a in range(e[2], e[2] + AB) if (e[1], a) in wide
                     for n in (0, 16)]
    sizes = [RP * KT, 3 * RS * KT, RX * KT, 3 * DT * RQ, 4 * DT * RM, 2 * RO, 2 * RL]
    _, SP, XP, QR, WR, OR, ML, NPB = [sum(sizes[:n]) for n in range(len(sizes) + 1)]
    if opts.get('verbose'):
        print('RP RS RQ RX RM', RP, RS, RQ, RX, RM, 'free tiles', (int(13.25 * 256) - NBIG - NPB))
    order1 = sorted(range(NP), key=lambda t: all(u[0] != t for u in xunits))

    def kernel(x_hbm, k_hbm, v_hbm, wq_hbm, wo_hbm, w3_hbm, w4_hbm, o_ref, *scratch):
        k_bufs, v_bufs, scratch = scratch[:NP], scratch[NP:2 * NP], scratch[2 * NP:]
        w4_bufs, scratch = scratch[:len(W4C)], scratch[len(W4C):]
        wq_buf, wo_buf, w3_buf, pbuf, cst, big, xres, hlast, x_buf, sems = scratch
        t0 = (Sk - W) // 128

        def kv_cp(kind, t):
            src, dst = (k_hbm, k_bufs[t]) if kind == 0 else (v_hbm, v_bufs[t])
            return [pltpu.make_async_copy(src.at[pl.ds(AP * t, AP), a, pl.ds(t0, KT)],
                                          dst.at[:, :, pl.ds(8 * a, 8), :], sems.at[2 * t + kind])
                    for a in range(2)]

        def w_cp(src, dst, n, sem):
            rows = src.shape[0] // n
            return [pltpu.make_async_copy(src.at[pl.ds(i * rows, rows), a],
                                          dst.at[pl.ds(i * rows, rows), :, pl.ds(8 * a, 8), :], sem)
                    for i in range(n) for a in range(2)]

        def wq_cp():
            cps = w_cp(wq_hbm, wq_buf, 1, sems.at[2 * NP])
            return cps[:1] + [pltpu.make_async_copy(x_hbm, x_buf, sems.at[2 * NP])] + cps[1:]

        def wo_cp():
            return w_cp(wo_hbm, wo_buf, 8, sems.at[2 * NP + 1])

        def w3_cp():
            return [pltpu.make_async_copy(w3_hbm, w3_buf, sems.at[2 * NP + 2])]

        def w4_cp(i):
            a, b = W4C[i]
            return [pltpu.make_async_copy(w4_hbm.at[pl.ds(128 * a, 128 * (b - a))], w4_bufs[i],
                                          sems.at[2 * NP + 3 + i])]

        def wait(cps):
            for cp in cps:
                cp.wait()

        cps = wq_cp()
        for t in order1:
            cps += kv_cp(0, t) + kv_cp(1, t) + (wo_cp() if t == order1[0] else [])
        for cp in cps + w3_cp() + [cp for i in range(len(W4C)) for cp in w4_cp(i)]:
            cp.start()

        ku = [r.bitcast(u32) for r in k_bufs]
        vu = [r.bitcast(u32) for r in v_bufs]
        wqu = wq_buf.bitcast(u32)
        wou = wo_buf.bitcast(u32)

        def top(n):
            return lax.broadcasted_iota(i32, (8, n), 0) < 4

        def left():
            return lax.broadcasted_iota(i32, (8, 128), 1) < 64

        def cols(n):
            return slice(128 * n, 128 * (n + 1))

        def rows(j):
            return slice(8 * j, 8 * j + 8)

        def masks():
            return [top(128), top(128) == left(), jnp.logical_not(top(128))]

        def mlp_hidden(x):
            lhs = jnp.where(top(D), x, 1.0)
            m1, xc, r1 = _stats(x)
            y = xc * r1
            m2 = jnp.mean(y, axis=-1, keepdims=True)
            r2 = lax.rsqrt(jnp.mean(y * y, axis=-1, keepdims=True) - m2 * m2 + _EPS)
            coef = jnp.where(top(128), r1 * r2, -(r2 * (r1 * m1 + m2)))
            hs = []
            for n in range(FT):
                u = _tree(jnp.add, [_mm(lhs[:, cols(j)], w3_buf[cols(j), cols(n)]) for j in range(DT)]) * coef
                hs.append(jax.nn.gelu(u + pltpu.roll(u, 4, 0), approximate=True))
            return y, hs

        def mlp_out(hs, ci, out):
            a0, a1 = W4C[ci]
            for n in range(a0, a1):
                out = [out[c] + _mm(hs[n], w4_bufs[ci][cols(n - a0), cols(c)]) for c in range(DT)]
            return out

        def layer1():
            for u, mask in enumerate(masks()):
                cst[u] = jnp.where(mask, cexp, 0.0).astype(f32)
            wait(wq_cp())
            x = jnp.broadcast_to(x_buf[...].astype(f32), (8, D))
            _, xc, r = _stats(x)
            xn = xc * r

            def q_body(t, c):
                for i in range(3):
                    q = _tree(jnp.add, [_mm(xn[:, cols(j)], _wtile(wqu[rows(j), 3 * t + i])) for j in range(DT)])
                    big[QP + 3 * t + i] = q * cst[i]
                return c
            lax.fori_loop(0, NP, q_body, 0)

            att = [jnp.zeros((8, 128), f32)] * DT
            for t in order1:
                def s_body(k, c, t=t, q=[big[QP + 3 * t + j] for j in range(3)]):
                    big[AL + k] = _tree(jnp.add, [_mm(q[j], _wtile(ku[t][rows(j), k])) for j in range(3)])
                    return c

                def o_body(k, o, t=t):
                    return [o[j] + _mm(big[AL + k], _wtile(vu[t][rows(j), k]), _NT) for j in range(3)]

                wait(kv_cp(0, t))
                lax.fori_loop(0, KT, s_body, 0, unroll=8)
                sc = big[AL:AL + KT]
                p = jnp.exp2(sc - jnp.max(jnp.max(sc, axis=0), axis=1, keepdims=True))
                big[AL:AL + KT] = p
                inv = 1.0 / jnp.sum(jnp.sum(p, axis=0), axis=1, keepdims=True)
                wait(kv_cp(1, t) + (wo_cp() if t == order1[0] else []))
                o = lax.fori_loop(0, KT, o_body, [jnp.zeros((8, 128), f32)] * 3, unroll=8)
                o = [jnp.where(mask, o[j] * inv, 0.0) for j, mask in enumerate(masks())]
                att = [att[c] + _tree(jnp.add, [_mm(o[j], _wtile(wou[rows(3 * t + j), c])) for j in range(3)])
                       for c in range(DT)]
                for j in [j for tt, j in xunits if tt == t]:
                    def t_body(k, c, t=t, j=j):
                        w = _wtile(vu[t][rows(j), k]).astype(f32).T.astype(bf16)
                        vu[t][rows(j), k] = pltpu.bitcast(w, u32).reshape(8, 8, 128)
                        return c
                    lax.fori_loop(0, nx[t, j], t_body, 0, unroll=4)
                for n, a in [(n, a) for n, (tt, a) in enumerate(wide) if tt == t]:
                    y = _wtile(vu[t][a]).astype(f32).reshape(KT, 16, 128)
                    big[WD + n * KT:WD + (n + 1) * KT] = y[:, 8:16]
                    vu[t][a] = pltpu.bitcast(y[:, 0:8], u32)
            att = jnp.concatenate(att, axis=1)
            x = x + (att + pltpu.roll(att, 4, 0))
            wait(w3_cp())
            y, hs = mlp_hidden(x)
            out = [(x + y)[:, cols(c)] for c in range(DT)]
            for ci in range(len(W4C) - 1):
                wait(w4_cp(ci))
                out = mlp_out(hs, ci, out)
            xres[...] = jnp.concatenate(out, axis=1)
            for n in range(*W4C[-1]):
                hlast[n - W4C[-1][0]] = hs[n]

        def layer2(z):
            wait(w4_cp(len(W4C) - 1))
            if opts.get('skip2'):
                o_ref[...] = xres[0:1, :].astype(o_ref.dtype)
                return
            hs = {n: hlast[n - W4C[-1][0]] for n in range(*W4C[-1])}
            x = jnp.concatenate(mlp_out(hs, len(W4C) - 1, [xres[:, cols(c)] for c in range(DT)]), axis=1)
            xres[...] = x
            m, xc, r = _stats(x)
            for j in range(DT):
                big[XL + j] = (xc * r)[:, cols(j)]
            xraw, coef0 = jnp.where(top(D), x, 1.0), jnp.where(top(128), 1.0, -m)
            coef = coef0 * r
            acc, val, fwd = {}, {}, []
            st = dict(pin=False, dirty=False, cnt=0, started=False, left=sum(e[0] == 'step' for e in events))

            def lhs(n):
                if st['pin']:
                    st['pin'] = False
                    return big[n + z]
                if n not in val:
                    val[n] = big[n]
                return val[n]

            def checkpoint():
                for (t, a), y in acc.items():
                    n = acc_at[t, a // 8] + 2 * (a % 8)
                    big[n:n + 2] = y.reshape(2, 8, 128)

            def put(n, r):
                fwd.append((st['cnt'], n, r))

            def flush(upto, pin=False):
                while fwd and fwd[0][0] <= upto:
                    _, n, r = fwd.pop(0)
                    pbuf[z if pin else 0, :, cols(n)] = r
                    if pin and st['left'] <= opts.get('vpin', 72):
                        vu[NP - 1][z, 2] = pltpu.bitcast(r, u32)
                    pin = False

            def get(n):
                flush(max([c for c, m, _ in fwd if m == n], default=-1))
                return pbuf[0, :, cols(n)]

            def ptile(t, k):
                return cols(sp[t] * KT + k)

            def prow(t, odd, k):
                return pbuf[0, 4 * odd:4 * odd + 1, ptile(t - (t + odd == 0), k)]

            def t_qraw(t, i):
                y = _tree(jnp.add, [_mm(xraw[:, cols(j)], _wtile(wqu[rows(j), 3 * t + i])) for j in range(DT)])
                y = y * (coef if t else coef0)
                big[QP + 3 * t + i] = (y + pltpu.roll(y, 4, 0)) * cst[i]
                st['cnt'] += DT - 1

            def t_q(t, i, j):
                put(QR + (sq[t] * 3 + i) * DT + j, _mm(lhs(XL + j), _wtile(wqu[rows(j), 3 * t + i])))

            def t_qk(t, j, k):
                put(SP + (3 * ss[t] + j) * KT + k, _mm(lhs(QP + 3 * t + j), _wtile(ku[t][rows(j), k])))

            def t_or(t, j):
                a = big[acc_at[t, j]:acc_at[t, j] + 16].reshape(128, 128)
                if j == 1:
                    r = _mm(jnp.concatenate([lhs(WB + 2 * t), lhs(WB + 2 * t + 1)], axis=0), a, _NT)
                    put(OR + 2 * so[t, j] + 1, r[8:16])
                else:
                    r = _mm(lhs(WB + 2 * t + j // 2), a, _NT)
                put(OR + 2 * so[t, j], r[0:8])

            def t_pvx(t, j, k):
                p = prow(t, j // 2, k) * lhs(WB + 2 * t + j // 2)
                put(XP + sx[t, j] * KT + k, _mm(p, _wtile(vu[t][rows(j), k])))

            def t_wo(units, n, c):
                t, j = units[n]
                put(WR + (sw[units] * 4 + n) * DT + c, _mm(lhs(OB + 3 * t + j), _wtile(wou[rows(3 * t + j), c])))

            def p_qfin(t, i):
                n = QR + (sq[t] * 3 + i) * DT
                big[QP + 3 * t + i] = _tree(jnp.add, [get(n + j) for j in range(DT)]) * cst[i]

            def p_sma(t, k0):
                n = SP + 3 * ss[max(t, 0)] * KT
                sv = []
                for k in range(k0, k0 + SG):
                    sc = get(n + k) + get(n + KT + k)
                    sc = sc + get(n + 2 * KT + k) if t >= 0 else sc
                    sv.append(sc * r if t <= 0 else sc)
                    pbuf[0, :, ptile(t, k)] = sv[-1]
                big[MB + 2 + 2 * t] = val['m'] = _tree(jnp.maximum, sv + ([val['m']] if k0 else []))

            def p_smb(t, k0):
                ps = []
                for k in range(k0, k0 + SG):
                    ps.append(jnp.exp2(pbuf[0, :, ptile(t, k)] - val['m']))
                    pbuf[0, :, ptile(t, k)] = ps[-1]
                if t >= 0:
                    big[MB + 3 + 2 * t] = val['l'] = _tree(jnp.add, ps + ([val['l']] if k0 else []))
                if t >= 0 and k0 + SG == KT:
                    pbuf[0, :, cols(ML + 2 * sl[t])] = val['m']
                    pbuf[0, :, cols(ML + 2 * sl[t] + 1)] = val['l']

            def p_wld(t):
                val['ml', t] = pbuf[0, :, cols(ML + 2 * sl[t])], pbuf[0, :, cols(ML + 2 * sl[t] + 1)]

            def p_w(t):
                m, l = val['ml', t]
                e = jnp.exp2(m - jnp.max(m, axis=1, keepdims=True))
                w = e / jnp.sum(e * l, axis=1, keepdims=True)
                for h in range(2):
                    big[WB + 2 * t + h] = jnp.broadcast_to(w[4 * h:4 * h + 1], (8, 128))

            def p_ofin(t, j):
                r = get(OR + 2 * so[t, j])
                r = jnp.where(left(), r, get(OR + 2 * so[t, j] + 1)) if j == 1 else r
                big[OB + 3 * t + j] = r + big[OB + 3 * t + j] if (t, j) in nx else r

            def p_xsum(t, j, k0):
                n = XP + sx[t, j] * KT + k0
                ys = [get(n + u) for u in range(4)] + ([val['y', t, j]] if k0 else [])
                big[OB + 3 * t + j] = val['y', t, j] = _tree(jnp.add, ys)

            def p_wacc(units, c):
                rs = [get(WR + (sw[units] * 4 + n) * DT + c) for n in range(len(units))]
                big[XA + c] = _tree(jnp.add, rs + ([big[XA + c]] if units != next(iter(sw)) else []))

            fns = {'qraw': t_qraw, 'q': t_q, 'qk': t_qk, 'or': t_or, 'pvx': t_pvx, 'wo': t_wo, 'qfin': p_qfin,
                   'sma': p_sma, 'smb': p_smb, 'wld': p_wld, 'w': p_w, 'ofin': p_ofin, 'xsum': p_xsum, 'wacc': p_wacc}
            for e in events:
                if e[0] == 'step':
                    _, t, a0, k = e
                    k0 = nx.get((t, a0 // 8), 0)
                    for a in range(a0, a0 + AB):
                        n = k + SKEW * (a - a0)
                        kk = k0 + (n - k0) % (KT - k0)
                        if ('p', t, a0, n) not in val:
                            val['p', t, a0, n] = prow(t, int(a0 >= AP // 2), kk)
                        if (t, a) in wide:
                            y = jnp.concatenate([pltpu.bitcast(vu[t][a, kk], f32),
                                                 big[WD + wide.index((t, a)) * KT + kk]])
                        else:
                            y = pltpu.bitcast(vu[t][a, kk], bf16).astype(f32)
                        y = y * val['p', t, a0, n]
                        acc[t, a] = acc[t, a] + y if (t, a) in acc else y
                    st.update(dirty=True, started=True, left=st['left'] - 1)
                    if k == KT - 1:
                        checkpoint()
                        acc.clear()
                elif e[0] == 'piece':
                    fns[e[1]](*e[2:])
                elif e[1] == 'gap':
                    st['cnt'] += 4
                else:
                    pinned = st['cnt'] % 4 == opts.get('ph', 2) and st['left'] > 0
                    if pinned and st['dirty']:
                        checkpoint()
                    st.update(pin=pinned and st['started'], dirty=st['dirty'] and not pinned)
                    fns[e[1]](*e[2:])
                    st['pin'] = False
                    if pinned:
                        flush(st['cnt'] - 4 * FD + 3, pin=st['started'])
                    st['cnt'] += 1
            assert not fwd
            x = xres[...] + jnp.concatenate([big[XA + c] for c in range(DT)], axis=1)
            y, hs = mlp_hidden(x)
            out = [(x + y)[:, cols(c)] for c in range(DT)]
            for ci in range(len(W4C)):
                out = mlp_out(hs, ci, out)
            o_ref[...] = jnp.concatenate(out, axis=1)[0:1].astype(o_ref.dtype)

        def body(it, carry):
            pl.when(it == 0)(layer1 if not opts.get('skip1') else lambda: None)
            pl.when(it == 1)(lambda: layer2(it >> 4))
            return carry

        lax.fori_loop(0, 2, body, 0)

    def V(*s, dt=f32):
        return pltpu.VMEM(s, dt)

    out = pl.pallas_call(
        kernel,
        out_shape=jax.ShapeDtypeStruct((1, D), A_x.dtype),
        in_specs=[pl.BlockSpec(memory_space=pl.ANY)] * 7,
        out_specs=pl.BlockSpec(memory_space=pltpu.VMEM),
        scratch_shapes=(
            [V(AP, KT, 16, 128, dt=bf16)] * (2 * NP)
            + [V(128 * (b - a), D, dt=bf16) for a, b in W4C]
            + [V(D // 16, 3 * NP, 16, 128, dt=bf16), V(AP * NP, DT, 16, 128, dt=bf16), V(D, F, dt=bf16),
               V(1, 8, -(-NPB // 4) * 512), V(4, 8, 128), V(-(-NBIG // 4) * 4, 8, 128),
               V(8, D), V(W4C[-1][1] - W4C[-1][0], 8, 128), V(1, D, dt=bf16),
               pltpu.SemaphoreType.DMA((2 * NP + 3 + len(W4C),))]),
        compiler_params=pltpu.CompilerParams(
            vmem_limit_bytes=int(opts.get('vmem', 128) * 1024 * 1024),
            disable_semaphore_checks=True, disable_bounds_checks=True),
        name='fused_decode_layers',
    )(A_x.reshape(1, D), _cache_view(A_k_cache), _cache_view(A_v_cache),
      _weight_view(A_wq), _weight_view(A_wo), B_w3, B_w4)
    return out.reshape(B, S, D)


@jax.jit
def pallas_interleave_layers__sliding_block_cached__mixer_s_mlp__decode_kernel(
    A_x: jax.Array,
    A_k_cache: jax.Array,
    A_v_cache: jax.Array,
    A_wq: jax.Array,
    A_wo: jax.Array,
    B_x: jax.Array,
    B_w1: jax.Array,
    B_w2: jax.Array,
    B_w3: jax.Array,
    B_w4: jax.Array,
):
    return _run(_OPTS, A_x, A_k_cache, A_v_cache, A_wq, A_wo, B_w3, B_w4)
```

```python
import jax
import jax.numpy as jnp
from jax import lax
import jax.experimental.pallas as pl
import jax.experimental.pallas.tpu as pltpu

f32, bf16, u32, i32 = jnp.float32, jnp.bfloat16, jnp.uint32, jnp.int32
_EPS = 1e-5
_LOG2E = 1.4426950408889634
_NN = (((1,), (0,)), ((), ()))
_NT = (((1,), (1,)), ((), ()))

_OPTS = dict(xunits=[(5, 0, 32), (7, 2, 32), (9, 2, 32), (11, 0, 32), (12, 2, 32), (13, 0, 32), (14, 2, 8)], nwide=76, qlead=2.0, keep=8,
             AD=100, LAT=205, LAT0=205, q2at=20, vpin=80)


def _stats(x):
    m = jnp.mean(x, axis=-1, keepdims=True)
    xc = x - m
    v = jnp.mean(xc * xc, axis=-1, keepdims=True)
    return m, xc, lax.rsqrt(v + _EPS)


def _tree(op, xs):
    xs = list(xs)
    while len(xs) > 1:
        nxt = [op(xs[i], xs[i + 1]) for i in range(0, len(xs) - 1, 2)]
        if len(xs) % 2:
            nxt.append(xs[-1])
        xs = nxt
    return xs[0]


def _wtile(u):
    return pltpu.bitcast(u.reshape(u.shape[0] * 8, 128), bf16)


def _mm(lhs, w, dims=_NN):
    return lax.dot_general(lhs, w, dims, preferred_element_type=f32)


def _cache_view(c):
    _, H, Sk, Dh = c.shape
    c = c.reshape(H, Sk // 128, 128, Dh // 16, 2, 8)
    c = jnp.transpose(c, (0, 3, 4, 1, 5, 2))
    return c.reshape(H * Dh // 16, 2, Sk // 128, 8, 128)


def _weight_view(w):
    R, N = w.shape
    w = w.reshape(R // 16, 2, 8, N // 128, 128)
    return jnp.transpose(w, (0, 1, 3, 2, 4))


def _schedule(NP, KT, DT, AP, AB, SG, xunits, qlead, keep, LAT=205, LAT0=165, LEAD=32, WD=60, WL=400, AD=160,
              vcost=5.95, pstride=2, nraw=8, q2at=40, ph=2, wide=(), part=None, **_):
    xs = {u[:2]: u[2] for u in xunits}
    grp = [(t, a) for t in range(NP) for a in range(0, AP, AB)]
    grp[-2:] = grp[:-3:-1]
    steps = [(t, a, k) for t, a in grp for k in range(xs.get((t, a // 8), 0), KT)]
    first_step = {}
    for i, s in enumerate(steps):
        first_step.setdefault(s[0], i)
    main = [('qraw', t, i) for t in range(nraw) for i in range(3)]
    for t in range(NP):
        qk = [('qk', t, j, k) for j in range(3) for k in range(KT)]
        main += qk[:q2at] + [('q', t + 1, i) for i in range(3) if nraw <= t + 1 < NP] + qk[q2at:]
    done = {('q', t): 3 for t in range(nraw)}
    or_left = [(t, j) for t in range(NP) for j in range(3) if xs.get((t, j), 0) < KT]
    wo_left = [(t, j) for t in range(NP) for j in range(3)]
    px_left = list(xs)
    ev, pend, wait, cur = [], [], [], []
    s = dict(tm=0.0, tv=0.0, i=0, mi=0, qk=0)

    def sm(t):
        return ([(('sma', t, k), 3 * SG, None, 0) for k in range(0, KT, SG)]
                + [(('smb', t, k), 3 * SG, ('p', t), SG) for k in range(0, KT, SG)])

    def g_wo(n):
        wo = tuple(u for u in wo_left if done.get(('o',) + u, 0) >= 1)[:4]
        if len(wo) < n:
            return None
        for u in wo:
            wo_left.remove(u)
        g = [(('wo', wo, n, c), 8, []) for n in range(len(wo)) for c in range(DT)]
        g[-1] = (g[-1][0], 8, [(('wacc', wo, c), len(wo), None, 0) for c in range(DT)])
        return g

    def g_or(n, last):
        rd = [u for u in or_left if done.get(('acc',) + u, 0) >= 8 // AB and done.get(('w', u[0]), 0)
              and (last or done[('acct',) + u] + AD <= s['tv'])
              and done.get(('y',) + u, 0) >= xs.get(u, 0)][:4]
        if len(rd) < n:
            return None
        for u in rd:
            or_left.remove(u)
        return [(('gap',), 8 * len(rd), [])] + [(('or',) + u, 8, [(('ofin',) + u, 1, ('o',) + u, 1)]) for u in rd]

    def g_px():
        rd = [u for u in px_left if done.get(('w', u[0]), 0)]
        if not rd:
            return None
        px_left.remove(rd[0])
        n = xs[rd[0]]
        g = [(('pvx',) + rd[0] + (k,), 8, []) for k in range(n)]
        e, inc = (('o',) + rd[0], 4 / KT) if n == KT else (('y',) + rd[0], 4)
        g[-1] = (g[-1][0], 8, [(('xsum',) + rd[0] + (k,), 4, e, inc) for k in range(0, n, 4)])
        return g

    def pick():
        last, endgame, nxt = s['i'] >= len(steps), s['mi'] >= len(main), s['qk']
        if last:
            return g_or(1, True) or g_px() or g_wo(1)
        if endgame:
            return g_or(4, False) or g_px() or g_wo(4) or g_wo(1)
        rem = sum(8 for m in main[s['mi']:s['mi'] + 200] if m[0] != 'qk' or m[1] == nxt)
        if (first_step[nxt] - s['i']) * vcost - rem > qlead * 500:
            g = (g_wo(4) if len(wo_left) > keep else None) or g_or(4, False) or g_px()
            if g:
                return g
        m = main[s['mi']]
        if m[0] == 'qk' and done.get(('q', m[1]), 0) < 3:
            return None
        s['mi'] += 1
        pcs = []
        if m[0] == 'q':
            pcs = [(('qfin',) + m[1:], 5, ('q', m[1]), 1)]
        if m[0] == 'qk' and (m[2] == 2 or m[1:3] == (0, 1)) and m[3] % SG == SG - 1:
            t = m[1] if m[2] == 2 else -1
            pcs = [sm(t)[m[3] // SG]] + (sm(t)[KT // SG:] if m[3] == KT - 1 else [])
        return [(m, 8, pcs)]

    def later(t, pcs):
        wait.append((t, pcs))
        wait.sort(key=lambda w: w[0])

    def piece():
        a, cv, e, inc = pend.pop(0)
        ev.append(('piece',) + a)
        s['tv'] += cv / 4
        if e is not None:
            done[e] = done.get(e, 0) + inc
        if a[0] == 'smb' and a[2] == KT - SG and a[1] >= 0:
            later(s['tv'] + WD, [(('wld', a[1]), 0, ('wld', a[1]), 1)])
            later(s['tv'] + WD + WL, [(('w', a[1]), 24, ('w', a[1]), 1)])

    def urgent(p):
        return p[2] is not None and p[2][0] != 'p'

    while True:
        while wait and wait[0][0] <= s['tv']:
            pcs = wait.pop(0)[1]
            pend[:] = [p for p in pcs if urgent(p)] + pend + [p for p in pcs if not urgent(p)]
        i = s['i']
        more = i < len(steps)
        blocked = not more or done.get(('p', steps[i][0] - (i < AP // 2 // AB * KT)), 0) < min(KT, steps[i][2] + 6)
        if not cur and (s['tm'] + LEAD <= s['tv'] or blocked):
            cur = pick() or []
        if not more and not pend and not wait and not cur:
            break
        if cur and (s['tm'] + LEAD <= s['tv']
                    or (blocked and not pend and (not wait or s['tm'] + LEAD <= wait[0][0]))):
            a, cm, pcs = cur.pop(0)
            ev.append(('tile',) + a)
            s['tm'] = max(s['tm'], s['tv'] - LEAD - 8) + cm
            s['tv'] += 0.25 * (a[0] == 'pvx')
            s['qk'] += a[0] == 'qk' and a[2:] == (2, KT - 1)
            if pcs:
                later(s['tm'] + (LAT if 0 < i < len(steps) else LAT0), pcs)
        elif blocked and pend:
            piece()
        elif blocked:
            s['tv'] = max(s['tv'], wait[0][0])
        else:
            if pend and (i % pstride == 0 or urgent(pend[0])):
                piece()
            t, a, k = steps[i]
            ev.append(('step', t, a, k))
            if k == KT - 1:
                done['acc', t, a // 8] = done.get(('acc', t, a // 8), 0) + 1
                done['acct', t, a // 8] = s['tv']
            s['tv'] += vcost - 0.5 * sum((t, b) in wide for b in range(a, a + AB))
            s['i'] += 1
    assert not or_left and not wo_left and not px_left

    out, cur, cnt = [], [], 0
    for e in ev + [None]:
        if e is None or (e[0] == 'tile' and e[1] != 'gap' and cnt % 4 == ph):
            if any(x[0] == 'step' for x in cur) and len(cur) < 32:
                cur = cur[:1] + [x for x in cur[1:] if x[0] == 'piece'] + [x for x in cur[1:] if x[0] != 'piece']
            out += cur
            cur = []
        if e is not None:
            cur.append(e)
            cnt += (4 if e[1] == 'gap' else 1) * (e[0] == 'tile')
    return out


def _slots(events, key):
    first, last = {}, {}
    for n, e in enumerate(events):
        k = key(e)
        if k is not None:
            first.setdefault(k, n)
            last[k] = n
    slot, busy = {}, []
    for k in first:
        free = [i for i, u in enumerate(busy) if u < first[k]]
        slot[k] = free[0] if free else len(busy)
        busy[slot[k]:slot[k] + 1] = [last[k]]
    return slot, len(busy)


def _run(opts, A_x, A_k_cache, A_v_cache, A_wq, A_wo, B_w3, B_w4):
    B, S, D = A_x.shape
    _, H, Sk, Dh = A_k_cache.shape
    F = B_w3.shape[1]
    W = min(4096, max(256, Sk // 4))
    assert (B, S, H, Dh, W) == (1, 1, 32, 192, 4096) and D % 128 == 0 and F % 128 == 0
    AP = Dh // 8
    KT = W // 128
    NP = H // 2
    DT, FT = D // 128, F // 128
    AB, SG, FD = 4, 2, opts.get('fd', 5)
    SKEW = opts.get('skew', 1)
    cexp = (Dh ** -0.5) * _LOG2E
    nx = {u[:2]: u[2] for u in opts['xunits']}
    xunits = list(nx)
    wide = [(t, a) for t in range(NP) for a in range(0, AP, AB) if (t, a // 8) not in xunits + [(NP - 1, 2)]]
    drop = [g for n, g in enumerate(wide) if n % 3][:max(0, len(wide) - opts['nwide'])]
    wide = [g for g in wide if g not in drop] + [(t, a + 2) for t, a in wide[::-1]][:max(0, opts['nwide'] - len(wide))]
    events = _schedule(NP, KT, DT, AP, AB, SG, wide=wide, **opts)
    sp, RP = _slots(events, lambda e: e[1] - (e[1] == 0 and e[2] < AP // 2) if e[0] == 'step'
                    else e[2] if e[1] in ('sma', 'smb', 'pvx') else None)
    ss, RS = _slots(events, lambda e: max(e[2], 0) if e[1] in ('qk', 'sma') else None)
    sq, RQ = _slots(events, lambda e: e[2] if e[1] in ('q', 'qfin') else None)
    sx, RX = _slots(events, lambda e: e[2:4] if e[1] in ('pvx', 'xsum') else None)
    sw, RM = _slots(events, lambda e: e[2] if e[1] in ('wo', 'wacc') else None)
    so, RO = _slots(events, lambda e: e[2:4] if e[1] in ('or', 'ofin') else None)
    sl, RL = _slots(events, lambda e: e[2] if e[1] in ('smb', 'wld') else None)
    assert _slots(events, lambda e: e[2] if e[1] in ('sma', 'smb') else None)[1] == 1
    sizes = [3 * NP, 3 * NP, 2 * NP, 3 * NP, 2, DT, 2 * NP + 3, KT, KT * len(wide)]
    QP, Q0, WB, OB, XL, XA, MB, AL, WD, NBIG = [sum(sizes[:n]) for n in range(len(sizes) + 1)]
    free, acc_at = [AL, AL + 16], {}
    for e in events:
        if e[0] == 'step' and (e[1], e[2] // 8) not in acc_at:
            acc_at[e[1], e[2] // 8] = free.pop(0)
        if e[0] == 'step' and e[3] == KT - 1:
            free += [WD + KT * wide.index((e[1], a)) + n for a in range(e[2], e[2] + AB) if (e[1], a) in wide
                     for n in (0, 16)]
    sizes = [RP * KT, 3 * RS * KT, RX * KT, 3 * RQ, 4 * DT * RM, 2 * RO, 2 * RL]
    _, SP, XP, QR, WR, OR, ML, NPB = [sum(sizes[:n]) for n in range(len(sizes) + 1)]
    if opts.get('verbose'):
        print('RP RS RQ RX RM', RP, RS, RQ, RX, RM, 'free tiles', (int(13.25 * 256) - NBIG - NPB))
    order1 = sorted(range(NP), key=lambda t: all(u[0] != t for u in xunits))

    def kernel(x_hbm, k_hbm, v_hbm, wq_hbm, wo_hbm, w3_hbm, w4_hbm, o_ref, *scratch):
        k_bufs, v_bufs, scratch = scratch[:NP], scratch[NP:2 * NP], scratch[2 * NP:]
        w4_bufs, scratch = scratch[:DT], scratch[DT:]
        wq_buf, wo_buf, w3_buf, pbuf, cst, big, hbuf, xres, x_buf, sems = scratch
        t0 = (Sk - W) // 128

        def kv_cp(kind, t):
            src, dst = (k_hbm, k_bufs[t]) if kind == 0 else (v_hbm, v_bufs[t])
            return [pltpu.make_async_copy(src.at[pl.ds(AP * t, AP), a, pl.ds(t0, KT)],
                                          dst.at[:, :, pl.ds(8 * a, 8), :], sems.at[2 * t + kind])
                    for a in range(2)]

        def w_cp(src, dst, n, sem):
            rows = src.shape[0] // n
            return [pltpu.make_async_copy(src.at[pl.ds(i * rows, rows), a],
                                          dst.at[pl.ds(i * rows, rows), :, pl.ds(8 * a, 8), :], sem)
                    for i in range(n) for a in range(2)]

        def wq_cp():
            cps = w_cp(wq_hbm, wq_buf, 1, sems.at[2 * NP])
            return cps[:1] + [pltpu.make_async_copy(x_hbm, x_buf, sems.at[2 * NP])] + cps[1:]

        def wo_cp():
            return w_cp(wo_hbm, wo_buf, 8, sems.at[2 * NP + 1])

        def w3_cp():
            return [pltpu.make_async_copy(w3_hbm, w3_buf, sems.at[2 * NP + 2])]

        def w4_cp(c):
            return [pltpu.make_async_copy(w4_hbm.at[:, pl.ds(128 * c, 128)], w4_bufs[c], sems.at[2 * NP + 3 + c])]

        def wait(cps):
            for cp in cps:
                cp.wait()

        cps = wq_cp()
        for t in order1:
            cps += kv_cp(0, t) + kv_cp(1, t) + (wo_cp() if t == order1[0] else [])
        for cp in cps + w3_cp() + [cp for c in range(DT) for cp in w4_cp(c)]:
            cp.start()

        ku = [r.bitcast(u32) for r in k_bufs]
        vu = [r.bitcast(u32) for r in v_bufs]
        wqu = wq_buf.bitcast(u32)
        wou = wo_buf.bitcast(u32)
        w4u = [r.bitcast(u32) for r in w4_bufs]

        def top(n):
            return lax.broadcasted_iota(i32, (8, n), 0) < 4

        def left():
            return lax.broadcasted_iota(i32, (8, 128), 1) < 64

        def cols(n):
            return slice(128 * n, 128 * (n + 1))

        def rows(j):
            return slice(8 * j, 8 * j + 8)

        def masks():
            return [top(128), top(128) == left(), jnp.logical_not(top(128))]

        def mlp_hidden(x):
            lhs = jnp.where(top(D), x, 1.0)
            m1, xc, r1 = _stats(x)
            y = xc * r1
            m2 = jnp.mean(y, axis=-1, keepdims=True)
            r2 = lax.rsqrt(jnp.mean(y * y, axis=-1, keepdims=True) - m2 * m2 + _EPS)
            coef = jnp.where(top(128), r1 * r2, -(r2 * (r1 * m1 + m2)))
            hs = []
            for n in range(FT):
                u = _tree(jnp.add, [_mm(lhs[:, cols(j)], w3_buf[cols(j), cols(n)]) for j in range(DT)]) * coef
                hs.append(jax.nn.gelu(u + pltpu.roll(u, 4, 0), approximate=True))
            return y, hs

        def w4_tile(n, c):
            return pltpu.bitcast(w4u[c][64 * n:64 * (n + 1)], bf16)

        def layer1():
            for u, mask in enumerate(masks()):
                cst[u] = jnp.where(mask, cexp, 0.0).astype(f32)
            wait(wq_cp())
            x = jnp.broadcast_to(x_buf[...].astype(f32), (8, D))
            _, xc, r = _stats(x)
            xn = xc * r

            def q_body(t, c):
                for i in range(3):
                    q = _tree(jnp.add, [_mm(xn[:, cols(j)], _wtile(wqu[rows(j), 3 * t + i])) for j in range(DT)])
                    big[QP + 3 * t + i] = q * cst[i]
                return c
            lax.fori_loop(0, NP, q_body, 0)

            att = [jnp.zeros((8, 128), f32)] * DT
            for t in order1:
                def s_body(k, c, t=t, q=[big[QP + 3 * t + j] for j in range(3)]):
                    big[AL + k] = _tree(jnp.add, [_mm(q[j], _wtile(ku[t][rows(j), k])) for j in range(3)])
                    return c

                def o_body(k, o, t=t):
                    return [o[j] + _mm(big[AL + k], _wtile(vu[t][rows(j), k]), _NT) for j in range(3)]

                wait(kv_cp(0, t))
                lax.fori_loop(0, KT, s_body, 0, unroll=8)
                sc = big[AL:AL + KT]
                p = jnp.exp2(sc - jnp.max(jnp.max(sc, axis=0), axis=1, keepdims=True))
                big[AL:AL + KT] = p
                inv = 1.0 / jnp.sum(jnp.sum(p, axis=0), axis=1, keepdims=True)
                wait(kv_cp(1, t) + (wo_cp() if t == order1[0] else []))
                o = lax.fori_loop(0, KT, o_body, [jnp.zeros((8, 128), f32)] * 3, unroll=8)
                o = [jnp.where(mask, o[j] * inv, 0.0) for j, mask in enumerate(masks())]
                att = [att[c] + _tree(jnp.add, [_mm(o[j], _wtile(wou[rows(3 * t + j), c])) for j in range(3)])
                       for c in range(DT)]
                for j in [j for tt, j in xunits if tt == t]:
                    def t_body(k, c, t=t, j=j):
                        w = _wtile(vu[t][rows(j), k]).astype(f32).T.astype(bf16)
                        vu[t][rows(j), k] = pltpu.bitcast(w, u32).reshape(8, 8, 128)
                        return c
                    lax.fori_loop(0, nx[t, j], t_body, 0, unroll=4)
                for n, a in [(n, a) for n, (tt, a) in enumerate(wide) if tt == t]:
                    y = _wtile(vu[t][a]).astype(f32).reshape(KT, 16, 128)
                    big[WD + n * KT:WD + (n + 1) * KT] = y[:, 8:16]
                    vu[t][a] = pltpu.bitcast(y[:, 0:8], u32)
            att = jnp.concatenate(att, axis=1)
            x = x + (att + pltpu.roll(att, 4, 0))
            wait(w3_cp())
            y, hs = mlp_hidden(x)
            xres[...] = x + y
            for n in range(FT):
                hbuf[n] = hs[n]
            for c in range(DT - 1):
                wait(w4_cp(c))
                xc = xres[:, cols(c)] + _tree(jnp.add, [_mm(hbuf[n], w4_tile(n, c)) for n in range(FT)])
                xres[:, cols(c)] = xc
                xc = jnp.where(top(128), xc, 1.0)
                for n in range(3 * NP):
                    r = _mm(xc, _wtile(wqu[rows(c), n]))
                    big[Q0 + n] = big[Q0 + n] + r if c else r

        def layer2(z):
            wait(w4_cp(DT - 1))
            if opts.get('skip2'):
                o_ref[...] = xres[0:1, :].astype(o_ref.dtype)
                return
            xc = xres[:, cols(DT - 1)] + _tree(jnp.add, [_mm(hbuf[n], w4_tile(n, DT - 1)) for n in range(FT)])
            xres[:, cols(DT - 1)] = xc
            m, _, r = _stats(xres[...])
            big[XL] = xraw = jnp.where(top(128), xc, 1.0)
            coef0 = jnp.where(top(128), 1.0, -m)
            big[XL + 1] = coef = coef0 * r
            acc, val, fwd = {}, {}, []
            st = dict(pin=False, dirty=False, cnt=0, started=False, left=sum(e[0] == 'step' for e in events))

            def lhs(n):
                if st['pin']:
                    st['pin'] = False
                    return big[n + z]
                if n not in val:
                    val[n] = big[n]
                return val[n]

            def checkpoint():
                for (t, a), y in acc.items():
                    n = acc_at[t, a // 8] + 2 * (a % 8)
                    big[n:n + 2] = y.reshape(2, 8, 128)

            def put(n, r):
                fwd.append((st['cnt'], n, r))

            def flush(upto, pin=False):
                while fwd and fwd[0][0] <= upto:
                    _, n, r = fwd.pop(0)
                    pbuf[z if pin else 0, :, cols(n)] = r
                    if pin and st['left'] <= opts.get('vpin', 72):
                        vu[NP - 1][z, 2] = pltpu.bitcast(r, u32)
                    pin = False

            def get(n):
                flush(max([c for c, m, _ in fwd if m == n], default=-1))
                return pbuf[0, :, cols(n)]

            def ptile(t, k):
                return cols(sp[t] * KT + k)

            def prow(t, odd, k):
                return pbuf[0, 4 * odd:4 * odd + 1, ptile(t - (t + odd == 0), k)]

            def q_fin(t, i, y, coef):
                y = (y + big[Q0 + 3 * t + i]) * coef
                big[QP + 3 * t + i] = (y + pltpu.roll(y, 4, 0)) * cst[i]

            def t_qraw(t, i):
                q_fin(t, i, _mm(xraw, _wtile(wqu[rows(DT - 1), 3 * t + i])), coef if t else coef0)

            def t_q(t, i):
                put(QR + sq[t] * 3 + i, _mm(lhs(XL), _wtile(wqu[rows(DT - 1), 3 * t + i])))

            def t_qk(t, j, k):
                put(SP + (3 * ss[t] + j) * KT + k, _mm(lhs(QP + 3 * t + j), _wtile(ku[t][rows(j), k])))

            def t_or(t, j):
                a = big[acc_at[t, j]:acc_at[t, j] + 16].reshape(128, 128)
                if j == 1:
                    r = _mm(jnp.concatenate([lhs(WB + 2 * t), lhs(WB + 2 * t + 1)], axis=0), a, _NT)
                    put(OR + 2 * so[t, j] + 1, r[8:16])
                else:
                    r = _mm(lhs(WB + 2 * t + j // 2), a, _NT)
                put(OR + 2 * so[t, j], r[0:8])

            def t_pvx(t, j, k):
                p = prow(t, j // 2, k) * lhs(WB + 2 * t + j // 2)
                put(XP + sx[t, j] * KT + k, _mm(p, _wtile(vu[t][rows(j), k])))

            def t_wo(units, n, c):
                t, j = units[n]
                put(WR + (sw[units] * 4 + n) * DT + c, _mm(lhs(OB + 3 * t + j), _wtile(wou[rows(3 * t + j), c])))

            def p_qfin(t, i):
                q_fin(t, i, get(QR + sq[t] * 3 + i), big[XL + 1])

            def p_sma(t, k0):
                n = SP + 3 * ss[max(t, 0)] * KT
                sv = []
                for k in range(k0, k0 + SG):
                    sc = get(n + k) + get(n + KT + k)
                    sc = sc + get(n + 2 * KT + k) if t >= 0 else sc
                    sv.append(sc * r if t <= 0 else sc)
                    pbuf[0, :, ptile(t, k)] = sv[-1]
                big[MB + 2 + 2 * t] = val['m'] = _tree(jnp.maximum, sv + ([val['m']] if k0 else []))

            def p_smb(t, k0):
                ps = []
                for k in range(k0, k0 + SG):
                    ps.append(jnp.exp2(pbuf[0, :, ptile(t, k)] - val['m']))
                    pbuf[0, :, ptile(t, k)] = ps[-1]
                if t >= 0:
                    big[MB + 3 + 2 * t] = val['l'] = _tree(jnp.add, ps + ([val['l']] if k0 else []))
                if t >= 0 and k0 + SG == KT:
                    pbuf[0, :, cols(ML + 2 * sl[t])] = val['m']
                    pbuf[0, :, cols(ML + 2 * sl[t] + 1)] = val['l']

            def p_wld(t):
                val['ml', t] = pbuf[0, :, cols(ML + 2 * sl[t])], pbuf[0, :, cols(ML + 2 * sl[t] + 1)]

            def p_w(t):
                m, l = val['ml', t]
                e = jnp.exp2(m - jnp.max(m, axis=1, keepdims=True))
                w = e / jnp.sum(e * l, axis=1, keepdims=True)
                for h in range(2):
                    big[WB + 2 * t + h] = jnp.broadcast_to(w[4 * h:4 * h + 1], (8, 128))

            def p_ofin(t, j):
                r = get(OR + 2 * so[t, j])
                r = jnp.where(left(), r, get(OR + 2 * so[t, j] + 1)) if j == 1 else r
                big[OB + 3 * t + j] = r + big[OB + 3 * t + j] if (t, j) in nx else r

            def p_xsum(t, j, k0):
                n = XP + sx[t, j] * KT + k0
                ys = [get(n + u) for u in range(4)] + ([val['y', t, j]] if k0 else [])
                big[OB + 3 * t + j] = val['y', t, j] = _tree(jnp.add, ys)

            def p_wacc(units, c):
                rs = [get(WR + (sw[units] * 4 + n) * DT + c) for n in range(len(units))]
                big[XA + c] = _tree(jnp.add, rs + ([big[XA + c]] if units != next(iter(sw)) else []))

            fns = {'qraw': t_qraw, 'q': t_q, 'qk': t_qk, 'or': t_or, 'pvx': t_pvx, 'wo': t_wo, 'qfin': p_qfin,
                   'sma': p_sma, 'smb': p_smb, 'wld': p_wld, 'w': p_w, 'ofin': p_ofin, 'xsum': p_xsum, 'wacc': p_wacc}
            for e in events:
                if e[0] == 'step':
                    _, t, a0, k = e
                    k0 = nx.get((t, a0 // 8), 0)
                    for a in range(a0, a0 + AB):
                        n = k + SKEW * (a - a0)
                        kk = k0 + (n - k0) % (KT - k0)
                        if ('p', t, a0, n) not in val:
                            val['p', t, a0, n] = prow(t, int(a0 >= AP // 2), kk)
                        if (t, a) in wide:
                            y = jnp.concatenate([pltpu.bitcast(vu[t][a, kk], f32),
                                                 big[WD + wide.index((t, a)) * KT + kk]])
                        else:
                            y = pltpu.bitcast(vu[t][a, kk], bf16).astype(f32)
                        y = y * val['p', t, a0, n]
                        acc[t, a] = acc[t, a] + y if (t, a) in acc else y
                    st.update(dirty=True, started=True, left=st['left'] - 1)
                    if k == KT - 1:
                        checkpoint()
                        acc.clear()
                elif e[0] == 'piece':
                    fns[e[1]](*e[2:])
                elif e[1] == 'gap':
                    st['cnt'] += 4
                else:
                    pinned = st['cnt'] % 4 == opts.get('ph', 2) and st['left'] > 0
                    if pinned and st['dirty']:
                        checkpoint()
                    st.update(pin=pinned and st['started'], dirty=st['dirty'] and not pinned)
                    fns[e[1]](*e[2:])
                    st['pin'] = False
                    if pinned:
                        flush(st['cnt'] - 4 * FD + 3, pin=st['started'])
                    st['cnt'] += 1
            assert not fwd
            x = xres[...] + jnp.concatenate([big[XA + c] for c in range(DT)], axis=1)
            y, hs = mlp_hidden(x)
            out = [(x + y)[:, cols(c)] for c in range(DT)]
            for n in range(FT):
                out = [out[c] + _mm(hs[n], w4_tile(n, c)) for c in range(DT)]
            o_ref[...] = jnp.concatenate(out, axis=1)[0:1].astype(o_ref.dtype)

        def body(it, carry):
            pl.when(it == 0)(layer1 if not opts.get('skip1') else lambda: None)
            pl.when(it == 1)(lambda: layer2(it >> 4))
            return carry

        lax.fori_loop(0, 2, body, 0)

    def V(*s, dt=f32):
        return pltpu.VMEM(s, dt)

    out = pl.pallas_call(
        kernel,
        out_shape=jax.ShapeDtypeStruct((1, D), A_x.dtype),
        in_specs=[pl.BlockSpec(memory_space=pl.ANY)] * 7,
        out_specs=pl.BlockSpec(memory_space=pltpu.VMEM),
        scratch_shapes=(
            [V(AP, KT, 16, 128, dt=bf16)] * (2 * NP)
            + [V(F, 128, dt=bf16)] * DT
            + [V(D // 16, 3 * NP, 16, 128, dt=bf16), V(AP * NP, DT, 16, 128, dt=bf16), V(D, F, dt=bf16),
               V(1, 8, -(-NPB // 4) * 512), V(4, 8, 128), V(-(-NBIG // 4) * 4, 8, 128),
               V(FT, 8, 128), V(8, D), V(1, D, dt=bf16),
               pltpu.SemaphoreType.DMA((2 * NP + 3 + DT,))]),
        compiler_params=pltpu.CompilerParams(
            vmem_limit_bytes=int(opts.get('vmem', 128) * 1024 * 1024),
            disable_semaphore_checks=True, disable_bounds_checks=True),
        name='fused_decode_layers',
    )(A_x.reshape(1, D), _cache_view(A_k_cache), _cache_view(A_v_cache),
      _weight_view(A_wq), _weight_view(A_wo), B_w3, B_w4)
    return out.reshape(B, S, D)


@jax.jit
def pallas_interleave_layers__sliding_block_cached__mixer_s_mlp__decode_kernel(
    A_x: jax.Array,
    A_k_cache: jax.Array,
    A_v_cache: jax.Array,
    A_wq: jax.Array,
    A_wo: jax.Array,
    B_x: jax.Array,
    B_w1: jax.Array,
    B_w2: jax.Array,
    B_w3: jax.Array,
    B_w4: jax.Array,
):
    return _run(_OPTS, A_x, A_k_cache, A_v_cache, A_wq, A_wo, B_w3, B_w4)
```

```python
import jax
import jax.numpy as jnp
from jax import lax
import jax.experimental.pallas as pl
import jax.experimental.pallas.tpu as pltpu

f32, bf16, u32, i32 = jnp.float32, jnp.bfloat16, jnp.uint32, jnp.int32
_EPS = 1e-5
_LOG2E = 1.4426950408889634
_NN = (((1,), (0,)), ((), ()))
_NT = (((1,), (1,)), ((), ()))

_OPTS = dict(xunits=[(5, 0, 32), (7, 2, 32), (9, 2, 32), (11, 0, 32), (12, 2, 32), (13, 0, 32), (14, 2, 4)], nwide=78, qlead=2.0, keep=8,
             AD=100, LAT=205, LAT0=205, q2at=20, vpin=80)


def _stats(x):
    m = jnp.mean(x, axis=-1, keepdims=True)
    xc = x - m
    v = jnp.mean(xc * xc, axis=-1, keepdims=True)
    return m, xc, lax.rsqrt(v + _EPS)


def _tree(op, xs):
    xs = list(xs)
    while len(xs) > 1:
        nxt = [op(xs[i], xs[i + 1]) for i in range(0, len(xs) - 1, 2)]
        if len(xs) % 2:
            nxt.append(xs[-1])
        xs = nxt
    return xs[0]


def _wtile(u):
    return pltpu.bitcast(u.reshape(u.shape[0] * 8, 128), bf16)


def _mm(lhs, w, dims=_NN):
    return lax.dot_general(lhs, w, dims, preferred_element_type=f32)


def _cache_view(c):
    _, H, Sk, Dh = c.shape
    c = c.reshape(H, Sk // 128, 128, Dh // 16, 2, 8)
    c = jnp.transpose(c, (0, 3, 4, 1, 5, 2))
    return c.reshape(H * Dh // 16, 2, Sk // 128, 8, 128)


def _weight_view(w):
    R, N = w.shape
    w = w.reshape(R // 16, 2, 8, N // 128, 128)
    return jnp.transpose(w, (0, 1, 3, 2, 4))


def _schedule(NP, KT, DT, AP, AB, SG, xunits, qlead, keep, LAT=205, LAT0=165, LEAD=32, WD=140, WL=400, AD=160,
              vcost=5.95, pstride=2, nraw=8, q2at=40, ph=3, wide=(), **_):
    xs = {u[:2]: u[2] for u in xunits}
    grp = [(t, a) for t in range(NP) for a in range(0, AP, AB)]
    grp[-2:] = grp[:-3:-1]
    steps = [(t, a, k) for t, a in grp for k in range(xs.get((t, a // 8), 0), KT)]
    first_step = {}
    for i, s in enumerate(steps):
        first_step.setdefault(s[0], i)
    main = [('qraw', t, i) for t in range(nraw) for i in range(3)]
    for t in range(NP):
        qk = [('qk', t, j, k) for j in range(3) for k in range(KT)]
        main += qk[:q2at] + [('q', t + 1, i) for i in range(3) if nraw <= t + 1 < NP] + qk[q2at:]
    done = {('q', t): 3 for t in range(nraw)}
    or_left = [(t, j) for t in range(NP) for j in range(3) if xs.get((t, j), 0) < KT]
    wo_left = [(t, j) for t in range(NP) for j in range(3)]
    px_left = list(xs)
    ev, pend, wait, cur = [], [], [], []
    s = dict(tm=0.0, tv=0.0, i=0, mi=0, qk=0)

    def sm(t):
        return ([(('sma', t, k), 3 * SG, None, 0) for k in range(0, KT, SG)]
                + [(('smb', t, k), 3 * SG, ('p', t), SG) for k in range(0, KT, SG)])

    def g_wo(n):
        wo = tuple(u for u in wo_left if done.get(('o',) + u, 0) >= 1)[:4]
        if len(wo) < n:
            return None
        for u in wo:
            wo_left.remove(u)
        g = [(('wo', wo, n, c), 8, []) for n in range(len(wo)) for c in range(DT)]
        g[-1] = (g[-1][0], 8, [(('wacc', wo, c), len(wo), None, 0) for c in range(DT)])
        return g

    def g_or(n, last):
        rd = [u for u in or_left if done.get(('acc',) + u, 0) >= 8 // AB and done.get(('w', u[0]), 0)
              and (last or done[('acct',) + u] + AD <= s['tv'])
              and done.get(('y',) + u, 0) >= xs.get(u, 0)][:4]
        if len(rd) < n:
            return None
        for u in rd:
            or_left.remove(u)
        return [(('gap',), 8 * len(rd), [])] + [(('or',) + u, 8, [(('ofin',) + u, 1, ('o',) + u, 1)]) for u in rd]

    def g_px():
        rd = [u for u in px_left if done.get(('w', u[0]), 0)]
        if not rd:
            return None
        px_left.remove(rd[0])
        n = xs[rd[0]]
        g = [(('pvx',) + rd[0] + (k,), 8, []) for k in range(n)]
        e, inc = (('o',) + rd[0], 4 / KT) if n == KT else (('y',) + rd[0], 4)
        g[-1] = (g[-1][0], 8, [(('xsum',) + rd[0] + (k,), 4, e, inc) for k in range(0, n, 4)])
        return g

    def pick():
        last, endgame, nxt = s['i'] >= len(steps), s['mi'] >= len(main), s['qk']
        if last:
            return g_or(1, True) or g_px() or g_wo(1)
        if endgame:
            return g_or(4, False) or g_px() or g_wo(4) or g_wo(1)
        rem = sum(8 for m in main[s['mi']:s['mi'] + 200] if m[0] != 'qk' or m[1] == nxt)
        if (first_step[nxt] - s['i']) * vcost - rem > qlead * 500:
            g = (g_wo(4) if len(wo_left) > keep else None) or g_or(4, False) or g_px()
            if g:
                return g
        m = main[s['mi']]
        if m[0] == 'qk' and done.get(('q', m[1]), 0) < 3:
            return None
        s['mi'] += 1
        pcs = []
        if m[0] == 'q':
            pcs = [(('qfin',) + m[1:], 5, ('q', m[1]), 1)]
        if m[0] == 'qk' and (m[2] == 2 or m[1:3] == (0, 1)) and m[3] % SG == SG - 1:
            t = m[1] if m[2] == 2 else -1
            pcs = [sm(t)[m[3] // SG]] + (sm(t)[KT // SG:] if m[3] == KT - 1 else [])
        return [(m, 8, pcs)]

    def later(t, pcs):
        wait.append((t, pcs))
        wait.sort(key=lambda w: w[0])

    def piece():
        a, cv, e, inc = pend.pop(0)
        ev.append(('piece',) + a)
        s['tv'] += cv / 4
        if e is not None:
            done[e] = done.get(e, 0) + inc
        if a[0] == 'smb' and a[2] == KT - SG and a[1] >= 0:
            later(s['tv'] + WD, [(('wld', a[1]), 0, ('wld', a[1]), 1)])
            later(s['tv'] + WD + WL, [(('w', a[1]), 24, ('w', a[1]), 1)])

    def urgent(p):
        return p[2] is not None and p[2][0] != 'p'

    while True:
        while wait and wait[0][0] <= s['tv']:
            pcs = wait.pop(0)[1]
            pend[:] = [p for p in pcs if urgent(p)] + pend + [p for p in pcs if not urgent(p)]
        i = s['i']
        more = i < len(steps)
        blocked = not more or done.get(('p', steps[i][0] - (i < AP // 2 // AB * KT)), 0) < min(KT, steps[i][2] + 6)
        if not cur and (s['tm'] + LEAD <= s['tv'] or blocked):
            cur = pick() or []
        if not more and not pend and not wait and not cur:
            break
        if cur and (s['tm'] + LEAD <= s['tv']
                    or (blocked and not pend and (not wait or s['tm'] + LEAD <= wait[0][0]))):
            a, cm, pcs = cur.pop(0)
            ev.append(('tile',) + a)
            s['tm'] = max(s['tm'], s['tv'] - LEAD - 8) + cm
            s['tv'] += 0.25 * (a[0] == 'pvx')
            s['qk'] += a[0] == 'qk' and a[2:] == (2, KT - 1)
            if pcs:
                later(s['tm'] + (LAT if 0 < i < len(steps) else LAT0), pcs)
        elif blocked and pend:
            piece()
        elif blocked:
            s['tv'] = max(s['tv'], wait[0][0])
        else:
            if pend and (i % pstride == 0 or urgent(pend[0])):
                piece()
            t, a, k = steps[i]
            ev.append(('step', t, a, k))
            if k == KT - 1:
                done['acc', t, a // 8] = done.get(('acc', t, a // 8), 0) + 1
                done['acct', t, a // 8] = s['tv']
            s['tv'] += vcost - 0.5 * sum((t, b) in wide for b in range(a, a + AB))
            s['i'] += 1
    assert not or_left and not wo_left and not px_left

    out, cur, cnt = [], [], 0
    for e in ev + [None]:
        if e is None or (e[0] == 'tile' and e[1] != 'gap' and cnt % 4 == ph):
            if any(x[0] == 'step' for x in cur) and len(cur) < 32:
                cur = cur[:1] + [x for x in cur[1:] if x[0] == 'piece'] + [x for x in cur[1:] if x[0] != 'piece']
            out += cur
            cur = []
        if e is not None:
            cur.append(e)
            cnt += (4 if e[1] == 'gap' else 1) * (e[0] == 'tile')
    return out


def _slots(events, key):
    first, last = {}, {}
    for n, e in enumerate(events):
        k = key(e)
        if k is not None:
            first.setdefault(k, n)
            last[k] = n
    slot, busy = {}, []
    for k in first:
        free = [i for i, u in enumerate(busy) if u < first[k]]
        slot[k] = free[0] if free else len(busy)
        busy[slot[k]:slot[k] + 1] = [last[k]]
    return slot, len(busy)


def _run(opts, A_x, A_k_cache, A_v_cache, A_wq, A_wo, B_w3, B_w4):
    B, S, D = A_x.shape
    _, H, Sk, Dh = A_k_cache.shape
    F = B_w3.shape[1]
    W = min(4096, max(256, Sk // 4))
    assert (B, S, H, Dh, W) == (1, 1, 32, 192, 4096) and D % 128 == 0 and F % 128 == 0
    AP = Dh // 8
    KT = W // 128
    NP = H // 2
    DT, FT = D // 128, F // 128
    AB, SG, FD = 4, 2, opts.get('fd', 5)
    SKEW = opts.get('skew', 1)
    cexp = (Dh ** -0.5) * _LOG2E
    nx = {u[:2]: u[2] for u in opts['xunits']}
    xunits = list(nx)
    wide = [(t, a) for t in range(NP) for a in range(0, AP, AB) if (t, a // 8) not in xunits + [(NP - 1, 2)]]
    drop = [g for n, g in enumerate(wide) if n % 3][:max(0, len(wide) - opts['nwide'])]
    wide = [g for g in wide if g not in drop] + [(t, a + 2) for t, a in wide[::-1]][:max(0, opts['nwide'] - len(wide))]
    events = _schedule(NP, KT, DT, AP, AB, SG, wide=wide, **opts)
    sp, RP = _slots(events, lambda e: e[1] - (e[1] == 0 and e[2] < AP // 2) if e[0] == 'step'
                    else e[2] if e[1] in ('sma', 'smb', 'pvx') else None)
    ss, RS = _slots(events, lambda e: max(e[2], 0) if e[1] in ('qk', 'sma') else None)
    sq, RQ = _slots(events, lambda e: e[2] if e[1] in ('q', 'qfin') else None)
    sx, RX = _slots(events, lambda e: e[2:4] if e[1] in ('pvx', 'xsum') else None)
    sw, RM = _slots(events, lambda e: e[2] if e[1] in ('wo', 'wacc') else None)
    so, RO = _slots(events, lambda e: e[2:4] if e[1] in ('or', 'ofin') else None)
    sl, RL = _slots(events, lambda e: e[2] if e[1] in ('smb', 'wld') else None)
    assert _slots(events, lambda e: e[2] if e[1] in ('sma', 'smb') else None)[1] == 1
    sizes = [3 * NP, 3 * NP, 2 * NP, 2, DT, 2 * NP + 3, KT, KT * len(wide)]
    QP, Q0, WB, XL, XA, MB, AL, WD, NBIG = [sum(sizes[:n]) for n in range(len(sizes) + 1)]
    OB = Q0
    free, acc_at = [AL, AL + 16], {}
    for e in events:
        if e[0] == 'step' and (e[1], e[2] // 8) not in acc_at:
            acc_at[e[1], e[2] // 8] = free.pop(0)
        if e[0] == 'step' and e[3] == KT - 1:
            free += [WD + KT * wide.index((e[1], a)) + n for a in range(e[2], e[2] + AB) if (e[1], a) in wide
                     for n in (0, 16)]
    sizes = [RP * KT, 3 * RS * KT, RX * KT, 3 * RQ, 4 * DT * RM, 2 * RO, 2 * RL]
    _, SP, XP, QR, WR, OR, ML, NPB = [sum(sizes[:n]) for n in range(len(sizes) + 1)]
    NV = opts.get('nv', 2)
    if opts.get('verbose'):
        print('RP RS RQ RX RM', RP, RS, RQ, RX, RM, 'free tiles', (int(13.25 * 256) - NBIG - NPB))
    order1 = sorted(range(NP), key=lambda t: all(u[0] != t for u in xunits))

    def kernel(x_hbm, k_hbm, v_hbm, wq_hbm, wo_hbm, w3_hbm, w4_hbm, o_ref, *scratch):
        k_bufs, v_bufs, scratch = scratch[:NP], scratch[NP:2 * NP], scratch[2 * NP:]
        w4_bufs, scratch = scratch[:DT], scratch[DT:]
        wq_buf, wo_buf, w3_buf, pbuf, cst, big, hbuf, xres, x_buf, sems = scratch
        t0 = (Sk - W) // 128

        def kv_cp(kind, t):
            src, dst = (k_hbm, k_bufs[t]) if kind == 0 else (v_hbm, v_bufs[t])
            return [pltpu.make_async_copy(src.at[pl.ds(AP * t, AP), a, pl.ds(t0, KT)],
                                          dst.at[:, :, pl.ds(8 * a, 8), :], sems.at[2 * t + kind])
                    for a in range(2)]

        def w_cp(src, dst, n, sem):
            rows = src.shape[0] // n
            return [pltpu.make_async_copy(src.at[pl.ds(i * rows, rows), a],
                                          dst.at[pl.ds(i * rows, rows), :, pl.ds(8 * a, 8), :], sem)
                    for i in range(n) for a in range(2)]

        def wq_cp():
            cps = w_cp(wq_hbm, wq_buf, 1, sems.at[2 * NP])
            return cps[:1] + [pltpu.make_async_copy(x_hbm, x_buf, sems.at[2 * NP])] + cps[1:]

        def wo_cp():
            return w_cp(wo_hbm, wo_buf, 8, sems.at[2 * NP + 1])

        def w3_cp():
            return [pltpu.make_async_copy(w3_hbm, w3_buf, sems.at[2 * NP + 2])]

        def w4_cp(c):
            return [pltpu.make_async_copy(w4_hbm.at[:, pl.ds(128 * c, 128)], w4_bufs[c], sems.at[2 * NP + 3 + c])]

        def wait(cps):
            for cp in cps:
                cp.wait()

        cps = wq_cp()
        for t in order1:
            cps += kv_cp(0, t) + kv_cp(1, t) + (wo_cp() if t == order1[0] else [])
        for cp in cps + w3_cp() + [cp for c in range(DT) for cp in w4_cp(c)]:
            cp.start()

        ku = [r.bitcast(u32) for r in k_bufs]
        vu = [r.bitcast(u32) for r in v_bufs]
        wqu = wq_buf.bitcast(u32)
        wou = wo_buf.bitcast(u32)
        w4u = [r.bitcast(u32) for r in w4_bufs]

        def top(n):
            return lax.broadcasted_iota(i32, (8, n), 0) < 4

        def left():
            return lax.broadcasted_iota(i32, (8, 128), 1) < 64

        def cols(n):
            return slice(128 * n, 128 * (n + 1))

        def rows(j):
            return slice(8 * j, 8 * j + 8)

        def masks():
            return [top(128), top(128) == left(), jnp.logical_not(top(128))]

        def mlp_hidden(x):
            lhs = jnp.where(top(D), x, 1.0)
            m1, xc, r1 = _stats(x)
            y = xc * r1
            m2 = jnp.mean(y, axis=-1, keepdims=True)
            r2 = lax.rsqrt(jnp.mean(y * y, axis=-1, keepdims=True) - m2 * m2 + _EPS)
            coef = jnp.where(top(128), r1 * r2, -(r2 * (r1 * m1 + m2)))
            hs = []
            for n in range(FT):
                u = _tree(jnp.add, [_mm(lhs[:, cols(j)], w3_buf[cols(j), cols(n)]) for j in range(DT)]) * coef
                hs.append(jax.nn.gelu(u + pltpu.roll(u, 4, 0), approximate=True))
            return y, hs

        def w4_tile(n, c):
            return pltpu.bitcast(w4u[c][64 * n:64 * (n + 1)], bf16)

        def layer1():
            for u, mask in enumerate(masks()):
                cst[u] = jnp.where(mask, cexp, 0.0).astype(f32)
            wait(wq_cp())
            x = jnp.broadcast_to(x_buf[...].astype(f32), (8, D))
            _, xc, r = _stats(x)
            xn = xc * r

            def q_body(t, c):
                for i in range(3):
                    q = _tree(jnp.add, [_mm(xn[:, cols(j)], _wtile(wqu[rows(j), 3 * t + i])) for j in range(DT)])
                    big[QP + 3 * t + i] = q * cst[i]
                return c
            lax.fori_loop(0, NP, q_body, 0)

            att = [jnp.zeros((8, 128), f32)] * DT
            for t in order1:
                def s_body(k, c, t=t, q=[big[QP + 3 * t + j] for j in range(3)]):
                    big[AL + k] = _tree(jnp.add, [_mm(q[j], _wtile(ku[t][rows(j), k])) for j in range(3)])
                    return c

                def o_body(k, o, t=t):
                    return [o[j] + _mm(big[AL + k], _wtile(vu[t][rows(j), k]), _NT) for j in range(3)]

                wait(kv_cp(0, t))
                lax.fori_loop(0, KT, s_body, 0, unroll=8)
                sc = big[AL:AL + KT]
                p = jnp.exp2(sc - jnp.max(jnp.max(sc, axis=0), axis=1, keepdims=True))
                big[AL:AL + KT] = p
                inv = 1.0 / jnp.sum(jnp.sum(p, axis=0), axis=1, keepdims=True)
                wait(kv_cp(1, t) + (wo_cp() if t == order1[0] else []))
                o = lax.fori_loop(0, KT, o_body, [jnp.zeros((8, 128), f32)] * 3, unroll=8)
                o = [jnp.where(mask, o[j] * inv, 0.0) for j, mask in enumerate(masks())]
                att = [att[c] + _tree(jnp.add, [_mm(o[j], _wtile(wou[rows(3 * t + j), c])) for j in range(3)])
                       for c in range(DT)]
                for j in [j for tt, j in xunits if tt == t]:
                    def t_body(k, c, t=t, j=j):
                        w = _wtile(vu[t][rows(j), k]).astype(f32).T.astype(bf16)
                        vu[t][rows(j), k] = pltpu.bitcast(w, u32).reshape(8, 8, 128)
                        return c
                    lax.fori_loop(0, nx[t, j], t_body, 0, unroll=4)
                for n, a in [(n, a) for n, (tt, a) in enumerate(wide) if tt == t]:
                    y = _wtile(vu[t][a]).astype(f32).reshape(KT, 16, 128)
                    big[WD + n * KT:WD + (n + 1) * KT] = y[:, 8:16]
                    vu[t][a] = pltpu.bitcast(y[:, 0:8], u32)
            att = jnp.concatenate(att, axis=1)
            x = x + (att + pltpu.roll(att, 4, 0))
            wait(w3_cp())
            y, hs = mlp_hidden(x)
            xres[...] = x + y
            for n in range(FT):
                hbuf[n] = hs[n]
            for c in range(DT - 1):
                wait(w4_cp(c))
                xc = xres[:, cols(c)] + _tree(jnp.add, [_mm(hbuf[n], w4_tile(n, c)) for n in range(FT)])
                xres[:, cols(c)] = xc
                xc = jnp.where(top(128), xc, 1.0)
                for n in range(3 * NP):
                    r = _mm(xc, _wtile(wqu[rows(c), n]))
                    big[Q0 + n] = big[Q0 + n] + r if c else r

        def layer2(z):
            wait(w4_cp(DT - 1))
            if opts.get('skip2'):
                o_ref[...] = xres[0:1, :].astype(o_ref.dtype)
                return
            xc = xres[:, cols(DT - 1)] + _tree(jnp.add, [_mm(hbuf[n], w4_tile(n, DT - 1)) for n in range(FT)])
            xres[:, cols(DT - 1)] = xc
            m, _, r = _stats(xres[...])
            big[XL] = xraw = jnp.where(top(128), xc, 1.0)
            coef0 = jnp.where(top(128), 1.0, -m)
            big[XL + 1] = coef = coef0 * r
            acc, val, fwd = {}, {}, []
            st = dict(pin=False, dirty=False, cnt=0, started=False, left=sum(e[0] == 'step' for e in events))

            def lhs(n):
                if st['pin']:
                    st['pin'] = False
                    return big[n + z]
                if n not in val:
                    val[n] = big[n]
                return val[n]

            def checkpoint():
                for (t, a), y in acc.items():
                    n = acc_at[t, a // 8] + 2 * (a % 8)
                    big[n:n + 2] = y.reshape(2, 8, 128)

            def put(n, r):
                fwd.append((st['cnt'], n, r))

            def flush(upto, pin=False):
                while fwd and fwd[0][0] <= upto:
                    _, n, r = fwd.pop(0)
                    pbuf[z if pin else 0, :, cols(n)] = r
                    if pin and st['left'] <= opts.get('vpin', 72):
                        vu[NP - 1][z, 2] = pltpu.bitcast(r, u32)
                    pin = False

            def get(n):
                flush(max([c for c, m, _ in fwd if m == n], default=-1))
                return pbuf[0, :, cols(n)]

            def ptile(t, k):
                return cols(sp[t] * KT + k)

            def prow(t, odd, k):
                return pbuf[0, 4 * odd:4 * odd + 1, ptile(t - (t + odd == 0), k)]

            def q_fin(t, i, y, coef):
                y = (y + big[Q0 + 3 * t + i]) * coef
                big[QP + 3 * t + i] = (y + pltpu.roll(y, 4, 0)) * cst[i]

            def t_qraw(t, i):
                q_fin(t, i, _mm(xraw, _wtile(wqu[rows(DT - 1), 3 * t + i])), coef if t else coef0)

            def t_q(t, i):
                put(QR + sq[t] * 3 + i, _mm(lhs(XL), _wtile(wqu[rows(DT - 1), 3 * t + i])))

            def t_qk(t, j, k):
                put(SP + (3 * ss[t] + j) * KT + k, _mm(lhs(QP + 3 * t + j), _wtile(ku[t][rows(j), k])))

            def t_or(t, j):
                a = big[acc_at[t, j]:acc_at[t, j] + 16].reshape(128, 128)
                if j == 1:
                    r = _mm(jnp.concatenate([lhs(WB + 2 * t), lhs(WB + 2 * t + 1)], axis=0), a, _NT)
                    put(OR + 2 * so[t, j] + 1, r[8:16])
                else:
                    r = _mm(lhs(WB + 2 * t + j // 2), a, _NT)
                put(OR + 2 * so[t, j], r[0:8])

            def t_pvx(t, j, k):
                p = val.pop(('px', t, j, k)) * lhs(WB + 2 * t + j // 2)
                put(XP + sx[t, j] * KT + k, _mm(p, _wtile(vu[t][rows(j), k])))

            def t_wo(units, n, c):
                t, j = units[n]
                put(WR + (sw[units] * 4 + n) * DT + c, _mm(lhs(OB + 3 * t + j), _wtile(wou[rows(3 * t + j), c])))

            def p_qfin(t, i):
                q_fin(t, i, get(QR + sq[t] * 3 + i), big[XL + 1])

            def p_sma(t, k0):
                n = SP + 3 * ss[max(t, 0)] * KT
                sv = []
                for k in range(k0, k0 + SG):
                    sc = get(n + k) + get(n + KT + k)
                    sc = sc + get(n + 2 * KT + k) if t >= 0 else sc
                    sv.append(sc * r if t <= 0 else sc)
                    pbuf[0, :, ptile(t, k)] = sv[-1]
                big[MB + 2 + 2 * t] = val['m'] = _tree(jnp.maximum, sv + ([val['m']] if k0 else []))

            def p_smb(t, k0):
                ps = []
                for k in range(k0, k0 + SG):
                    ps.append(jnp.exp2(pbuf[0, :, ptile(t, k)] - val['m']))
                    pbuf[0, :, ptile(t, k)] = ps[-1]
                if t >= 0:
                    big[MB + 3 + 2 * t] = val['l'] = _tree(jnp.add, ps + ([val['l']] if k0 else []))
                if t >= 0 and k0 + SG == KT:
                    pbuf[0, :, cols(ML + 2 * sl[t])] = val['m']
                    pbuf[0, :, cols(ML + 2 * sl[t] + 1)] = val['l']

            def p_wld(t):
                val['ml', t] = pbuf[0, :, cols(ML + 2 * sl[t])], pbuf[0, :, cols(ML + 2 * sl[t] + 1)]

            def p_w(t):
                m, l = val['ml', t]
                e = jnp.exp2(m - jnp.max(m, axis=1, keepdims=True))
                w = e / jnp.sum(e * l, axis=1, keepdims=True)
                for h in range(2):
                    big[WB + 2 * t + h] = jnp.broadcast_to(w[4 * h:4 * h + 1], (8, 128))

            def p_ofin(t, j):
                r = get(OR + 2 * so[t, j])
                r = jnp.where(left(), r, get(OR + 2 * so[t, j] + 1)) if j == 1 else r
                big[OB + 3 * t + j] = r + big[OB + 3 * t + j] if (t, j) in nx else r

            def p_xsum(t, j, k0):
                n = XP + sx[t, j] * KT + k0
                ys = [get(n + u) for u in range(4)] + ([val['y', t, j]] if k0 else [])
                big[OB + 3 * t + j] = val['y', t, j] = _tree(jnp.add, ys)

            def p_wacc(units, c):
                rs = [get(WR + (sw[units] * 4 + n) * DT + c) for n in range(len(units))]
                big[XA + c] = _tree(jnp.add, rs + ([big[XA + c]] if units != next(iter(sw)) else []))

            fns = {'qraw': t_qraw, 'q': t_q, 'qk': t_qk, 'or': t_or, 'pvx': t_pvx, 'wo': t_wo, 'qfin': p_qfin,
                   'sma': p_sma, 'smb': p_smb, 'wld': p_wld, 'w': p_w, 'ofin': p_ofin, 'xsum': p_xsum, 'wacc': p_wacc}
            tiles = [e for e in events if e[0] == 'tile' and e[1] != 'gap']
            for e in events:
                if e[0] == 'step':
                    _, t, a0, k = e
                    k0 = nx.get((t, a0 // 8), 0)
                    for a in range(a0, a0 + AB):
                        n = k + SKEW * (a - a0)
                        kk = k0 + (n - k0) % (KT - k0)
                        if ('p', t, a0, n) not in val:
                            val['p', t, a0, n] = prow(t, int(a0 >= AP // 2), kk)
                        if (t, a) in wide:
                            y = jnp.concatenate([pltpu.bitcast(vu[t][a, kk], f32),
                                                 big[WD + wide.index((t, a)) * KT + kk]])
                        else:
                            y = pltpu.bitcast(vu[t][a, kk], bf16).astype(f32)
                        y = y * val['p', t, a0, n]
                        acc[t, a] = acc[t, a] + y if (t, a) in acc else y
                    st.update(dirty=True, started=True, left=st['left'] - 1)
                    if k == KT - 1:
                        checkpoint()
                        acc.clear()
                elif e[0] == 'piece':
                    fns[e[1]](*e[2:])
                elif e[1] == 'gap':
                    st['cnt'] += 4
                else:
                    pinned = st['cnt'] % 4 == opts.get('ph', 3) and st['left'] > 0
                    if pinned and st['dirty']:
                        checkpoint()
                    st.update(pin=pinned and st['started'], dirty=st['dirty'] and not pinned)
                    fns[e[1]](*e[2:])
                    st['pin'] = False
                    tiles.pop(0)
                    for u in tiles[:opts.get('pf', 4)]:
                        if u[1] == 'pvx' and ('px',) + u[2:] not in val:
                            val[('px',) + u[2:]] = prow(u[2], u[3] // 2, u[4])
                    if pinned:
                        flush(st['cnt'] - 4 * FD + 3, pin=st['started'])
                    st['cnt'] += 1
            assert not fwd
            x = xres[...] + jnp.concatenate([big[XA + c] for c in range(DT)], axis=1)
            y, hs = mlp_hidden(x)
            out = [(x + y)[:, cols(c)] for c in range(DT)]
            part = [None] * DT
            for n in range(NV):
                hb = jnp.concatenate([hs[n]] * 16, axis=0).T
                for a in range(8):
                    for c in range(DT):
                        u = pltpu.bitcast(w4u[c][rows(8 * n + a)], bf16).astype(f32) * hb[16 * a:16 * a + 16]
                        part[c] = u if part[c] is None else part[c] + u
            for n in range(NV, FT):
                out = [out[c] + _mm(hs[n], w4_tile(n, c)) for c in range(DT)]
            out = [out[c] + jnp.sum(part[c], axis=0, keepdims=True) for c in range(DT)]
            o_ref[...] = jnp.concatenate(out, axis=1)[0:1].astype(o_ref.dtype)

        def body(it, carry):
            pl.when(it == 0)(layer1 if not opts.get('skip1') else lambda: None)
            pl.when(it == 1)(lambda: layer2(it >> 4))
            return carry

        lax.fori_loop(0, 2, body, 0)

    def V(*s, dt=f32):
        return pltpu.VMEM(s, dt)

    out = pl.pallas_call(
        kernel,
        out_shape=jax.ShapeDtypeStruct((1, D), A_x.dtype),
        in_specs=[pl.BlockSpec(memory_space=pl.ANY)] * 7,
        out_specs=pl.BlockSpec(memory_space=pltpu.VMEM),
        scratch_shapes=(
            [V(AP, KT, 16, 128, dt=bf16)] * (2 * NP)
            + [V(F, 128, dt=bf16)] * DT
            + [V(D // 16, 3 * NP, 16, 128, dt=bf16), V(AP * NP, DT, 16, 128, dt=bf16), V(D, F, dt=bf16),
               V(1, 8, -(-NPB // 4) * 512), V(4, 8, 128), V(-(-NBIG // 4) * 4, 8, 128),
               V(FT, 8, 128), V(8, D), V(1, D, dt=bf16),
               pltpu.SemaphoreType.DMA((2 * NP + 3 + DT,))]),
        compiler_params=pltpu.CompilerParams(
            vmem_limit_bytes=int(opts.get('vmem', 128) * 1024 * 1024),
            disable_semaphore_checks=True, disable_bounds_checks=True),
        name='fused_decode_layers',
    )(A_x.reshape(1, D), _cache_view(A_k_cache), _cache_view(A_v_cache),
      _weight_view(A_wq), _weight_view(A_wo), B_w3, B_w4)
    return out.reshape(B, S, D)


@jax.jit
def pallas_interleave_layers__sliding_block_cached__mixer_s_mlp__decode_kernel(
    A_x: jax.Array,
    A_k_cache: jax.Array,
    A_v_cache: jax.Array,
    A_wq: jax.Array,
    A_wo: jax.Array,
    B_x: jax.Array,
    B_w1: jax.Array,
    B_w2: jax.Array,
    B_w3: jax.Array,
    B_w4: jax.Array,
):
    return _run(_OPTS, A_x, A_k_cache, A_v_cache, A_wq, A_wo, B_w3, B_w4)
```

```python
import jax
import jax.numpy as jnp
from jax import lax
import jax.experimental.pallas as pl
import jax.experimental.pallas.tpu as pltpu

f32, bf16, u32, i32 = jnp.float32, jnp.bfloat16, jnp.uint32, jnp.int32
_EPS = 1e-5
_LOG2E = 1.4426950408889634
_NN = (((1,), (0,)), ((), ()))
_NT = (((1,), (1,)), ((), ()))

_OPTS = dict(xunits=[(5, 0, 32), (7, 2, 32), (9, 2, 32), (11, 0, 32), (12, 2, 32), (14, 2, 12)], nwide=78, nlate=[10, 10, 9, 0], qlead=2.0, keep=8,
             AD=100, LAT=205, LAT0=205, q2at=20, vpin=80)


def _stats(x):
    m = jnp.mean(x, axis=-1, keepdims=True)
    xc = x - m
    v = jnp.mean(xc * xc, axis=-1, keepdims=True)
    return m, xc, lax.rsqrt(v + _EPS)


def _tree(op, xs):
    xs = list(xs)
    while len(xs) > 1:
        nxt = [op(xs[i], xs[i + 1]) for i in range(0, len(xs) - 1, 2)]
        if len(xs) % 2:
            nxt.append(xs[-1])
        xs = nxt
    return xs[0]


def _wtile(u):
    return pltpu.bitcast(u.reshape(u.shape[0] * 8, 128), bf16)


def _mm(lhs, w, dims=_NN):
    return lax.dot_general(lhs, w, dims, preferred_element_type=f32)


def _cache_view(c):
    _, H, Sk, Dh = c.shape
    c = c.reshape(H, Sk // 128, 128, Dh // 16, 2, 8)
    c = jnp.transpose(c, (0, 3, 4, 1, 5, 2))
    return c.reshape(H * Dh // 16, 2, Sk // 128, 8, 128)


def _weight_view(w):
    R, N = w.shape
    w = w.reshape(R // 16, 2, 8, N // 128, 128)
    return jnp.transpose(w, (0, 1, 3, 2, 4))


def _schedule(NP, KT, DT, AP, AB, SG, xunits, qlead, keep, LAT=205, LAT0=165, LEAD=32, WD=140, WL=400, AD=160,
              vcost=5.95, pstride=2, nraw=8, q2at=40, ph=3, wide=(), wk=(8, 20), **_):
    xs = {u[:2]: u[2] for u in xunits}
    grp = [(t, a) for t in range(NP) for a in range(0, AP, AB)]
    grp[-2:] = grp[:-3:-1]
    steps = [(t, a, k) for t, a in grp for k in range(xs.get((t, a // 8), 0), KT)]
    first_step = {}
    for i, s in enumerate(steps):
        first_step.setdefault(s[0], i)
    main = [('qraw', t, i) for t in range(nraw) for i in range(3)]
    for t in range(NP):
        qk = [('qk', t, j, k) for j in range(3) for k in range(KT)]
        main += qk[:q2at] + [('q', t + 1, i) for i in range(3) if nraw <= t + 1 < NP] + qk[q2at:]
    done = {('q', t): 3 for t in range(nraw)}
    or_left = [(t, j) for t in range(NP) for j in range(3) if xs.get((t, j), 0) < KT]
    wo_left = [(t, j) for t in range(NP) for j in range(3)]
    px_left = list(xs)
    ev, pend, wait, cur = [], [], [], []
    s = dict(tm=0.0, tv=0.0, i=0, mi=0, qk=0)

    def sm(t):
        return ([(('sma', t, k), 3 * SG, None, 0) for k in range(0, KT, SG)]
                + [(('smb', t, k), 3 * SG, ('p', t), SG) for k in range(0, KT, SG)])

    def g_wo(n):
        wo = tuple(u for u in wo_left if done.get(('o',) + u, 0) >= 1)[:4]
        if len(wo) < n:
            return None
        for u in wo:
            wo_left.remove(u)
        g = [(('wo', wo, n, c), 8, []) for n in range(len(wo)) for c in range(DT)]
        g[-1] = (g[-1][0], 8, [(('wacc', wo, c), len(wo), None, 0) for c in range(DT)])
        return g

    def g_or(n, last):
        rd = [u for u in or_left if done.get(('acc',) + u, 0) >= 8 // AB and done.get(('w', u[0]), 0)
              and (last or done[('acct',) + u] + AD <= s['tv'])
              and done.get(('y',) + u, 0) >= xs.get(u, 0)][:4]
        if len(rd) < n:
            return None
        for u in rd:
            or_left.remove(u)
        return [(('gap',), 8 * len(rd), [])] + [(('or',) + u, 8, [(('ofin',) + u, 1, ('o',) + u, 1)]) for u in rd]

    def g_px():
        rd = [u for u in px_left if done.get(('w', u[0]), 0)]
        if not rd:
            return None
        px_left.remove(rd[0])
        n = xs[rd[0]]
        g = [(('pvx',) + rd[0] + (k,), 8, []) for k in range(n)]
        e, inc = (('o',) + rd[0], 4 / KT) if n == KT else (('y',) + rd[0], 4)
        g[-1] = (g[-1][0], 8, [(('xsum',) + rd[0] + (k,), 4, e, inc) for k in range(0, n, 4)])
        return g

    def pick():
        last, endgame, nxt = s['i'] >= len(steps), s['mi'] >= len(main), s['qk']
        if last:
            return g_or(1, True) or g_px() or g_wo(1)
        if endgame:
            return g_or(4, False) or g_px() or g_wo(4) or g_wo(1)
        rem = sum(8 for m in main[s['mi']:s['mi'] + 200] if m[0] != 'qk' or m[1] == nxt)
        if (first_step[nxt] - s['i']) * vcost - rem > qlead * 500:
            g = (g_wo(4) if len(wo_left) > keep else None) or g_or(4, False) or g_px()
            if g:
                return g
        m = main[s['mi']]
        if m[0] == 'qk' and done.get(('q', m[1]), 0) < 3:
            return None
        s['mi'] += 1
        pcs = []
        if m[0] == 'q':
            pcs = [(('qfin',) + m[1:], 5, ('q', m[1]), 1)]
        if m[0] == 'qk' and (m[2] == 2 or m[1:3] == (0, 1)) and m[3] % SG == SG - 1:
            t = m[1] if m[2] == 2 else -1
            pcs = [sm(t)[m[3] // SG]] + (sm(t)[KT // SG:] if m[3] == KT - 1 else [])
        return [(m, 8, pcs)]

    def later(t, pcs):
        wait.append((t, pcs))
        wait.sort(key=lambda w: w[0])

    def piece():
        a, cv, e, inc = pend.pop(0)
        if a[0] == 'wld' and s['i'] < len(steps) and not wk[0] <= steps[s['i']][2] <= wk[1]:
            return later(s['tv'] + 30, [(a, cv, e, inc)])
        ev.append(('piece',) + a)
        s['tv'] += cv / 4
        if e is not None:
            done[e] = done.get(e, 0) + inc
        if a[0] == 'smb' and a[2] == KT - SG and a[1] >= 0:
            later(s['tv'] + WD, [(('wld', a[1]), 0, ('wld', a[1]), 1)])
        if a[0] == 'wld':
            later(s['tv'] + WL, [(('w', a[1]), 24, ('w', a[1]), 1)])

    def urgent(p):
        return p[2] is not None and p[2][0] != 'p'

    while True:
        while wait and wait[0][0] <= s['tv']:
            pcs = wait.pop(0)[1]
            pend[:] = [p for p in pcs if urgent(p)] + pend + [p for p in pcs if not urgent(p)]
        i = s['i']
        more = i < len(steps)
        blocked = not more or done.get(('p', steps[i][0] - (i < AP // 2 // AB * KT)), 0) < min(KT, steps[i][2] + 6)
        if not cur and (s['tm'] + LEAD <= s['tv'] or blocked):
            cur = pick() or []
        if not more and not pend and not wait and not cur:
            break
        if cur and (s['tm'] + LEAD <= s['tv']
                    or (blocked and not pend and (not wait or s['tm'] + LEAD <= wait[0][0]))):
            a, cm, pcs = cur.pop(0)
            ev.append(('tile',) + a)
            s['tm'] = max(s['tm'], s['tv'] - LEAD - 8) + cm
            s['tv'] += 0.25 * (a[0] == 'pvx')
            s['qk'] += a[0] == 'qk' and a[2:] == (2, KT - 1)
            if pcs:
                later(s['tm'] + (LAT if 0 < i < len(steps) else LAT0), pcs)
        elif blocked and pend:
            piece()
        elif blocked:
            s['tv'] = max(s['tv'], wait[0][0])
        else:
            if pend and (i % pstride == 0 or urgent(pend[0])):
                piece()
            t, a, k = steps[i]
            ev.append(('step', t, a, k))
            if k == KT - 1:
                done['acc', t, a // 8] = done.get(('acc', t, a // 8), 0) + 1
                done['acct', t, a // 8] = s['tv']
            s['tv'] += vcost - 0.5 * sum((t, b) in wide for b in range(a, a + AB))
            s['i'] += 1
    assert not or_left and not wo_left and not px_left

    out, cur, cnt = [], [], 0
    for e in ev + [None]:
        if e is None or (e[0] == 'tile' and e[1] != 'gap' and cnt % 4 == ph):
            if any(x[0] == 'step' for x in cur) and len(cur) < 32:
                cur = cur[:1] + [x for x in cur[1:] if x[0] == 'piece'] + [x for x in cur[1:] if x[0] != 'piece']
            out += cur
            cur = []
        if e is not None:
            cur.append(e)
            cnt += (4 if e[1] == 'gap' else 1) * (e[0] == 'tile')
    return out


def _slots(events, key):
    first, last = {}, {}
    for n, e in enumerate(events):
        k = key(e)
        if k is not None:
            first.setdefault(k, n)
            last[k] = n
    slot, busy = {}, []
    for k in first:
        free = [i for i, u in enumerate(busy) if u < first[k]]
        slot[k] = free[0] if free else len(busy)
        busy[slot[k]:slot[k] + 1] = [last[k]]
    return slot, len(busy)


def _run(opts, A_x, A_k_cache, A_v_cache, A_wq, A_wo, B_w3, B_w4):
    B, S, D = A_x.shape
    _, H, Sk, Dh = A_k_cache.shape
    F = B_w3.shape[1]
    W = min(4096, max(256, Sk // 4))
    assert (B, S, H, Dh, W) == (1, 1, 32, 192, 4096) and D % 128 == 0 and F % 128 == 0
    AP = Dh // 8
    KT = W // 128
    NP = H // 2
    DT, FT = D // 128, F // 128
    AB, SG, FD = 4, 2, opts.get('fd', 5)
    SKEW = opts.get('skew', 1)
    cexp = (Dh ** -0.5) * _LOG2E
    nx = {u[:2]: u[2] for u in opts['xunits']}
    xunits = list(nx)
    wide = [(t, a) for t in range(NP) for a in range(0, AP, AB) if (t, a // 8) not in xunits + [(NP - 1, 2)]]
    drop = [g for n, g in enumerate(wide) if n % 3][:max(0, len(wide) - opts['nwide'])]
    wide = [g for g in wide if g not in drop] + [(t, a + 2) for t, a in wide[::-1]][:max(0, opts['nwide'] - len(wide))]
    late = [(t, a) for b in (0, 2) for t in range(NP - 1, 0, -1) for a in range(b, AP, AB)
            if (t, a // 8) not in xunits + [(NP - 1, 2)] and (t, a) not in wide]
    nlate = opts['nlate']
    late = {g: (c, n) for c in range(DT - 1) for n, g in enumerate(late[sum(nlate[:c]):sum(nlate[:c + 1])])}
    events = _schedule(NP, KT, DT, AP, AB, SG, wide=wide + list(late), **opts)
    sp, RP = _slots(events, lambda e: e[1] - (e[1] == 0 and e[2] < AP // 2) if e[0] == 'step'
                    else e[2] if e[1] in ('sma', 'smb', 'pvx') else None)
    ss, RS = _slots(events, lambda e: max(e[2], 0) if e[1] in ('qk', 'sma') else None)
    sq, RQ = _slots(events, lambda e: e[2] if e[1] in ('q', 'qfin') else None)
    sx, RX = _slots(events, lambda e: e[2:4] if e[1] in ('pvx', 'xsum') else None)
    sw, RM = _slots(events, lambda e: e[2] if e[1] in ('wo', 'wacc') else None)
    so, RO = _slots(events, lambda e: e[2:4] if e[1] in ('or', 'ofin') else None)
    sl, RL = _slots(events, lambda e: e[2] if e[1] in ('smb', 'wld') else None)
    assert _slots(events, lambda e: e[2] if e[1] in ('sma', 'smb') else None)[1] == 1
    sizes = [3 * NP, 3 * NP, 2 * NP, 2, DT, 2 * NP + 3, KT, KT * len(wide)]
    QP, Q0, WB, XL, XA, MB, AL, WD, NBIG = [sum(sizes[:n]) for n in range(len(sizes) + 1)]
    OB = Q0
    free, acc_at = [AL, AL + 16], {}
    for e in events:
        if e[0] == 'step' and (e[1], e[2] // 8) not in acc_at:
            acc_at[e[1], e[2] // 8] = free.pop(0)
        if e[0] == 'step' and e[3] == KT - 1:
            free += [WD + KT * wide.index((e[1], a)) + n for a in range(e[2], e[2] + AB) if (e[1], a) in wide
                     for n in (0, 16)]
    sizes = [RP * KT, 3 * RS * KT, RX * KT, 3 * RQ, 4 * DT * RM, 2 * RO, 2 * RL]
    _, SP, XP, QR, WR, OR, ML, NPB = [sum(sizes[:n]) for n in range(len(sizes) + 1)]
    NV, NQ = opts.get('nv', 2), opts.get('nq', 8)
    assert nlate[DT - 2] == 0 and 2 * nlate[DT - 3] <= 11 + (3 * NP - NQ) // 4
    if opts.get('verbose'):
        print('RP RS RQ RX RM', RP, RS, RQ, RX, RM, 'free tiles', (int(13.25 * 256) - NBIG - NPB))
    order1 = sorted(range(NP), key=lambda t: all(u[0] != t for u in xunits))

    def kernel(x_hbm, k_hbm, v_hbm, wq_hbm, wo_hbm, w3_hbm, w4_hbm, o_ref, *scratch):
        k_bufs, v_bufs, scratch = scratch[:NP], scratch[NP:2 * NP], scratch[2 * NP:]
        w4_bufs, wq_bufs, scratch = scratch[:DT], scratch[DT:2 * DT], scratch[2 * DT:]
        wo_buf, w3_buf, pbuf, cst, big, hbuf, xres, x_buf, sems = scratch
        t0 = (Sk - W) // 128

        def kv_cp(kind, t):
            src, dst = (k_hbm, k_bufs[t]) if kind == 0 else (v_hbm, v_bufs[t])
            return [pltpu.make_async_copy(src.at[pl.ds(AP * t, AP), a, pl.ds(t0, KT)],
                                          dst.at[:, :, pl.ds(8 * a, 8), :], sems.at[2 * t + kind])
                    for a in range(2)]

        def w_cp(src, dst, n, sem):
            rows = src.shape[0] // n
            return [pltpu.make_async_copy(src.at[pl.ds(i * rows, rows), a],
                                          dst.at[pl.ds(i * rows, rows), :, pl.ds(8 * a, 8), :], sem)
                    for i in range(n) for a in range(2)]

        def wq_cp():
            cps = [cp for j in range(DT) for cp in w_cp(wq_hbm.at[pl.ds(8 * j, 8)], wq_bufs[j], 1, sems.at[2 * NP])]
            return cps[:1] + [pltpu.make_async_copy(x_hbm, x_buf, sems.at[2 * NP])] + cps[1:]

        def wo_cp():
            return w_cp(wo_hbm, wo_buf, 8, sems.at[2 * NP + 1])

        def w3_cp():
            return [pltpu.make_async_copy(w3_hbm, w3_buf, sems.at[2 * NP + 2])]

        def w4_cp(c):
            return [pltpu.make_async_copy(w4_hbm.at[:, pl.ds(128 * c, 128)], w4_bufs[c], sems.at[2 * NP + 3 + c])]

        def wait(cps):
            for cp in cps:
                cp.wait()

        cps = wq_cp()
        for t in order1:
            cps += kv_cp(0, t) + kv_cp(1, t) + (wo_cp() if t == order1[0] else [])
        for cp in cps + w3_cp() + [cp for c in range(DT) for cp in w4_cp(c)]:
            cp.start()

        ku = [r.bitcast(u32) for r in k_bufs]
        vu = [r.bitcast(u32) for r in v_bufs]
        wqu = [r.bitcast(u32) for r in wq_bufs]
        wou = wo_buf.bitcast(u32)
        w4u = [r.bitcast(u32) for r in w4_bufs]

        def top(n):
            return lax.broadcasted_iota(i32, (8, n), 0) < 4

        def left():
            return lax.broadcasted_iota(i32, (8, 128), 1) < 64

        def cols(n):
            return slice(128 * n, 128 * (n + 1))

        def rows(j):
            return slice(8 * j, 8 * j + 8)

        def masks():
            return [top(128), top(128) == left(), jnp.logical_not(top(128))]

        def mlp_hidden(x):
            lhs = jnp.where(top(D), x, 1.0)
            m1, xc, r1 = _stats(x)
            y = xc * r1
            m2 = jnp.mean(y, axis=-1, keepdims=True)
            r2 = lax.rsqrt(jnp.mean(y * y, axis=-1, keepdims=True) - m2 * m2 + _EPS)
            coef = jnp.where(top(128), r1 * r2, -(r2 * (r1 * m1 + m2)))
            hs = []
            for n in range(FT):
                u = _tree(jnp.add, [_mm(lhs[:, cols(j)], w3_buf[cols(j), cols(n)]) for j in range(DT)]) * coef
                hs.append(jax.nn.gelu(u + pltpu.roll(u, 4, 0), approximate=True))
            return y, hs

        def w4_tile(n, c):
            return pltpu.bitcast(w4u[c][64 * n:64 * (n + 1)], bf16)

        def late_at(n, k):
            return ((n * KT + k + 2) % (24 * NP)) // (3 * NP), (n * KT + k + 2) % (3 * NP)

        def unpack_late(c, n0, n1, after=None):
            todo = [(g, n, k) for g, (cc, n) in late.items() if cc == c for k in range(KT)][16 * n0:16 * n1]
            if todo and after is not None:
                wqu[c][after[0], 0] = pltpu.bitcast(after[1], u32)
            for (t, a), n, k in todo:
                y = pltpu.bitcast(pltpu.bitcast(vu[t][a, k], bf16).astype(f32), u32)
                wqu[c][late_at(n, k)] = y[8:16]
                vu[t][a, k] = y[0:8]

        def layer1(z):
            for u, mask in enumerate(masks()):
                cst[u] = jnp.where(mask, cexp, 0.0).astype(f32)
            wait(wq_cp())
            x = jnp.broadcast_to(x_buf[...].astype(f32), (8, D))
            _, xc, r = _stats(x)
            xn = xc * r

            def q_body(t, c):
                for i in range(3):
                    q = _tree(jnp.add, [_mm(xn[:, cols(j)], _wtile(wqu[j][:, 3 * t + i])) for j in range(DT)])
                    big[QP + 3 * t + i] = q * cst[i]
                return c
            lax.fori_loop(0, NP, q_body, 0)

            att = [jnp.zeros((8, 128), f32)] * DT
            for t in order1:
                def s_body(k, c, t=t, q=[big[QP + 3 * t + j] for j in range(3)]):
                    big[AL + k] = _tree(jnp.add, [_mm(q[j], _wtile(ku[t][rows(j), k])) for j in range(3)])
                    return c

                def o_body(k, o, t=t):
                    return [o[j] + _mm(big[AL + k], _wtile(vu[t][rows(j), k]), _NT) for j in range(3)]

                wait(kv_cp(0, t))
                lax.fori_loop(0, KT, s_body, 0, unroll=8)
                sc = big[AL:AL + KT]
                p = jnp.exp2(sc - jnp.max(jnp.max(sc, axis=0), axis=1, keepdims=True))
                big[AL:AL + KT] = p
                inv = 1.0 / jnp.sum(jnp.sum(p, axis=0), axis=1, keepdims=True)
                wait(kv_cp(1, t) + (wo_cp() if t == order1[0] else []))
                o = lax.fori_loop(0, KT, o_body, [jnp.zeros((8, 128), f32)] * 3, unroll=8)
                o = [jnp.where(mask, o[j] * inv, 0.0) for j, mask in enumerate(masks())]
                att = [att[c] + _tree(jnp.add, [_mm(o[j], _wtile(wou[rows(3 * t + j), c])) for j in range(3)])
                       for c in range(DT)]
                for j in [j for tt, j in xunits if tt == t]:
                    def t_body(k, c, t=t, j=j):
                        w = _wtile(vu[t][rows(j), k]).astype(f32).T.astype(bf16)
                        vu[t][rows(j), k] = pltpu.bitcast(w, u32).reshape(8, 8, 128)
                        return c
                    lax.fori_loop(0, nx[t, j], t_body, 0, unroll=4)
                for n, a in [(n, a) for n, (tt, a) in enumerate(wide) if tt == t]:
                    y = _wtile(vu[t][a]).astype(f32).reshape(KT, 16, 128)
                    big[WD + n * KT:WD + (n + 1) * KT] = y[:, 8:16]
                    vu[t][a] = pltpu.bitcast(y[:, 0:8], u32)
            att = jnp.concatenate(att, axis=1)
            x = x + (att + pltpu.roll(att, 4, 0))
            wait(w3_cp())
            y, hs = mlp_hidden(x)
            xres[...] = x + y
            for n in range(FT):
                hbuf[n] = hs[n]
            for c in range(DT - 1):
                wait(w4_cp(c))
                unpack_late(c - 1, 0, 7)
                xc = xres[:, cols(c)] + _tree(jnp.add, [_mm(hbuf[n], w4_tile(n, c)) for n in range(FT)])
                xres[:, cols(c)] = xc
                xc = jnp.where(top(128), xc, 1.0)
                unpack_late(c - 1, 7, 11, (z, xc))
                for n in range(3 * NP - (NQ if c == DT - 2 else 0)):
                    r = _mm(xc, _wtile(wqu[c][:, n]))
                    big[Q0 + n] = big[Q0 + n] + r if c else r
                    if n % 4 == 0:
                        unpack_late(c - 1, 11 + n // 4, 12 + n // 4, (z, r))

        def layer2(z):
            wait(w4_cp(DT - 1))
            if opts.get('skip2'):
                keep = big[Q0 + z] + sum(pltpu.bitcast(r[z, 1], f32) for r in wqu + vu)
                o_ref[...] = (xres[0:1, :] + jnp.concatenate([keep[0:1]] * DT, axis=1)).astype(o_ref.dtype)
                return
            xc = xres[:, cols(DT - 1)] + _tree(jnp.add, [_mm(hbuf[n], w4_tile(n, DT - 1)) for n in range(FT)])
            for n in range(3 * NP - NQ, 3 * NP):
                xp = jnp.where(top(128), xres[:, cols(DT - 2)], 1.0)
                big[Q0 + n] = big[Q0 + n] + _mm(xp, _wtile(wqu[DT - 2][:, n]))
            xres[:, cols(DT - 1)] = xc
            m, _, r = _stats(xres[...])
            big[XL] = xraw = jnp.where(top(128), xc, 1.0)
            coef0 = jnp.where(top(128), 1.0, -m)
            big[XL + 1] = coef = coef0 * r
            acc, val, fwd = {}, {}, []
            st = dict(pin=False, dirty=False, cnt=0, started=False, left=sum(e[0] == 'step' for e in events))

            def lhs(n):
                if st['pin']:
                    st['pin'] = False
                    return big[n + z]
                if n not in val:
                    val[n] = big[n]
                return val[n]

            def checkpoint():
                for (t, a), y in acc.items():
                    n = acc_at[t, a // 8] + 2 * (a % 8)
                    big[n:n + 2] = y.reshape(2, 8, 128)

            def put(n, r):
                fwd.append((st['cnt'], n, r))

            def flush(upto, pin=False):
                while fwd and fwd[0][0] <= upto:
                    _, n, r = fwd.pop(0)
                    pbuf[z if pin else 0, :, cols(n)] = r
                    if pin and st['left'] <= opts.get('vpin', 72):
                        vu[NP - 1][z, 2] = pltpu.bitcast(r, u32)
                    pin = False

            def get(n):
                flush(max([c for c, m, _ in fwd if m == n], default=-1))
                return pbuf[0, :, cols(n)]

            def ptile(t, k):
                return cols(sp[t] * KT + k)

            def prow(t, odd, k):
                return pbuf[0, 4 * odd:4 * odd + 1, ptile(t - (t + odd == 0), k)]

            def q_fin(t, i, y, coef):
                y = (y + big[Q0 + 3 * t + i]) * coef
                big[QP + 3 * t + i] = (y + pltpu.roll(y, 4, 0)) * cst[i]

            def t_qraw(t, i):
                q_fin(t, i, _mm(xraw, _wtile(wqu[DT - 1][:, 3 * t + i])), coef if t else coef0)

            def t_q(t, i):
                put(QR + sq[t] * 3 + i, _mm(lhs(XL), _wtile(wqu[DT - 1][:, 3 * t + i])))

            def t_qk(t, j, k):
                put(SP + (3 * ss[t] + j) * KT + k, _mm(lhs(QP + 3 * t + j), _wtile(ku[t][rows(j), k])))

            def t_or(t, j):
                a = big[acc_at[t, j]:acc_at[t, j] + 16].reshape(128, 128)
                if j == 1:
                    r = _mm(jnp.concatenate([lhs(WB + 2 * t), lhs(WB + 2 * t + 1)], axis=0), a, _NT)
                    put(OR + 2 * so[t, j] + 1, r[8:16])
                else:
                    r = _mm(lhs(WB + 2 * t + j // 2), a, _NT)
                put(OR + 2 * so[t, j], r[0:8])

            def t_pvx(t, j, k):
                p = val.pop(('px', t, j, k)) * lhs(WB + 2 * t + j // 2)
                put(XP + sx[t, j] * KT + k, _mm(p, _wtile(vu[t][rows(j), k])))

            def t_wo(units, n, c):
                t, j = units[n]
                put(WR + (sw[units] * 4 + n) * DT + c, _mm(lhs(OB + 3 * t + j), _wtile(wou[rows(3 * t + j), c])))

            def p_qfin(t, i):
                q_fin(t, i, get(QR + sq[t] * 3 + i), big[XL + 1])

            def p_sma(t, k0):
                n = SP + 3 * ss[max(t, 0)] * KT
                sv = []
                for k in range(k0, k0 + SG):
                    sc = get(n + k) + get(n + KT + k)
                    sc = sc + get(n + 2 * KT + k) if t >= 0 else sc
                    sv.append(sc * r if t <= 0 else sc)
                    pbuf[0, :, ptile(t, k)] = sv[-1]
                big[MB + 2 + 2 * t] = val['m'] = _tree(jnp.maximum, sv + ([val['m']] if k0 else []))

            def p_smb(t, k0):
                ps = []
                for k in range(k0, k0 + SG):
                    ps.append(jnp.exp2(pbuf[0, :, ptile(t, k)] - val['m']))
                    pbuf[0, :, ptile(t, k)] = ps[-1]
                if t >= 0:
                    big[MB + 3 + 2 * t] = val['l'] = _tree(jnp.add, ps + ([val['l']] if k0 else []))
                if t >= 0 and k0 + SG == KT:
                    pbuf[0, :, cols(ML + 2 * sl[t])] = val['m']
                    pbuf[0, :, cols(ML + 2 * sl[t] + 1)] = val['l']

            def p_wld(t):
                val['ml', t] = pbuf[0, :, cols(ML + 2 * sl[t])], pbuf[0, :, cols(ML + 2 * sl[t] + 1)]

            def p_w(t):
                m, l = val['ml', t]
                e = jnp.exp2(m - jnp.max(m, axis=1, keepdims=True))
                w = e / jnp.sum(e * l, axis=1, keepdims=True)
                for h in range(2):
                    big[WB + 2 * t + h] = jnp.broadcast_to(w[4 * h:4 * h + 1], (8, 128))

            def p_ofin(t, j):
                r = get(OR + 2 * so[t, j])
                r = jnp.where(left(), r, get(OR + 2 * so[t, j] + 1)) if j == 1 else r
                big[OB + 3 * t + j] = r + big[OB + 3 * t + j] if (t, j) in nx else r

            def p_xsum(t, j, k0):
                n = XP + sx[t, j] * KT + k0
                ys = [get(n + u) for u in range(4)] + ([val['y', t, j]] if k0 else [])
                big[OB + 3 * t + j] = val['y', t, j] = _tree(jnp.add, ys)

            def p_wacc(units, c):
                rs = [get(WR + (sw[units] * 4 + n) * DT + c) for n in range(len(units))]
                big[XA + c] = _tree(jnp.add, rs + ([big[XA + c]] if units != next(iter(sw)) else []))

            fns = {'qraw': t_qraw, 'q': t_q, 'qk': t_qk, 'or': t_or, 'pvx': t_pvx, 'wo': t_wo, 'qfin': p_qfin,
                   'sma': p_sma, 'smb': p_smb, 'wld': p_wld, 'w': p_w, 'ofin': p_ofin, 'xsum': p_xsum, 'wacc': p_wacc}
            tiles = [e for e in events if e[0] == 'tile' and e[1] != 'gap']
            for e in events:
                if e[0] == 'step':
                    _, t, a0, k = e
                    k0 = nx.get((t, a0 // 8), 0)
                    for a in range(a0, a0 + AB):
                        n = k + SKEW * (a - a0)
                        kk = k0 + (n - k0) % (KT - k0)
                        if ('p', t, a0, n) not in val:
                            val['p', t, a0, n] = prow(t, int(a0 >= AP // 2), kk)
                        if (t, a) in wide:
                            y = jnp.concatenate([pltpu.bitcast(vu[t][a, kk], f32),
                                                 big[WD + wide.index((t, a)) * KT + kk]])
                        elif (t, a) in late:
                            c, u = late[t, a]
                            y = pltpu.bitcast(jnp.concatenate([vu[t][a, kk], wqu[c][late_at(u, kk)]]), f32)
                        else:
                            y = pltpu.bitcast(vu[t][a, kk], bf16).astype(f32)
                        y = y * val['p', t, a0, n]
                        acc[t, a] = acc[t, a] + y if (t, a) in acc else y
                    st.update(dirty=True, started=True, left=st['left'] - 1)
                    if k == KT - 1:
                        checkpoint()
                        acc.clear()
                elif e[0] == 'piece':
                    fns[e[1]](*e[2:])
                elif e[1] == 'gap':
                    st['cnt'] += 4
                else:
                    pinned = st['cnt'] % 4 == opts.get('ph', 3) and st['left'] > 0
                    if pinned and st['dirty']:
                        checkpoint()
                    st.update(pin=pinned and st['started'], dirty=st['dirty'] and not pinned)
                    fns[e[1]](*e[2:])
                    st['pin'] = False
                    tiles.pop(0)
                    for u in tiles[:opts.get('pf', 4)]:
                        if u[1] == 'pvx' and ('px',) + u[2:] not in val:
                            val[('px',) + u[2:]] = prow(u[2], u[3] // 2, u[4])
                    if pinned:
                        flush(st['cnt'] - 4 * FD + 3, pin=st['started'])
                    st['cnt'] += 1
            assert not fwd
            x = xres[...] + jnp.concatenate([big[XA + c] for c in range(DT)], axis=1)
            y, hs = mlp_hidden(x)
            out = [(x + y)[:, cols(c)] for c in range(DT)]
            part = [None] * DT
            for n in range(NV):
                hb = jnp.concatenate([hs[n]] * 16, axis=0).T
                for a in range(8):
                    for c in range(DT):
                        u = pltpu.bitcast(w4u[c][rows(8 * n + a)], bf16).astype(f32) * hb[16 * a:16 * a + 16]
                        part[c] = u if part[c] is None else part[c] + u
            for n in range(NV, FT):
                out = [out[c] + _mm(hs[n], w4_tile(n, c)) for c in range(DT)]
            out = [out[c] + jnp.sum(part[c], axis=0, keepdims=True) for c in range(DT)]
            o_ref[...] = jnp.concatenate(out, axis=1)[0:1].astype(o_ref.dtype)

        def body(it, carry):
            pl.when(it == 0)(lambda: layer1(it >> 4) if not opts.get('skip1') else None)
            pl.when(it == 1)(lambda: layer2(it >> 4))
            return carry

        lax.fori_loop(0, 2, body, 0)

    def V(*s, dt=f32):
        return pltpu.VMEM(s, dt)

    out = pl.pallas_call(
        kernel,
        out_shape=jax.ShapeDtypeStruct((1, D), A_x.dtype),
        in_specs=[pl.BlockSpec(memory_space=pl.ANY)] * 7,
        out_specs=pl.BlockSpec(memory_space=pltpu.VMEM),
        scratch_shapes=(
            [V(AP, KT, 16, 128, dt=bf16)] * (2 * NP)
            + [V(F, 128, dt=bf16)] * DT + [V(8, 3 * NP, 16, 128, dt=bf16)] * DT
            + [V(AP * NP, DT, 16, 128, dt=bf16), V(D, F, dt=bf16),
               V(1, 8, -(-NPB // 4) * 512), V(4, 8, 128), V(-(-NBIG // 4) * 4, 8, 128),
               V(FT, 8, 128), V(8, D), V(1, D, dt=bf16),
               pltpu.SemaphoreType.DMA((2 * NP + 3 + DT,))]),
        compiler_params=pltpu.CompilerParams(
            vmem_limit_bytes=int(opts.get('vmem', 128) * 1024 * 1024),
            disable_semaphore_checks=True, disable_bounds_checks=True),
        name='fused_decode_layers',
    )(A_x.reshape(1, D), _cache_view(A_k_cache), _cache_view(A_v_cache),
      _weight_view(A_wq), _weight_view(A_wo), B_w3, B_w4)
    return out.reshape(B, S, D)


@jax.jit
def pallas_interleave_layers__sliding_block_cached__mixer_s_mlp__decode_kernel(
    A_x: jax.Array,
    A_k_cache: jax.Array,
    A_v_cache: jax.Array,
    A_wq: jax.Array,
    A_wo: jax.Array,
    B_x: jax.Array,
    B_w1: jax.Array,
    B_w2: jax.Array,
    B_w3: jax.Array,
    B_w4: jax.Array,
):
    return _run(_OPTS, A_x, A_k_cache, A_v_cache, A_wq, A_wo, B_w3, B_w4)
```

```python
import jax
import jax.numpy as jnp
from jax import lax
import jax.experimental.pallas as pl
import jax.experimental.pallas.tpu as pltpu

f32, bf16, u32, i32 = jnp.float32, jnp.bfloat16, jnp.uint32, jnp.int32
_EPS = 1e-5
_LOG2E = 1.4426950408889634
_NN = (((1,), (0,)), ((), ()))
_NT = (((1,), (1,)), ((), ()))

_OPTS = dict(xunits=[(5, 0, 32), (7, 2, 32), (9, 2, 32), (11, 0, 32), (12, 2, 32), (14, 2, 12)], nwide=78, nlate=[10, 10, 9, 0], qlead=2.0, keep=8,
             AD=100, LAT=205, LAT0=205, q2at=20, vpin=80)


def _stats(x):
    m = jnp.mean(x, axis=-1, keepdims=True)
    xc = x - m
    v = jnp.mean(xc * xc, axis=-1, keepdims=True)
    return m, xc, lax.rsqrt(v + _EPS)


def _tree(op, xs):
    xs = list(xs)
    while len(xs) > 1:
        nxt = [op(xs[i], xs[i + 1]) for i in range(0, len(xs) - 1, 2)]
        if len(xs) % 2:
            nxt.append(xs[-1])
        xs = nxt
    return xs[0]


def _wtile(u):
    return pltpu.bitcast(u.reshape(u.shape[0] * 8, 128), bf16)


def _mm(lhs, w, dims=_NN):
    return lax.dot_general(lhs, w, dims, preferred_element_type=f32)


def _cache_view(c):
    _, H, Sk, Dh = c.shape
    c = c.reshape(H, Sk // 128, 128, Dh // 16, 2, 8)
    c = jnp.transpose(c, (0, 3, 4, 1, 5, 2))
    return c.reshape(H * Dh // 16, 2, Sk // 128, 8, 128)


def _weight_view(w):
    R, N = w.shape
    w = w.reshape(R // 16, 2, 8, N // 128, 128)
    return jnp.transpose(w, (0, 1, 3, 2, 4))


def _schedule(NP, KT, DT, AP, AB, SG, xunits, qlead, keep, LAT=205, LAT0=165, LEAD=32, WD=140, WL=400, AD=160,
              vcost=5.95, pstride=2, nraw=8, q2at=40, ph=3, wide=(), wk=(8, 20), **_):
    xs = {u[:2]: u[2] for u in xunits}
    grp = [(t, a) for t in range(NP) for a in range(0, AP, AB)]
    grp[-2:] = grp[:-3:-1]
    steps = [(t, a, k) for t, a in grp for k in range(xs.get((t, a // 8), 0), KT)]
    first_step = {}
    for i, s in enumerate(steps):
        first_step.setdefault(s[0], i)
    main = [('qraw', t, i) for t in range(nraw) for i in range(3)]
    for t in range(NP):
        qk = [('qk', t, j, k) for j in range(3) for k in range(KT)]
        main += qk[:q2at] + [('q', t + 1, i) for i in range(3) if nraw <= t + 1 < NP] + qk[q2at:]
    done = {('q', t): 3 for t in range(nraw)}
    or_left = [(t, j) for t in range(NP) for j in range(3) if xs.get((t, j), 0) < KT]
    wo_left = [(t, j) for t in range(NP) for j in range(3)]
    px_left = list(xs)
    ev, pend, wait, cur = [], [], [], []
    s = dict(tm=0.0, tv=0.0, i=0, mi=0, qk=0)

    def sm(t):
        return ([(('sma', t, k), 3 * SG, None, 0) for k in range(0, KT, SG)]
                + [(('smb', t, k), 3 * SG, ('p', t), SG) for k in range(0, KT, SG)])

    def g_wo(n):
        wo = tuple(u for u in wo_left if done.get(('o',) + u, 0) >= 1)[:4]
        if len(wo) < n:
            return None
        for u in wo:
            wo_left.remove(u)
        g = [(('wo', wo, n, c), 8, []) for n in range(len(wo)) for c in range(DT)]
        g[-1] = (g[-1][0], 8, [(('wacc', wo, c), len(wo), None, 0) for c in range(DT)])
        return g

    def g_or(n, last):
        rd = [u for u in or_left if done.get(('acc',) + u, 0) >= 8 // AB and done.get(('w', u[0]), 0)
              and (last or done[('acct',) + u] + AD <= s['tv'])
              and done.get(('y',) + u, 0) >= xs.get(u, 0)][:4]
        if len(rd) < n:
            return None
        for u in rd:
            or_left.remove(u)
        return [(('gap',), 8 * len(rd), [])] + [(('or',) + u, 8, [(('ofin',) + u, 1, ('o',) + u, 1)]) for u in rd]

    def g_px():
        rd = [u for u in px_left if done.get(('w', u[0]), 0)]
        if not rd:
            return None
        px_left.remove(rd[0])
        n = xs[rd[0]]
        g = [(('pvx',) + rd[0] + (k,), 8, []) for k in range(n)]
        e, inc = (('o',) + rd[0], 4 / KT) if n == KT else (('y',) + rd[0], 4)
        g[-1] = (g[-1][0], 8, [(('xsum',) + rd[0] + (k,), 4, e, inc) for k in range(0, n, 4)])
        return g

    def pick():
        last, endgame, nxt = s['i'] >= len(steps), s['mi'] >= len(main), s['qk']
        if last:
            return g_or(1, True) or g_px() or g_wo(1)
        if endgame:
            return g_or(4, False) or g_px() or g_wo(4) or g_wo(1)
        rem = sum(8 for m in main[s['mi']:s['mi'] + 200] if m[0] != 'qk' or m[1] == nxt)
        if (first_step[nxt] - s['i']) * vcost - rem > qlead * 500:
            g = (g_wo(4) if len(wo_left) > keep else None) or g_or(4, False) or g_px()
            if g:
                return g
        m = main[s['mi']]
        if m[0] == 'qk' and done.get(('q', m[1]), 0) < 3:
            return None
        s['mi'] += 1
        pcs = []
        if m[0] == 'q':
            pcs = [(('qfin',) + m[1:], 5, ('q', m[1]), 1)]
        if m[0] == 'qk' and (m[2] == 2 or m[1:3] == (0, 1)) and m[3] % SG == SG - 1:
            t = m[1] if m[2] == 2 else -1
            pcs = [sm(t)[m[3] // SG]] + (sm(t)[KT // SG:] if m[3] == KT - 1 else [])
        return [(m, 8, pcs)]

    def later(t, pcs):
        wait.append((t, pcs))
        wait.sort(key=lambda w: w[0])

    def piece():
        a, cv, e, inc = pend.pop(0)
        if a[0] == 'wld' and s['i'] < len(steps) and not wk[0] <= steps[s['i']][2] <= wk[1]:
            return later(s['tv'] + 30, [(a, cv, e, inc)])
        ev.append(('piece',) + a)
        s['tv'] += cv / 4
        if e is not None:
            done[e] = done.get(e, 0) + inc
        if a[0] == 'smb' and a[2] == KT - SG and a[1] >= 0:
            later(s['tv'] + WD, [(('wld', a[1]), 0, ('wld', a[1]), 1)])
        if a[0] == 'wld':
            later(s['tv'] + WL, [(('w', a[1]), 24, ('w', a[1]), 1)])

    def urgent(p):
        return p[2] is not None and p[2][0] != 'p'

    while True:
        while wait and wait[0][0] <= s['tv']:
            pcs = wait.pop(0)[1]
            pend[:] = [p for p in pcs if urgent(p)] + pend + [p for p in pcs if not urgent(p)]
        i = s['i']
        more = i < len(steps)
        blocked = not more or done.get(('p', steps[i][0] - (i < AP // 2 // AB * KT)), 0) < min(KT, steps[i][2] + 6)
        if not cur and (s['tm'] + LEAD <= s['tv'] or blocked):
            cur = pick() or []
        if not more and not pend and not wait and not cur:
            break
        if cur and (s['tm'] + LEAD <= s['tv']
                    or (blocked and not pend and (not wait or s['tm'] + LEAD <= wait[0][0]))):
            a, cm, pcs = cur.pop(0)
            ev.append(('tile',) + a)
            s['tm'] = max(s['tm'], s['tv'] - LEAD - 8) + cm
            s['tv'] += 0.25 * (a[0] == 'pvx')
            s['qk'] += a[0] == 'qk' and a[2:] == (2, KT - 1)
            if pcs:
                later(s['tm'] + (LAT if 0 < i < len(steps) else LAT0), pcs)
        elif blocked and pend:
            piece()
        elif blocked:
            s['tv'] = max(s['tv'], wait[0][0])
        else:
            if pend and (i % pstride == 0 or urgent(pend[0])):
                piece()
            t, a, k = steps[i]
            ev.append(('step', t, a, k))
            if k == KT - 1:
                done['acc', t, a // 8] = done.get(('acc', t, a // 8), 0) + 1
                done['acct', t, a // 8] = s['tv']
            s['tv'] += vcost - 0.5 * sum((t, b) in wide for b in range(a, a + AB))
            s['i'] += 1
    assert not or_left and not wo_left and not px_left

    out, cur, cnt = [], [], 0
    for e in ev + [None]:
        if e is None or (e[0] == 'tile' and e[1] != 'gap' and cnt % 4 == ph):
            if any(x[0] == 'step' for x in cur) and len(cur) < 32:
                cur = cur[:1] + [x for x in cur[1:] if x[0] == 'piece'] + [x for x in cur[1:] if x[0] != 'piece']
            out += cur
            cur = []
        if e is not None:
            cur.append(e)
            cnt += (4 if e[1] == 'gap' else 1) * (e[0] == 'tile')
    return out


def _slots(events, key):
    first, last = {}, {}
    for n, e in enumerate(events):
        k = key(e)
        if k is not None:
            first.setdefault(k, n)
            last[k] = n
    slot, busy = {}, []
    for k in first:
        free = [i for i, u in enumerate(busy) if u < first[k]]
        slot[k] = free[0] if free else len(busy)
        busy[slot[k]:slot[k] + 1] = [last[k]]
    return slot, len(busy)


def _run(opts, A_x, A_k_cache, A_v_cache, A_wq, A_wo, B_w3, B_w4):
    B, S, D = A_x.shape
    _, H, Sk, Dh = A_k_cache.shape
    F = B_w3.shape[1]
    W = min(4096, max(256, Sk // 4))
    assert (B, S, H, Dh, W) == (1, 1, 32, 192, 4096) and D % 128 == 0 and F % 128 == 0
    AP = Dh // 8
    KT = W // 128
    NP = H // 2
    DT, FT = D // 128, F // 128
    AB, SG, FD = 4, 2, opts.get('fd', 5)
    SKEW = opts.get('skew', 1)
    cexp = (Dh ** -0.5) * _LOG2E
    nx = {u[:2]: u[2] for u in opts['xunits']}
    xunits = list(nx)
    wide = [(t, a) for t in range(NP) for a in range(0, AP, AB) if (t, a // 8) not in xunits + [(NP - 1, 2)]]
    drop = [g for n, g in enumerate(wide) if n % 3][:max(0, len(wide) - opts['nwide'])]
    wide = [g for g in wide if g not in drop] + [(t, a + 2) for t, a in wide[::-1]][:max(0, opts['nwide'] - len(wide))]
    late = [(t, a) for b in (0, 2) for t in range(NP - 1, 0, -1) for a in range(b, AP, AB)
            if (t, a // 8) not in xunits + [(NP - 1, 2)] and (t, a) not in wide]
    nlate = opts['nlate']
    late = {g: (c, n) for c in range(DT - 1) for n, g in enumerate(late[sum(nlate[:c]):sum(nlate[:c + 1])])}
    events = _schedule(NP, KT, DT, AP, AB, SG, wide=wide + list(late), **opts)
    sp, RP = _slots(events, lambda e: e[1] - (e[1] == 0 and e[2] < AP // 2) if e[0] == 'step'
                    else e[2] if e[1] in ('sma', 'smb', 'pvx') else None)
    ss, RS = _slots(events, lambda e: max(e[2], 0) if e[1] in ('qk', 'sma') else None)
    sq, RQ = _slots(events, lambda e: e[2] if e[1] in ('q', 'qfin') else None)
    sx, RX = _slots(events, lambda e: e[2:4] if e[1] in ('pvx', 'xsum') else None)
    sw, RM = _slots(events, lambda e: e[2] if e[1] in ('wo', 'wacc') else None)
    so, RO = _slots(events, lambda e: e[2:4] if e[1] in ('or', 'ofin') else None)
    sl, RL = _slots(events, lambda e: e[2] if e[1] in ('smb', 'wld') else None)
    assert _slots(events, lambda e: e[2] if e[1] in ('sma', 'smb') else None)[1] == 1
    sizes = [3 * NP, 3 * NP, 2 * NP, 2, DT, 2 * NP + 3, KT, KT * len(wide)]
    QP, Q0, WB, XL, XA, MB, AL, WD, NBIG = [sum(sizes[:n]) for n in range(len(sizes) + 1)]
    OB = Q0
    free, acc_at = [AL, AL + 16], {}
    for e in events:
        if e[0] == 'step' and (e[1], e[2] // 8) not in acc_at:
            acc_at[e[1], e[2] // 8] = free.pop(0)
        if e[0] == 'step' and e[3] == KT - 1:
            free += [WD + KT * wide.index((e[1], a)) + n for a in range(e[2], e[2] + AB) if (e[1], a) in wide
                     for n in (0, 16)]
    sizes = [RP * KT, 3 * RS * KT, RX * KT, 3 * RQ, 4 * DT * RM, 2 * RO, 2 * RL]
    _, SP, XP, QR, WR, OR, ML, NPB = [sum(sizes[:n]) for n in range(len(sizes) + 1)]
    NV, NQ = opts.get('nv', 5), opts.get('nq', 8)
    assert nlate[DT - 2] == 0 and 2 * nlate[DT - 3] <= 11 + (3 * NP - NQ) // 4
    if opts.get('verbose'):
        print('RP RS RQ RX RM', RP, RS, RQ, RX, RM, 'free tiles', (int(13.25 * 256) - NBIG - NPB))
    order1 = sorted(range(NP), key=lambda t: all(u[0] != t for u in xunits))

    def kernel(x_hbm, k_hbm, v_hbm, wq_hbm, wo_hbm, w3_hbm, w4_hbm, o_ref, *scratch):
        k_bufs, v_bufs, scratch = scratch[:NP], scratch[NP:2 * NP], scratch[2 * NP:]
        w4_bufs, wq_bufs, scratch = scratch[:DT], scratch[DT:2 * DT], scratch[2 * DT:]
        wo_buf, w3_buf, pbuf, cst, big, hbuf, xres, x_buf, sems = scratch
        t0 = (Sk - W) // 128

        def kv_cp(kind, t):
            src, dst = (k_hbm, k_bufs[t]) if kind == 0 else (v_hbm, v_bufs[t])
            return [pltpu.make_async_copy(src.at[pl.ds(AP * t, AP), a, pl.ds(t0, KT)],
                                          dst.at[:, :, pl.ds(8 * a, 8), :], sems.at[2 * t + kind])
                    for a in range(2)]

        def w_cp(src, dst, n, sem):
            rows = src.shape[0] // n
            return [pltpu.make_async_copy(src.at[pl.ds(i * rows, rows), a],
                                          dst.at[pl.ds(i * rows, rows), :, pl.ds(8 * a, 8), :], sem)
                    for i in range(n) for a in range(2)]

        def wq_cp():
            cps = [cp for j in range(DT) for cp in w_cp(wq_hbm.at[pl.ds(8 * j, 8)], wq_bufs[j], 1, sems.at[2 * NP])]
            return cps[:1] + [pltpu.make_async_copy(x_hbm, x_buf, sems.at[2 * NP])] + cps[1:]

        def wo_cp():
            return w_cp(wo_hbm, wo_buf, 8, sems.at[2 * NP + 1])

        def w3_cp():
            return [pltpu.make_async_copy(w3_hbm, w3_buf, sems.at[2 * NP + 2])]

        def w4_cp(c):
            return [pltpu.make_async_copy(w4_hbm.at[:, pl.ds(128 * c, 128)], w4_bufs[c], sems.at[2 * NP + 3 + c])]

        def wait(cps):
            for cp in cps:
                cp.wait()

        cps = wq_cp()
        for t in order1:
            cps += kv_cp(0, t) + kv_cp(1, t) + (wo_cp() if t == order1[0] else [])
        for cp in cps + w3_cp() + [cp for c in range(DT) for cp in w4_cp(c)]:
            cp.start()

        ku = [r.bitcast(u32) for r in k_bufs]
        vu = [r.bitcast(u32) for r in v_bufs]
        wqu = [r.bitcast(u32) for r in wq_bufs]
        wou = wo_buf.bitcast(u32)
        w4u = [r.bitcast(u32) for r in w4_bufs]

        def top(n):
            return lax.broadcasted_iota(i32, (8, n), 0) < 4

        def left():
            return lax.broadcasted_iota(i32, (8, 128), 1) < 64

        def cols(n):
            return slice(128 * n, 128 * (n + 1))

        def rows(j):
            return slice(8 * j, 8 * j + 8)

        def masks():
            return [top(128), top(128) == left(), jnp.logical_not(top(128))]

        def mlp_hidden(x):
            lhs = jnp.where(top(D), x, 1.0)
            m1 = jnp.mean(x, axis=-1, keepdims=True)
            xc = x - m1
            v1 = jnp.mean(xc * xc, axis=-1, keepdims=True)
            r1 = lax.rsqrt(v1 + _EPS)
            y = xc * r1
            m2 = jnp.mean(xc, axis=-1, keepdims=True) * r1
            r2 = lax.rsqrt(v1 * r1 * r1 - m2 * m2 + _EPS)
            coef = jnp.where(top(128), r1 * r2, -(r2 * (r1 * m1 + m2)))
            hs = []
            for n in range(FT):
                u = _tree(jnp.add, [_mm(lhs[:, cols(j)], w3_buf[cols(j), cols(n)]) for j in range(DT)]) * coef
                hs.append(jax.nn.gelu(u + pltpu.roll(u, 4, 0), approximate=True))
            return y, hs

        def w4_tile(n, c):
            return pltpu.bitcast(w4u[c][64 * n:64 * (n + 1)], bf16)

        def late_at(n, k):
            return ((n * KT + k + 2) % (24 * NP)) // (3 * NP), (n * KT + k + 2) % (3 * NP)

        def unpack_late(c, n0, n1, after=None):
            todo = [(g, n, k) for g, (cc, n) in late.items() if cc == c for k in range(KT)][16 * n0:16 * n1]
            if todo and after is not None:
                wqu[c][after[0], 0] = pltpu.bitcast(after[1], u32)
            for (t, a), n, k in todo:
                y = pltpu.bitcast(pltpu.bitcast(vu[t][a, k], bf16).astype(f32), u32)
                wqu[c][late_at(n, k)] = y[8:16]
                vu[t][a, k] = y[0:8]

        def layer1(z):
            for u, mask in enumerate(masks()):
                cst[u] = jnp.where(mask, cexp, 0.0).astype(f32)
            wait(wq_cp())
            x = jnp.broadcast_to(x_buf[...].astype(f32), (8, D))
            _, xc, r = _stats(x)
            xn = xc * r

            def q_body(t, c):
                for i in range(3):
                    q = _tree(jnp.add, [_mm(xn[:, cols(j)], _wtile(wqu[j][:, 3 * t + i])) for j in range(DT)])
                    big[QP + 3 * t + i] = q * cst[i]
                return c
            lax.fori_loop(0, NP, q_body, 0)

            att = [jnp.zeros((8, 128), f32)] * DT
            for t in order1:
                def s_body(k, c, t=t, q=[big[QP + 3 * t + j] for j in range(3)]):
                    big[AL + k] = _tree(jnp.add, [_mm(q[j], _wtile(ku[t][rows(j), k])) for j in range(3)])
                    return c

                def o_body(k, o, t=t):
                    return [o[j] + _mm(big[AL + k], _wtile(vu[t][rows(j), k]), _NT) for j in range(3)]

                wait(kv_cp(0, t))
                lax.fori_loop(0, KT, s_body, 0, unroll=8)
                sc = big[AL:AL + KT]
                p = jnp.exp2(sc - jnp.max(jnp.max(sc, axis=0), axis=1, keepdims=True))
                big[AL:AL + KT] = p
                inv = 1.0 / jnp.sum(jnp.sum(p, axis=0), axis=1, keepdims=True)
                wait(kv_cp(1, t) + (wo_cp() if t == order1[0] else []))
                o = lax.fori_loop(0, KT, o_body, [jnp.zeros((8, 128), f32)] * 3, unroll=8)
                o = [jnp.where(mask, o[j] * inv, 0.0) for j, mask in enumerate(masks())]
                att = [att[c] + _tree(jnp.add, [_mm(o[j], _wtile(wou[rows(3 * t + j), c])) for j in range(3)])
                       for c in range(DT)]
                for j in [j for tt, j in xunits if tt == t]:
                    def t_body(k, c, t=t, j=j):
                        w = _wtile(vu[t][rows(j), k]).astype(f32).T.astype(bf16)
                        vu[t][rows(j), k] = pltpu.bitcast(w, u32).reshape(8, 8, 128)
                        return c
                    lax.fori_loop(0, nx[t, j], t_body, 0, unroll=4)
                for n, a in [(n, a) for n, (tt, a) in enumerate(wide) if tt == t]:
                    y = _wtile(vu[t][a]).astype(f32).reshape(KT, 16, 128)
                    big[WD + n * KT:WD + (n + 1) * KT] = y[:, 8:16]
                    vu[t][a] = pltpu.bitcast(y[:, 0:8], u32)
            att = jnp.concatenate(att, axis=1)
            x = x + (att + pltpu.roll(att, 4, 0))
            wait(w3_cp())
            y, hs = mlp_hidden(x)
            xres[...] = x + y
            for n in range(FT):
                hbuf[n] = hs[n]
            for c in range(DT - 1):
                wait(w4_cp(c))
                unpack_late(c - 1, 0, 7)
                xc = xres[:, cols(c)] + _tree(jnp.add, [_mm(hbuf[n], w4_tile(n, c)) for n in range(FT)])
                xres[:, cols(c)] = xc
                xc = jnp.where(top(128), xc, 1.0)
                unpack_late(c - 1, 7, 11, (z, xc))
                for n in range(3 * NP - (NQ if c == DT - 2 else 0)):
                    r = _mm(xc, _wtile(wqu[c][:, n]))
                    big[Q0 + n] = big[Q0 + n] + r if c else r
                    if n % 4 == 0:
                        unpack_late(c - 1, 11 + n // 4, 12 + n // 4, (z, r))

        def layer2(z):
            wait(w4_cp(DT - 1))
            if opts.get('skip2'):
                keep = big[Q0 + z] + sum(pltpu.bitcast(r[z, 1], f32) for r in wqu + vu)
                o_ref[...] = (xres[0:1, :] + jnp.concatenate([keep[0:1]] * DT, axis=1)).astype(o_ref.dtype)
                return
            xc = xres[:, cols(DT - 1)] + _tree(jnp.add, [_mm(hbuf[n], w4_tile(n, DT - 1)) for n in range(FT)])
            for n in range(3 * NP - NQ, 3 * NP):
                xp = jnp.where(top(128), xres[:, cols(DT - 2)], 1.0)
                big[Q0 + n] = big[Q0 + n] + _mm(xp, _wtile(wqu[DT - 2][:, n]))
            xres[:, cols(DT - 1)] = xc
            m, _, r = _stats(xres[...])
            big[XL] = xraw = jnp.where(top(128), xc, 1.0)
            coef0 = jnp.where(top(128), 1.0, -m)
            big[XL + 1] = coef = coef0 * r
            acc, val, fwd = {}, {}, []
            st = dict(pin=False, dirty=False, cnt=0, started=False, left=sum(e[0] == 'step' for e in events))

            def lhs(n):
                if st['pin']:
                    st['pin'] = False
                    return big[n + z]
                if n not in val:
                    val[n] = big[n]
                return val[n]

            def checkpoint():
                for (t, a), y in acc.items():
                    n = acc_at[t, a // 8] + 2 * (a % 8)
                    big[n:n + 2] = y.reshape(2, 8, 128)

            def put(n, r):
                fwd.append((st['cnt'], n, r))

            def flush(upto, pin=False):
                while fwd and fwd[0][0] <= upto:
                    _, n, r = fwd.pop(0)
                    pbuf[z if pin else 0, :, cols(n)] = r
                    if pin and st['left'] <= opts.get('vpin', 72):
                        vu[NP - 1][z, 2] = pltpu.bitcast(r, u32)
                    pin = False

            def get(n):
                flush(max([c for c, m, _ in fwd if m == n], default=-1))
                return pbuf[0, :, cols(n)]

            def ptile(t, k):
                return cols(sp[t] * KT + k)

            def prow(t, odd, k):
                return pbuf[0, 4 * odd:4 * odd + 1, ptile(t - (t + odd == 0), k)]

            def q_fin(t, i, y, coef):
                y = (y + big[Q0 + 3 * t + i]) * coef
                big[QP + 3 * t + i] = (y + pltpu.roll(y, 4, 0)) * cst[i]

            def t_qraw(t, i):
                q_fin(t, i, _mm(xraw, _wtile(wqu[DT - 1][:, 3 * t + i])), coef if t else coef0)

            def t_q(t, i):
                put(QR + sq[t] * 3 + i, _mm(lhs(XL), _wtile(wqu[DT - 1][:, 3 * t + i])))

            def t_qk(t, j, k):
                put(SP + (3 * ss[t] + j) * KT + k, _mm(lhs(QP + 3 * t + j), _wtile(ku[t][rows(j), k])))

            def t_or(t, j):
                a = big[acc_at[t, j]:acc_at[t, j] + 16].reshape(128, 128)
                if j == 1:
                    r = _mm(jnp.concatenate([lhs(WB + 2 * t), lhs(WB + 2 * t + 1)], axis=0), a, _NT)
                    put(OR + 2 * so[t, j] + 1, r[8:16])
                else:
                    r = _mm(lhs(WB + 2 * t + j // 2), a, _NT)
                put(OR + 2 * so[t, j], r[0:8])

            def t_pvx(t, j, k):
                p = val.pop(('px', t, j, k)) * lhs(WB + 2 * t + j // 2)
                put(XP + sx[t, j] * KT + k, _mm(p, _wtile(vu[t][rows(j), k])))

            def t_wo(units, n, c):
                t, j = units[n]
                put(WR + (sw[units] * 4 + n) * DT + c, _mm(lhs(OB + 3 * t + j), _wtile(wou[rows(3 * t + j), c])))

            def p_qfin(t, i):
                q_fin(t, i, get(QR + sq[t] * 3 + i), big[XL + 1])

            def p_sma(t, k0):
                n = SP + 3 * ss[max(t, 0)] * KT
                sv = []
                for k in range(k0, k0 + SG):
                    sc = get(n + k) + get(n + KT + k)
                    sc = sc + get(n + 2 * KT + k) if t >= 0 else sc
                    sv.append(sc * r if t <= 0 else sc)
                    pbuf[0, :, ptile(t, k)] = sv[-1]
                big[MB + 2 + 2 * t] = val['m'] = _tree(jnp.maximum, sv + ([val['m']] if k0 else []))

            def p_smb(t, k0):
                ps = []
                for k in range(k0, k0 + SG):
                    ps.append(jnp.exp2(pbuf[0, :, ptile(t, k)] - val['m']))
                    pbuf[0, :, ptile(t, k)] = ps[-1]
                if t >= 0:
                    big[MB + 3 + 2 * t] = val['l'] = _tree(jnp.add, ps + ([val['l']] if k0 else []))
                if t >= 0 and k0 + SG == KT:
                    pbuf[0, :, cols(ML + 2 * sl[t])] = val['m']
                    pbuf[0, :, cols(ML + 2 * sl[t] + 1)] = val['l']

            def p_wld(t):
                val['ml', t] = pbuf[0, :, cols(ML + 2 * sl[t])], pbuf[0, :, cols(ML + 2 * sl[t] + 1)]

            def p_w(t):
                m, l = val['ml', t]
                e = jnp.exp2(m - jnp.max(m, axis=1, keepdims=True))
                w = e / jnp.sum(e * l, axis=1, keepdims=True)
                for h in range(2):
                    big[WB + 2 * t + h] = jnp.broadcast_to(w[4 * h:4 * h + 1], (8, 128))

            def p_ofin(t, j):
                r = get(OR + 2 * so[t, j])
                r = jnp.where(left(), r, get(OR + 2 * so[t, j] + 1)) if j == 1 else r
                big[OB + 3 * t + j] = r + big[OB + 3 * t + j] if (t, j) in nx else r

            def p_xsum(t, j, k0):
                n = XP + sx[t, j] * KT + k0
                ys = [get(n + u) for u in range(4)] + ([val['y', t, j]] if k0 else [])
                big[OB + 3 * t + j] = val['y', t, j] = _tree(jnp.add, ys)

            def p_wacc(units, c):
                rs = [get(WR + (sw[units] * 4 + n) * DT + c) for n in range(len(units))]
                big[XA + c] = _tree(jnp.add, rs + ([big[XA + c]] if units != next(iter(sw)) else []))

            fns = {'qraw': t_qraw, 'q': t_q, 'qk': t_qk, 'or': t_or, 'pvx': t_pvx, 'wo': t_wo, 'qfin': p_qfin,
                   'sma': p_sma, 'smb': p_smb, 'wld': p_wld, 'w': p_w, 'ofin': p_ofin, 'xsum': p_xsum, 'wacc': p_wacc}
            tiles = [e for e in events if e[0] == 'tile' and e[1] != 'gap']
            for e in events:
                if e[0] == 'step':
                    _, t, a0, k = e
                    k0 = nx.get((t, a0 // 8), 0)
                    for a in range(a0, a0 + AB):
                        n = k + SKEW * (a - a0)
                        kk = k0 + (n - k0) % (KT - k0)
                        if ('p', t, a0, n) not in val:
                            val['p', t, a0, n] = prow(t, int(a0 >= AP // 2), kk)
                        if (t, a) in wide:
                            y = jnp.concatenate([pltpu.bitcast(vu[t][a, kk], f32),
                                                 big[WD + wide.index((t, a)) * KT + kk]])
                        elif (t, a) in late:
                            c, u = late[t, a]
                            y = pltpu.bitcast(jnp.concatenate([vu[t][a, kk], wqu[c][late_at(u, kk)]]), f32)
                        else:
                            y = pltpu.bitcast(vu[t][a, kk], bf16).astype(f32)
                        y = y * val['p', t, a0, n]
                        acc[t, a] = acc[t, a] + y if (t, a) in acc else y
                    st.update(dirty=True, started=True, left=st['left'] - 1)
                    if k == KT - 1:
                        checkpoint()
                        acc.clear()
                elif e[0] == 'piece':
                    fns[e[1]](*e[2:])
                elif e[1] == 'gap':
                    st['cnt'] += 4
                else:
                    pinned = st['cnt'] % 4 == opts.get('ph', 3) and st['left'] > 0
                    if pinned and st['dirty']:
                        checkpoint()
                    st.update(pin=pinned and st['started'], dirty=st['dirty'] and not pinned)
                    fns[e[1]](*e[2:])
                    st['pin'] = False
                    tiles.pop(0)
                    for u in tiles[:opts.get('pf', 4)]:
                        if u[1] == 'pvx' and ('px',) + u[2:] not in val:
                            val[('px',) + u[2:]] = prow(u[2], u[3] // 2, u[4])
                    if pinned:
                        flush(st['cnt'] - 4 * FD + 3, pin=st['started'])
                    st['cnt'] += 1
            assert not fwd
            x = xres[...] + jnp.concatenate([big[XA + c] for c in range(DT)], axis=1)
            y, hs = mlp_hidden(x)
            out = [(x + y)[:, cols(c)] for c in range(DT)]
            part = [None] * DT
            hb = [jnp.concatenate([hs[n]] * 16, axis=0).T for n in range(NV)]
            for n0 in range(0, NV, 3):
                for a in range(8):
                    for n in range(n0, min(n0 + 3, NV)):
                        for c in range(DT):
                            u = pltpu.bitcast(w4u[c][rows(8 * n + a)], bf16).astype(f32) * hb[n][16 * a:16 * a + 16]
                            part[c] = u if part[c] is None else part[c] + u
            for n in range(NV, FT):
                out = [out[c] + _mm(hs[n], w4_tile(n, c)) for c in range(DT)]
            out = [out[c] + jnp.sum(part[c], axis=0, keepdims=True) for c in range(DT)]
            o_ref[...] = jnp.concatenate(out, axis=1)[0:1].astype(o_ref.dtype)

        def body(it, carry):
            pl.when(it == 0)(lambda: layer1(it >> 4) if not opts.get('skip1') else None)
            pl.when(it == 1)(lambda: layer2(it >> 4))
            return carry

        lax.fori_loop(0, 2, body, 0)

    def V(*s, dt=f32):
        return pltpu.VMEM(s, dt)

    out = pl.pallas_call(
        kernel,
        out_shape=jax.ShapeDtypeStruct((1, D), A_x.dtype),
        in_specs=[pl.BlockSpec(memory_space=pl.ANY)] * 7,
        out_specs=pl.BlockSpec(memory_space=pltpu.VMEM),
        scratch_shapes=(
            [V(AP, KT, 16, 128, dt=bf16)] * (2 * NP)
            + [V(F, 128, dt=bf16)] * DT + [V(8, 3 * NP, 16, 128, dt=bf16)] * DT
            + [V(AP * NP, DT, 16, 128, dt=bf16), V(D, F, dt=bf16),
               V(1, 8, -(-NPB // 4) * 512), V(4, 8, 128), V(-(-NBIG // 4) * 4, 8, 128),
               V(FT, 8, 128), V(8, D), V(1, D, dt=bf16),
               pltpu.SemaphoreType.DMA((2 * NP + 3 + DT,))]),
        compiler_params=pltpu.CompilerParams(
            vmem_limit_bytes=int(opts.get('vmem', 128) * 1024 * 1024),
            disable_semaphore_checks=True, disable_bounds_checks=True),
        name='fused_decode_layers',
    )(A_x.reshape(1, D), _cache_view(A_k_cache), _cache_view(A_v_cache),
      _weight_view(A_wq), _weight_view(A_wo), B_w3, B_w4)
    return out.reshape(B, S, D)


@jax.jit
def pallas_interleave_layers__sliding_block_cached__mixer_s_mlp__decode_kernel(
    A_x: jax.Array,
    A_k_cache: jax.Array,
    A_v_cache: jax.Array,
    A_wq: jax.Array,
    A_wo: jax.Array,
    B_x: jax.Array,
    B_w1: jax.Array,
    B_w2: jax.Array,
    B_w3: jax.Array,
    B_w4: jax.Array,
):
    return _run(_OPTS, A_x, A_k_cache, A_v_cache, A_wq, A_wo, B_w3, B_w4)
```

```python
import jax
import jax.numpy as jnp
from jax import lax
import jax.experimental.pallas as pl
import jax.experimental.pallas.tpu as pltpu

f32, bf16, u32, i32 = jnp.float32, jnp.bfloat16, jnp.uint32, jnp.int32
_EPS = 1e-5
_LOG2E = 1.4426950408889634
_NN = (((1,), (0,)), ((), ()))
_NT = (((1,), (1,)), ((), ()))

_OPTS = dict(xunits=[(5, 0, 32), (7, 2, 32), (9, 2, 32), (11, 0, 32), (12, 2, 32), (14, 2, 12)], nwide=78, nlate=[10, 10, 9, 0], qlead=2.0, keep=8,
             AD=100, LAT=205, LAT0=205, q2at=20, vpin=72)


def _stats(x):
    m = jnp.mean(x, axis=-1, keepdims=True)
    xc = x - m
    v = jnp.mean(xc * xc, axis=-1, keepdims=True)
    return m, xc, lax.rsqrt(v + _EPS)


def _tree(op, xs):
    xs = list(xs)
    while len(xs) > 1:
        nxt = [op(xs[i], xs[i + 1]) for i in range(0, len(xs) - 1, 2)]
        if len(xs) % 2:
            nxt.append(xs[-1])
        xs = nxt
    return xs[0]


def _wtile(u):
    return pltpu.bitcast(u.reshape(u.shape[0] * 8, 128), bf16)


def _mm(lhs, w, dims=_NN):
    return lax.dot_general(lhs, w, dims, preferred_element_type=f32)


def _cache_view(c):
    _, H, Sk, Dh = c.shape
    c = c.reshape(H, Sk // 128, 128, Dh // 16, 2, 8)
    c = jnp.transpose(c, (0, 3, 4, 1, 5, 2))
    return c.reshape(H * Dh // 16, 2, Sk // 128, 8, 128)


def _weight_view(w):
    R, N = w.shape
    w = w.reshape(R // 16, 2, 8, N // 128, 128)
    return jnp.transpose(w, (0, 1, 3, 2, 4))


def _schedule(NP, KT, DT, AP, AB, SG, xunits, qlead, keep, LAT=205, LAT0=165, LEAD=32, WD=140, WL=400, AD=160,
              vcost=5.95, pstride=2, nraw=8, q2at=40, ph=3, wide=(), wk=(8, 20), cmaj=4, **_):
    xs = {u[:2]: u[2] for u in xunits}
    grp = [(t, a) for t in range(NP) for a in range(0, AP, AB)]
    grp[-2:] = grp[:-3:-1]
    steps = [(t, a, k) for t, a in grp for k in range(xs.get((t, a // 8), 0), KT)]
    first_step = {}
    for i, s in enumerate(steps):
        first_step.setdefault(s[0], i)
    main = [('qraw', t, i) for t in range(nraw) for i in range(3)]
    for t in range(NP):
        qk = [('qk', t, j, k) for j in range(3) for k in range(KT)]
        main += qk[:q2at] + [('q', t + 1, i) for i in range(3) if nraw <= t + 1 < NP] + qk[q2at:]
    done = {('q', t): 3 for t in range(nraw)}
    or_left = [(t, j) for t in range(NP) for j in range(3) if xs.get((t, j), 0) < KT]
    wo_left = [(t, j) for t in range(NP) for j in range(3)]
    px_left = list(xs)
    ev, pend, wait, cur = [], [], [], []
    s = dict(tm=0.0, tv=0.0, i=0, mi=0, qk=0)

    def sm(t):
        return ([(('sma', t, k), 3 * SG, None, 0) for k in range(0, KT, SG)]
                + [(('smb', t, k), 3 * SG, ('p', t), SG) for k in range(0, KT, SG)])

    def g_wo(n):
        wo = tuple(u for u in wo_left if done.get(('o',) + u, 0) >= 1)[:4]
        if len(wo_left) > cmaj:
            wo = wo[:len(wo_left) - cmaj]
        if len(wo) < n:
            return None
        for u in wo:
            wo_left.remove(u)
        g = [(('wo', wo, n, c), 8, []) for n in range(len(wo)) for c in range(DT)]
        if not wo_left and cmaj:
            g.sort(key=lambda x: x[0][3])
        g[-1] = (g[-1][0], 8, [(('wacc', wo, c), len(wo), None, 0) for c in range(DT)])
        return g

    def g_or(n, last):
        rd = [u for u in or_left if done.get(('acc',) + u, 0) >= 8 // AB and done.get(('w', u[0]), 0)
              and (last or done[('acct',) + u] + AD <= s['tv'])
              and done.get(('y',) + u, 0) >= xs.get(u, 0)][:4]
        if len(rd) < n:
            return None
        for u in rd:
            or_left.remove(u)
        return [(('gap',), 8 * len(rd), [])] + [(('or',) + u, 8, [(('ofin',) + u, 1, ('o',) + u, 1)]) for u in rd]

    def g_px():
        rd = [u for u in px_left if done.get(('w', u[0]), 0)]
        if not rd:
            return None
        px_left.remove(rd[0])
        n = xs[rd[0]]
        g = [(('pvx',) + rd[0] + (k,), 8, []) for k in range(n)]
        e, inc = (('o',) + rd[0], 4 / KT) if n == KT else (('y',) + rd[0], 4)
        g[-1] = (g[-1][0], 8, [(('xsum',) + rd[0] + (k,), 4, e, inc) for k in range(0, n, 4)])
        return g

    def pick():
        last, endgame, nxt = s['i'] >= len(steps), s['mi'] >= len(main), s['qk']
        if last:
            return g_or(1, True) or g_px() or g_wo(len(wo_left) if 0 < len(wo_left) <= cmaj else 1)
        if endgame:
            return g_or(4, False) or g_px() or g_wo(4) or (g_wo(1) if len(wo_left) > cmaj else None)
        rem = sum(8 for m in main[s['mi']:s['mi'] + 200] if m[0] != 'qk' or m[1] == nxt)
        if (first_step[nxt] - s['i']) * vcost - rem > qlead * 500:
            g = (g_wo(4) if len(wo_left) > keep else None) or g_or(4, False) or g_px()
            if g:
                return g
        m = main[s['mi']]
        if m[0] == 'qk' and done.get(('q', m[1]), 0) < 3:
            return None
        s['mi'] += 1
        pcs = []
        if m[0] == 'q':
            pcs = [(('qfin',) + m[1:], 5, ('q', m[1]), 1)]
        if m[0] == 'qk' and (m[2] == 2 or m[1:3] == (0, 1)) and m[3] % SG == SG - 1:
            t = m[1] if m[2] == 2 else -1
            pcs = [sm(t)[m[3] // SG]] + (sm(t)[KT // SG:] if m[3] == KT - 1 else [])
        return [(m, 8, pcs)]

    def later(t, pcs):
        wait.append((t, pcs))
        wait.sort(key=lambda w: w[0])

    def piece():
        a, cv, e, inc = pend.pop(0)
        if a[0] == 'wld' and s['i'] < len(steps) and not wk[0] <= steps[s['i']][2] <= wk[1]:
            return later(s['tv'] + 30, [(a, cv, e, inc)])
        ev.append(('piece',) + a)
        s['tv'] += cv / 4
        if e is not None:
            done[e] = done.get(e, 0) + inc
        if a[0] == 'smb' and a[2] == KT - SG and a[1] >= 0:
            later(s['tv'] + WD, [(('wld', a[1]), 0, ('wld', a[1]), 1)])
        if a[0] == 'wld':
            later(s['tv'] + WL, [(('w', a[1]), 24, ('w', a[1]), 1)])

    def urgent(p):
        return p[2] is not None and p[2][0] != 'p'

    while True:
        while wait and wait[0][0] <= s['tv']:
            pcs = wait.pop(0)[1]
            pend[:] = [p for p in pcs if urgent(p)] + pend + [p for p in pcs if not urgent(p)]
        i = s['i']
        more = i < len(steps)
        blocked = not more or done.get(('p', steps[i][0] - (i < AP // 2 // AB * KT)), 0) < min(KT, steps[i][2] + 6)
        if not cur and (s['tm'] + LEAD <= s['tv'] or blocked):
            cur = pick() or []
        if not more and not pend and not wait and not cur:
            break
        if cur and (s['tm'] + LEAD <= s['tv']
                    or (blocked and not pend and (not wait or s['tm'] + LEAD <= wait[0][0]))):
            a, cm, pcs = cur.pop(0)
            ev.append(('tile',) + a)
            s['tm'] = max(s['tm'], s['tv'] - LEAD - 8) + cm
            s['tv'] += 0.25 * (a[0] == 'pvx')
            s['qk'] += a[0] == 'qk' and a[2:] == (2, KT - 1)
            if pcs:
                later(s['tm'] + (LAT if 0 < i < len(steps) else LAT0), pcs)
        elif blocked and pend:
            piece()
        elif blocked:
            s['tv'] = max(s['tv'], wait[0][0])
        else:
            if pend and (i % pstride == 0 or urgent(pend[0])):
                piece()
            t, a, k = steps[i]
            ev.append(('step', t, a, k))
            if k == KT - 1:
                done['acc', t, a // 8] = done.get(('acc', t, a // 8), 0) + 1
                done['acct', t, a // 8] = s['tv']
            s['tv'] += vcost - 0.5 * sum((t, b) in wide for b in range(a, a + AB))
            s['i'] += 1
    assert not or_left and not wo_left and not px_left

    out, cur, cnt = [], [], 0
    for e in ev + [None]:
        if e is None or (e[0] == 'tile' and e[1] != 'gap' and cnt % 4 == ph):
            if any(x[0] == 'step' for x in cur) and len(cur) < 32:
                cur = cur[:1] + [x for x in cur[1:] if x[0] == 'piece'] + [x for x in cur[1:] if x[0] != 'piece']
            out += cur
            cur = []
        if e is not None:
            cur.append(e)
            cnt += (4 if e[1] == 'gap' else 1) * (e[0] == 'tile')
    return out


def _slots(events, key):
    first, last = {}, {}
    for n, e in enumerate(events):
        k = key(e)
        if k is not None:
            first.setdefault(k, n)
            last[k] = n
    slot, busy = {}, []
    for k in first:
        free = [i for i, u in enumerate(busy) if u < first[k]]
        slot[k] = free[0] if free else len(busy)
        busy[slot[k]:slot[k] + 1] = [last[k]]
    return slot, len(busy)


def _run(opts, A_x, A_k_cache, A_v_cache, A_wq, A_wo, B_w3, B_w4):
    B, S, D = A_x.shape
    _, H, Sk, Dh = A_k_cache.shape
    F = B_w3.shape[1]
    W = min(4096, max(256, Sk // 4))
    assert (B, S, H, Dh, W) == (1, 1, 32, 192, 4096) and D % 128 == 0 and F % 128 == 0
    AP = Dh // 8
    KT = W // 128
    NP = H // 2
    DT, FT = D // 128, F // 128
    AB, SG, FD = 4, 2, opts.get('fd', 5)
    SKEW = opts.get('skew', 1)
    cexp = (Dh ** -0.5) * _LOG2E
    nx = {u[:2]: u[2] for u in opts['xunits']}
    xunits = list(nx)
    wide = [(t, a) for t in range(NP) for a in range(0, AP, AB) if (t, a // 8) not in xunits + [(NP - 1, 2)]]
    drop = [g for n, g in enumerate(wide) if n % 3][:max(0, len(wide) - opts['nwide'])]
    wide = [g for g in wide if g not in drop] + [(t, a + 2) for t, a in wide[::-1]][:max(0, opts['nwide'] - len(wide))]
    late = [(t, a) for b in (0, 2) for t in range(NP - 1, 0, -1) for a in range(b, AP, AB)
            if (t, a // 8) not in xunits + [(NP - 1, 2)] and (t, a) not in wide]
    nlate = opts['nlate']
    late = {g: (c, n) for c in range(DT - 1) for n, g in enumerate(late[sum(nlate[:c]):sum(nlate[:c + 1])])}
    events = _schedule(NP, KT, DT, AP, AB, SG, wide=wide + list(late), **opts)
    sp, RP = _slots(events, lambda e: e[1] - (e[1] == 0 and e[2] < AP // 2) if e[0] == 'step'
                    else e[2] if e[1] in ('sma', 'smb', 'pvx') else None)
    ss, RS = _slots(events, lambda e: max(e[2], 0) if e[1] in ('qk', 'sma') else None)
    sq, RQ = _slots(events, lambda e: e[2] if e[1] in ('q', 'qfin') else None)
    sx, RX = _slots(events, lambda e: e[2:4] if e[1] in ('pvx', 'xsum') else None)
    sw, RM = _slots(events, lambda e: e[2] if e[1] in ('wo', 'wacc') else None)
    so, RO = _slots(events, lambda e: e[2:4] if e[1] in ('or', 'ofin') else None)
    sl, RL = _slots(events, lambda e: e[2] if e[1] in ('smb', 'wld') else None)
    assert _slots(events, lambda e: e[2] if e[1] in ('sma', 'smb') else None)[1] == 1
    sizes = [3 * NP, 3 * NP, 2 * NP, 2, DT, 2 * NP + 3, KT, KT * len(wide)]
    QP, Q0, WB, XL, XA, MB, AL, WD, NBIG = [sum(sizes[:n]) for n in range(len(sizes) + 1)]
    OB = Q0
    free, acc_at = [AL, AL + 16], {}
    for e in events:
        if e[0] == 'step' and (e[1], e[2] // 8) not in acc_at:
            acc_at[e[1], e[2] // 8] = free.pop(0)
        if e[0] == 'step' and e[3] == KT - 1:
            free += [WD + KT * wide.index((e[1], a)) + n for a in range(e[2], e[2] + AB) if (e[1], a) in wide
                     for n in (0, 16)]
    sizes = [RP * KT, 3 * RS * KT, RX * KT, 3 * RQ, 4 * DT * RM, 2 * RO, 2 * RL]
    _, SP, XP, QR, WR, OR, ML, NPB = [sum(sizes[:n]) for n in range(len(sizes) + 1)]
    NV, NQ = opts.get('nv', 4), opts.get('nq', 8)
    assert nlate[DT - 2] == 0 and 2 * nlate[DT - 3] <= 11 + (3 * NP - NQ) // 4
    if opts.get('verbose'):
        print('RP RS RQ RX RM', RP, RS, RQ, RX, RM, 'free tiles', (int(13.25 * 256) - NBIG - NPB))
    order1 = sorted(range(NP), key=lambda t: all(u[0] != t for u in xunits))

    def kernel(x_hbm, k_hbm, v_hbm, wq_hbm, wo_hbm, w3_hbm, w4_hbm, o_ref, *scratch):
        k_bufs, v_bufs, scratch = scratch[:NP], scratch[NP:2 * NP], scratch[2 * NP:]
        w4_bufs, wq_bufs, scratch = scratch[:DT], scratch[DT:2 * DT], scratch[2 * DT:]
        wo_buf, w3_buf, pbuf, cst, big, hbuf, xres, x_buf, sems = scratch
        t0 = (Sk - W) // 128

        def kv_cp(kind, t):
            src, dst = (k_hbm, k_bufs[t]) if kind == 0 else (v_hbm, v_bufs[t])
            return [pltpu.make_async_copy(src.at[pl.ds(AP * t, AP), a, pl.ds(t0, KT)],
                                          dst.at[:, :, pl.ds(8 * a, 8), :], sems.at[2 * t + kind])
                    for a in range(2)]

        def w_cp(src, dst, n, sem):
            rows = src.shape[0] // n
            return [pltpu.make_async_copy(src.at[pl.ds(i * rows, rows), a],
                                          dst.at[pl.ds(i * rows, rows), :, pl.ds(8 * a, 8), :], sem)
                    for i in range(n) for a in range(2)]

        def wq_cp():
            cps = [cp for j in range(DT) for cp in w_cp(wq_hbm.at[pl.ds(8 * j, 8)], wq_bufs[j], 1, sems.at[2 * NP])]
            return cps[:1] + [pltpu.make_async_copy(x_hbm, x_buf, sems.at[2 * NP])] + cps[1:]

        def wo_cp():
            return w_cp(wo_hbm, wo_buf, 8, sems.at[2 * NP + 1])

        def w3_cp():
            return [pltpu.make_async_copy(w3_hbm, w3_buf, sems.at[2 * NP + 2])]

        def w4_cp(c):
            return [pltpu.make_async_copy(w4_hbm.at[:, pl.ds(128 * c, 128)], w4_bufs[c], sems.at[2 * NP + 3 + c])]

        def wait(cps):
            for cp in cps:
                cp.wait()

        cps = wq_cp()
        for t in order1:
            cps += kv_cp(0, t) + kv_cp(1, t) + (wo_cp() if t == order1[0] else [])
        for cp in cps + w3_cp() + [cp for c in range(DT) for cp in w4_cp(c)]:
            cp.start()

        ku = [r.bitcast(u32) for r in k_bufs]
        vu = [r.bitcast(u32) for r in v_bufs]
        wqu = [r.bitcast(u32) for r in wq_bufs]
        wou = wo_buf.bitcast(u32)
        w4u = [r.bitcast(u32) for r in w4_bufs]

        def top(n):
            return lax.broadcasted_iota(i32, (8, n), 0) < 4

        def left():
            return lax.broadcasted_iota(i32, (8, 128), 1) < 64

        def cols(n):
            return slice(128 * n, 128 * (n + 1))

        def rows(j):
            return slice(8 * j, 8 * j + 8)

        def masks():
            return [top(128), top(128) == left(), jnp.logical_not(top(128))]

        def mlp_hidden(x):
            lhs = jnp.where(top(D), x, 1.0)
            m1 = jnp.mean(x, axis=-1, keepdims=True)
            xc = x - m1
            v1 = jnp.mean(xc * xc, axis=-1, keepdims=True)
            r1 = lax.rsqrt(v1 + _EPS)
            y = xc * r1
            m2 = jnp.mean(xc, axis=-1, keepdims=True) * r1
            r2 = lax.rsqrt(v1 * r1 * r1 - m2 * m2 + _EPS)
            coef = jnp.where(top(128), r1 * r2, -(r2 * (r1 * m1 + m2)))
            hs, NF = [], opts.get('nf', 4)
            first = {(n, j): _mm(lhs[:, cols(j)], w3_buf[cols(j), cols(n)]) for j in range(DT) for n in range(NF)}
            for n in range(FT):
                u = _tree(jnp.add, [first[n, j] if n < NF else _mm(lhs[:, cols(j)], w3_buf[cols(j), cols(n)])
                                    for j in range(DT)]) * coef
                hs.append(jax.nn.gelu(u + pltpu.roll(u, 4, 0), approximate=True))
            return y, hs

        def w4_tile(n, c):
            return pltpu.bitcast(w4u[c][64 * n:64 * (n + 1)], bf16)

        def late_at(n, k):
            return ((n * KT + k + 2) % (24 * NP)) // (3 * NP), (n * KT + k + 2) % (3 * NP)

        def unpack_late(c, n0, n1, after=None):
            todo = [(g, n, k) for g, (cc, n) in late.items() if cc == c for k in range(KT)][16 * n0:16 * n1]
            if todo and after is not None:
                wqu[c][after[0], 0] = pltpu.bitcast(after[1], u32)
            for (t, a), n, k in todo:
                y = pltpu.bitcast(pltpu.bitcast(vu[t][a, k], bf16).astype(f32), u32)
                wqu[c][late_at(n, k)] = y[8:16]
                vu[t][a, k] = y[0:8]

        def layer1(z):
            for u, mask in enumerate(masks()):
                cst[u] = jnp.where(mask, cexp, 0.0).astype(f32)
            wait(wq_cp())
            x = jnp.broadcast_to(x_buf[...].astype(f32), (8, D))
            _, xc, r = _stats(x)
            xn = xc * r

            def q_body(t, c):
                for i in range(3):
                    q = _tree(jnp.add, [_mm(xn[:, cols(j)], _wtile(wqu[j][:, 3 * t + i])) for j in range(DT)])
                    big[QP + 3 * t + i] = q * cst[i]
                return c
            lax.fori_loop(0, NP, q_body, 0)

            att = [jnp.zeros((8, 128), f32)] * DT
            for t in order1:
                def s_body(k, c, t=t, q=[big[QP + 3 * t + j] for j in range(3)]):
                    big[AL + k] = _tree(jnp.add, [_mm(q[j], _wtile(ku[t][rows(j), k])) for j in range(3)])
                    return c

                def o_body(k, o, t=t):
                    return [o[j] + _mm(big[AL + k], _wtile(vu[t][rows(j), k]), _NT) for j in range(3)]

                wait(kv_cp(0, t))
                lax.fori_loop(0, KT, s_body, 0, unroll=8)
                sc = big[AL:AL + KT]
                p = jnp.exp2(sc - jnp.max(jnp.max(sc, axis=0), axis=1, keepdims=True))
                big[AL:AL + KT] = p
                inv = 1.0 / jnp.sum(jnp.sum(p, axis=0), axis=1, keepdims=True)
                wait(kv_cp(1, t) + (wo_cp() if t == order1[0] else []))
                o = lax.fori_loop(0, KT, o_body, [jnp.zeros((8, 128), f32)] * 3, unroll=8)
                o = [jnp.where(mask, o[j] * inv, 0.0) for j, mask in enumerate(masks())]
                att = [att[c] + _tree(jnp.add, [_mm(o[j], _wtile(wou[rows(3 * t + j), c])) for j in range(3)])
                       for c in range(DT)]
                for j in [j for tt, j in xunits if tt == t]:
                    def t_body(k, c, t=t, j=j):
                        w = _wtile(vu[t][rows(j), k]).astype(f32).T.astype(bf16)
                        vu[t][rows(j), k] = pltpu.bitcast(w, u32).reshape(8, 8, 128)
                        return c
                    lax.fori_loop(0, nx[t, j], t_body, 0, unroll=4)
                for n, a in [(n, a) for n, (tt, a) in enumerate(wide) if tt == t]:
                    y = _wtile(vu[t][a]).astype(f32).reshape(KT, 16, 128)
                    big[WD + n * KT:WD + (n + 1) * KT] = y[:, 8:16]
                    vu[t][a] = pltpu.bitcast(y[:, 0:8], u32)
            att = jnp.concatenate(att, axis=1)
            x = x + (att + pltpu.roll(att, 4, 0))
            wait(w3_cp())
            y, hs = mlp_hidden(x)
            xres[...] = x + y
            for n in range(FT):
                hbuf[n] = hs[n]
            for c in range(DT - 1):
                wait(w4_cp(c))
                unpack_late(c - 1, 0, 7)
                xc = xres[:, cols(c)] + _tree(jnp.add, [_mm(hbuf[n], w4_tile(n, c)) for n in range(FT)])
                xres[:, cols(c)] = xc
                xc = jnp.where(top(128), xc, 1.0)
                unpack_late(c - 1, 7, 11, (z, xc))
                for n in range(3 * NP - (NQ if c == DT - 2 else 0)):
                    r = _mm(xc, _wtile(wqu[c][:, n]))
                    big[Q0 + n] = big[Q0 + n] + r if c else r
                    if n % 4 == 0:
                        unpack_late(c - 1, 11 + n // 4, 12 + n // 4, (z, r))

        def layer2(z):
            wait(w4_cp(DT - 1))
            if opts.get('skip2'):
                keep = big[Q0 + z] + sum(pltpu.bitcast(r[z, 1], f32) for r in wqu + vu)
                o_ref[...] = (xres[0:1, :] + jnp.concatenate([keep[0:1]] * DT, axis=1)).astype(o_ref.dtype)
                return
            xc = xres[:, cols(DT - 1)] + _tree(jnp.add, [_mm(hbuf[n], w4_tile(n, DT - 1)) for n in range(FT)])
            for n in range(3 * NP - NQ, 3 * NP):
                xp = jnp.where(top(128), xres[:, cols(DT - 2)], 1.0)
                big[Q0 + n] = big[Q0 + n] + _mm(xp, _wtile(wqu[DT - 2][:, n]))
            xres[:, cols(DT - 1)] = xc
            m, _, r = _stats(xres[...])
            big[XL] = xraw = jnp.where(top(128), xc, 1.0)
            coef0 = jnp.where(top(128), 1.0, -m)
            big[XL + 1] = coef = coef0 * r
            acc, val, fwd = {}, {}, []
            st = dict(pin=False, dirty=False, cnt=0, started=False, left=sum(e[0] == 'step' for e in events))

            def lhs(n):
                if st['pin']:
                    st['pin'] = False
                    return big[n + z]
                if n not in val:
                    val[n] = big[n]
                return val[n]

            def checkpoint():
                for (t, a), y in acc.items():
                    n = acc_at[t, a // 8] + 2 * (a % 8)
                    big[n:n + 2] = y.reshape(2, 8, 128)

            def put(n, r):
                fwd.append((st['cnt'], n, r))

            def flush(upto, pin=False):
                while fwd and fwd[0][0] <= upto:
                    _, n, r = fwd.pop(0)
                    pbuf[z if pin else 0, :, cols(n)] = r
                    if pin and st['left'] <= opts.get('vpin', 72):
                        vu[NP - 1][z, 2] = pltpu.bitcast(r, u32)
                    pin = False

            def get(n):
                flush(max([c for c, m, _ in fwd if m == n], default=-1))
                return pbuf[0, :, cols(n)]

            def ptile(t, k):
                return cols(sp[t] * KT + k)

            def prow(t, odd, k):
                return pbuf[0, 4 * odd:4 * odd + 1, ptile(t - (t + odd == 0), k)]

            def q_fin(t, i, y, coef):
                y = (y + big[Q0 + 3 * t + i]) * coef
                big[QP + 3 * t + i] = (y + pltpu.roll(y, 4, 0)) * cst[i]

            def t_qraw(t, i):
                q_fin(t, i, _mm(xraw, _wtile(wqu[DT - 1][:, 3 * t + i])), coef if t else coef0)

            def t_q(t, i):
                put(QR + sq[t] * 3 + i, _mm(lhs(XL), _wtile(wqu[DT - 1][:, 3 * t + i])))

            def t_qk(t, j, k):
                put(SP + (3 * ss[t] + j) * KT + k, _mm(lhs(QP + 3 * t + j), _wtile(ku[t][rows(j), k])))

            def t_or(t, j):
                a = big[acc_at[t, j]:acc_at[t, j] + 16].reshape(128, 128)
                if j == 1:
                    r = _mm(jnp.concatenate([lhs(WB + 2 * t), lhs(WB + 2 * t + 1)], axis=0), a, _NT)
                    put(OR + 2 * so[t, j] + 1, r[8:16])
                else:
                    r = _mm(lhs(WB + 2 * t + j // 2), a, _NT)
                put(OR + 2 * so[t, j], r[0:8])

            def t_pvx(t, j, k):
                p = val.pop(('px', t, j, k)) * lhs(WB + 2 * t + j // 2)
                put(XP + sx[t, j] * KT + k, _mm(p, _wtile(vu[t][rows(j), k])))

            def t_wo(units, n, c):
                t, j = units[n]
                put(WR + (sw[units] * 4 + n) * DT + c, _mm(lhs(OB + 3 * t + j), _wtile(wou[rows(3 * t + j), c])))

            def p_qfin(t, i):
                q_fin(t, i, get(QR + sq[t] * 3 + i), big[XL + 1])

            def p_sma(t, k0):
                n = SP + 3 * ss[max(t, 0)] * KT
                sv = []
                for k in range(k0, k0 + SG):
                    sc = get(n + k) + get(n + KT + k)
                    sc = sc + get(n + 2 * KT + k) if t >= 0 else sc
                    sv.append(sc * r if t <= 0 else sc)
                    pbuf[0, :, ptile(t, k)] = sv[-1]
                big[MB + 2 + 2 * t] = val['m'] = _tree(jnp.maximum, sv + ([val['m']] if k0 else []))

            def p_smb(t, k0):
                ps = []
                for k in range(k0, k0 + SG):
                    ps.append(jnp.exp2(pbuf[0, :, ptile(t, k)] - val['m']))
                    pbuf[0, :, ptile(t, k)] = ps[-1]
                if t >= 0:
                    big[MB + 3 + 2 * t] = val['l'] = _tree(jnp.add, ps + ([val['l']] if k0 else []))
                if t >= 0 and k0 + SG == KT:
                    pbuf[0, :, cols(ML + 2 * sl[t])] = val['m']
                    pbuf[0, :, cols(ML + 2 * sl[t] + 1)] = val['l']

            def p_wld(t):
                val['ml', t] = pbuf[0, :, cols(ML + 2 * sl[t])], pbuf[0, :, cols(ML + 2 * sl[t] + 1)]

            def p_w(t):
                m, l = val['ml', t]
                e = jnp.exp2(m - jnp.max(m, axis=1, keepdims=True))
                w = e / jnp.sum(e * l, axis=1, keepdims=True)
                for h in range(2):
                    big[WB + 2 * t + h] = jnp.broadcast_to(w[4 * h:4 * h + 1], (8, 128))

            def p_ofin(t, j):
                r = get(OR + 2 * so[t, j])
                r = jnp.where(left(), r, get(OR + 2 * so[t, j] + 1)) if j == 1 else r
                big[OB + 3 * t + j] = r + big[OB + 3 * t + j] if (t, j) in nx else r

            def p_xsum(t, j, k0):
                n = XP + sx[t, j] * KT + k0
                ys = [get(n + u) for u in range(4)] + ([val['y', t, j]] if k0 else [])
                big[OB + 3 * t + j] = val['y', t, j] = _tree(jnp.add, ys)

            def p_wacc(units, c):
                rs = [get(WR + (sw[units] * 4 + n) * DT + c) for n in range(len(units))]
                big[XA + c] = _tree(jnp.add, rs + ([big[XA + c]] if units != next(iter(sw)) else []))

            fns = {'qraw': t_qraw, 'q': t_q, 'qk': t_qk, 'or': t_or, 'pvx': t_pvx, 'wo': t_wo, 'qfin': p_qfin,
                   'sma': p_sma, 'smb': p_smb, 'wld': p_wld, 'w': p_w, 'ofin': p_ofin, 'xsum': p_xsum, 'wacc': p_wacc}
            tiles = [e for e in events if e[0] == 'tile' and e[1] != 'gap']
            for e in events:
                if e[0] == 'step':
                    _, t, a0, k = e
                    k0 = nx.get((t, a0 // 8), 0)
                    for a in range(a0, a0 + AB):
                        n = k + SKEW * (a - a0)
                        kk = k0 + (n - k0) % (KT - k0)
                        if ('p', t, a0, n) not in val:
                            val['p', t, a0, n] = prow(t, int(a0 >= AP // 2), kk)
                        if (t, a) in wide:
                            y = jnp.concatenate([pltpu.bitcast(vu[t][a, kk], f32),
                                                 big[WD + wide.index((t, a)) * KT + kk]])
                        elif (t, a) in late:
                            c, u = late[t, a]
                            y = pltpu.bitcast(jnp.concatenate([vu[t][a, kk], wqu[c][late_at(u, kk)]]), f32)
                        else:
                            y = pltpu.bitcast(vu[t][a, kk], bf16).astype(f32)
                        y = y * val['p', t, a0, n]
                        acc[t, a] = acc[t, a] + y if (t, a) in acc else y
                    st.update(dirty=True, started=True, left=st['left'] - 1)
                    if k == KT - 1:
                        checkpoint()
                        acc.clear()
                elif e[0] == 'piece':
                    fns[e[1]](*e[2:])
                elif e[1] == 'gap':
                    st['cnt'] += 4
                else:
                    pinned = st['cnt'] % 4 == opts.get('ph', 3) and st['left'] > 0
                    if pinned and st['dirty']:
                        checkpoint()
                    st.update(pin=pinned and st['started'], dirty=st['dirty'] and not pinned)
                    fns[e[1]](*e[2:])
                    st['pin'] = False
                    tiles.pop(0)
                    for u in tiles[:opts.get('pf', 4)]:
                        if u[1] == 'pvx' and ('px',) + u[2:] not in val:
                            val[('px',) + u[2:]] = prow(u[2], u[3] // 2, u[4])
                    if pinned:
                        flush(st['cnt'] - 4 * FD + 3, pin=st['started'])
                    st['cnt'] += 1
            assert not fwd
            x = xres[...] + jnp.concatenate([big[XA + c] for c in range(DT)], axis=1)
            y, hs = mlp_hidden(x)
            out = [(x + y)[:, cols(c)] for c in range(DT)]
            part = [None] * DT
            hb = [jnp.concatenate([hs[n]] * 16, axis=0).T for n in range(NV)]
            for n0 in range(0, NV, 3):
                for a in range(8):
                    for n in range(n0, min(n0 + 3, NV)):
                        for c in range(DT):
                            u = pltpu.bitcast(w4u[c][rows(8 * n + a)], bf16).astype(f32) * hb[n][16 * a:16 * a + 16]
                            part[c] = u if part[c] is None else part[c] + u
            for n in range(NV, FT):
                out = [out[c] + _mm(hs[n], w4_tile(n, c)) for c in range(DT)]
            out = [out[c] + jnp.sum(part[c], axis=0, keepdims=True) for c in range(DT)]
            o_ref[...] = jnp.concatenate(out, axis=1)[0:1].astype(o_ref.dtype)

        def body(it, carry):
            pl.when(it == 0)(lambda: layer1(it >> 4) if not opts.get('skip1') else None)
            pl.when(it == 1)(lambda: layer2(it >> 4))
            return carry

        lax.fori_loop(0, 2, body, 0)

    def V(*s, dt=f32):
        return pltpu.VMEM(s, dt)

    out = pl.pallas_call(
        kernel,
        out_shape=jax.ShapeDtypeStruct((1, D), A_x.dtype),
        in_specs=[pl.BlockSpec(memory_space=pl.ANY)] * 7,
        out_specs=pl.BlockSpec(memory_space=pltpu.VMEM),
        scratch_shapes=(
            [V(AP, KT, 16, 128, dt=bf16)] * (2 * NP)
            + [V(F, 128, dt=bf16)] * DT + [V(8, 3 * NP, 16, 128, dt=bf16)] * DT
            + [V(AP * NP, DT, 16, 128, dt=bf16), V(D, F, dt=bf16),
               V(1, 8, -(-NPB // 4) * 512), V(4, 8, 128), V(-(-NBIG // 4) * 4, 8, 128),
               V(FT, 8, 128), V(8, D), V(1, D, dt=bf16),
               pltpu.SemaphoreType.DMA((2 * NP + 3 + DT,))]),
        compiler_params=pltpu.CompilerParams(
            vmem_limit_bytes=int(opts.get('vmem', 128) * 1024 * 1024),
            disable_semaphore_checks=True, disable_bounds_checks=True),
        name='fused_decode_layers',
    )(A_x.reshape(1, D), _cache_view(A_k_cache), _cache_view(A_v_cache),
      _weight_view(A_wq), _weight_view(A_wo), B_w3, B_w4)
    return out.reshape(B, S, D)


@jax.jit
def pallas_interleave_layers__sliding_block_cached__mixer_s_mlp__decode_kernel(
    A_x: jax.Array,
    A_k_cache: jax.Array,
    A_v_cache: jax.Array,
    A_wq: jax.Array,
    A_wo: jax.Array,
    B_x: jax.Array,
    B_w1: jax.Array,
    B_w2: jax.Array,
    B_w3: jax.Array,
    B_w4: jax.Array,
):
    return _run(_OPTS, A_x, A_k_cache, A_v_cache, A_wq, A_wo, B_w3, B_w4)
```

```python
import jax
import jax.numpy as jnp
from jax import lax
import jax.experimental.pallas as pl
import jax.experimental.pallas.tpu as pltpu

f32, bf16, u32, i32 = jnp.float32, jnp.bfloat16, jnp.uint32, jnp.int32
_EPS = 1e-5
_LOG2E = 1.4426950408889634
_NN = (((1,), (0,)), ((), ()))
_NT = (((1,), (1,)), ((), ()))

_OPTS = dict(xunits=[(5, 0, 32), (7, 2, 32), (9, 2, 32), (11, 0, 32), (12, 2, 32), (14, 2, 16)], nwide=78, nlate=[10, 10, 9, 0], qlead=2.0, keep=8,
             AD=60, LAT=205, LAT0=205, q2at=20, vpin=36)


def _stats(x):
    m = jnp.mean(x, axis=-1, keepdims=True)
    xc = x - m
    v = jnp.mean(xc * xc, axis=-1, keepdims=True)
    return m, xc, lax.rsqrt(v + _EPS)


def _tree(op, xs):
    xs = list(xs)
    while len(xs) > 1:
        nxt = [op(xs[i], xs[i + 1]) for i in range(0, len(xs) - 1, 2)]
        if len(xs) % 2:
            nxt.append(xs[-1])
        xs = nxt
    return xs[0]


def _wtile(u):
    return pltpu.bitcast(u.reshape(u.shape[0] * 8, 128), bf16)


def _mm(lhs, w, dims=_NN):
    return lax.dot_general(lhs, w, dims, preferred_element_type=f32)


def _cache_view(c):
    _, H, Sk, Dh = c.shape
    c = c.reshape(H, Sk // 128, 128, Dh // 16, 2, 8)
    c = jnp.transpose(c, (0, 3, 4, 1, 5, 2))
    return c.reshape(H * Dh // 16, 2, Sk // 128, 8, 128)


def _weight_view(w):
    R, N = w.shape
    w = w.reshape(R // 16, 2, 8, N // 128, 128)
    return jnp.transpose(w, (0, 1, 3, 2, 4))


def _schedule(NP, KT, DT, AP, AB, SG, xunits, qlead, keep, LAT=205, LAT0=165, LEAD=32, WD=140, WL=400, AD=160,
              vcost=5.95, pstride=2, nraw=8, q2at=40, ph=3, wide=(), wk=(8, 20), cmaj=4, **_):
    xs = {u[:2]: u[2] for u in xunits}
    grp = [(t, a) for t in range(NP) for a in range(0, AP, AB)]
    grp[-2:] = grp[:-3:-1]
    steps = [(t, a, k) for t, a in grp for k in range(xs.get((t, a // 8), 0), KT)]
    first_step = {}
    for i, s in enumerate(steps):
        first_step.setdefault(s[0], i)
    main = [('qraw', t, i) for t in range(nraw) for i in range(3)]
    for t in range(NP):
        qk = [('qk', t, j, k) for j in range(3) for k in range(KT)]
        main += qk[:q2at] + [('q', t + 1, i) for i in range(3) if nraw <= t + 1 < NP] + qk[q2at:]
    done = {('q', t): 3 for t in range(nraw)}
    or_left = [(t, j) for t in range(NP) for j in range(3) if xs.get((t, j), 0) < KT]
    wo_left = [(t, j) for t in range(NP) for j in range(3)]
    px_left = list(xs)
    ev, pend, wait, cur, src = [], [], [], [], {}
    s = dict(tm=0.0, tv=0.0, i=0, mi=0, qk=0)

    def sm(t):
        return ([(('sma', t, k), 3 * SG, None, 0) for k in range(0, KT, SG)]
                + [(('smb', t, k), 3 * SG, ('p', t), SG) for k in range(0, KT, SG)])

    def g_wo(n):
        wo = tuple(u for u in wo_left if done.get(('o',) + u, 0) >= 1)[:4]
        if len(wo_left) > cmaj:
            wo = wo[:len(wo_left) - cmaj]
        if len(wo) < n:
            return None
        for u in wo:
            wo_left.remove(u)
        g = [(('wo', wo, n, c), 8, []) for n in range(len(wo)) for c in range(DT)]
        if not wo_left and cmaj:
            g.sort(key=lambda x: x[0][3])
        g[-1] = (g[-1][0], 8, [(('wacc', wo, c), len(wo), None, 0) for c in range(DT)])
        return g

    def g_or(n, last):
        rd = [u for u in or_left if done.get(('acc',) + u, 0) >= 8 // AB and done.get(('w', u[0]), 0)
              and (last or done[('acct',) + u] + AD <= s['tv'])
              and done.get(('y',) + u, 0) >= xs.get(u, 0)][:4]
        if len(rd) < n:
            return None
        for u in rd:
            or_left.remove(u)
        return [(('gap',), 8 * len(rd), [])] + [(('or',) + u, 8, [(('ofin',) + u, 1, ('o',) + u, 1)]) for u in rd]

    def g_px():
        rd = [u for u in px_left if done.get(('w', u[0]), 0)]
        if not rd:
            return None
        px_left.remove(rd[0])
        n = xs[rd[0]]
        g = [(('pvx',) + rd[0] + (k,), 8, []) for k in range(n)]
        e, inc = (('o',) + rd[0], 4 / KT) if n == KT else (('y',) + rd[0], 4)
        g[-1] = (g[-1][0], 8, [(('xsum',) + rd[0] + (k,), 4, e, inc) for k in range(0, n, 4)])
        return g

    def pick():
        last, endgame, nxt = s['i'] >= len(steps), s['mi'] >= len(main), s['qk']
        if last:
            return g_or(1, True) or g_px() or g_wo(len(wo_left) if 0 < len(wo_left) <= cmaj else 1)
        if endgame:
            return g_or(4, False) or g_px() or g_wo(4) or (g_wo(1) if len(wo_left) > cmaj else None)
        rem = sum(8 for m in main[s['mi']:s['mi'] + 200] if m[0] != 'qk' or m[1] == nxt)
        if (first_step[nxt] - s['i']) * vcost - rem > qlead * 500:
            g = (g_wo(4) if len(wo_left) > keep else None) or g_or(4, False) or g_px()
            if g:
                return g
        m = main[s['mi']]
        if m[0] == 'qk' and done.get(('q', m[1]), 0) < 3:
            return None
        s['mi'] += 1
        pcs = []
        if m[0] == 'q':
            pcs = [(('qfin',) + m[1:], 5, ('q', m[1]), 1)]
        if m[0] == 'qk' and (m[2] == 2 or m[1:3] == (0, 1)) and m[3] % SG == SG - 1:
            t = m[1] if m[2] == 2 else -1
            pcs = [sm(t)[m[3] // SG]] + (sm(t)[KT // SG:] if m[3] == KT - 1 else [])
        return [(m, 8, pcs)]

    def later(t, pcs):
        wait.append((t, pcs))
        wait.sort(key=lambda w: w[0])

    def piece():
        a, cv, e, inc = pend.pop(0)
        if a[0] == 'wld' and s['i'] < len(steps) and not wk[0] <= steps[s['i']][2] <= wk[1]:
            return later(s['tv'] + 30, [(a, cv, e, inc)])
        ev.append(('piece',) + a)
        s['tv'] += cv / 4
        if e is not None:
            done[e] = done.get(e, 0) + inc
        if a[0] == 'smb' and a[2] == KT - SG and a[1] >= 0:
            later(s['tv'] + WD, [(('wld', a[1]), 0, ('wld', a[1]), 1)])
        if a[0] == 'wld':
            later(s['tv'] + WL, [(('w', a[1]), 24, ('w', a[1]), 1)])

    def urgent(p):
        return p[2] is not None and p[2][0] != 'p'

    while True:
        while wait and wait[0][0] <= s['tv']:
            pcs = wait.pop(0)[1]
            pend[:] = [p for p in pcs if urgent(p)] + pend + [p for p in pcs if not urgent(p)]
        i = s['i']
        more = i < len(steps)
        blocked = not more or done.get(('p', steps[i][0] - (i < AP // 2 // AB * KT)), 0) < min(KT, steps[i][2] + 6)
        if not more and or_left:
            cur = (g_or(1, True) or []) + cur
        if not cur and (s['tm'] + LEAD <= s['tv'] or blocked):
            cur = pick() or []
        if not more and not pend and not wait and not cur:
            break
        if cur and (s['tm'] + LEAD <= s['tv']
                    or (blocked and not pend and (not wait or s['tm'] + LEAD <= wait[0][0]))):
            a, cm, pcs = cur.pop(0)
            ev.append(('tile',) + a)
            s['tm'] = max(s['tm'], s['tv'] - LEAD - 8) + cm
            s['tv'] += 0.25 * (a[0] == 'pvx')
            s['qk'] += a[0] == 'qk' and a[2:] == (2, KT - 1)
            src.update({('piece',) + pc[0]: ev[-1] for pc in pcs})
            if pcs:
                later(s['tm'] + (LAT if 0 < i < len(steps) else LAT0), pcs)
        elif blocked and pend:
            piece()
        elif blocked:
            s['tv'] = max(s['tv'], wait[0][0])
        else:
            if pend and (i % pstride == 0 or urgent(pend[0])):
                piece()
            t, a, k = steps[i]
            ev.append(('step', t, a, k))
            if k == KT - 1:
                done['acc', t, a // 8] = done.get(('acc', t, a // 8), 0) + 1
                done['acct', t, a // 8] = s['tv']
            s['tv'] += vcost - 0.5 * sum((t, b) in wide for b in range(a, a + AB))
            s['i'] += 1
    assert not or_left and not wo_left and not px_left

    out, cur, cnt = [], [], 0
    for e in ev + [None]:
        if e is None or (e[0] == 'tile' and e[1] != 'gap' and cnt % 4 == ph):
            if any(x[0] == 'step' for x in cur) and len(cur) < 32 and not any(src.get(x) in cur for x in cur):
                cur = cur[:1] + [x for x in cur[1:] if x[0] == 'piece'] + [x for x in cur[1:] if x[0] != 'piece']
            out += cur
            cur = []
        if e is not None:
            cur.append(e)
            cnt += (4 if e[1] == 'gap' else 1) * (e[0] == 'tile')
    pos = {e: n for n, e in enumerate(out)}
    assert all(pos[a] < pos[b] for b, a in src.items())
    return out


def _slots(events, key):
    first, last = {}, {}
    for n, e in enumerate(events):
        k = key(e)
        if k is not None:
            first.setdefault(k, n)
            last[k] = n
    slot, busy = {}, []
    for k in first:
        free = [i for i, u in enumerate(busy) if u < first[k]]
        slot[k] = free[0] if free else len(busy)
        busy[slot[k]:slot[k] + 1] = [last[k]]
    return slot, len(busy)


def _run(opts, A_x, A_k_cache, A_v_cache, A_wq, A_wo, B_w3, B_w4):
    B, S, D = A_x.shape
    _, H, Sk, Dh = A_k_cache.shape
    F = B_w3.shape[1]
    W = min(4096, max(256, Sk // 4))
    assert (B, S, H, Dh, W) == (1, 1, 32, 192, 4096) and D % 128 == 0 and F % 128 == 0
    AP = Dh // 8
    KT = W // 128
    NP = H // 2
    DT, FT = D // 128, F // 128
    AB, SG, FD = 4, 2, opts.get('fd', 5)
    SKEW = opts.get('skew', 1)
    cexp = (Dh ** -0.5) * _LOG2E
    nx = {u[:2]: u[2] for u in opts['xunits']}
    xunits = list(nx)
    wide = [(t, a) for t in range(NP) for a in range(0, AP, AB) if (t, a // 8) not in xunits + [(NP - 1, 2)]]
    drop = [g for n, g in enumerate(wide) if n % 3][:max(0, len(wide) - opts['nwide'])]
    wide = [g for g in wide if g not in drop] + [(t, a + 2) for t, a in wide[::-1]][:max(0, opts['nwide'] - len(wide))]
    late = [(t, a) for b in (0, 2) for t in range(NP - 1, 0, -1) for a in range(b, AP, AB)
            if (t, a // 8) not in xunits + [(NP - 1, 2)] and (t, a) not in wide]
    nlate = opts['nlate']
    late = {g: (c, n) for c in range(DT - 1) for n, g in enumerate(late[sum(nlate[:c]):sum(nlate[:c + 1])])}
    events = _schedule(NP, KT, DT, AP, AB, SG, wide=wide + list(late), **opts)
    sp, RP = _slots(events, lambda e: e[1] - (e[1] == 0 and e[2] < AP // 2) if e[0] == 'step'
                    else e[2] if e[1] in ('sma', 'smb', 'pvx') else None)
    ss, RS = _slots(events, lambda e: max(e[2], 0) if e[1] in ('qk', 'sma') else None)
    sq, RQ = _slots(events, lambda e: e[2] if e[1] in ('q', 'qfin') else None)
    sx, RX = _slots(events, lambda e: e[2:4] if e[1] in ('pvx', 'xsum') else None)
    sw, RM = _slots(events, lambda e: e[2] if e[1] in ('wo', 'wacc') else None)
    so, RO = _slots(events, lambda e: e[2:4] if e[1] in ('or', 'ofin') else None)
    sl, RL = _slots(events, lambda e: e[2] if e[1] in ('smb', 'wld') else None)
    assert _slots(events, lambda e: e[2] if e[1] in ('sma', 'smb') else None)[1] == 1
    sizes = [3 * NP, 3 * NP, 2 * NP, 2, DT, 2 * NP + 3, KT, KT * len(wide)]
    QP, Q0, WB, XL, XA, MB, AL, WD, NBIG = [sum(sizes[:n]) for n in range(len(sizes) + 1)]
    OB = Q0
    free, acc_at = [AL, AL + 16], {}
    for e in events:
        if e[0] == 'step' and (e[1], e[2] // 8) not in acc_at:
            acc_at[e[1], e[2] // 8] = free.pop(0)
        if e[0] == 'step' and e[3] == KT - 1:
            free += [WD + KT * wide.index((e[1], a)) + n for a in range(e[2], e[2] + AB) if (e[1], a) in wide
                     for n in (0, 16)]
    sizes = [RP * KT, 3 * RS * KT, RX * KT, 3 * RQ, 4 * DT * RM, 2 * RO, 2 * RL]
    _, SP, XP, QR, WR, OR, ML, NPB = [sum(sizes[:n]) for n in range(len(sizes) + 1)]
    NV, NQ = opts.get('nv', 4), opts.get('nq', 8)
    assert nlate[DT - 2] == 0 and 2 * nlate[DT - 3] <= 11 + (3 * NP - NQ) // 4
    if opts.get('verbose'):
        print('RP RS RQ RX RM', RP, RS, RQ, RX, RM, 'free tiles', (int(13.25 * 256) - NBIG - NPB))
    order1 = sorted(range(NP), key=lambda t: all(u[0] != t for u in xunits))

    def kernel(x_hbm, k_hbm, v_hbm, wq_hbm, wo_hbm, w3_hbm, w4_hbm, o_ref, *scratch):
        k_bufs, v_bufs, scratch = scratch[:NP], scratch[NP:2 * NP], scratch[2 * NP:]
        w4_bufs, wq_bufs, scratch = scratch[:DT], scratch[DT:2 * DT], scratch[2 * DT:]
        wo_buf, w3_buf, pbuf, cst, big, hbuf, xres, x_buf, sems = scratch
        t0 = (Sk - W) // 128

        def kv_cp(kind, t):
            src, dst = (k_hbm, k_bufs[t]) if kind == 0 else (v_hbm, v_bufs[t])
            return [pltpu.make_async_copy(src.at[pl.ds(AP * t, AP), a, pl.ds(t0, KT)],
                                          dst.at[:, :, pl.ds(8 * a, 8), :], sems.at[2 * t + kind])
                    for a in range(2)]

        def w_cp(src, dst, n, sem):
            rows = src.shape[0] // n
            return [pltpu.make_async_copy(src.at[pl.ds(i * rows, rows), a],
                                          dst.at[pl.ds(i * rows, rows), :, pl.ds(8 * a, 8), :], sem)
                    for i in range(n) for a in range(2)]

        def wq_cp():
            cps = [cp for j in range(DT) for cp in w_cp(wq_hbm.at[pl.ds(8 * j, 8)], wq_bufs[j], 1, sems.at[2 * NP])]
            return cps[:1] + [pltpu.make_async_copy(x_hbm, x_buf, sems.at[2 * NP])] + cps[1:]

        def wo_cp():
            return w_cp(wo_hbm, wo_buf, 8, sems.at[2 * NP + 1])

        def w3_cp():
            return [pltpu.make_async_copy(w3_hbm, w3_buf, sems.at[2 * NP + 2])]

        def w4_cp(c):
            return [pltpu.make_async_copy(w4_hbm.at[:, pl.ds(128 * c, 128)], w4_bufs[c], sems.at[2 * NP + 3 + c])]

        def wait(cps):
            for cp in cps:
                cp.wait()

        cps = wq_cp()
        for t in order1:
            cps += kv_cp(0, t) + kv_cp(1, t) + (wo_cp() if t == order1[0] else [])
        for cp in cps + w3_cp() + [cp for c in range(DT) for cp in w4_cp(c)]:
            cp.start()

        ku = [r.bitcast(u32) for r in k_bufs]
        vu = [r.bitcast(u32) for r in v_bufs]
        wqu = [r.bitcast(u32) for r in wq_bufs]
        wou = wo_buf.bitcast(u32)
        w4u = [r.bitcast(u32) for r in w4_bufs]

        def top(n):
            return lax.broadcasted_iota(i32, (8, n), 0) < 4

        def left():
            return lax.broadcasted_iota(i32, (8, 128), 1) < 64

        def cols(n):
            return slice(128 * n, 128 * (n + 1))

        def rows(j):
            return slice(8 * j, 8 * j + 8)

        def masks():
            return [top(128), top(128) == left(), jnp.logical_not(top(128))]

        def mlp_hidden(x):
            lhs = jnp.where(top(D), x, 1.0)
            m1 = jnp.mean(x, axis=-1, keepdims=True)
            xc = x - m1
            v1 = jnp.mean(xc * xc, axis=-1, keepdims=True)
            r1 = lax.rsqrt(v1 + _EPS)
            y = xc * r1
            m2 = jnp.mean(xc, axis=-1, keepdims=True) * r1
            r2 = lax.rsqrt(v1 * r1 * r1 - m2 * m2 + _EPS)
            coef = jnp.where(top(128), r1 * r2, -(r2 * (r1 * m1 + m2)))
            hs, NF = [], opts.get('nf', 4)
            first = {(n, j): _mm(lhs[:, cols(j)], w3_buf[cols(j), cols(n)]) for j in range(DT) for n in range(NF)}
            for n in range(FT):
                u = _tree(jnp.add, [first[n, j] if n < NF else _mm(lhs[:, cols(j)], w3_buf[cols(j), cols(n)])
                                    for j in range(DT)]) * coef
                hs.append(jax.nn.gelu(u + pltpu.roll(u, 4, 0), approximate=True))
            return y, hs

        def w4_tile(n, c):
            return pltpu.bitcast(w4u[c][64 * n:64 * (n + 1)], bf16)

        def late_at(n, k):
            return ((n * KT + k + 2) % (24 * NP)) // (3 * NP), (n * KT + k + 2) % (3 * NP)

        def unpack_late(c, n0, n1, after=None):
            todo = [(g, n, k) for g, (cc, n) in late.items() if cc == c for k in range(KT)][16 * n0:16 * n1]
            if todo and after is not None:
                wqu[c][after[0], 0] = pltpu.bitcast(after[1], u32)
            for (t, a), n, k in todo:
                y = pltpu.bitcast(pltpu.bitcast(vu[t][a, k], bf16).astype(f32), u32)
                wqu[c][late_at(n, k)] = y[8:16]
                vu[t][a, k] = y[0:8]

        def layer1(z):
            for u, mask in enumerate(masks()):
                cst[u] = jnp.where(mask, cexp, 0.0).astype(f32)
            wait(wq_cp())
            x = jnp.broadcast_to(x_buf[...].astype(f32), (8, D))
            _, xc, r = _stats(x)
            xn = xc * r

            def q_body(t, c):
                for i in range(3):
                    q = _tree(jnp.add, [_mm(xn[:, cols(j)], _wtile(wqu[j][:, 3 * t + i])) for j in range(DT)])
                    big[QP + 3 * t + i] = q * cst[i]
                return c
            lax.fori_loop(0, NP, q_body, 0)

            att = [jnp.zeros((8, 128), f32)] * DT
            for t in order1:
                def s_body(k, c, t=t, q=[big[QP + 3 * t + j] for j in range(3)]):
                    big[AL + k] = _tree(jnp.add, [_mm(q[j], _wtile(ku[t][rows(j), k])) for j in range(3)])
                    return c

                def o_body(k, o, t=t):
                    return [o[j] + _mm(big[AL + k], _wtile(vu[t][rows(j), k]), _NT) for j in range(3)]

                wait(kv_cp(0, t))
                lax.fori_loop(0, KT, s_body, 0, unroll=8)
                sc = big[AL:AL + KT]
                p = jnp.exp2(sc - jnp.max(jnp.max(sc, axis=0), axis=1, keepdims=True))
                big[AL:AL + KT] = p
                inv = 1.0 / jnp.sum(jnp.sum(p, axis=0), axis=1, keepdims=True)
                wait(kv_cp(1, t) + (wo_cp() if t == order1[0] else []))
                o = lax.fori_loop(0, KT, o_body, [jnp.zeros((8, 128), f32)] * 3, unroll=8)
                o = [jnp.where(mask, o[j] * inv, 0.0) for j, mask in enumerate(masks())]
                att = [att[c] + _tree(jnp.add, [_mm(o[j], _wtile(wou[rows(3 * t + j), c])) for j in range(3)])
                       for c in range(DT)]
                for j in [j for tt, j in xunits if tt == t]:
                    def t_body(k, c, t=t, j=j):
                        w = _wtile(vu[t][rows(j), k]).astype(f32).T.astype(bf16)
                        vu[t][rows(j), k] = pltpu.bitcast(w, u32).reshape(8, 8, 128)
                        return c
                    lax.fori_loop(0, nx[t, j], t_body, 0, unroll=4)
                for n, a in [(n, a) for n, (tt, a) in enumerate(wide) if tt == t]:
                    y = _wtile(vu[t][a]).astype(f32).reshape(KT, 16, 128)
                    big[WD + n * KT:WD + (n + 1) * KT] = y[:, 8:16]
                    vu[t][a] = pltpu.bitcast(y[:, 0:8], u32)
            att = jnp.concatenate(att, axis=1)
            x = x + (att + pltpu.roll(att, 4, 0))
            wait(w3_cp())
            y, hs = mlp_hidden(x)
            xres[...] = x + y
            for n in range(FT):
                hbuf[n] = hs[n]
            for c in range(DT - 1):
                wait(w4_cp(c))
                unpack_late(c - 1, 0, 7)
                xc = xres[:, cols(c)] + _tree(jnp.add, [_mm(hbuf[n], w4_tile(n, c)) for n in range(FT)])
                xres[:, cols(c)] = xc
                xc = jnp.where(top(128), xc, 1.0)
                unpack_late(c - 1, 7, 11, (z, xc))
                for n in range(3 * NP - (NQ if c == DT - 2 else 0)):
                    r = _mm(xc, _wtile(wqu[c][:, n]))
                    big[Q0 + n] = big[Q0 + n] + r if c else r
                    if n % 4 == 0:
                        unpack_late(c - 1, 11 + n // 4, 12 + n // 4, (z, r))

        def layer2(z):
            wait(w4_cp(DT - 1))
            if opts.get('skip2'):
                keep = big[Q0 + z] + sum(pltpu.bitcast(r[z, 1], f32) for r in wqu + vu)
                o_ref[...] = (xres[0:1, :] + jnp.concatenate([keep[0:1]] * DT, axis=1)).astype(o_ref.dtype)
                return
            xc = xres[:, cols(DT - 1)] + _tree(jnp.add, [_mm(hbuf[n], w4_tile(n, DT - 1)) for n in range(FT)])
            for n in range(3 * NP - NQ, 3 * NP):
                xp = jnp.where(top(128), xres[:, cols(DT - 2)], 1.0)
                big[Q0 + n] = big[Q0 + n] + _mm(xp, _wtile(wqu[DT - 2][:, n]))
            xres[:, cols(DT - 1)] = xc
            m, _, r = _stats(xres[...])
            big[XL] = xraw = jnp.where(top(128), xc, 1.0)
            coef0 = jnp.where(top(128), 1.0, -m)
            big[XL + 1] = coef = coef0 * r
            acc, val, fwd = {}, {}, []
            st = dict(pin=False, dirty=False, cnt=0, started=False, left=sum(e[0] == 'step' for e in events))

            def lhs(n):
                if st['pin']:
                    st['pin'] = False
                    return big[n + z]
                if n not in val:
                    val[n] = big[n]
                return val[n]

            def checkpoint():
                for (t, a), y in acc.items():
                    n = acc_at[t, a // 8] + 2 * (a % 8)
                    big[n:n + 2] = y.reshape(2, 8, 128)

            def put(n, r):
                fwd.append((st['cnt'], n, r))

            def flush(upto, pin=False):
                while fwd and fwd[0][0] <= upto:
                    _, n, r = fwd.pop(0)
                    pbuf[z if pin else 0, :, cols(n)] = r
                    if pin and st['left'] <= opts.get('vpin', 72):
                        vu[NP - 1][z, 2] = pltpu.bitcast(r, u32)
                    pin = False

            def get(n):
                flush(max([c for c, m, _ in fwd if m == n], default=-1))
                return pbuf[0, :, cols(n)]

            def ptile(t, k):
                return cols(sp[t] * KT + k)

            def prow(t, odd, k):
                return pbuf[0, 4 * odd:4 * odd + 1, ptile(t - (t + odd == 0), k)]

            def q_fin(t, i, y, coef):
                y = (y + big[Q0 + 3 * t + i]) * coef
                big[QP + 3 * t + i] = (y + pltpu.roll(y, 4, 0)) * cst[i]

            def t_qraw(t, i):
                q_fin(t, i, _mm(xraw, _wtile(wqu[DT - 1][:, 3 * t + i])), coef if t else coef0)

            def t_q(t, i):
                put(QR + sq[t] * 3 + i, _mm(lhs(XL), _wtile(wqu[DT - 1][:, 3 * t + i])))

            def t_qk(t, j, k):
                put(SP + (3 * ss[t] + j) * KT + k, _mm(lhs(QP + 3 * t + j), _wtile(ku[t][rows(j), k])))

            def t_or(t, j):
                a = big[acc_at[t, j]:acc_at[t, j] + 16].reshape(128, 128)
                if j == 1:
                    r = _mm(jnp.concatenate([lhs(WB + 2 * t), lhs(WB + 2 * t + 1)], axis=0), a, _NT)
                    put(OR + 2 * so[t, j] + 1, r[8:16])
                else:
                    r = _mm(lhs(WB + 2 * t + j // 2), a, _NT)
                put(OR + 2 * so[t, j], r[0:8])

            def t_pvx(t, j, k):
                p = val.pop(('px', t, j, k)) * lhs(WB + 2 * t + j // 2)
                put(XP + sx[t, j] * KT + k, _mm(p, _wtile(vu[t][rows(j), k])))

            def t_wo(units, n, c):
                t, j = units[n]
                put(WR + (sw[units] * 4 + n) * DT + c, _mm(lhs(OB + 3 * t + j), _wtile(wou[rows(3 * t + j), c])))

            def p_qfin(t, i):
                q_fin(t, i, get(QR + sq[t] * 3 + i), big[XL + 1])

            def p_sma(t, k0):
                n = SP + 3 * ss[max(t, 0)] * KT
                sv = []
                for k in range(k0, k0 + SG):
                    sc = get(n + k) + get(n + KT + k)
                    sc = sc + get(n + 2 * KT + k) if t >= 0 else sc
                    sv.append(sc * r if t <= 0 else sc)
                    pbuf[0, :, ptile(t, k)] = sv[-1]
                big[MB + 2 + 2 * t] = val['m'] = _tree(jnp.maximum, sv + ([val['m']] if k0 else []))

            def p_smb(t, k0):
                ps = []
                for k in range(k0, k0 + SG):
                    ps.append(jnp.exp2(pbuf[0, :, ptile(t, k)] - val['m']))
                    pbuf[0, :, ptile(t, k)] = ps[-1]
                if t >= 0:
                    big[MB + 3 + 2 * t] = val['l'] = _tree(jnp.add, ps + ([val['l']] if k0 else []))
                if t >= 0 and k0 + SG == KT:
                    pbuf[0, :, cols(ML + 2 * sl[t])] = val['m']
                    pbuf[0, :, cols(ML + 2 * sl[t] + 1)] = val['l']

            def p_wld(t):
                val['ml', t] = pbuf[0, :, cols(ML + 2 * sl[t])], pbuf[0, :, cols(ML + 2 * sl[t] + 1)]

            def p_w(t):
                m, l = val['ml', t]
                e = jnp.exp2(m - jnp.max(m, axis=1, keepdims=True))
                w = e / jnp.sum(e * l, axis=1, keepdims=True)
                for h in range(2):
                    big[WB + 2 * t + h] = jnp.broadcast_to(w[4 * h:4 * h + 1], (8, 128))

            def p_ofin(t, j):
                r = get(OR + 2 * so[t, j])
                r = jnp.where(left(), r, get(OR + 2 * so[t, j] + 1)) if j == 1 else r
                big[OB + 3 * t + j] = r + big[OB + 3 * t + j] if (t, j) in nx else r

            def p_xsum(t, j, k0):
                n = XP + sx[t, j] * KT + k0
                ys = [get(n + u) for u in range(4)] + ([val['y', t, j]] if k0 else [])
                big[OB + 3 * t + j] = val['y', t, j] = _tree(jnp.add, ys)

            def p_wacc(units, c):
                rs = [get(WR + (sw[units] * 4 + n) * DT + c) for n in range(len(units))]
                big[XA + c] = _tree(jnp.add, rs + ([big[XA + c]] if units != next(iter(sw)) else []))

            fns = {'qraw': t_qraw, 'q': t_q, 'qk': t_qk, 'or': t_or, 'pvx': t_pvx, 'wo': t_wo, 'qfin': p_qfin,
                   'sma': p_sma, 'smb': p_smb, 'wld': p_wld, 'w': p_w, 'ofin': p_ofin, 'xsum': p_xsum, 'wacc': p_wacc}
            tiles = [e for e in events if e[0] == 'tile' and e[1] != 'gap']
            for e in events:
                if e[0] == 'step':
                    _, t, a0, k = e
                    k0 = nx.get((t, a0 // 8), 0)
                    for a in range(a0, a0 + AB):
                        n = k + SKEW * (a - a0)
                        kk = k0 + (n - k0) % (KT - k0)
                        if ('p', t, a0, n) not in val:
                            val['p', t, a0, n] = prow(t, int(a0 >= AP // 2), kk)
                        if (t, a) in wide:
                            y = jnp.concatenate([pltpu.bitcast(vu[t][a, kk], f32),
                                                 big[WD + wide.index((t, a)) * KT + kk]])
                        elif (t, a) in late:
                            c, u = late[t, a]
                            y = pltpu.bitcast(jnp.concatenate([vu[t][a, kk], wqu[c][late_at(u, kk)]]), f32)
                        else:
                            y = pltpu.bitcast(vu[t][a, kk], bf16).astype(f32)
                        y = y * val['p', t, a0, n]
                        acc[t, a] = acc[t, a] + y if (t, a) in acc else y
                    st.update(dirty=True, started=True, left=st['left'] - 1)
                    if k == KT - 1:
                        checkpoint()
                        acc.clear()
                elif e[0] == 'piece':
                    fns[e[1]](*e[2:])
                elif e[1] == 'gap':
                    st['cnt'] += 4
                else:
                    pinned = st['cnt'] % 4 == opts.get('ph', 3) and st['left'] > 0
                    if pinned and st['dirty']:
                        checkpoint()
                    st.update(pin=pinned and st['started'], dirty=st['dirty'] and not pinned)
                    fns[e[1]](*e[2:])
                    st['pin'] = False
                    tiles.pop(0)
                    for u in tiles[:opts.get('pf', 4)]:
                        if u[1] == 'pvx' and ('px',) + u[2:] not in val:
                            val[('px',) + u[2:]] = prow(u[2], u[3] // 2, u[4])
                    if pinned:
                        flush(st['cnt'] - 4 * FD + 3, pin=st['started'])
                    st['cnt'] += 1
            assert not fwd
            x = xres[...] + jnp.concatenate([big[XA + c] for c in range(DT)], axis=1)
            y, hs = mlp_hidden(x)
            out = [(x + y)[:, cols(c)] for c in range(DT)]
            part = [None] * DT
            hb = [jnp.concatenate([hs[n]] * 16, axis=0).T for n in range(NV)]
            for n0 in range(0, NV, 3):
                for a in range(8):
                    for n in range(n0, min(n0 + 3, NV)):
                        for c in range(DT):
                            u = pltpu.bitcast(w4u[c][rows(8 * n + a)], bf16).astype(f32) * hb[n][16 * a:16 * a + 16]
                            part[c] = u if part[c] is None else part[c] + u
            for n in range(NV, FT):
                out = [out[c] + _mm(hs[n], w4_tile(n, c)) for c in range(DT)]
            out = [out[c] + jnp.sum(part[c], axis=0, keepdims=True) for c in range(DT)]
            o_ref[...] = jnp.concatenate(out, axis=1)[0:1].astype(o_ref.dtype)

        def body(it, carry):
            pl.when(it == 0)(lambda: layer1(it >> 4) if not opts.get('skip1') else None)
            pl.when(it == 1)(lambda: layer2(it >> 4))
            return carry

        lax.fori_loop(0, 2, body, 0)

    def V(*s, dt=f32):
        return pltpu.VMEM(s, dt)

    out = pl.pallas_call(
        kernel,
        out_shape=jax.ShapeDtypeStruct((1, D), A_x.dtype),
        in_specs=[pl.BlockSpec(memory_space=pl.ANY)] * 7,
        out_specs=pl.BlockSpec(memory_space=pltpu.VMEM),
        scratch_shapes=(
            [V(AP, KT, 16, 128, dt=bf16)] * (2 * NP)
            + [V(F, 128, dt=bf16)] * DT + [V(8, 3 * NP, 16, 128, dt=bf16)] * DT
            + [V(AP * NP, DT, 16, 128, dt=bf16), V(D, F, dt=bf16),
               V(1, 8, -(-NPB // 4) * 512), V(4, 8, 128), V(-(-NBIG // 4) * 4, 8, 128),
               V(FT, 8, 128), V(8, D), V(1, D, dt=bf16),
               pltpu.SemaphoreType.DMA((2 * NP + 3 + DT,))]),
        compiler_params=pltpu.CompilerParams(
            vmem_limit_bytes=int(opts.get('vmem', 128) * 1024 * 1024),
            disable_semaphore_checks=True, disable_bounds_checks=True),
        name='fused_decode_layers',
    )(A_x.reshape(1, D), _cache_view(A_k_cache), _cache_view(A_v_cache),
      _weight_view(A_wq), _weight_view(A_wo), B_w3, B_w4)
    return out.reshape(B, S, D)


@jax.jit
def pallas_interleave_layers__sliding_block_cached__mixer_s_mlp__decode_kernel(
    A_x: jax.Array,
    A_k_cache: jax.Array,
    A_v_cache: jax.Array,
    A_wq: jax.Array,
    A_wo: jax.Array,
    B_x: jax.Array,
    B_w1: jax.Array,
    B_w2: jax.Array,
    B_w3: jax.Array,
    B_w4: jax.Array,
):
    return _run(_OPTS, A_x, A_k_cache, A_v_cache, A_wq, A_wo, B_w3, B_w4)
```

```python
import jax
import jax.numpy as jnp
from jax import lax
import jax.experimental.pallas as pl
import jax.experimental.pallas.tpu as pltpu

f32, bf16, u32, i32 = jnp.float32, jnp.bfloat16, jnp.uint32, jnp.int32
_EPS = 1e-5
_LOG2E = 1.4426950408889634
_NN = (((1,), (0,)), ((), ()))
_NT = (((1,), (1,)), ((), ()))

_OPTS = dict(xunits=[(5, 0, 32), (7, 2, 32), (9, 2, 32), (11, 0, 32), (14, 2, 12)], nwide=87, nlate=[10, 10, 9, 0], qlead=2.0, keep=8,
             AD=60, LAT=205, LAT0=205, q2at=20, vpin=36)


def _stats(x):
    m = jnp.mean(x, axis=-1, keepdims=True)
    xc = x - m
    v = jnp.mean(xc * xc, axis=-1, keepdims=True)
    return m, xc, lax.rsqrt(v + _EPS)


def _tree(op, xs):
    xs = list(xs)
    while len(xs) > 1:
        nxt = [op(xs[i], xs[i + 1]) for i in range(0, len(xs) - 1, 2)]
        if len(xs) % 2:
            nxt.append(xs[-1])
        xs = nxt
    return xs[0]


def _wtile(u):
    return pltpu.bitcast(u.reshape(u.shape[0] * 8, 128), bf16)


def _mm(lhs, w, dims=_NN):
    return lax.dot_general(lhs, w, dims, preferred_element_type=f32)


def _cache_view(c):
    _, H, Sk, Dh = c.shape
    c = c.reshape(H, Sk // 128, 128, Dh // 16, 2, 8)
    c = jnp.transpose(c, (0, 3, 4, 1, 5, 2))
    return c.reshape(H * Dh // 16, 2, Sk // 128, 8, 128)


def _weight_view(w):
    R, N = w.shape
    w = w.reshape(R // 16, 2, 8, N // 128, 128)
    return jnp.transpose(w, (0, 1, 3, 2, 4))


def _schedule(NP, KT, DT, AP, AB, SG, xunits, qlead, keep, LAT=205, LAT0=165, LEAD=32, WD=140, WL=400, AD=160,
              vcost=5.95, pstride=2, nraw=8, q2at=40, ph=0, wide=(), wk=(8, 20), cmaj=4, **_):
    xs = {u[:2]: u[2] for u in xunits}
    grp = [(t, a) for t in range(NP) for a in range(0, AP, AB)]
    grp[-2:] = grp[:-3:-1]
    steps = [(t, a, k) for t, a in grp for k in range(xs.get((t, a // 8), 0), KT)]
    first_step = {}
    for i, s in enumerate(steps):
        first_step.setdefault(s[0], i)
    main = [('qraw', t, i) for t in range(nraw) for i in range(3)]
    for t in range(NP):
        qk = [('qk', t, j, k) for j in range(3) for k in range(KT)]
        main += qk[:q2at] + [('q', t + 1, i) for i in range(3) if nraw <= t + 1 < NP] + qk[q2at:]
    done = {('q', t): 3 for t in range(nraw)}
    or_left = [(t, j) for t in range(NP) for j in range(3) if xs.get((t, j), 0) < KT]
    wo_left = [(t, j) for t in range(NP) for j in range(3)]
    px_left = list(xs)
    ev, pend, wait, cur, src = [], [], [], [], {}
    s = dict(tm=0.0, tv=0.0, i=0, mi=0, qk=0)

    def sm(t):
        return ([(('sma', t, k), 3 + 4 * (k == KT - SG), None, 0) for k in range(0, KT, SG)]
                + [(('smb', t, k), 3, ('p', t), SG) for k in range(0, KT, SG)])

    def g_wo(n):
        wo = tuple(u for u in wo_left if done.get(('o',) + u, 0) >= 1)[:4]
        if len(wo_left) > cmaj:
            wo = wo[:len(wo_left) - cmaj]
        if len(wo) < n:
            return None
        for u in wo:
            wo_left.remove(u)
        g = [(('wo', wo, n, c), 8, []) for n in range(len(wo)) for c in range(DT)]
        if not wo_left and cmaj:
            g.sort(key=lambda x: x[0][3])
        g[-1] = (g[-1][0], 8, [(('wacc', wo, c), len(wo), None, 0) for c in range(DT)])
        return g

    def g_or(n, last):
        rd = [u for u in or_left if done.get(('acc',) + u, 0) >= 8 // AB and done.get(('w', u[0]), 0)
              and (last or done[('acct',) + u] + AD <= s['tv'])
              and done.get(('y',) + u, 0) >= xs.get(u, 0)][:4]
        if len(rd) < n:
            return None
        for u in rd:
            or_left.remove(u)
        return [(('gap',), 8 * len(rd), [])] + [(('or',) + u, 8, [(('ofin',) + u, 1, ('o',) + u, 1)]) for u in rd]

    def g_px():
        rd = [u for u in px_left if done.get(('w', u[0]), 0)]
        if not rd:
            return None
        px_left.remove(rd[0])
        n = xs[rd[0]]
        g = [(('pvx',) + rd[0] + (k,), 8, []) for k in range(n)]
        e, inc = (('o',) + rd[0], 4 / KT) if n == KT else (('y',) + rd[0], 4)
        g[-1] = (g[-1][0], 8, [(('xsum',) + rd[0] + (k,), 4, e, inc) for k in range(0, n, 4)])
        return g

    def pick():
        last, endgame, nxt = s['i'] >= len(steps), s['mi'] >= len(main), s['qk']
        if last:
            return g_or(1, True) or g_px() or g_wo(len(wo_left) if 0 < len(wo_left) <= cmaj else 1)
        if endgame:
            return g_or(4, False) or g_px() or g_wo(4) or (g_wo(1) if len(wo_left) > cmaj else None)
        rem = sum(8 for m in main[s['mi']:s['mi'] + 200] if m[0] != 'qk' or m[1] == nxt)
        if (first_step[nxt] - s['i']) * vcost - rem > qlead * 500:
            g = (g_wo(4) if len(wo_left) > keep else None) or g_or(4, False) or g_px()
            if g:
                return g
        m = main[s['mi']]
        if m[0] == 'qk' and done.get(('q', m[1]), 0) < 3:
            return None
        s['mi'] += 1
        pcs = []
        if m[0] == 'q':
            pcs = [(('qfin',) + m[1:], 5, ('q', m[1]), 1)]
        if m[0] == 'qk' and (m[2] == 2 or m[1:3] == (0, 1)) and m[3] % SG == SG - 1:
            t = m[1] if m[2] == 2 else -1
            pcs = [sm(t)[m[3] // SG]] + (sm(t)[KT // SG:] if m[3] == KT - 1 else [])
        return [(m, 8, pcs)]

    def later(t, pcs):
        wait.append((t, pcs))
        wait.sort(key=lambda w: w[0])

    def piece():
        a, cv, e, inc = pend.pop(0)
        if a[0] == 'wld' and s['i'] < len(steps) and not wk[0] <= steps[s['i']][2] <= wk[1]:
            return later(s['tv'] + 30, [(a, cv, e, inc)])
        ev.append(('piece',) + a)
        s['tv'] += cv / 4
        if e is not None:
            done[e] = done.get(e, 0) + inc
        if a[0] == 'smb' and a[2] == KT - SG and a[1] >= 0:
            later(s['tv'] + WD, [(('wld', a[1]), 0, ('wld', a[1]), 1)])
        if a[0] == 'wld':
            later(s['tv'] + WL, [(('w', a[1]), 28, ('w', a[1]), 1)])

    def urgent(p):
        return p[2] is not None and p[2][0] != 'p'

    while True:
        while wait and wait[0][0] <= s['tv']:
            pcs = wait.pop(0)[1]
            pend[:] = [p for p in pcs if urgent(p)] + pend + [p for p in pcs if not urgent(p)]
        i = s['i']
        more = i < len(steps)
        blocked = not more or done.get(('p', steps[i][0] - (i < AP // 2 // AB * KT)), 0) < min(KT, steps[i][2] + 6)
        if not more and or_left:
            cur = (g_or(1, True) or []) + cur
        if not cur and (s['tm'] + LEAD <= s['tv'] or blocked):
            cur = pick() or []
        if not more and not pend and not wait and not cur:
            break
        if cur and (s['tm'] + LEAD <= s['tv']
                    or (blocked and not pend and (not wait or s['tm'] + LEAD <= wait[0][0]))):
            a, cm, pcs = cur.pop(0)
            ev.append(('tile',) + a)
            s['tm'] = max(s['tm'], s['tv'] - LEAD - 8) + cm
            s['tv'] += 0.25 * (a[0] == 'pvx')
            s['qk'] += a[0] == 'qk' and a[2:] == (2, KT - 1)
            src.update({('piece',) + pc[0]: ev[-1] for pc in pcs})
            if pcs:
                later(s['tm'] + (LAT if 0 < i < len(steps) else LAT0), pcs)
        elif blocked and pend:
            piece()
        elif blocked:
            s['tv'] = max(s['tv'], wait[0][0])
        else:
            if pend and (i % pstride == 0 or urgent(pend[0])):
                piece()
            t, a, k = steps[i]
            ev.append(('step', t, a, k))
            if k == KT - 1:
                done['acc', t, a // 8] = done.get(('acc', t, a // 8), 0) + 1
                done['acct', t, a // 8] = s['tv']
            s['tv'] += vcost - 0.5 * sum((t, b) in wide for b in range(a, a + AB))
            s['i'] += 1
    assert not or_left and not wo_left and not px_left

    out, cur, cnt = [], [], 0
    for e in ev + [None]:
        if e is None or (e[0] == 'tile' and e[1] != 'gap' and cnt % 4 == ph):
            if any(x[0] == 'step' for x in cur) and len(cur) < 32 and not any(src.get(x) in cur for x in cur):
                cur = cur[:1] + [x for x in cur[1:] if x[0] == 'piece'] + [x for x in cur[1:] if x[0] != 'piece']
            out += cur
            cur = []
        if e is not None:
            cur.append(e)
            cnt += (4 if e[1] == 'gap' else 1) * (e[0] == 'tile')
    pos = {e: n for n, e in enumerate(out)}
    assert all(pos[a] < pos[b] for b, a in src.items())
    return out


def _slots(events, key):
    first, last = {}, {}
    for n, e in enumerate(events):
        k = key(e)
        if k is not None:
            first.setdefault(k, n)
            last[k] = n
    slot, busy = {}, []
    for k in first:
        free = [i for i, u in enumerate(busy) if u < first[k]]
        slot[k] = free[0] if free else len(busy)
        busy[slot[k]:slot[k] + 1] = [last[k]]
    return slot, len(busy)


def _run(opts, A_x, A_k_cache, A_v_cache, A_wq, A_wo, B_w3, B_w4):
    B, S, D = A_x.shape
    _, H, Sk, Dh = A_k_cache.shape
    F = B_w3.shape[1]
    W = min(4096, max(256, Sk // 4))
    assert (B, S, H, Dh, W) == (1, 1, 32, 192, 4096) and D % 128 == 0 and F % 128 == 0
    AP = Dh // 8
    KT = W // 128
    NP = H // 2
    DT, FT = D // 128, F // 128
    AB, SG, FD = 4, 4, opts.get('fd', 5)
    KP = KT // SG
    SKEW = opts.get('skew', 1)
    cexp = (Dh ** -0.5) * _LOG2E
    nx = {u[:2]: u[2] for u in opts['xunits']}
    xunits = list(nx)
    wide = [(t, a) for t in range(NP) for a in range(0, AP, AB) if (t, a // 8) not in xunits + [(NP - 1, 2)]]
    drop = [g for n, g in enumerate(wide) if n % 3][:max(0, len(wide) - opts['nwide'])]
    wide = [g for g in wide if g not in drop] + [(t, a + 2) for t, a in wide[::-1]][:max(0, opts['nwide'] - len(wide))]
    late = [(t, a) for b in (0, 2) for t in range(NP - 1, 0, -1) for a in range(b, AP, AB)
            if (t, a // 8) not in xunits + [(NP - 1, 2)] and (t, a) not in wide]
    nlate = opts['nlate']
    late = {g: (c, n) for c in range(DT - 1) for n, g in enumerate(late[sum(nlate[:c]):sum(nlate[:c + 1])])}
    events = _schedule(NP, KT, DT, AP, AB, SG, wide=wide + list(late), **opts)
    sp, RP = _slots(events, lambda e: e[1] - (e[1] == 0 and e[2] < AP // 2) if e[0] == 'step'
                    else e[2] if e[1] in ('sma', 'smb', 'pvx') else None)
    ss, RS = _slots(events, lambda e: max(e[2], 0) if e[1] in ('qk', 'sma') else None)
    sq, RQ = _slots(events, lambda e: e[2] if e[1] in ('q', 'qfin') else None)
    sx, RX = _slots(events, lambda e: e[2:4] if e[1] in ('pvx', 'xsum') else None)
    sw, RM = _slots(events, lambda e: e[2] if e[1] in ('wo', 'wacc') else None)
    so, RO = _slots(events, lambda e: e[2:4] if e[1] in ('or', 'ofin') else None)
    sl, RL = _slots(events, lambda e: e[2] if e[1] in ('smb', 'wld') else None)
    assert _slots(events, lambda e: e[2] if e[1] in ('sma', 'smb') else None)[1] == 1
    sizes = [3 * NP, 3 * NP, 2 * NP, 2, DT, 2 * NP + 3, KT, KT * len(wide)]
    QP, Q0, WB, XL, XA, MB, AL, WD, NBIG = [sum(sizes[:n]) for n in range(len(sizes) + 1)]
    OB = Q0
    free, acc_at = [AL, AL + 16], {}
    for e in events:
        if e[0] == 'step' and (e[1], e[2] // 8) not in acc_at:
            acc_at[e[1], e[2] // 8] = free.pop(0)
        if e[0] == 'step' and e[3] == KT - 1:
            free += [WD + KT * wide.index((e[1], a)) + n for a in range(e[2], e[2] + AB) if (e[1], a) in wide
                     for n in (0, 16)]
    sizes = [RP * KP, 3 * RS * KP, RX * KT, 3 * RQ, 4 * DT * RM, 2 * RO, 2 * RL]
    _, SP, XP, QR, WR, OR, ML, NPB = [sum(sizes[:n]) for n in range(len(sizes) + 1)]
    NV, NQ = opts.get('nv', 4), opts.get('nq', 8)
    assert nlate[DT - 2] == 0 and 2 * nlate[DT - 3] <= 11 + (3 * NP - NQ) // 4
    if opts.get('verbose'):
        print('RP RS RQ RX RM', RP, RS, RQ, RX, RM, 'free tiles', (int(13.25 * 256) - NBIG - NPB))
    order1 = sorted(range(NP), key=lambda t: all(u[0] != t for u in xunits))

    def kernel(x_hbm, k_hbm, v_hbm, wq_hbm, wo_hbm, w3_hbm, w4_hbm, o_ref, *scratch):
        k_bufs, v_bufs, scratch = scratch[:NP], scratch[NP:2 * NP], scratch[2 * NP:]
        w4_bufs, wq_bufs, scratch = scratch[:DT], scratch[DT:2 * DT], scratch[2 * DT:]
        wo_buf, w3_buf, pbuf, cst, big, hbuf, xres, x_buf, sems = scratch
        t0 = (Sk - W) // 128

        def kv_cp(kind, t):
            src, dst = (k_hbm, k_bufs[t]) if kind == 0 else (v_hbm, v_bufs[t])
            return [pltpu.make_async_copy(src.at[pl.ds(AP * t, AP), a, pl.ds(t0, KT)],
                                          dst.at[:, :, pl.ds(8 * a, 8), :], sems.at[2 * t + kind])
                    for a in range(2)]

        def w_cp(src, dst, n, sem):
            rows = src.shape[0] // n
            return [pltpu.make_async_copy(src.at[pl.ds(i * rows, rows), a],
                                          dst.at[pl.ds(i * rows, rows), :, pl.ds(8 * a, 8), :], sem)
                    for i in range(n) for a in range(2)]

        def wq_cp():
            cps = [cp for j in range(DT) for cp in w_cp(wq_hbm.at[pl.ds(8 * j, 8)], wq_bufs[j], 1, sems.at[2 * NP])]
            return cps[:1] + [pltpu.make_async_copy(x_hbm, x_buf, sems.at[2 * NP])] + cps[1:]

        def wo_cp():
            return w_cp(wo_hbm, wo_buf, 8, sems.at[2 * NP + 1])

        def w3_cp():
            return [pltpu.make_async_copy(w3_hbm, w3_buf, sems.at[2 * NP + 2])]

        def w4_cp(c):
            return [pltpu.make_async_copy(w4_hbm.at[:, pl.ds(128 * c, 128)], w4_bufs[c], sems.at[2 * NP + 3 + c])]

        def wait(cps):
            for cp in cps:
                cp.wait()

        cps = wq_cp()
        for t in order1:
            cps += kv_cp(0, t) + kv_cp(1, t) + (wo_cp() if t == order1[0] else [])
        for cp in cps + w3_cp() + [cp for c in range(DT) for cp in w4_cp(c)]:
            cp.start()

        ku = [r.bitcast(u32) for r in k_bufs]
        vu = [r.bitcast(u32) for r in v_bufs]
        wqu = [r.bitcast(u32) for r in wq_bufs]
        wou = wo_buf.bitcast(u32)
        w4u = [r.bitcast(u32) for r in w4_bufs]

        def top(n):
            return lax.broadcasted_iota(i32, (8, n), 0) < 4

        def left():
            return lax.broadcasted_iota(i32, (8, 128), 1) < 64

        def cols(n):
            return slice(128 * n, 128 * (n + 1))

        def rows(j):
            return slice(8 * j, 8 * j + 8)

        def masks():
            even = lax.broadcasted_iota(i32, (8, 128), 0) % 2 == 0
            return [even, even == left(), jnp.logical_not(even)]

        def mlp_hidden(x):
            lhs = jnp.where(top(D), x, 1.0)
            m1 = jnp.mean(x, axis=-1, keepdims=True)
            xc = x - m1
            v1 = jnp.mean(xc * xc, axis=-1, keepdims=True)
            r1 = lax.rsqrt(v1 + _EPS)
            y = xc * r1
            m2 = jnp.mean(xc, axis=-1, keepdims=True) * r1
            r2 = lax.rsqrt(v1 * r1 * r1 - m2 * m2 + _EPS)
            coef = jnp.where(top(128), r1 * r2, -(r2 * (r1 * m1 + m2)))
            hs, NF = [], opts.get('nf', 4)
            first = {(n, j): _mm(lhs[:, cols(j)], w3_buf[cols(j), cols(n)]) for j in range(DT) for n in range(NF)}
            for n in range(FT):
                u = _tree(jnp.add, [first[n, j] if n < NF else _mm(lhs[:, cols(j)], w3_buf[cols(j), cols(n)])
                                    for j in range(DT)]) * coef
                hs.append(jax.nn.gelu(u + pltpu.roll(u, 4, 0), approximate=True))
            return y, hs

        def w4_tile(n, c):
            return pltpu.bitcast(w4u[c][64 * n:64 * (n + 1)], bf16)

        def late_at(n, k):
            return ((n * KT + k + 2) % (24 * NP)) // (3 * NP), (n * KT + k + 2) % (3 * NP)

        def unpack_late(c, n0, n1, after=None):
            todo = [(g, n, k) for g, (cc, n) in late.items() if cc == c for k in range(KT)][16 * n0:16 * n1]
            if todo and after is not None:
                wqu[c][after[0], 0] = pltpu.bitcast(after[1], u32)
            for (t, a), n, k in todo:
                y = pltpu.bitcast(pltpu.bitcast(vu[t][a, k], bf16).astype(f32), u32)
                wqu[c][late_at(n, k)] = y[8:16]
                vu[t][a, k] = y[0:8]

        def layer1(z):
            for u, mask in enumerate(masks()):
                cst[u] = jnp.where(mask, cexp, 0.0).astype(f32)
            wait(wq_cp())
            x = jnp.broadcast_to(x_buf[...].astype(f32), (8, D))
            _, xc, r = _stats(x)
            xn = xc * r

            def q_body(t, c):
                for i in range(3):
                    q = _tree(jnp.add, [_mm(xn[:, cols(j)], _wtile(wqu[j][:, 3 * t + i])) for j in range(DT)])
                    big[QP + 3 * t + i] = q * cst[i]
                return c
            lax.fori_loop(0, NP, q_body, 0)

            att = [jnp.zeros((8, 128), f32)] * DT
            for t in order1:
                def s_body(k, c, t=t, q=[big[QP + 3 * t + j] for j in range(3)]):
                    big[AL + k] = _tree(jnp.add, [_mm(q[j], _wtile(ku[t][rows(j), k])) for j in range(3)])
                    return c

                def o_body(k, o, t=t):
                    return [o[j] + _mm(big[AL + k], _wtile(vu[t][rows(j), k]), _NT) for j in range(3)]

                wait(kv_cp(0, t))
                lax.fori_loop(0, KT, s_body, 0, unroll=8)
                sc = big[AL:AL + KT]
                p = jnp.exp2(sc - jnp.max(jnp.max(sc, axis=0), axis=1, keepdims=True))
                big[AL:AL + KT] = p
                inv = 1.0 / jnp.sum(jnp.sum(p, axis=0), axis=1, keepdims=True)
                wait(kv_cp(1, t) + (wo_cp() if t == order1[0] else []))
                o = lax.fori_loop(0, KT, o_body, [jnp.zeros((8, 128), f32)] * 3, unroll=8)
                o = [jnp.where(mask, o[j] * inv, 0.0) for j, mask in enumerate(masks())]
                att = [att[c] + _tree(jnp.add, [_mm(o[j], _wtile(wou[rows(3 * t + j), c])) for j in range(3)])
                       for c in range(DT)]
                for j in [j for tt, j in xunits if tt == t]:
                    def t_body(k, c, t=t, j=j):
                        w = _wtile(vu[t][rows(j), k]).astype(f32).T.astype(bf16)
                        vu[t][rows(j), k] = pltpu.bitcast(w, u32).reshape(8, 8, 128)
                        return c
                    lax.fori_loop(0, nx[t, j], t_body, 0, unroll=4)
                for n, a in [(n, a) for n, (tt, a) in enumerate(wide) if tt == t]:
                    y = _wtile(vu[t][a]).astype(f32).reshape(KT, 16, 128)
                    big[WD + n * KT:WD + (n + 1) * KT] = y[:, 8:16]
                    vu[t][a] = pltpu.bitcast(y[:, 0:8], u32)
            att = jnp.concatenate(att, axis=1)
            x = x + (att + pltpu.roll(att, 1, 0))
            wait(w3_cp())
            y, hs = mlp_hidden(x)
            xres[...] = x + y
            for n in range(FT):
                hbuf[n] = hs[n]
            for c in range(DT - 1):
                wait(w4_cp(c))
                unpack_late(c - 1, 0, 7)
                xc = xres[:, cols(c)] + _tree(jnp.add, [_mm(hbuf[n], w4_tile(n, c)) for n in range(FT)])
                xres[:, cols(c)] = xc
                if c == DT - 2:
                    cst[3] = jnp.broadcast_to(jnp.mean(xres[:, :D - 128], axis=-1, keepdims=True), (8, 128))
                xc = jnp.where(top(128), xc, 1.0)
                unpack_late(c - 1, 7, 11, (z, xc))
                for n in range(3 * NP - (NQ if c == DT - 2 else 0)):
                    r = _mm(xc, _wtile(wqu[c][:, n]))
                    big[Q0 + n] = big[Q0 + n] + r if c else r
                    if n % 4 == 0:
                        unpack_late(c - 1, 11 + n // 4, 12 + n // 4, (z, r))

        def layer2(z):
            wait(w4_cp(DT - 1))
            if opts.get('skip2'):
                keep = big[Q0 + z] + sum(pltpu.bitcast(r[z, 1], f32) for r in wqu + vu)
                o_ref[...] = (xres[0:1, :] + jnp.concatenate([keep[0:1]] * DT, axis=1)).astype(o_ref.dtype)
                return
            xc = xres[:, cols(DT - 1)] + _tree(jnp.add, [_mm(hbuf[n], w4_tile(n, DT - 1)) for n in range(FT)])
            for n in range(3 * NP - NQ, 3 * NP):
                xp = jnp.where(top(128), xres[:, cols(DT - 2)], 1.0)
                big[Q0 + n] = big[Q0 + n] + _mm(xp, _wtile(wqu[DT - 2][:, n]))
            xres[:, cols(DT - 1)] = xc
            d = xres[...] - jnp.concatenate([cst[3]] * DT, axis=1)
            md = jnp.mean(d, axis=-1, keepdims=True)
            r = lax.rsqrt(jnp.mean(d * d, axis=-1, keepdims=True) - md * md + _EPS)
            big[XL] = xraw = jnp.where(top(128), xc, 1.0)
            big[XL + 1] = coef = jnp.where(top(128), r, -(r * (cst[3] + md)))
            acc, val, fwd = {}, {}, []
            st = dict(pin=False, dirty=False, cnt=0, started=False, left=sum(e[0] == 'step' for e in events))

            def lhs(n):
                if st['pin']:
                    st['pin'] = False
                    return big[n + z]
                if n not in val:
                    val[n] = big[n]
                return val[n]

            def checkpoint():
                for (t, a), y in acc.items():
                    n = acc_at[t, a // 8] + 2 * (a % 8)
                    big[n:n + 2] = y.reshape(2, 8, 128)

            def put(n, r, rs=slice(0, 8)):
                fwd.append((st['cnt'], n, r, rs))

            def flush(upto, pin=False):
                while fwd and fwd[0][0] <= upto:
                    _, n, r, rs = fwd.pop(0)
                    pbuf[z if pin else 0, rs, cols(n)] = r[rs]
                    if pin and st['left'] <= opts.get('vpin', 72):
                        vu[NP - 1][z, 2] = pltpu.bitcast(r, u32)
                    pin = False

            def get(n):
                flush(max([f[0] for f in fwd if f[1] == n], default=-1))
                return pbuf[0, :, cols(n)]

            def ptile(t, k):
                return cols(sp[t] * KP + k // SG)

            def prow(t, odd, k):
                r = 2 * (k % SG) + odd
                return pbuf[0, r:r + 1, ptile(t - (t + odd == 0), k)]

            def q_fin(t, i, y, coef):
                y = (y + big[Q0 + 3 * t + i]) * coef
                big[QP + 3 * t + i] = (y + pltpu.roll(y, 4, 0)) * cst[i]

            def t_qraw(t, i):
                q_fin(t, i, _mm(xraw, _wtile(wqu[DT - 1][:, 3 * t + i])), coef)

            def t_q(t, i):
                put(QR + sq[t] * 3 + i, _mm(lhs(XL), _wtile(wqu[DT - 1][:, 3 * t + i])))

            def t_qk(t, j, k):
                put(SP + (3 * ss[t] + j) * KP + k // SG, _mm(lhs(QP + 3 * t + j), _wtile(ku[t][rows(j), k])),
                    slice(2 * (k % SG), 2 * (k % SG) + 2))

            def t_or(t, j):
                a = big[acc_at[t, j]:acc_at[t, j] + 16].reshape(128, 128)
                if j == 1:
                    r = _mm(jnp.concatenate([lhs(WB + 2 * t), lhs(WB + 2 * t + 1)], axis=0), a, _NT)
                    put(OR + 2 * so[t, j] + 1, r[8:16])
                else:
                    r = _mm(lhs(WB + 2 * t + j // 2), a, _NT)
                put(OR + 2 * so[t, j], r[0:8])

            def t_pvx(t, j, k):
                p = val.pop(('px', t, j, k)) * lhs(WB + 2 * t + j // 2)
                put(XP + sx[t, j] * KT + k, _mm(p, _wtile(vu[t][rows(j), k])))

            def t_wo(units, n, c):
                t, j = units[n]
                put(WR + (sw[units] * 4 + n) * DT + c, _mm(lhs(OB + 3 * t + j), _wtile(wou[rows(3 * t + j), c])))

            def p_qfin(t, i):
                q_fin(t, i, get(QR + sq[t] * 3 + i), big[XL + 1])

            def over_tiles(op, y):
                y = op(y, pltpu.roll(y, 2, 0))
                return op(y, pltpu.roll(y, 4, 0))

            def p_sma(t, k0):
                n = SP + 3 * ss[max(t, 0)] * KP + k0 // SG
                sc = get(n) + get(n + KP)
                sc = sc + get(n + 2 * KP) if t >= 0 else sc
                pbuf[0, :, ptile(t, k0)] = sc
                m = jnp.maximum(sc, val['m']) if k0 else sc
                big[MB + 2 + 2 * t] = val['m'] = over_tiles(jnp.maximum, m) if k0 + SG == KT else m

            def p_smb(t, k0):
                pbuf[0, :, ptile(t, k0)] = p = jnp.exp2(pbuf[0, :, ptile(t, k0)] - val['m'])
                if t >= 0:
                    big[MB + 3 + 2 * t] = val['l'] = p + val['l'] if k0 else p
                if t >= 0 and k0 + SG == KT:
                    pbuf[0, :, cols(ML + 2 * sl[t])] = val['m']
                    pbuf[0, :, cols(ML + 2 * sl[t] + 1)] = val['l']

            def p_wld(t):
                val['ml', t] = pbuf[0, :, cols(ML + 2 * sl[t])], pbuf[0, :, cols(ML + 2 * sl[t] + 1)]

            def p_w(t):
                m, l = val['ml', t]
                e = jnp.exp2(m - jnp.max(m, axis=1, keepdims=True))
                w = e / jnp.sum(e * over_tiles(jnp.add, l), axis=1, keepdims=True)
                for h in range(2):
                    big[WB + 2 * t + h] = jnp.broadcast_to(w[h:h + 1], (8, 128))

            def p_ofin(t, j):
                r = get(OR + 2 * so[t, j])
                r = jnp.where(left(), r, get(OR + 2 * so[t, j] + 1)) if j == 1 else r
                big[OB + 3 * t + j] = r + big[OB + 3 * t + j] if (t, j) in nx else r

            def p_xsum(t, j, k0):
                n = XP + sx[t, j] * KT + k0
                ys = [get(n + u) for u in range(4)] + ([val['y', t, j]] if k0 else [])
                big[OB + 3 * t + j] = val['y', t, j] = _tree(jnp.add, ys)

            def p_wacc(units, c):
                rs = [get(WR + (sw[units] * 4 + n) * DT + c) for n in range(len(units))]
                big[XA + c] = _tree(jnp.add, rs + ([big[XA + c]] if units != next(iter(sw)) else []))

            fns = {'qraw': t_qraw, 'q': t_q, 'qk': t_qk, 'or': t_or, 'pvx': t_pvx, 'wo': t_wo, 'qfin': p_qfin,
                   'sma': p_sma, 'smb': p_smb, 'wld': p_wld, 'w': p_w, 'ofin': p_ofin, 'xsum': p_xsum, 'wacc': p_wacc}
            tiles = [e for e in events if e[0] == 'tile' and e[1] != 'gap']
            for e in events:
                if e[0] == 'step':
                    _, t, a0, k = e
                    k0 = nx.get((t, a0 // 8), 0)
                    for a in range(a0, a0 + AB):
                        n = k + SKEW * (a - a0)
                        kk = k0 + (n - k0) % (KT - k0)
                        if ('p', t, a0, n) not in val:
                            val['p', t, a0, n] = prow(t, int(a0 >= AP // 2), kk)
                        if (t, a) in wide:
                            y = jnp.concatenate([pltpu.bitcast(vu[t][a, kk], f32),
                                                 big[WD + wide.index((t, a)) * KT + kk]])
                        elif (t, a) in late:
                            c, u = late[t, a]
                            y = pltpu.bitcast(jnp.concatenate([vu[t][a, kk], wqu[c][late_at(u, kk)]]), f32)
                        else:
                            y = pltpu.bitcast(vu[t][a, kk], bf16).astype(f32)
                        y = y * val['p', t, a0, n]
                        acc[t, a] = acc[t, a] + y if (t, a) in acc else y
                    st.update(dirty=True, started=True, left=st['left'] - 1)
                    if k == KT - 1:
                        checkpoint()
                        acc.clear()
                elif e[0] == 'piece':
                    fns[e[1]](*e[2:])
                elif e[1] == 'gap':
                    st['cnt'] += 4
                else:
                    pinned = st['cnt'] % 4 == opts.get('ph', 0) and st['left'] > 0
                    if pinned and st['dirty']:
                        checkpoint()
                    st.update(pin=pinned and st['started'], dirty=st['dirty'] and not pinned)
                    fns[e[1]](*e[2:])
                    st['pin'] = False
                    tiles.pop(0)
                    for u in tiles[:opts.get('pf', 4)]:
                        if u[1] == 'pvx' and ('px',) + u[2:] not in val:
                            val[('px',) + u[2:]] = prow(u[2], u[3] // 2, u[4])
                    if pinned:
                        flush(st['cnt'] - 4 * FD + 3, pin=st['started'])
                    st['cnt'] += 1
            assert not fwd
            x = xres[...] + jnp.concatenate([big[XA + c] for c in range(DT)], axis=1)
            y, hs = mlp_hidden(x)
            out = [(x + y)[:, cols(c)] for c in range(DT)]
            part = [None] * DT
            hb = [jnp.concatenate([hs[n]] * 16, axis=0).T for n in range(NV)]
            for n0 in range(0, NV, 3):
                for a in range(8):
                    for n in range(n0, min(n0 + 3, NV)):
                        for c in range(DT):
                            u = pltpu.bitcast(w4u[c][rows(8 * n + a)], bf16).astype(f32) * hb[n][16 * a:16 * a + 16]
                            part[c] = u if part[c] is None else part[c] + u
            for n in range(NV, FT):
                out = [out[c] + _mm(hs[n], w4_tile(n, c)) for c in range(DT)]
            out = [out[c] + jnp.sum(part[c], axis=0, keepdims=True) for c in range(DT)]
            o_ref[...] = jnp.concatenate(out, axis=1)[0:1].astype(o_ref.dtype)

        def body(it, carry):
            pl.when(it == 0)(lambda: layer1(it >> 4) if not opts.get('skip1') else None)
            pl.when(it == 1)(lambda: layer2(it >> 4))
            return carry

        lax.fori_loop(0, 2, body, 0)

    def V(*s, dt=f32):
        return pltpu.VMEM(s, dt)

    out = pl.pallas_call(
        kernel,
        out_shape=jax.ShapeDtypeStruct((1, D), A_x.dtype),
        in_specs=[pl.BlockSpec(memory_space=pl.ANY)] * 7,
        out_specs=pl.BlockSpec(memory_space=pltpu.VMEM),
        scratch_shapes=(
            [V(AP, KT, 16, 128, dt=bf16)] * (2 * NP)
            + [V(F, 128, dt=bf16)] * DT + [V(8, 3 * NP, 16, 128, dt=bf16)] * DT
            + [V(AP * NP, DT, 16, 128, dt=bf16), V(D, F, dt=bf16),
               V(1, 8, -(-NPB // 4) * 512), V(4, 8, 128), V(-(-NBIG // 4) * 4, 8, 128),
               V(FT, 8, 128), V(8, D), V(1, D, dt=bf16),
               pltpu.SemaphoreType.DMA((2 * NP + 3 + DT,))]),
        compiler_params=pltpu.CompilerParams(
            vmem_limit_bytes=int(opts.get('vmem', 128) * 1024 * 1024),
            disable_semaphore_checks=True, disable_bounds_checks=True),
        name='fused_decode_layers',
    )(A_x.reshape(1, D), _cache_view(A_k_cache), _cache_view(A_v_cache),
      _weight_view(A_wq), _weight_view(A_wo), B_w3, B_w4)
    return out.reshape(B, S, D)


@jax.jit
def pallas_interleave_layers__sliding_block_cached__mixer_s_mlp__decode_kernel(
    A_x: jax.Array,
    A_k_cache: jax.Array,
    A_v_cache: jax.Array,
    A_wq: jax.Array,
    A_wo: jax.Array,
    B_x: jax.Array,
    B_w1: jax.Array,
    B_w2: jax.Array,
    B_w3: jax.Array,
    B_w4: jax.Array,
):
    return _run(_OPTS, A_x, A_k_cache, A_v_cache, A_wq, A_wo, B_w3, B_w4)
```

```python
import jax
import jax.numpy as jnp
from jax import lax
import jax.experimental.pallas as pl
import jax.experimental.pallas.tpu as pltpu

f32, bf16, u32, i32 = jnp.float32, jnp.bfloat16, jnp.uint32, jnp.int32
_EPS = 1e-5
_LOG2E = 1.4426950408889634
_NN = (((1,), (0,)), ((), ()))
_NT = (((1,), (1,)), ((), ()))

_OPTS = dict(xunits=[(5, 0, 32), (7, 2, 32), (9, 2, 32), (11, 0, 32), (14, 2, 4)], nwide=89, nlate=[10, 10, 9, 0], wlast=[3, 7, 11, 14, 15], qlead=2.0, keep=8,
             AD=60, LAT=205, LAT0=205, q2at=20, vpin=36)


def _stats(x):
    m = jnp.mean(x, axis=-1, keepdims=True)
    xc = x - m
    v = jnp.mean(xc * xc, axis=-1, keepdims=True)
    return m, xc, lax.rsqrt(v + _EPS)


def _tree(op, xs):
    xs = list(xs)
    while len(xs) > 1:
        nxt = [op(xs[i], xs[i + 1]) for i in range(0, len(xs) - 1, 2)]
        if len(xs) % 2:
            nxt.append(xs[-1])
        xs = nxt
    return xs[0]


def _wtile(u):
    return pltpu.bitcast(u.reshape(u.shape[0] * 8, 128), bf16)


def _mm(lhs, w, dims=_NN):
    return lax.dot_general(lhs, w, dims, preferred_element_type=f32)


def _cache_view(c):
    _, H, Sk, Dh = c.shape
    c = c.reshape(H, Sk // 128, 128, Dh // 16, 2, 8)
    c = jnp.transpose(c, (0, 3, 4, 1, 5, 2))
    return c.reshape(H * Dh // 16, 2, Sk // 128, 8, 128)


def _weight_view(w):
    R, N = w.shape
    w = w.reshape(R // 16, 2, 8, N // 128, 128)
    return jnp.transpose(w, (0, 1, 3, 2, 4))


def _schedule(NP, KT, DT, AP, AB, SG, xunits, qlead, keep, LAT=205, LAT0=165, LEAD=32, WD=140, WL=400, AD=160,
              vcost=5.95, pstride=2, nraw=8, q2at=40, ph=0, wide=(), wk=(8, 20), cmaj=4, wlast=(), **_):
    xs = {u[:2]: u[2] for u in xunits}
    grp = [(t, a) for t in range(NP) for a in range(0, AP, AB)]
    grp[-2:] = grp[:-3:-1]
    steps = [(t, a, k) for t, a in grp for k in range(xs.get((t, a // 8), 0), KT)]
    first_step = {}
    for i, s in enumerate(steps):
        first_step.setdefault(s[0], i)
    main = [('qraw', t, i) for t in range(nraw) for i in range(3)]
    for t in range(NP):
        qk = [('qk', t, j, k) for j in range(3) for k in range(KT)]
        main += qk[:q2at] + [('q', t + 1, i) for i in range(3) if nraw <= t + 1 < NP] + qk[q2at:]
    done = {('q', t): 3 for t in range(nraw)}
    or_left = [(t, j) for t in range(NP) for j in range(3) if xs.get((t, j), 0) < KT]
    wo_left = [(t, j) for t in range(NP) for j in range(3)]
    px_left = list(xs)
    ev, pend, wait, cur, src = [], [], [], [], {}
    s = dict(tm=0.0, tv=0.0, i=0, mi=0, qk=0)

    def sm(t):
        return ([(('sma', t, k), 3 + 4 * (k == KT - SG), None, 0) for k in range(0, KT, SG)]
                + [(('smb', t, k), 3 + 4 * (k == KT - SG), ('p', t), SG) for k in range(0, KT, SG)])

    def g_wo(n):
        wo = tuple(u for u in wo_left if done.get(('o',) + u, 0) >= 1)[:4]
        if len(wo_left) > cmaj:
            wo = wo[:len(wo_left) - cmaj]
        if len(wo) < n:
            return None
        for u in wo:
            wo_left.remove(u)
        g = [(('wo', wo, n, c), 8, []) for n in range(len(wo)) for c in range(DT)]
        if not wo_left and cmaj:
            g.sort(key=lambda x: x[0][3])
        g[-1] = (g[-1][0], 8, [(('wacc', wo, c), 1, None, 0) for c in range(DT)])
        return g

    def g_or(n, last):
        rd = [u for u in or_left if done.get(('acc',) + u, 0) >= 8 // AB and done.get(('w', min(t for t in wlast if t >= u[0])), 0)
              and (last or done[('acct',) + u] + AD <= s['tv'])
              and done.get(('y',) + u, 0) >= xs.get(u, 0)][:4]
        if len(rd) < n:
            return None
        for u in rd:
            or_left.remove(u)
        return [(('gap',), 8 * len(rd), [])] + [(('or',) + u, 8, [(('ofin',) + u, 1, ('o',) + u, 1)]) for u in rd]

    def g_px():
        rd = [u for u in px_left if done.get(('w', min(t for t in wlast if t >= u[0])), 0)]
        if not rd:
            return None
        px_left.remove(rd[0])
        n = xs[rd[0]]
        g = [(('pvx',) + rd[0] + (k,), 8, []) for k in range(n)]
        g[-1] = (g[-1][0], 8, [(('xsum',) + rd[0], n // 4 + 3, ('o' if n == KT else 'y',) + rd[0], n)])
        return g

    def pick():
        last, endgame, nxt = s['i'] >= len(steps), s['mi'] >= len(main), s['qk']
        if last:
            return g_or(1, True) or g_px() or g_wo(len(wo_left) if 0 < len(wo_left) <= cmaj else 1)
        if endgame:
            return g_or(4, False) or g_px() or g_wo(4) or (g_wo(1) if len(wo_left) > cmaj else None)
        rem = sum(8 for m in main[s['mi']:s['mi'] + 200] if m[0] != 'qk' or m[1] == nxt)
        if (first_step[nxt] - s['i']) * vcost - rem > qlead * 500:
            g = (g_wo(4) if len(wo_left) > keep else None) or g_or(4, False) or g_px()
            if g:
                return g
        m = main[s['mi']]
        if m[0] == 'qk' and done.get(('q', m[1]), 0) < 3:
            return None
        s['mi'] += 1
        pcs = []
        if m[0] == 'q':
            pcs = [(('qfin',) + m[1:], 5, ('q', m[1]), 1)]
        if m[0] == 'qk' and (m[2] == 2 or m[1:3] == (0, 1)) and m[3] % SG == SG - 1:
            t = m[1] if m[2] == 2 else -1
            pcs = [sm(t)[m[3] // SG]] + (sm(t)[KT // SG:] if m[3] == KT - 1 else [])
        return [(m, 8, pcs)]

    def later(t, pcs):
        wait.append((t, pcs))
        wait.sort(key=lambda w: w[0])

    def piece():
        a, cv, e, inc = pend.pop(0)
        if a[0] == 'wld' and s['i'] < len(steps) and not wk[0] <= steps[s['i']][2] <= wk[1]:
            return later(s['tv'] + 30, [(a, cv, e, inc)])
        ev.append(('piece',) + a)
        s['tv'] += cv / 4
        if e is not None:
            done[e] = done.get(e, 0) + inc
        if a[0] == 'smb' and a[2] == KT - SG and a[1] in wlast:
            later(s['tv'] + WD, [(('wld', a[1]), 0, ('wld', a[1]), 1)])
        if a[0] == 'wld':
            later(s['tv'] + WL, [(('w', a[1]), 26, ('w', a[1]), 1)])

    def urgent(p):
        return p[2] is not None and p[2][0] != 'p'

    while True:
        while wait and wait[0][0] <= s['tv']:
            pcs = wait.pop(0)[1]
            pend[:] = [p for p in pcs if urgent(p)] + pend + [p for p in pcs if not urgent(p)]
        i = s['i']
        more = i < len(steps)
        blocked = not more or done.get(('p', steps[i][0] - (i < AP // 2 // AB * KT)), 0) < min(KT, steps[i][2] + 6)
        if not more and or_left:
            cur = (g_or(1, True) or []) + cur
        if not cur and (s['tm'] + LEAD <= s['tv'] or blocked):
            cur = pick() or []
        if not more and not pend and not wait and not cur:
            break
        if cur and (s['tm'] + LEAD <= s['tv']
                    or (blocked and not pend and (not wait or s['tm'] + LEAD <= wait[0][0]))):
            a, cm, pcs = cur.pop(0)
            ev.append(('tile',) + a)
            s['tm'] = max(s['tm'], s['tv'] - LEAD - 8) + cm
            s['tv'] += 0.25 * (a[0] == 'pvx')
            s['qk'] += a[0] == 'qk' and a[2:] == (2, KT - 1)
            src.update({('piece',) + pc[0]: ev[-1] for pc in pcs})
            if pcs:
                later(s['tm'] + (LAT if 0 < i < len(steps) else LAT0), pcs)
        elif blocked and pend:
            piece()
        elif blocked:
            s['tv'] = max(s['tv'], wait[0][0])
        else:
            if pend and (i % pstride == 0 or urgent(pend[0])):
                piece()
            t, a, k = steps[i]
            ev.append(('step', t, a, k))
            if k == KT - 1:
                done['acc', t, a // 8] = done.get(('acc', t, a // 8), 0) + 1
                done['acct', t, a // 8] = s['tv']
            s['tv'] += vcost - 0.5 * sum((t, b) in wide for b in range(a, a + AB))
            s['i'] += 1
    assert not or_left and not wo_left and not px_left

    out, cur, cnt = [], [], 0
    for e in ev + [None]:
        if e is None or (e[0] == 'tile' and e[1] != 'gap' and cnt % 4 == ph):
            if any(x[0] == 'step' for x in cur) and len(cur) < 32 and not any(src.get(x) in cur for x in cur):
                cur = cur[:1] + [x for x in cur[1:] if x[0] == 'piece'] + [x for x in cur[1:] if x[0] != 'piece']
            out += cur
            cur = []
        if e is not None:
            cur.append(e)
            cnt += (4 if e[1] == 'gap' else 1) * (e[0] == 'tile')
    pos = {e: n for n, e in enumerate(out)}
    assert all(pos[a] < pos[b] for b, a in src.items())
    return out


def _slots(events, key):
    first, last = {}, {}
    for n, e in enumerate(events):
        k = key(e)
        if k is not None:
            first.setdefault(k, n)
            last[k] = n
    slot, busy = {}, []
    for k in first:
        free = [i for i, u in enumerate(busy) if u < first[k]]
        slot[k] = free[0] if free else len(busy)
        busy[slot[k]:slot[k] + 1] = [last[k]]
    return slot, len(busy)


def _run(opts, A_x, A_k_cache, A_v_cache, A_wq, A_wo, B_w3, B_w4):
    B, S, D = A_x.shape
    _, H, Sk, Dh = A_k_cache.shape
    F = B_w3.shape[1]
    W = min(4096, max(256, Sk // 4))
    assert (B, S, H, Dh, W) == (1, 1, 32, 192, 4096) and D % 128 == 0 and F % 128 == 0
    AP = Dh // 8
    KT = W // 128
    NP = H // 2
    DT, FT = D // 128, F // 128
    AB, SG, FD = 4, 4, opts.get('fd', 5)
    KP = KT // SG
    SKEW = opts.get('skew', 1)
    cexp = (Dh ** -0.5) * _LOG2E
    nx = {u[:2]: u[2] for u in opts['xunits']}
    xunits = list(nx)
    wide = [(t, a) for t in range(NP) for a in range(0, AP, AB) if (t, a // 8) not in xunits + [(NP - 1, 2)]]
    drop = [g for n, g in enumerate(wide) if n % 3][:max(0, len(wide) - opts['nwide'])]
    wide = [g for g in wide if g not in drop] + [(t, a + 2) for t, a in wide[::-1]][:max(0, opts['nwide'] - len(wide))]
    late = [(t, a) for b in (0, 2) for t in range(NP - 1, 0, -1) for a in range(b, AP, AB)
            if (t, a // 8) not in xunits + [(NP - 1, 2)] and (t, a) not in wide]
    nlate = opts['nlate']
    late = {g: (c, n) for c in range(DT - 1) for n, g in enumerate(late[sum(nlate[:c]):sum(nlate[:c + 1])])}
    events = _schedule(NP, KT, DT, AP, AB, SG, wide=wide + list(late), **opts)
    sp, RP = _slots(events, lambda e: e[1] - (e[1] == 0 and e[2] < AP // 2) if e[0] == 'step'
                    else e[2] if e[1] in ('sma', 'smb', 'pvx') else None)
    ss, RS = _slots(events, lambda e: max(e[2], 0) if e[1] in ('qk', 'sma') else None)
    sq, RQ = _slots(events, lambda e: e[2] if e[1] in ('q', 'qfin') else None)
    sx, RX = _slots(events, lambda e: e[2:4] if e[1] in ('pvx', 'xsum') else None)
    sw, RM = _slots(events, lambda e: e[2] if e[1] in ('wo', 'wacc') else None)
    so, RO = _slots(events, lambda e: e[2:4] if e[1] in ('or', 'ofin') else None)
    wlast = opts['wlast']
    wgrp = {t: [u for u in range(NP) if max([-1] + [v for v in wlast if v < t]) < u <= min(v for v in wlast if v >= t)]
            for t in range(NP)}
    sl, RL = _slots(events, lambda e: wgrp[e[2]][-1] if e[1] in ('smb', 'wld') and e[2] >= 0 else None)
    assert _slots(events, lambda e: e[2] if e[1] in ('sma', 'smb') else None)[1] == 1
    sizes = [3 * NP, 3 * NP, 2 * NP, 2, DT, 2 * NP + 3, KT, KT * len(wide)]
    QP, Q0, WB, XL, XA, MB, AL, WD, NBIG = [sum(sizes[:n]) for n in range(len(sizes) + 1)]
    OB = Q0
    free, acc_at = [AL, AL + 16], {}
    for e in events:
        if e[0] == 'step' and (e[1], e[2] // 8) not in acc_at:
            acc_at[e[1], e[2] // 8] = free.pop(0)
        if e[0] == 'step' and e[3] == KT - 1:
            free += [WD + KT * wide.index((e[1], a)) + n for a in range(e[2], e[2] + AB) if (e[1], a) in wide
                     for n in (0, 16)]
    sizes = [RP * KP, 3 * RS * KP, RX * KP, 3 * RQ, DT * (RM + 4), 2 * RO, 2 * RL]
    _, SP, XP, QR, WR, OR, ML, NPB = [sum(sizes[:n]) for n in range(len(sizes) + 1)]
    NV, NQ = opts.get('nv', 4), opts.get('nq', 8)
    assert nlate[DT - 2] == 0 and 2 * nlate[DT - 3] <= 11 + (3 * NP - NQ) // 4
    if opts.get('verbose'):
        print('RP RS RQ RX RM', RP, RS, RQ, RX, RM, 'free tiles', (int(13.25 * 256) - NBIG - NPB))
    order1 = sorted(range(NP), key=lambda t: all(u[0] != t for u in xunits))

    def kernel(x_hbm, k_hbm, v_hbm, wq_hbm, wo_hbm, w3_hbm, w4_hbm, o_ref, *scratch):
        k_bufs, v_bufs, scratch = scratch[:NP], scratch[NP:2 * NP], scratch[2 * NP:]
        w4_bufs, wq_bufs, scratch = scratch[:DT], scratch[DT:2 * DT], scratch[2 * DT:]
        wo_buf, w3_buf, pbuf, cst, big, hbuf, xres, x_buf, sems = scratch
        t0 = (Sk - W) // 128

        def kv_cp(kind, t):
            src, dst = (k_hbm, k_bufs[t]) if kind == 0 else (v_hbm, v_bufs[t])
            return [pltpu.make_async_copy(src.at[pl.ds(AP * t, AP), a, pl.ds(t0, KT)],
                                          dst.at[:, :, pl.ds(8 * a, 8), :], sems.at[2 * t + kind])
                    for a in range(2)]

        def w_cp(src, dst, n, sem):
            rows = src.shape[0] // n
            return [pltpu.make_async_copy(src.at[pl.ds(i * rows, rows), a],
                                          dst.at[pl.ds(i * rows, rows), :, pl.ds(8 * a, 8), :], sem)
                    for i in range(n) for a in range(2)]

        def wq_cp():
            cps = [cp for j in range(DT) for cp in w_cp(wq_hbm.at[pl.ds(8 * j, 8)], wq_bufs[j], 1, sems.at[2 * NP])]
            return cps[:1] + [pltpu.make_async_copy(x_hbm, x_buf, sems.at[2 * NP])] + cps[1:]

        def wo_cp():
            return w_cp(wo_hbm, wo_buf, 8, sems.at[2 * NP + 1])

        def w3_cp():
            return [pltpu.make_async_copy(w3_hbm, w3_buf, sems.at[2 * NP + 2])]

        def w4_cp(c):
            return [pltpu.make_async_copy(w4_hbm.at[:, pl.ds(128 * c, 128)], w4_bufs[c], sems.at[2 * NP + 3 + c])]

        def wait(cps):
            for cp in cps:
                cp.wait()

        cps = wq_cp()
        for t in order1:
            cps += kv_cp(0, t) + kv_cp(1, t) + (wo_cp() if t == order1[0] else [])
        for cp in cps + w3_cp() + [cp for c in range(DT) for cp in w4_cp(c)]:
            cp.start()

        ku = [r.bitcast(u32) for r in k_bufs]
        vu = [r.bitcast(u32) for r in v_bufs]
        wqu = [r.bitcast(u32) for r in wq_bufs]
        wou = wo_buf.bitcast(u32)
        w4u = [r.bitcast(u32) for r in w4_bufs]

        def top(n):
            return lax.broadcasted_iota(i32, (8, n), 0) < 4

        def left():
            return lax.broadcasted_iota(i32, (8, 128), 1) < 64

        def cols(n):
            return slice(128 * n, 128 * (n + 1))

        def rows(j):
            return slice(8 * j, 8 * j + 8)

        def masks():
            even = lax.broadcasted_iota(i32, (8, 128), 0) % 2 == 0
            return [even, even == left(), jnp.logical_not(even)]

        def mlp_hidden(x):
            lhs = jnp.where(top(D), x, 1.0)
            m1 = jnp.mean(x, axis=-1, keepdims=True)
            xc = x - m1
            v1 = jnp.mean(xc * xc, axis=-1, keepdims=True)
            r1 = lax.rsqrt(v1 + _EPS)
            y = xc * r1
            m2 = jnp.mean(xc, axis=-1, keepdims=True) * r1
            r2 = lax.rsqrt(v1 * r1 * r1 - m2 * m2 + _EPS)
            coef = jnp.where(top(128), r1 * r2, -(r2 * (r1 * m1 + m2)))
            hs, NF = [], opts.get('nf', 4)
            first = {(n, j): _mm(lhs[:, cols(j)], w3_buf[cols(j), cols(n)]) for j in range(DT) for n in range(NF)}
            for n in range(FT):
                u = _tree(jnp.add, [first[n, j] if n < NF else _mm(lhs[:, cols(j)], w3_buf[cols(j), cols(n)])
                                    for j in range(DT)]) * coef
                hs.append(jax.nn.gelu(u + pltpu.roll(u, 4, 0), approximate=True))
            return y, hs

        def w4_tile(n, c):
            return pltpu.bitcast(w4u[c][64 * n:64 * (n + 1)], bf16)

        def late_at(n, k):
            return ((n * KT + k + 2) % (24 * NP)) // (3 * NP), (n * KT + k + 2) % (3 * NP)

        def unpack_late(c, n0, n1, after=None):
            todo = [(g, n, k) for g, (cc, n) in late.items() if cc == c for k in range(KT)][16 * n0:16 * n1]
            if todo and after is not None:
                wqu[c][after[0], 0] = pltpu.bitcast(after[1], u32)
            for (t, a), n, k in todo:
                y = pltpu.bitcast(pltpu.bitcast(vu[t][a, k], bf16).astype(f32), u32)
                wqu[c][late_at(n, k)] = y[8:16]
                vu[t][a, k] = y[0:8]

        def layer1(z):
            for u, mask in enumerate(masks()):
                cst[u] = jnp.where(mask, cexp, 0.0).astype(f32)
            wait(wq_cp())
            x = jnp.broadcast_to(x_buf[...].astype(f32), (8, D))
            _, xc, r = _stats(x)
            xn = xc * r

            def q_body(t, c):
                for i in range(3):
                    q = _tree(jnp.add, [_mm(xn[:, cols(j)], _wtile(wqu[j][:, 3 * t + i])) for j in range(DT)])
                    big[QP + 3 * t + i] = q * cst[i]
                return c
            lax.fori_loop(0, NP, q_body, 0)

            att = [jnp.zeros((8, 128), f32)] * DT
            for t in order1:
                def s_body(k, c, t=t, q=[big[QP + 3 * t + j] for j in range(3)]):
                    big[AL + k] = _tree(jnp.add, [_mm(q[j], _wtile(ku[t][rows(j), k])) for j in range(3)])
                    return c

                def o_body(k, o, t=t):
                    return [o[j] + _mm(big[AL + k], _wtile(vu[t][rows(j), k]), _NT) for j in range(3)]

                wait(kv_cp(0, t))
                lax.fori_loop(0, KT, s_body, 0, unroll=8)
                sc = big[AL:AL + KT]
                p = jnp.exp2(sc - jnp.max(jnp.max(sc, axis=0), axis=1, keepdims=True))
                big[AL:AL + KT] = p
                inv = 1.0 / jnp.sum(jnp.sum(p, axis=0), axis=1, keepdims=True)
                wait(kv_cp(1, t) + (wo_cp() if t == order1[0] else []))
                o = lax.fori_loop(0, KT, o_body, [jnp.zeros((8, 128), f32)] * 3, unroll=8)
                o = [jnp.where(mask, o[j] * inv, 0.0) for j, mask in enumerate(masks())]
                att = [att[c] + _tree(jnp.add, [_mm(o[j], _wtile(wou[rows(3 * t + j), c])) for j in range(3)])
                       for c in range(DT)]
                for j in [j for tt, j in xunits if tt == t]:
                    def t_body(k, c, t=t, j=j):
                        w = _wtile(vu[t][rows(j), k]).astype(f32).T.astype(bf16)
                        vu[t][rows(j), k] = pltpu.bitcast(w, u32).reshape(8, 8, 128)
                        return c
                    lax.fori_loop(0, nx[t, j], t_body, 0, unroll=4)
                for n, a in [(n, a) for n, (tt, a) in enumerate(wide) if tt == t]:
                    y = _wtile(vu[t][a]).astype(f32).reshape(KT, 16, 128)
                    big[WD + n * KT:WD + (n + 1) * KT] = y[:, 8:16]
                    vu[t][a] = pltpu.bitcast(y[:, 0:8], u32)
            att = jnp.concatenate(att, axis=1)
            x = x + (att + pltpu.roll(att, 1, 0))
            wait(w3_cp())
            y, hs = mlp_hidden(x)
            xres[...] = x + y
            for n in range(FT):
                hbuf[n] = hs[n]
            for c in range(DT - 1):
                wait(w4_cp(c))
                unpack_late(c - 1, 0, 7)
                xc = xres[:, cols(c)] + _tree(jnp.add, [_mm(hbuf[n], w4_tile(n, c)) for n in range(FT)])
                xres[:, cols(c)] = xc
                if c == DT - 2:
                    cst[3] = jnp.broadcast_to(jnp.mean(xres[:, :D - 128], axis=-1, keepdims=True), (8, 128))
                xc = jnp.where(top(128), xc, 1.0)
                unpack_late(c - 1, 7, 11, (z, xc))
                for n in range(3 * NP - (NQ if c == DT - 2 else 0)):
                    r = _mm(xc, _wtile(wqu[c][:, n]))
                    big[Q0 + n] = big[Q0 + n] + r if c else r
                    if n % 4 == 0:
                        unpack_late(c - 1, 11 + n // 4, 12 + n // 4, (z, r))

        def layer2(z):
            wait(w4_cp(DT - 1))
            if opts.get('skip2'):
                keep = big[Q0 + z] + sum(pltpu.bitcast(r[z, 1], f32) for r in wqu + vu)
                o_ref[...] = (xres[0:1, :] + jnp.concatenate([keep[0:1]] * DT, axis=1)).astype(o_ref.dtype)
                return
            xc = xres[:, cols(DT - 1)] + _tree(jnp.add, [_mm(hbuf[n], w4_tile(n, DT - 1)) for n in range(FT)])
            for n in range(3 * NP - NQ, 3 * NP):
                xp = jnp.where(top(128), xres[:, cols(DT - 2)], 1.0)
                big[Q0 + n] = big[Q0 + n] + _mm(xp, _wtile(wqu[DT - 2][:, n]))
            xres[:, cols(DT - 1)] = xc
            d = xres[...] - jnp.concatenate([cst[3]] * DT, axis=1)
            md = jnp.mean(d, axis=-1, keepdims=True)
            r = lax.rsqrt(jnp.mean(d * d, axis=-1, keepdims=True) - md * md + _EPS)
            big[XL] = xraw = jnp.where(top(128), xc, 1.0)
            big[XL + 1] = coef = jnp.where(top(128), r, -(r * (cst[3] + md)))
            acc, val, fwd = {}, {}, []
            st = dict(pin=False, dirty=False, cnt=0, started=False, left=sum(e[0] == 'step' for e in events))

            def lhs(n):
                if st['pin']:
                    st['pin'] = False
                    return big[n + z]
                if n not in val:
                    val[n] = big[n]
                return val[n]

            def checkpoint():
                for (t, a), y in acc.items():
                    n = acc_at[t, a // 8] + 2 * (a % 8)
                    big[n:n + 2] = y.reshape(2, 8, 128)

            def two(n):
                return slice(2 * n, 2 * n + 2)

            def put(n, r, rs=slice(0, 8)):
                fwd.append((st['cnt'], n, r, rs))

            def flush(upto, pin=False):
                while fwd and fwd[0][0] <= upto:
                    _, n, r, rs = fwd.pop(0)
                    pbuf[z if pin else 0, rs, cols(n)] = r[rs]
                    if pin and st['left'] <= opts.get('vpin', 72):
                        vu[NP - 1][z, 2] = pltpu.bitcast(r, u32)
                    pin = False

            def get(n, rs=slice(0, 8)):
                flush(max([f[0] for f in fwd if f[1] == n], default=-1))
                return pbuf[0, rs, cols(n)]

            def ptile(t, k):
                return cols(sp[t] * KP + k // SG)

            def prow(t, odd, k):
                r = 2 * (k % SG) + odd
                return pbuf[0, r:r + 1, ptile(t - (t + odd == 0), k)]

            def q_fin(t, i, y, coef):
                y = (y + big[Q0 + 3 * t + i]) * coef
                big[QP + 3 * t + i] = (y + pltpu.roll(y, 4, 0)) * cst[i]

            def t_qraw(t, i):
                q_fin(t, i, _mm(xraw, _wtile(wqu[DT - 1][:, 3 * t + i])), coef)

            def t_q(t, i):
                put(QR + sq[t] * 3 + i, _mm(lhs(XL), _wtile(wqu[DT - 1][:, 3 * t + i])))

            def t_qk(t, j, k):
                put(SP + (3 * ss[t] + j) * KP + k // SG, _mm(lhs(QP + 3 * t + j), _wtile(ku[t][rows(j), k])),
                    two(k % SG))

            def t_or(t, j):
                a = big[acc_at[t, j]:acc_at[t, j] + 16].reshape(128, 128)
                if j == 1:
                    r = _mm(jnp.concatenate([lhs(WB + 2 * t), lhs(WB + 2 * t + 1)], axis=0), a, _NT)
                    put(OR + 2 * so[t, j] + 1, r[8:16])
                else:
                    r = _mm(lhs(WB + 2 * t + j // 2), a, _NT)
                put(OR + 2 * so[t, j], r[0:8])

            def t_pvx(t, j, k):
                p = val.pop(('px', t, j, k)) * lhs(WB + 2 * t + j // 2)
                put(XP + sx[t, j] * KP + k // 4, _mm(p, _wtile(vu[t][rows(j), k])), two(k % 4))

            def t_wo(units, n, c):
                t, j = units[n]
                r = _mm(lhs(OB + 3 * t + j), _wtile(wou[rows(3 * t + j), c]))
                if units == list(sw)[-1]:
                    put(WR + (RM + n) * DT + c, r)
                else:
                    put(WR + sw[units] * DT + c, r, two(n))

            def p_qfin(t, i):
                q_fin(t, i, get(QR + sq[t] * 3 + i), big[XL + 1])

            def over_tiles(op, y):
                y = op(y, pltpu.roll(y, 2, 0))
                return op(y, pltpu.roll(y, 4, 0))

            def p_sma(t, k0):
                n = SP + 3 * ss[max(t, 0)] * KP + k0 // SG
                sc = get(n) + get(n + KP)
                sc = sc + get(n + 2 * KP) if t >= 0 else sc
                pbuf[0, :, ptile(t, k0)] = sc
                m = jnp.maximum(sc, val['m']) if k0 else sc
                big[MB + 2 + 2 * t] = val['m'] = over_tiles(jnp.maximum, m) if k0 + SG == KT else m

            def p_smb(t, k0):
                pbuf[0, :, ptile(t, k0)] = p = jnp.exp2(pbuf[0, :, ptile(t, k0)] - val['m'])
                if t >= 0:
                    big[MB + 3 + 2 * t] = val['l'] = p + val['l'] if k0 else p
                if t >= 0 and k0 + SG == KT:
                    n, rs = ML + 2 * sl[wgrp[t][-1]], two(wgrp[t].index(t))
                    pbuf[0, rs, cols(n)] = val['m'][rs]
                    pbuf[0, rs, cols(n + 1)] = over_tiles(jnp.add, val['l'])[rs]

            def p_wld(t):
                val['ml', t] = [pbuf[0, 0:2 * len(wgrp[t]), cols(ML + 2 * sl[t] + n)] for n in range(2)]

            def p_w(t):
                m, l = val['ml', t]
                e = jnp.exp2(m - jnp.max(m, axis=1, keepdims=True))
                w = e / jnp.sum(e * l, axis=1, keepdims=True)
                for h in range(2 * len(wgrp[t])):
                    big[WB + 2 * wgrp[t][0] + h] = jnp.broadcast_to(w[h:h + 1], (8, 128))

            def p_ofin(t, j):
                r = get(OR + 2 * so[t, j])
                r = jnp.where(left(), r, get(OR + 2 * so[t, j] + 1)) if j == 1 else r
                big[OB + 3 * t + j] = r + big[OB + 3 * t + j] if (t, j) in nx else r

            def p_xsum(t, j):
                ys = [get(XP + sx[t, j] * KP + u) for u in range(nx[t, j] // 4)]
                big[OB + 3 * t + j] = over_tiles(jnp.add, _tree(jnp.add, ys))

            def p_wacc(units, c):
                if units == list(sw)[-1]:
                    rs = [get(WR + (RM + n) * DT + c) for n in range(len(units))]
                    big[XA + c] = _tree(jnp.add, rs + [over_tiles(jnp.add, big[XA + c])])
                elif units == list(sw)[0]:
                    assert len(units) == 4
                    big[XA + c] = get(WR + sw[units] * DT + c)
                else:
                    rs = slice(0, 2 * len(units))
                    big[XA + c, rs] = big[XA + c, rs] + get(WR + sw[units] * DT + c, rs)

            fns = {'qraw': t_qraw, 'q': t_q, 'qk': t_qk, 'or': t_or, 'pvx': t_pvx, 'wo': t_wo, 'qfin': p_qfin,
                   'sma': p_sma, 'smb': p_smb, 'wld': p_wld, 'w': p_w, 'ofin': p_ofin, 'xsum': p_xsum, 'wacc': p_wacc}
            tiles = [e for e in events if e[0] == 'tile' and e[1] != 'gap']
            for e in events:
                if e[0] == 'step':
                    _, t, a0, k = e
                    k0 = nx.get((t, a0 // 8), 0)
                    for a in range(a0, a0 + AB):
                        n = k + SKEW * (a - a0)
                        kk = k0 + (n - k0) % (KT - k0)
                        if ('p', t, a0, n) not in val:
                            val['p', t, a0, n] = prow(t, int(a0 >= AP // 2), kk)
                        if (t, a) in wide:
                            y = jnp.concatenate([pltpu.bitcast(vu[t][a, kk], f32),
                                                 big[WD + wide.index((t, a)) * KT + kk]])
                        elif (t, a) in late:
                            c, u = late[t, a]
                            y = pltpu.bitcast(jnp.concatenate([vu[t][a, kk], wqu[c][late_at(u, kk)]]), f32)
                        else:
                            y = pltpu.bitcast(vu[t][a, kk], bf16).astype(f32)
                        y = y * val['p', t, a0, n]
                        acc[t, a] = acc[t, a] + y if (t, a) in acc else y
                    st.update(dirty=True, started=True, left=st['left'] - 1)
                    if k == KT - 1:
                        checkpoint()
                        acc.clear()
                elif e[0] == 'piece':
                    fns[e[1]](*e[2:])
                elif e[1] == 'gap':
                    st['cnt'] += 4
                else:
                    pinned = st['cnt'] % 4 == opts.get('ph', 0) and st['left'] > 0
                    if pinned and st['dirty']:
                        checkpoint()
                    st.update(pin=pinned and st['started'], dirty=st['dirty'] and not pinned)
                    fns[e[1]](*e[2:])
                    st['pin'] = False
                    tiles.pop(0)
                    for u in tiles[:opts.get('pf', 4)]:
                        if u[1] == 'pvx' and ('px',) + u[2:] not in val:
                            val[('px',) + u[2:]] = prow(u[2], u[3] // 2, u[4])
                    if pinned:
                        flush(st['cnt'] - 4 * FD + 3, pin=st['started'])
                    st['cnt'] += 1
            assert not fwd
            x = xres[...] + jnp.concatenate([big[XA + c] for c in range(DT)], axis=1)
            y, hs = mlp_hidden(x)
            out = [(x + y)[:, cols(c)] for c in range(DT)]
            part = [None] * DT
            hb = [jnp.concatenate([hs[n]] * 16, axis=0).T for n in range(NV)]
            for n0 in range(0, NV, 3):
                for a in range(8):
                    for n in range(n0, min(n0 + 3, NV)):
                        for c in range(DT):
                            u = pltpu.bitcast(w4u[c][rows(8 * n + a)], bf16).astype(f32) * hb[n][16 * a:16 * a + 16]
                            part[c] = u if part[c] is None else part[c] + u
            for n in range(NV, FT):
                out = [out[c] + _mm(hs[n], w4_tile(n, c)) for c in range(DT)]
            out = [out[c] + jnp.sum(part[c], axis=0, keepdims=True) for c in range(DT)]
            o_ref[...] = jnp.concatenate(out, axis=1)[0:1].astype(o_ref.dtype)

        def body(it, carry):
            pl.when(it == 0)(lambda: layer1(it >> 4) if not opts.get('skip1') else None)
            pl.when(it == 1)(lambda: layer2(it >> 4))
            return carry

        lax.fori_loop(0, 2, body, 0)

    def V(*s, dt=f32):
        return pltpu.VMEM(s, dt)

    out = pl.pallas_call(
        kernel,
        out_shape=jax.ShapeDtypeStruct((1, D), A_x.dtype),
        in_specs=[pl.BlockSpec(memory_space=pl.ANY)] * 7,
        out_specs=pl.BlockSpec(memory_space=pltpu.VMEM),
        scratch_shapes=(
            [V(AP, KT, 16, 128, dt=bf16)] * (2 * NP)
            + [V(F, 128, dt=bf16)] * DT + [V(8, 3 * NP, 16, 128, dt=bf16)] * DT
            + [V(AP * NP, DT, 16, 128, dt=bf16), V(D, F, dt=bf16),
               V(1, 8, -(-NPB // 4) * 512), V(4, 8, 128), V(-(-NBIG // 4) * 4, 8, 128),
               V(FT, 8, 128), V(8, D), V(1, D, dt=bf16),
               pltpu.SemaphoreType.DMA((2 * NP + 3 + DT,))]),
        compiler_params=pltpu.CompilerParams(
            vmem_limit_bytes=int(opts.get('vmem', 128) * 1024 * 1024),
            disable_semaphore_checks=True, disable_bounds_checks=True),
        name='fused_decode_layers',
    )(A_x.reshape(1, D), _cache_view(A_k_cache), _cache_view(A_v_cache),
      _weight_view(A_wq), _weight_view(A_wo), B_w3, B_w4)
    return out.reshape(B, S, D)


@jax.jit
def pallas_interleave_layers__sliding_block_cached__mixer_s_mlp__decode_kernel(
    A_x: jax.Array,
    A_k_cache: jax.Array,
    A_v_cache: jax.Array,
    A_wq: jax.Array,
    A_wo: jax.Array,
    B_x: jax.Array,
    B_w1: jax.Array,
    B_w2: jax.Array,
    B_w3: jax.Array,
    B_w4: jax.Array,
):
    return _run(_OPTS, A_x, A_k_cache, A_v_cache, A_wq, A_wo, B_w3, B_w4)
```

```python
import jax
import jax.numpy as jnp
from jax import lax
import jax.experimental.pallas as pl
import jax.experimental.pallas.tpu as pltpu

f32, bf16, u32, i32 = jnp.float32, jnp.bfloat16, jnp.uint32, jnp.int32
_EPS = 1e-5
_LOG2E = 1.4426950408889634
_NN = (((1,), (0,)), ((), ()))
_NT = (((1,), (1,)), ((), ()))

_OPTS = dict(
    xunits=[(5, 0, 32), (7, 2, 32), (9, 2, 32), (11, 0, 32), (13, 2, 8)],
    vunits=[(14, 2), (15, 0), (15, 1), (15, 2)], vlead=16,
    nwide=90, nlate=[10, 10, 9, 0],
    wlast=[3, 7, 11, 13, 15], qlead=2.0, keep=8, AD=60, LAT=205, LAT0=165, q2at=20, vpin=36)


def _stats(x):
    m = jnp.mean(x, axis=-1, keepdims=True)
    xc = x - m
    v = jnp.mean(xc * xc, axis=-1, keepdims=True)
    return m, xc, lax.rsqrt(v + _EPS)


def _tree(op, xs):
    xs = list(xs)
    while len(xs) > 1:
        nxt = [op(xs[i], xs[i + 1]) for i in range(0, len(xs) - 1, 2)]
        if len(xs) % 2:
            nxt.append(xs[-1])
        xs = nxt
    return xs[0]


def _wtile(u):
    return pltpu.bitcast(u.reshape(u.shape[0] * 8, 128), bf16)


def _mm(lhs, w, dims=_NN):
    return lax.dot_general(lhs, w, dims, preferred_element_type=f32)


def _cache_view(c):
    _, H, Sk, Dh = c.shape
    c = c.reshape(H, Sk // 128, 128, Dh // 16, 2, 8)
    c = jnp.transpose(c, (0, 3, 4, 1, 5, 2))
    return c.reshape(H * Dh // 16, 2, Sk // 128, 8, 128)


def _weight_view(w):
    R, N = w.shape
    w = w.reshape(R // 16, 2, 8, N // 128, 128)
    return jnp.transpose(w, (0, 1, 3, 2, 4))


def _schedule(NP, KT, DT, AP, AB, SG, xunits, qlead, keep, LAT=205, LAT0=165, LEAD=32, WD=140, WL=400, AD=160,
              vcost=5.95, pstride=2, nraw=8, q2at=40, ph=0, wide=(), wk=(8, 20), cmaj=4, wlast=(), vunits=(), **_):
    xs = {u[:2]: u[2] for u in xunits}
    grp = [(t, a) for t in range(NP) for a in range(0, AP, AB)]
    grp[-2:] = grp[:-3:-1]
    steps = [(t, a, k) for t, a in grp for k in range(xs.get((t, a // 8), 0), KT)]
    first_step = {}
    for i, s in enumerate(steps):
        first_step.setdefault(s[0], i)
    main = [('qraw', t, i) for t in range(nraw) for i in range(3)]
    for t in range(NP):
        qk = [('qk', t, j, k) for j in range(3) for k in range(KT)]
        main += qk[:q2at] + [('q', t + 1, i) for i in range(3) if nraw <= t + 1 < NP] + qk[q2at:]
    done = {('q', t): 3 for t in range(nraw)}
    or_left = [(t, j) for t in range(NP) for j in range(3) if xs.get((t, j), 0) < KT]
    or_left = [u for u in or_left if u not in vunits]
    wo_left = [(t, j) for t in range(NP) for j in range(3) if (t, j) not in vunits]
    px_left = list(xs)
    ev, pend, wait, cur, src = [], [], [], [], {}
    s = dict(tm=0.0, tv=0.0, i=0, mi=0, qk=0)

    def sm(t):
        return ([(('sma', t, k), 3 + 4 * (k == KT - SG), None, 0) for k in range(0, KT, SG)]
                + [(('smb', t, k), 3 + 4 * (k == KT - SG), ('p', t), SG) for k in range(0, KT, SG)])

    def g_wo(n):
        wo = tuple(u for u in wo_left if done.get(('o',) + u, 0) >= 1)[:4]
        if len(wo_left) > cmaj:
            wo = wo[:len(wo_left) - cmaj]
        if len(wo) < n:
            return None
        for u in wo:
            wo_left.remove(u)
        g = [(('wo', wo, n, c), 8, []) for n in range(len(wo)) for c in range(DT)]
        if not wo_left and cmaj:
            g.sort(key=lambda x: x[0][3])
        g[-1] = (g[-1][0], 8, [(('wacc', wo, c), 1, None, 0) for c in range(DT)])
        return g

    def g_or(n, last):
        rd = [u for u in or_left if done.get(('acc',) + u, 0) >= 8 // AB and done.get(('w', min(t for t in wlast if t >= u[0])), 0)
              and (last or done[('acct',) + u] + AD <= s['tv'])
              and done.get(('y',) + u, 0) >= xs.get(u, 0)][:4]
        if len(rd) < n:
            return None
        for u in rd:
            or_left.remove(u)
        return [(('gap',), 8 * len(rd), [])] + [(('or',) + u, 8, [(('ofin',) + u, 1, ('o',) + u, 1)]) for u in rd]

    def g_px():
        rd = [u for u in px_left if done.get(('w', min(t for t in wlast if t >= u[0])), 0)]
        if not rd:
            return None
        px_left.remove(rd[0])
        n = xs[rd[0]]
        g = [(('pvx',) + rd[0] + (k,), 8, []) for k in range(n)]
        g[-1] = (g[-1][0], 8, [(('xsum',) + rd[0], n // 4 + 3, ('o' if n == KT else 'y',) + rd[0], n)])
        return g

    def pick():
        last, endgame, nxt = s['i'] >= len(steps), s['mi'] >= len(main), s['qk']
        if last:
            return g_or(1, True) or g_px() or g_wo(len(wo_left) if 0 < len(wo_left) <= cmaj else 1)
        if endgame:
            return (g_or(min(4, len(or_left)) if vunits and or_left else 4, False) or g_px() or g_wo(4)
                    or (g_wo(1) if len(wo_left) > cmaj else None))
        rem = sum(8 for m in main[s['mi']:s['mi'] + 200] if m[0] != 'qk' or m[1] == nxt)
        if (first_step[nxt] - s['i']) * vcost - rem > qlead * 500:
            g = (g_wo(4) if len(wo_left) > keep else None) or g_or(4, False) or g_px()
            if g:
                return g
        m = main[s['mi']]
        if m[0] == 'qk' and done.get(('q', m[1]), 0) < 3:
            return None
        s['mi'] += 1
        pcs = []
        if m[0] == 'q':
            pcs = [(('qfin',) + m[1:], 5, ('q', m[1]), 1)]
        if m[0] == 'qk' and (m[2] == 2 or m[1:3] == (0, 1)) and m[3] % SG == SG - 1:
            t = m[1] if m[2] == 2 else -1
            pcs = [sm(t)[m[3] // SG]] + (sm(t)[KT // SG:] if m[3] == KT - 1 else [])
        return [(m, 8, pcs)]

    def later(t, pcs):
        wait.append((t, pcs))
        wait.sort(key=lambda w: w[0])

    def piece():
        a, cv, e, inc = pend.pop(0)
        if a[0] == 'wld' and s['i'] < len(steps) and not wk[0] <= steps[s['i']][2] <= wk[1]:
            return later(s['tv'] + 30, [(a, cv, e, inc)])
        ev.append(('piece',) + a)
        s['tv'] += cv / 4
        if e is not None:
            done[e] = done.get(e, 0) + inc
        if a[0] == 'smb' and a[2] == KT - SG and a[1] in wlast:
            later(s['tv'] + WD, [(('wld', a[1]), 0, ('wld', a[1]), 1)])
        if a[0] == 'wld':
            later(s['tv'] + WL, [(('w', a[1]), 26, ('w', a[1]), 1)])

    def urgent(p):
        return p[2] is not None and p[2][0] != 'p'

    while True:
        while wait and wait[0][0] <= s['tv']:
            pcs = wait.pop(0)[1]
            pend[:] = [p for p in pcs if urgent(p)] + pend + [p for p in pcs if not urgent(p)]
        i = s['i']
        more = i < len(steps)
        blocked = not more or done.get(('p', steps[i][0] - (i < AP // 2 // AB * KT)), 0) < min(KT, steps[i][2] + 6)
        if not more and or_left:
            cur = (g_or(1, True) or []) + cur
        if not cur and (s['tm'] + LEAD <= s['tv'] or blocked):
            cur = pick() or []
        if not more and not pend and not wait and not cur:
            break
        if cur and (s['tm'] + LEAD <= s['tv']
                    or (blocked and not pend and (not wait or s['tm'] + LEAD <= wait[0][0]))):
            a, cm, pcs = cur.pop(0)
            ev.append(('tile',) + a)
            s['tm'] = max(s['tm'], s['tv'] - LEAD - 8) + cm
            s['tv'] += 0.25 * (a[0] == 'pvx')
            s['qk'] += a[0] == 'qk' and a[2:] == (2, KT - 1)
            src.update({('piece',) + pc[0]: ev[-1] for pc in pcs})
            if pcs:
                later(s['tm'] + (LAT if 0 < i < len(steps) else LAT0), pcs)
        elif blocked and pend:
            piece()
        elif blocked:
            s['tv'] = max(s['tv'], wait[0][0])
        else:
            if pend and (i % pstride == 0 or urgent(pend[0])):
                piece()
            t, a, k = steps[i]
            ev.append(('step', t, a, k))
            if k == KT - 1:
                done['acc', t, a // 8] = done.get(('acc', t, a // 8), 0) + 1
                done['acct', t, a // 8] = s['tv']
            s['tv'] += vcost - 0.5 * sum((t, b) in wide for b in range(a, a + AB))
            s['i'] += 1
    assert not or_left and not wo_left and not px_left

    out, cur, cnt = [], [], 0
    for e in ev + [None]:
        if e is None or (e[0] == 'tile' and e[1] != 'gap' and cnt % 4 == ph):
            if any(x[0] == 'step' for x in cur) and len(cur) < 32 and not any(src.get(x) in cur for x in cur):
                cur = cur[:1] + [x for x in cur[1:] if x[0] == 'piece'] + [x for x in cur[1:] if x[0] != 'piece']
            out += cur
            cur = []
        if e is not None:
            cur.append(e)
            cnt += (4 if e[1] == 'gap' else 1) * (e[0] == 'tile')
    pos = {e: n for n, e in enumerate(out)}
    assert all(pos[a] < pos[b] for b, a in src.items())
    return out


def _slots(events, key):
    first, last = {}, {}
    for n, e in enumerate(events):
        k = key(e)
        if k is not None:
            first.setdefault(k, n)
            last[k] = n
    slot, busy = {}, []
    for k in first:
        free = [i for i, u in enumerate(busy) if u < first[k]]
        slot[k] = free[0] if free else len(busy)
        busy[slot[k]:slot[k] + 1] = [last[k]]
    return slot, len(busy)


def _run(opts, A_x, A_k_cache, A_v_cache, A_wq, A_wo, B_w3, B_w4):
    B, S, D = A_x.shape
    _, H, Sk, Dh = A_k_cache.shape
    F = B_w3.shape[1]
    W = min(4096, max(256, Sk // 4))
    assert (B, S, H, Dh, W) == (1, 1, 32, 192, 4096) and D % 128 == 0 and F % 128 == 0
    AP = Dh // 8
    KT = W // 128
    NP = H // 2
    DT, FT = D // 128, F // 128
    AB, SG, FD = 4, 4, opts.get('fd', 5)
    KP = KT // SG
    SKEW = opts.get('skew', 1)
    cexp = (Dh ** -0.5) * _LOG2E
    nx = {u[:2]: u[2] for u in opts['xunits']}
    xunits, vunits = list(nx), opts.get('vunits', [])
    wide = [(t, a) for t in range(NP) for a in range(0, AP, AB) if (t, a // 8) not in xunits + [(NP - 1, 2)]]
    drop = [g for n, g in enumerate(wide) if n % 3][:max(0, len(wide) - opts['nwide'])]
    wide = [g for g in wide if g not in drop] + [(t, a + 2) for t, a in wide[::-1]][:max(0, opts['nwide'] - len(wide))]
    late = [(t, a) for b in (0, 2) for t in range(NP - 1, 0, -1) for a in range(b, AP, AB)
            if (t, a // 8) not in xunits + [(NP - 1, 2)] and (t, a) not in wide]
    nlate = opts['nlate']
    late = {g: (c, n) for c in range(DT - 1) for n, g in enumerate(late[sum(nlate[:c]):sum(nlate[:c + 1])])}
    events = _schedule(NP, KT, DT, AP, AB, SG, wide=wide + list(late), **opts)
    sp, RP = _slots(events, lambda e: e[1] - (e[1] == 0 and e[2] < AP // 2) if e[0] == 'step'
                    else e[2] if e[1] in ('sma', 'smb', 'pvx') else None)
    ss, RS = _slots(events, lambda e: max(e[2], 0) if e[1] in ('qk', 'sma') else None)
    sq, RQ = _slots(events, lambda e: e[2] if e[1] in ('q', 'qfin') else None)
    sx, RX = _slots(events, lambda e: e[2:4] if e[1] in ('pvx', 'xsum') else None)
    sw, RM = _slots(events, lambda e: e[2] if e[1] in ('wo', 'wacc') else None)
    so, RO = _slots(events, lambda e: e[2:4] if e[1] in ('or', 'ofin') else None)
    wlast = opts['wlast']
    wgrp = {t: [u for u in range(NP) if max([-1] + [v for v in wlast if v < t]) < u <= min(v for v in wlast if v >= t)]
            for t in range(NP)}
    sl, RL = _slots(events, lambda e: wgrp[e[2]][-1] if e[1] in ('smb', 'wld') and e[2] >= 0 else None)
    assert _slots(events, lambda e: e[2] if e[1] in ('sma', 'smb') else None)[1] == 1
    sizes = [3 * NP, 3 * NP, 2 * NP, 2, DT, 2 * NP + 3, KT, KT * len(wide)]
    QP, Q0, WB, XL, XA, MB, AL, WD, NBIG = [sum(sizes[:n]) for n in range(len(sizes) + 1)]
    OB = Q0
    free, acc_at = [AL, AL + 16], {}
    for e in events:
        if e[0] == 'step' and (e[1], e[2] // 8) not in acc_at:
            acc_at[e[1], e[2] // 8] = free.pop(0)
        if e[0] == 'step' and e[3] == KT - 1:
            free += [WD + KT * wide.index((e[1], a)) + n for a in range(e[2], e[2] + AB) if (e[1], a) in wide
                     for n in (0, 16)]
    sizes = [RP * KP, 3 * RS * KP, RX * KP, 3 * RQ, DT * (RM + 4), 2 * RO, 2 * RL, 2]
    _, SP, XP, QR, WR, OR, ML, WL, NPB = [sum(sizes[:n]) for n in range(len(sizes) + 1)]
    NV, NQ = opts.get('nv', 4), opts.get('nq', 8)
    assert nlate[DT - 2] == 0 and 2 * nlate[DT - 3] <= 11 + (3 * NP - NQ) // 4
    if opts.get('verbose'):
        print('RP RS RQ RX RM', RP, RS, RQ, RX, RM, 'free tiles', (int(13.25 * 256) - NBIG - NPB))
    order1 = sorted(range(NP), key=lambda t: all(u[0] != t for u in xunits))

    def kernel(x_hbm, k_hbm, v_hbm, wq_hbm, wo_hbm, w3_hbm, w4_hbm, o_ref, *scratch):
        k_bufs, v_bufs, scratch = scratch[:NP], scratch[NP:2 * NP], scratch[2 * NP:]
        w4_bufs, wq_bufs, scratch = scratch[:DT], scratch[DT:2 * DT], scratch[2 * DT:]
        wo_buf, w3_buf, pbuf, cst, big, hbuf, xres, x_buf, sems = scratch
        t0 = (Sk - W) // 128

        def kv_cp(kind, t):
            src, dst = (k_hbm, k_bufs[t]) if kind == 0 else (v_hbm, v_bufs[t])
            return [pltpu.make_async_copy(src.at[pl.ds(AP * t, AP), a, pl.ds(t0, KT)],
                                          dst.at[:, :, pl.ds(8 * a, 8), :], sems.at[2 * t + kind])
                    for a in range(2)]

        def w_cp(src, dst, n, sem):
            rows = src.shape[0] // n
            return [pltpu.make_async_copy(src.at[pl.ds(i * rows, rows), a],
                                          dst.at[pl.ds(i * rows, rows), :, pl.ds(8 * a, 8), :], sem)
                    for i in range(n) for a in range(2)]

        def wq_cp():
            cps = [cp for j in range(DT) for cp in w_cp(wq_hbm.at[pl.ds(8 * j, 8)], wq_bufs[j], 1, sems.at[2 * NP])]
            return cps[:1] + [pltpu.make_async_copy(x_hbm, x_buf, sems.at[2 * NP])] + cps[1:]

        def wo_cp():
            return w_cp(wo_hbm, wo_buf, 8, sems.at[2 * NP + 1])

        def w3_cp():
            return [pltpu.make_async_copy(w3_hbm, w3_buf, sems.at[2 * NP + 2])]

        def w4_cp(c):
            return [pltpu.make_async_copy(w4_hbm.at[:, pl.ds(128 * c, 128)], w4_bufs[c], sems.at[2 * NP + 3 + c])]

        def wait(cps):
            for cp in cps:
                cp.wait()

        cps = wq_cp()
        for t in order1:
            cps += kv_cp(0, t) + kv_cp(1, t) + (wo_cp() if t == order1[0] else [])
        for cp in cps + w3_cp() + [cp for c in range(DT) for cp in w4_cp(c)]:
            cp.start()

        ku = [r.bitcast(u32) for r in k_bufs]
        vu = [r.bitcast(u32) for r in v_bufs]
        wqu = [r.bitcast(u32) for r in wq_bufs]
        wou = wo_buf.bitcast(u32)
        w4u = [r.bitcast(u32) for r in w4_bufs]

        def top(n):
            return lax.broadcasted_iota(i32, (8, n), 0) < 4

        def left():
            return lax.broadcasted_iota(i32, (8, 128), 1) < 64

        def cols(n):
            return slice(128 * n, 128 * (n + 1))

        def rows(j):
            return slice(8 * j, 8 * j + 8)

        def masks():
            even = lax.broadcasted_iota(i32, (8, 128), 0) % 2 == 0
            return [even, even == left(), jnp.logical_not(even)]

        def mlp_hidden(x):
            lhs = jnp.where(top(D), x, 1.0)
            m1 = jnp.mean(x, axis=-1, keepdims=True)
            xc = x - m1
            v1 = jnp.mean(xc * xc, axis=-1, keepdims=True)
            r1 = lax.rsqrt(v1 + _EPS)
            y = xc * r1
            m2 = jnp.mean(xc, axis=-1, keepdims=True) * r1
            r2 = lax.rsqrt(v1 * r1 * r1 - m2 * m2 + _EPS)
            coef = jnp.where(top(128), r1 * r2, -(r2 * (r1 * m1 + m2)))
            hs, NF = [], opts.get('nf', 4)
            first = {(n, j): _mm(lhs[:, cols(j)], w3_buf[cols(j), cols(n)]) for j in range(DT) for n in range(NF)}
            for n in range(FT):
                u = _tree(jnp.add, [first[n, j] if n < NF else _mm(lhs[:, cols(j)], w3_buf[cols(j), cols(n)])
                                    for j in range(DT)]) * coef
                hs.append(jax.nn.gelu(u + pltpu.roll(u, 4, 0), approximate=True))
            return y, hs

        def w4_tile(n, c):
            return pltpu.bitcast(w4u[c][64 * n:64 * (n + 1)], bf16)

        def late_at(n, k):
            return ((n * KT + k + 2) % (24 * NP)) // (3 * NP), (n * KT + k + 2) % (3 * NP)

        def unpack_late(c, n0, n1, after=None):
            todo = [(g, n, k) for g, (cc, n) in late.items() if cc == c for k in range(KT)][16 * n0:16 * n1]
            if todo and after is not None:
                wqu[c][after[0], 0] = pltpu.bitcast(after[1], u32)
            for (t, a), n, k in todo:
                y = pltpu.bitcast(pltpu.bitcast(vu[t][a, k], bf16).astype(f32), u32)
                wqu[c][late_at(n, k)] = y[8:16]
                vu[t][a, k] = y[0:8]

        def layer1(z):
            for u, mask in enumerate(masks()):
                cst[u] = jnp.where(mask, cexp, 0.0).astype(f32)
            wait(wq_cp())
            x = jnp.broadcast_to(x_buf[...].astype(f32), (8, D))
            _, xc, r = _stats(x)
            xn = xc * r

            def q_body(t, c):
                for i in range(3):
                    q = _tree(jnp.add, [_mm(xn[:, cols(j)], _wtile(wqu[j][:, 3 * t + i])) for j in range(DT)])
                    big[QP + 3 * t + i] = q * cst[i]
                return c
            lax.fori_loop(0, NP, q_body, 0)

            att = [jnp.zeros((8, 128), f32)] * DT
            for t in order1:
                def s_body(k, c, t=t, q=[big[QP + 3 * t + j] for j in range(3)]):
                    big[AL + k] = _tree(jnp.add, [_mm(q[j], _wtile(ku[t][rows(j), k])) for j in range(3)])
                    return c

                def o_body(k, o, t=t):
                    return [o[j] + _mm(big[AL + k], _wtile(vu[t][rows(j), k]), _NT) for j in range(3)]

                wait(kv_cp(0, t))
                lax.fori_loop(0, KT, s_body, 0, unroll=8)
                sc = big[AL:AL + KT]
                p = jnp.exp2(sc - jnp.max(jnp.max(sc, axis=0), axis=1, keepdims=True))
                big[AL:AL + KT] = p
                inv = 1.0 / jnp.sum(jnp.sum(p, axis=0), axis=1, keepdims=True)
                wait(kv_cp(1, t) + (wo_cp() if t == order1[0] else []))
                o = lax.fori_loop(0, KT, o_body, [jnp.zeros((8, 128), f32)] * 3, unroll=8)
                o = [jnp.where(mask, o[j] * inv, 0.0) for j, mask in enumerate(masks())]
                att = [att[c] + _tree(jnp.add, [_mm(o[j], _wtile(wou[rows(3 * t + j), c])) for j in range(3)])
                       for c in range(DT)]
                for j in [j for tt, j in xunits if tt == t]:
                    def t_body(k, c, t=t, j=j):
                        w = _wtile(vu[t][rows(j), k]).astype(f32).T.astype(bf16)
                        vu[t][rows(j), k] = pltpu.bitcast(w, u32).reshape(8, 8, 128)
                        return c
                    lax.fori_loop(0, nx[t, j], t_body, 0, unroll=4)
                for n, a in [(n, a) for n, (tt, a) in enumerate(wide) if tt == t]:
                    y = _wtile(vu[t][a]).astype(f32).reshape(KT, 16, 128)
                    big[WD + n * KT:WD + (n + 1) * KT] = y[:, 8:16]
                    vu[t][a] = pltpu.bitcast(y[:, 0:8], u32)
            att = jnp.concatenate(att, axis=1)
            x = x + (att + pltpu.roll(att, 1, 0))
            wait(w3_cp())
            y, hs = mlp_hidden(x)
            xres[...] = x + y
            for n in range(FT):
                hbuf[n] = hs[n]
            for c in range(DT - 1):
                wait(w4_cp(c))
                unpack_late(c - 1, 0, 7)
                xc = xres[:, cols(c)] + _tree(jnp.add, [_mm(hbuf[n], w4_tile(n, c)) for n in range(FT)])
                xres[:, cols(c)] = xc
                if c == DT - 2:
                    cst[3] = jnp.broadcast_to(jnp.mean(xres[:, :D - 128], axis=-1, keepdims=True), (8, 128))
                xc = jnp.where(top(128), xc, 1.0)
                unpack_late(c - 1, 7, 11, (z, xc))
                for n in range(3 * NP - (NQ if c == DT - 2 else 0)):
                    r = _mm(xc, _wtile(wqu[c][:, n]))
                    big[Q0 + n] = big[Q0 + n] + r if c else r
                    if n % 4 == 0:
                        unpack_late(c - 1, 11 + n // 4, 12 + n // 4, (z, r))

        def layer2(z):
            wait(w4_cp(DT - 1))
            if opts.get('skip2'):
                keep = big[Q0 + z] + sum(pltpu.bitcast(r[z, 1], f32) for r in wqu + vu)
                o_ref[...] = (xres[0:1, :] + jnp.concatenate([keep[0:1]] * DT, axis=1)).astype(o_ref.dtype)
                return
            xc = xres[:, cols(DT - 1)] + _tree(jnp.add, [_mm(hbuf[n], w4_tile(n, DT - 1)) for n in range(FT)])
            for n in range(3 * NP - NQ, 3 * NP):
                xp = jnp.where(top(128), xres[:, cols(DT - 2)], 1.0)
                big[Q0 + n] = big[Q0 + n] + _mm(xp, _wtile(wqu[DT - 2][:, n]))
            xres[:, cols(DT - 1)] = xc
            d = xres[...] - jnp.concatenate([cst[3]] * DT, axis=1)
            md = jnp.mean(d, axis=-1, keepdims=True)
            r = lax.rsqrt(jnp.mean(d * d, axis=-1, keepdims=True) - md * md + _EPS)
            big[XL] = xraw = jnp.where(top(128), xc, 1.0)
            big[XL + 1] = coef = jnp.where(top(128), r, -(r * (cst[3] + md)))
            acc, val, fwd = {}, {}, []
            st = dict(pin=False, dirty=False, cnt=0, started=False, left=sum(e[0] == 'step' for e in events))

            def lhs(n):
                if st['pin']:
                    st['pin'] = False
                    return big[n + z]
                if n not in val:
                    val[n] = big[n]
                return val[n]

            def checkpoint():
                for (t, a), y in acc.items():
                    n = acc_at[t, a // 8] + 2 * (a % 8)
                    big[n:n + 2] = y.reshape(2, 8, 128)

            def two(n):
                return slice(2 * n, 2 * n + 2)

            def put(n, r, rs=slice(0, 8)):
                fwd.append((st['cnt'], n, r, rs))

            def flush(upto, pin=False):
                while fwd and fwd[0][0] <= upto:
                    _, n, r, rs = fwd.pop(0)
                    pbuf[z if pin else 0, rs, cols(n)] = r[rs]
                    if pin and st['left'] <= opts.get('vpin', 72):
                        vu[NP - 1][z, 2] = pltpu.bitcast(r, u32)
                    pin = False

            def get(n, rs=slice(0, 8)):
                flush(max([f[0] for f in fwd if f[1] == n], default=-1))
                return pbuf[0, rs, cols(n)]

            def ptile(t, k):
                return cols(sp[t] * KP + k // SG)

            def prow(t, odd, k):
                r = 2 * (k % SG) + odd
                return pbuf[0, r:r + 1, ptile(t - (t + odd == 0), k)]

            def q_fin(t, i, y, coef):
                y = (y + big[Q0 + 3 * t + i]) * coef
                big[QP + 3 * t + i] = (y + pltpu.roll(y, 4, 0)) * cst[i]

            def t_qraw(t, i):
                q_fin(t, i, _mm(xraw, _wtile(wqu[DT - 1][:, 3 * t + i])), coef)

            def t_q(t, i):
                put(QR + sq[t] * 3 + i, _mm(lhs(XL), _wtile(wqu[DT - 1][:, 3 * t + i])))

            def t_qk(t, j, k):
                put(SP + (3 * ss[t] + j) * KP + k // SG, _mm(lhs(QP + 3 * t + j), _wtile(ku[t][rows(j), k])),
                    two(k % SG))

            def t_or(t, j):
                a = big[acc_at[t, j]:acc_at[t, j] + 16].reshape(128, 128)
                if j == 1:
                    r = _mm(jnp.concatenate([lhs(WB + 2 * t), lhs(WB + 2 * t + 1)], axis=0), a, _NT)
                    put(OR + 2 * so[t, j] + 1, r[8:16])
                else:
                    r = _mm(lhs(WB + 2 * t + j // 2), a, _NT)
                put(OR + 2 * so[t, j], r[0:8])

            def t_pvx(t, j, k):
                p = val.pop(('px', t, j, k)) * lhs(WB + 2 * t + j // 2)
                put(XP + sx[t, j] * KP + k // 4, _mm(p, _wtile(vu[t][rows(j), k])), two(k % 4))

            def t_wo(units, n, c):
                t, j = units[n]
                r = _mm(lhs(OB + 3 * t + j), _wtile(wou[rows(3 * t + j), c]))
                if units == list(sw)[-1]:
                    put(WR + (RM + n) * DT + c, r)
                else:
                    put(WR + sw[units] * DT + c, r, two(n))

            def p_qfin(t, i):
                q_fin(t, i, get(QR + sq[t] * 3 + i), big[XL + 1])

            def over_tiles(op, y):
                y = op(y, pltpu.roll(y, 2, 0))
                return op(y, pltpu.roll(y, 4, 0))

            def p_sma(t, k0):
                n = SP + 3 * ss[max(t, 0)] * KP + k0 // SG
                sc = get(n) + get(n + KP)
                sc = sc + get(n + 2 * KP) if t >= 0 else sc
                pbuf[0, :, ptile(t, k0)] = sc
                m = jnp.maximum(sc, val['m']) if k0 else sc
                big[MB + 2 + 2 * t] = val['m'] = over_tiles(jnp.maximum, m) if k0 + SG == KT else m

            def p_smb(t, k0):
                pbuf[0, :, ptile(t, k0)] = p = jnp.exp2(pbuf[0, :, ptile(t, k0)] - val['m'])
                if t >= 0:
                    big[MB + 3 + 2 * t] = val['l'] = p + val['l'] if k0 else p
                if t >= 0 and k0 + SG == KT:
                    n, rs = ML + 2 * sl[wgrp[t][-1]], two(wgrp[t].index(t))
                    pbuf[0, rs, cols(n)] = val['m'][rs]
                    pbuf[0, rs, cols(n + 1)] = over_tiles(jnp.add, val['l'])[rs]

            def p_wld(t):
                val['ml', t] = [pbuf[0, 0:2 * len(wgrp[t]), cols(ML + 2 * sl[t] + n)] for n in range(2)]

            def p_w(t):
                m, l = val['ml', t]
                e = jnp.exp2(m - jnp.max(m, axis=1, keepdims=True))
                w = e / jnp.sum(e * l, axis=1, keepdims=True)
                for h in range(2 * len(wgrp[t])):
                    big[WB + 2 * wgrp[t][0] + h] = jnp.broadcast_to(w[h:h + 1], (8, 128))
                if t == NP - 1:
                    pbuf[0, 0:2 * len(wgrp[t]), cols(WL)] = w
                    st['wl'] = True

            def p_ofin(t, j):
                r = get(OR + 2 * so[t, j])
                r = jnp.where(left(), r, get(OR + 2 * so[t, j] + 1)) if j == 1 else r
                big[OB + 3 * t + j] = r + big[OB + 3 * t + j] if (t, j) in nx else r

            def p_xsum(t, j):
                ys = [get(XP + sx[t, j] * KP + u) for u in range(nx[t, j] // 4)]
                big[OB + 3 * t + j] = over_tiles(jnp.add, _tree(jnp.add, ys))

            def p_wacc(units, c):
                if units == list(sw)[-1]:
                    rs = [get(WR + (RM + n) * DT + c) for n in range(len(units))]
                    big[XA + c] = _tree(jnp.add, rs + [over_tiles(jnp.add, big[XA + c])])
                elif units == list(sw)[0]:
                    assert len(units) == 4
                    big[XA + c] = get(WR + sw[units] * DT + c)
                else:
                    rs = slice(0, 2 * len(units))
                    big[XA + c, rs] = big[XA + c, rs] + get(WR + sw[units] * DT + c, rs)

            fns = {'qraw': t_qraw, 'q': t_q, 'qk': t_qk, 'or': t_or, 'pvx': t_pvx, 'wo': t_wo, 'qfin': p_qfin,
                   'sma': p_sma, 'smb': p_smb, 'wld': p_wld, 'w': p_w, 'ofin': p_ofin, 'xsum': p_xsum, 'wacc': p_wacc}
            tiles = [e for e in events if e[0] == 'tile' and e[1] != 'gap']
            for e in events:
                if e[0] == 'step':
                    _, t, a0, k = e
                    k0 = nx.get((t, a0 // 8), 0)
                    for a in range(a0, a0 + AB):
                        n = k + SKEW * (a - a0)
                        kk = k0 + (n - k0) % (KT - k0)
                        if ('p', t, a0, n) not in val:
                            val['p', t, a0, n] = prow(t, int(a0 >= AP // 2), kk)
                        if (t, a) in wide:
                            y = jnp.concatenate([pltpu.bitcast(vu[t][a, kk], f32),
                                                 big[WD + wide.index((t, a)) * KT + kk]])
                        elif (t, a) in late:
                            c, u = late[t, a]
                            y = pltpu.bitcast(jnp.concatenate([vu[t][a, kk], wqu[c][late_at(u, kk)]]), f32)
                        else:
                            y = pltpu.bitcast(vu[t][a, kk], bf16).astype(f32)
                        y = y * val['p', t, a0, n]
                        acc[t, a] = acc[t, a] + y if (t, a) in acc else y
                    st.update(dirty=True, started=True, left=st['left'] - 1)
                    if st['left'] == opts.get('vlead', 24) and vunits:
                        assert st['wl']
                        val['wl'] = [pbuf[0, h:h + 1, cols(WL)] for h in range(2 * len(wgrp[NP - 1]))]
                    if k == KT - 1:
                        checkpoint()
                        acc.clear()
                elif e[0] == 'piece':
                    fns[e[1]](*e[2:])
                elif e[1] == 'gap':
                    st['cnt'] += 4
                else:
                    pinned = st['cnt'] % 4 == opts.get('ph', 0) and st['left'] > 0
                    if pinned and st['dirty']:
                        checkpoint()
                    st.update(pin=pinned and st['started'], dirty=st['dirty'] and not pinned)
                    fns[e[1]](*e[2:])
                    st['pin'] = False
                    tiles.pop(0)
                    for u in tiles[:opts.get('pf', 4)]:
                        if u[1] == 'pvx' and ('px',) + u[2:] not in val:
                            val[('px',) + u[2:]] = prow(u[2], u[3] // 2, u[4])
                    if pinned:
                        flush(st['cnt'] - 4 * FD + 3, pin=st['started'])
                    st['cnt'] += 1
            assert not fwd
            att = [big[XA + c] for c in range(DT)]
            part = [None] * DT
            for t, a0 in [e[1:3] for e in events if e[0] == 'step' and e[3] == KT - 1 and (e[1], e[2] // 8) in vunits]:
                for a in range(a0, a0 + AB):
                    n = acc_at[t, a // 8] + 2 * (a % 8)
                    o = jnp.sum(big[n:n + 2].reshape(16, 128) * val['wl'][2 * wgrp[NP - 1].index(t) + (a >= AP // 2)],
                                axis=1, keepdims=True)
                    for c in range(DT):
                        u = pltpu.bitcast(wou[AP * t + a, c], bf16).astype(f32) * o
                        part[c] = u if part[c] is None else part[c] + u
            if vunits:
                att = [att[c] + jnp.sum(part[c], axis=0, keepdims=True) for c in range(DT)]
            x = xres[...] + jnp.concatenate(att, axis=1)
            y, hs = mlp_hidden(x)
            out = [(x + y)[:, cols(c)] for c in range(DT)]
            part = [None] * DT
            hb = [jnp.concatenate([hs[n]] * 16, axis=0).T for n in range(NV)]
            for n0 in range(0, NV, 3):
                for a in range(8):
                    for n in range(n0, min(n0 + 3, NV)):
                        for c in range(DT):
                            u = pltpu.bitcast(w4u[c][rows(8 * n + a)], bf16).astype(f32) * hb[n][16 * a:16 * a + 16]
                            part[c] = u if part[c] is None else part[c] + u
            for n in range(NV, FT):
                out = [out[c] + _mm(hs[n], w4_tile(n, c)) for c in range(DT)]
            out = [out[c] + jnp.sum(part[c], axis=0, keepdims=True) for c in range(DT)]
            o_ref[...] = jnp.concatenate(out, axis=1)[0:1].astype(o_ref.dtype)

        def body(it, carry):
            pl.when(it == 0)(lambda: layer1(it >> 4) if not opts.get('skip1') else None)
            pl.when(it == 1)(lambda: layer2(it >> 4))
            return carry

        lax.fori_loop(0, 2, body, 0)

    def V(*s, dt=f32):
        return pltpu.VMEM(s, dt)

    out = pl.pallas_call(
        kernel,
        out_shape=jax.ShapeDtypeStruct((1, D), A_x.dtype),
        in_specs=[pl.BlockSpec(memory_space=pl.ANY)] * 7,
        out_specs=pl.BlockSpec(memory_space=pltpu.VMEM),
        scratch_shapes=(
            [V(AP, KT, 16, 128, dt=bf16)] * (2 * NP)
            + [V(F, 128, dt=bf16)] * DT + [V(8, 3 * NP, 16, 128, dt=bf16)] * DT
            + [V(AP * NP, DT, 16, 128, dt=bf16), V(D, F, dt=bf16),
               V(1, 8, -(-NPB // 4) * 512), V(4, 8, 128), V(-(-NBIG // 4) * 4, 8, 128),
               V(FT, 8, 128), V(8, D), V(1, D, dt=bf16),
               pltpu.SemaphoreType.DMA((2 * NP + 3 + DT,))]),
        compiler_params=pltpu.CompilerParams(
            vmem_limit_bytes=int(opts.get('vmem', 128) * 1024 * 1024),
            disable_semaphore_checks=True, disable_bounds_checks=True),
        name='fused_decode_layers',
    )(A_x.reshape(1, D), _cache_view(A_k_cache), _cache_view(A_v_cache),
      _weight_view(A_wq), _weight_view(A_wo), B_w3, B_w4)
    return out.reshape(B, S, D)


@jax.jit
def pallas_interleave_layers__sliding_block_cached__mixer_s_mlp__decode_kernel(
    A_x: jax.Array,
    A_k_cache: jax.Array,
    A_v_cache: jax.Array,
    A_wq: jax.Array,
    A_wo: jax.Array,
    B_x: jax.Array,
    B_w1: jax.Array,
    B_w2: jax.Array,
    B_w3: jax.Array,
    B_w4: jax.Array,
):
    return _run(_OPTS, A_x, A_k_cache, A_v_cache, A_wq, A_wo, B_w3, B_w4)
```

```python
import jax
import jax.numpy as jnp
from jax import lax
import jax.experimental.pallas as pl
import jax.experimental.pallas.tpu as pltpu

f32, bf16, u32, i32 = jnp.float32, jnp.bfloat16, jnp.uint32, jnp.int32
_EPS = 1e-5
_LOG2E = 1.4426950408889634
_NN = (((1,), (0,)), ((), ()))
_NT = (((1,), (1,)), ((), ()))

_OPTS = dict(
    xunits=[(5, 0, 32), (7, 2, 32), (9, 2, 32), (11, 0, 32), (13, 2, 8)],
    vunits=[(14, 2), (15, 0), (15, 1), (15, 2)], vlead=16,
    nwide=90, nlate=[10, 10, 9, 0],
    wlast=[3, 7, 11, 13, 15], qlead=2.0, keep=8, AD=60, LAT=205, LAT0=165, q2at=20)


def _stats(x):
    m = jnp.mean(x, axis=-1, keepdims=True)
    xc = x - m
    v = jnp.mean(xc * xc, axis=-1, keepdims=True)
    return m, xc, lax.rsqrt(v + _EPS)


def _tree(op, xs):
    xs = list(xs)
    while len(xs) > 1:
        nxt = [op(xs[i], xs[i + 1]) for i in range(0, len(xs) - 1, 2)]
        if len(xs) % 2:
            nxt.append(xs[-1])
        xs = nxt
    return xs[0]


def _wtile(u):
    return pltpu.bitcast(u.reshape(u.shape[0] * 8, 128), bf16)


def _mm(lhs, w, dims=_NN):
    return lax.dot_general(lhs, w, dims, preferred_element_type=f32)


def _cache_view(c):
    _, H, Sk, Dh = c.shape
    c = c.reshape(H, Sk // 128, 128, Dh // 16, 2, 8)
    c = jnp.transpose(c, (0, 3, 4, 1, 5, 2))
    return c.reshape(H * Dh // 16, 2, Sk // 128, 8, 128)


def _weight_view(w):
    R, N = w.shape
    w = w.reshape(R // 16, 2, 8, N // 128, 128)
    return jnp.transpose(w, (0, 1, 3, 2, 4))


def _schedule(NP, KT, DT, AP, AB, SG, xunits, qlead, keep, LAT=205, LAT0=165, LEAD=32, WD=140, WL=400, AD=160,
              vcost=5.95, pstride=2, nraw=8, q2at=40, ph=0, wide=(), wk=(8, 20), cmaj=4, wlast=(), vunits=(), **_):
    xs = {u[:2]: u[2] for u in xunits}
    grp = [(t, a) for t in range(NP) for a in range(0, AP, AB)]
    grp[-2:] = grp[:-3:-1]
    steps = [(t, a, k) for t, a in grp for k in range(xs.get((t, a // 8), 0), KT)]
    first_step = {}
    for i, s in enumerate(steps):
        first_step.setdefault(s[0], i)
    main = [('qraw', t, i) for t in range(nraw) for i in range(3)]
    for t in range(NP):
        qk = [('qk', t, j, k) for j in range(3) for k in range(KT)]
        main += qk[:q2at] + [('q', t + 1, i) for i in range(3) if nraw <= t + 1 < NP] + qk[q2at:]
    done = {('q', t): 3 for t in range(nraw)}
    or_left = [(t, j) for t in range(NP) for j in range(3) if xs.get((t, j), 0) < KT]
    or_left = [u for u in or_left if u not in vunits]
    wo_left = [(t, j) for t in range(NP) for j in range(3) if (t, j) not in vunits]
    px_left = list(xs)
    ev, pend, wait, cur, src = [], [], [], [], {}
    s = dict(tm=0.0, tv=0.0, i=0, mi=0, qk=0)

    def sm(t):
        return ([(('sma', t, k), 3 + 4 * (k == KT - SG), None, 0) for k in range(0, KT, SG)]
                + [(('smb', t, k), 3 + 4 * (k == KT - SG), ('p', t), SG) for k in range(0, KT, SG)])

    def g_wo(n):
        wo = tuple(u for u in wo_left if done.get(('o',) + u, 0) >= 1)[:4]
        if len(wo_left) > cmaj:
            wo = wo[:len(wo_left) - cmaj]
        if len(wo) < n:
            return None
        for u in wo:
            wo_left.remove(u)
        g = [(('wo', wo, n, c), 8, []) for n in range(len(wo)) for c in range(DT)]
        if not wo_left and cmaj:
            g.sort(key=lambda x: x[0][3])
        g[-1] = (g[-1][0], 8, [(('wacc', wo, c), 1, None, 0) for c in range(DT)])
        return g

    def g_or(n, last):
        rd = [u for u in or_left if done.get(('acc',) + u, 0) >= 8 // AB and done.get(('w', min(t for t in wlast if t >= u[0])), 0)
              and (last or done[('acct',) + u] + AD <= s['tv'])
              and done.get(('y',) + u, 0) >= xs.get(u, 0)][:4]
        if len(rd) < n:
            return None
        for u in rd:
            or_left.remove(u)
        return [(('gap',), 8 * len(rd), [])] + [(('or',) + u, 8, [(('ofin',) + u, 1, ('o',) + u, 1)]) for u in rd]

    def g_px():
        rd = [u for u in px_left if done.get(('w', min(t for t in wlast if t >= u[0])), 0)]
        if not rd:
            return None
        px_left.remove(rd[0])
        n = xs[rd[0]]
        g = [(('pvx',) + rd[0] + (k,), 8, []) for k in range(n)]
        g[-1] = (g[-1][0], 8, [(('xsum',) + rd[0], n // 4 + 3, ('o' if n == KT else 'y',) + rd[0], n)])
        return g

    def pick():
        last, endgame, nxt = s['i'] >= len(steps), s['mi'] >= len(main), s['qk']
        if last:
            return g_or(1, True) or g_px() or g_wo(len(wo_left) if 0 < len(wo_left) <= cmaj else 1)
        if endgame:
            return (g_or(min(4, len(or_left)) if vunits and or_left else 4, False) or g_px() or g_wo(4)
                    or (g_wo(1) if len(wo_left) > cmaj else None))
        rem = sum(8 for m in main[s['mi']:s['mi'] + 200] if m[0] != 'qk' or m[1] == nxt)
        if (first_step[nxt] - s['i']) * vcost - rem > qlead * 500:
            g = (g_wo(4) if len(wo_left) > keep else None) or g_or(4, False) or g_px()
            if g:
                return g
        m = main[s['mi']]
        if m[0] == 'qk' and done.get(('q', m[1]), 0) < 3:
            return None
        s['mi'] += 1
        pcs = []
        if m[0] == 'q':
            pcs = [(('qfin',) + m[1:], 5, ('q', m[1]), 1)]
        if m[0] == 'qk' and (m[2] == 2 or m[1:3] == (0, 1)) and m[3] % SG == SG - 1:
            t = m[1] if m[2] == 2 else -1
            pcs = [sm(t)[m[3] // SG]] + (sm(t)[KT // SG:] if m[3] == KT - 1 else [])
        return [(m, 8, pcs)]

    def later(t, pcs):
        wait.append((t, pcs))
        wait.sort(key=lambda w: w[0])

    def piece():
        a, cv, e, inc = pend.pop(0)
        if a[0] == 'wld' and s['i'] < len(steps) and not wk[0] <= steps[s['i']][2] <= wk[1]:
            return later(s['tv'] + 30, [(a, cv, e, inc)])
        ev.append(('piece',) + a)
        s['tv'] += cv / 4
        if e is not None:
            done[e] = done.get(e, 0) + inc
        if a[0] == 'smb' and a[2] == KT - SG and a[1] in wlast:
            later(s['tv'] + WD, [(('wld', a[1]), 0, ('wld', a[1]), 1)])
        if a[0] == 'wld':
            later(s['tv'] + WL, [(('w', a[1]), 26, ('w', a[1]), 1)])

    def urgent(p):
        return p[2] is not None and p[2][0] != 'p'

    while True:
        while wait and wait[0][0] <= s['tv']:
            pcs = wait.pop(0)[1]
            pend[:] = [p for p in pcs if urgent(p)] + pend + [p for p in pcs if not urgent(p)]
        i = s['i']
        more = i < len(steps)
        blocked = not more or done.get(('p', steps[i][0] - (i < AP // 2 // AB * KT)), 0) < min(KT, steps[i][2] + 6)
        if not more and or_left:
            cur = (g_or(1, True) or []) + cur
        if not cur and (s['tm'] + LEAD <= s['tv'] or blocked):
            cur = pick() or []
        if not more and not pend and not wait and not cur:
            break
        if cur and (s['tm'] + LEAD <= s['tv']
                    or (blocked and not pend and (not wait or s['tm'] + LEAD <= wait[0][0]))):
            a, cm, pcs = cur.pop(0)
            ev.append(('tile',) + a)
            s['tm'] = max(s['tm'], s['tv'] - LEAD - 8) + cm
            s['tv'] += 0.25 * (a[0] == 'pvx')
            s['qk'] += a[0] == 'qk' and a[2:] == (2, KT - 1)
            src.update({('piece',) + pc[0]: ev[-1] for pc in pcs})
            if pcs:
                later(s['tm'] + (LAT if 0 < i < len(steps) else LAT0), pcs)
        elif blocked and pend:
            piece()
        elif blocked:
            s['tv'] = max(s['tv'], wait[0][0])
        else:
            if pend and (i % pstride == 0 or urgent(pend[0])):
                piece()
            t, a, k = steps[i]
            ev.append(('step', t, a, k))
            if k == KT - 1:
                done['acc', t, a // 8] = done.get(('acc', t, a // 8), 0) + 1
                done['acct', t, a // 8] = s['tv']
            s['tv'] += vcost - 0.5 * sum((t, b) in wide for b in range(a, a + AB))
            s['i'] += 1
    assert not or_left and not wo_left and not px_left

    out, cur, cnt = [], [], 0
    for e in ev + [None]:
        if e is None or (e[0] == 'tile' and e[1] != 'gap' and cnt % 4 == ph):
            if any(x[0] == 'step' for x in cur) and len(cur) < 32 and not any(src.get(x) in cur for x in cur):
                cur = cur[:1] + [x for x in cur[1:] if x[0] == 'piece'] + [x for x in cur[1:] if x[0] != 'piece']
            out += cur
            cur = []
        if e is not None:
            cur.append(e)
            cnt += (4 if e[1] == 'gap' else 1) * (e[0] == 'tile')
    pos = {e: n for n, e in enumerate(out)}
    assert all(pos[a] < pos[b] for b, a in src.items())
    return out


def _slots(events, key):
    first, last = {}, {}
    for n, e in enumerate(events):
        k = key(e)
        if k is not None:
            first.setdefault(k, n)
            last[k] = n
    slot, busy = {}, []
    for k in first:
        free = [i for i, u in enumerate(busy) if u < first[k]]
        slot[k] = free[0] if free else len(busy)
        busy[slot[k]:slot[k] + 1] = [last[k]]
    return slot, len(busy)


def _run(opts, A_x, A_k_cache, A_v_cache, A_wq, A_wo, B_w3, B_w4):
    B, S, D = A_x.shape
    _, H, Sk, Dh = A_k_cache.shape
    F = B_w3.shape[1]
    W = min(4096, max(256, Sk // 4))
    assert (B, S, H, Dh, W) == (1, 1, 32, 192, 4096) and D % 128 == 0 and F % 128 == 0
    AP = Dh // 8
    KT = W // 128
    NP = H // 2
    DT, FT = D // 128, F // 128
    AB, SG, FD = 4, 4, opts.get('fd', 5)
    KP = KT // SG
    SKEW = opts.get('skew', 1)
    cexp = (Dh ** -0.5) * _LOG2E
    nx = {u[:2]: u[2] for u in opts['xunits']}
    xunits, vunits = list(nx), opts.get('vunits', [])
    wide = [(t, a) for t in range(NP) for a in range(0, AP, AB) if (t, a // 8) not in xunits + [(NP - 1, 2)]]
    drop = [g for n, g in enumerate(wide) if n % 3][:max(0, len(wide) - opts['nwide'])]
    wide = [g for g in wide if g not in drop] + [(t, a + 2) for t, a in wide[::-1]][:max(0, opts['nwide'] - len(wide))]
    late = [(t, a) for b in (0, 2) for t in range(NP - 1, 0, -1) for a in range(b, AP, AB)
            if (t, a // 8) not in xunits + [(NP - 1, 2)] and (t, a) not in wide]
    nlate = opts['nlate']
    late = {g: (c, n) for c in range(DT - 1) for n, g in enumerate(late[sum(nlate[:c]):sum(nlate[:c + 1])])}
    events = _schedule(NP, KT, DT, AP, AB, SG, wide=wide + list(late), **opts)
    sp, RP = _slots(events, lambda e: e[1] - (e[1] == 0 and e[2] < AP // 2) if e[0] == 'step'
                    else e[2] if e[1] in ('sma', 'smb', 'pvx') else None)
    ss, RS = _slots(events, lambda e: max(e[2], 0) if e[1] in ('qk', 'sma') else None)
    sq, RQ = _slots(events, lambda e: e[2] if e[1] in ('q', 'qfin') else None)
    sx, RX = _slots(events, lambda e: e[2:4] if e[1] in ('pvx', 'xsum') else None)
    sw, RM = _slots(events, lambda e: e[2] if e[1] in ('wo', 'wacc') else None)
    so, RO = _slots(events, lambda e: e[2:4] if e[1] in ('or', 'ofin') else None)
    wlast = opts['wlast']
    wgrp = {t: [u for u in range(NP) if max([-1] + [v for v in wlast if v < t]) < u <= min(v for v in wlast if v >= t)]
            for t in range(NP)}
    sl, RL = _slots(events, lambda e: wgrp[e[2]][-1] if e[1] in ('smb', 'wld') and e[2] >= 0 else None)
    assert _slots(events, lambda e: e[2] if e[1] in ('sma', 'smb') else None)[1] == 1
    sizes = [3 * NP, 3 * NP, 2 * NP, 2, DT, 2 * NP + 3, KT, KT * len(wide)]
    QP, Q0, WB, XL, XA, MB, AL, WD, NBIG = [sum(sizes[:n]) for n in range(len(sizes) + 1)]
    OB = Q0
    free, acc_at = [AL, AL + 16], {}
    for e in events:
        if e[0] == 'step' and (e[1], e[2] // 8) not in acc_at:
            acc_at[e[1], e[2] // 8] = free.pop(0)
        if e[0] == 'step' and e[3] == KT - 1:
            free += [WD + KT * wide.index((e[1], a)) + n for a in range(e[2], e[2] + AB) if (e[1], a) in wide
                     for n in (0, 16)]
    sizes = [RP * KP, 3 * RS * KP, RX * KP, 3 * RQ, DT * (RM + 4), 2 * RO, 2 * RL, 2]
    _, SP, XP, QR, WR, OR, ML, WL, NPB = [sum(sizes[:n]) for n in range(len(sizes) + 1)]
    NV, NQ = opts.get('nv', 6), opts.get('nq', 8)
    assert nlate[DT - 2] == 0 and 2 * nlate[DT - 3] <= 11 + (3 * NP - NQ) // 4
    if opts.get('verbose'):
        print('RP RS RQ RX RM', RP, RS, RQ, RX, RM, 'free tiles', (int(13.25 * 256) - NBIG - NPB))
    order1 = sorted(range(NP), key=lambda t: all(u[0] != t for u in xunits))

    def kernel(x_hbm, k_hbm, v_hbm, wq_hbm, wo_hbm, w3_hbm, w4_hbm, o_ref, *scratch):
        k_bufs, v_bufs, scratch = scratch[:NP], scratch[NP:2 * NP], scratch[2 * NP:]
        w4_bufs, wq_bufs, scratch = scratch[:DT], scratch[DT:2 * DT], scratch[2 * DT:]
        wo_buf, w3_buf, pbuf, cst, big, hbuf, xres, x_buf, sems = scratch
        t0 = (Sk - W) // 128

        def kv_cp(kind, t):
            src, dst = (k_hbm, k_bufs[t]) if kind == 0 else (v_hbm, v_bufs[t])
            return [pltpu.make_async_copy(src.at[pl.ds(AP * t, AP), a, pl.ds(t0, KT)],
                                          dst.at[:, :, pl.ds(8 * a, 8), :], sems.at[2 * t + kind])
                    for a in range(2)]

        def w_cp(src, dst, n, sem):
            rows = src.shape[0] // n
            return [pltpu.make_async_copy(src.at[pl.ds(i * rows, rows), a],
                                          dst.at[pl.ds(i * rows, rows), :, pl.ds(8 * a, 8), :], sem)
                    for i in range(n) for a in range(2)]

        def wq_cp():
            cps = [cp for j in range(DT) for cp in w_cp(wq_hbm.at[pl.ds(8 * j, 8)], wq_bufs[j], 1, sems.at[2 * NP])]
            return cps[:1] + [pltpu.make_async_copy(x_hbm, x_buf, sems.at[2 * NP])] + cps[1:]

        def wo_cp():
            return w_cp(wo_hbm, wo_buf, 8, sems.at[2 * NP + 1])

        def w3_cp():
            return [pltpu.make_async_copy(w3_hbm, w3_buf, sems.at[2 * NP + 2])]

        def w4_cp(c):
            return [pltpu.make_async_copy(w4_hbm.at[:, pl.ds(128 * c, 128)], w4_bufs[c], sems.at[2 * NP + 3 + c])]

        def wait(cps):
            for cp in cps:
                cp.wait()

        cps = wq_cp()
        for t in order1:
            cps += kv_cp(0, t) + kv_cp(1, t) + (wo_cp() if t == order1[0] else [])
        for cp in cps + w3_cp() + [cp for c in range(DT) for cp in w4_cp(c)]:
            cp.start()

        ku = [r.bitcast(u32) for r in k_bufs]
        vu = [r.bitcast(u32) for r in v_bufs]
        wqu = [r.bitcast(u32) for r in wq_bufs]
        wou = wo_buf.bitcast(u32)
        w4u = [r.bitcast(u32) for r in w4_bufs]

        def top(n):
            return lax.broadcasted_iota(i32, (8, n), 0) < 4

        def left():
            return lax.broadcasted_iota(i32, (8, 128), 1) < 64

        def cols(n):
            return slice(128 * n, 128 * (n + 1))

        def rows(j):
            return slice(8 * j, 8 * j + 8)

        def masks():
            even = lax.broadcasted_iota(i32, (8, 128), 0) % 2 == 0
            return [even, even == left(), jnp.logical_not(even)]

        def moments(x, c):
            d = x - jnp.concatenate([c] * DT, axis=1)
            md = jnp.mean(d, axis=-1, keepdims=True)
            return d - md, c + md, jnp.mean(d * d, axis=-1, keepdims=True) - md * md

        def mlp_hidden(x, c):
            lhs = jnp.where(top(D), x, 1.0)
            xc, m1, v1 = moments(x, c)
            r1 = lax.rsqrt(v1 + _EPS)
            y = xc * r1
            r2 = lax.rsqrt(v1 * r1 * r1 + _EPS)
            coef = jnp.where(top(128), 1.0, -m1) * (r1 * r2)
            hs, NF = [], opts.get('nf', 4)
            first = {(n, j): _mm(lhs[:, cols(j)], w3_buf[cols(j), cols(n)]) for j in range(DT) for n in range(NF)}
            for n in range(FT):
                u = _tree(jnp.add, [first[n, j] if n < NF else _mm(lhs[:, cols(j)], w3_buf[cols(j), cols(n)])
                                    for j in range(DT)]) * coef
                hs.append(jax.nn.gelu(u + pltpu.roll(u, 4, 0), approximate=True))
            return y, hs

        def w4_tile(n, c):
            return pltpu.bitcast(w4u[c][64 * n:64 * (n + 1)], bf16)

        def late_at(n, k):
            return ((n * KT + k + 2) % (24 * NP)) // (3 * NP), (n * KT + k + 2) % (3 * NP)

        def unpack_late(c, n0, n1, after=None):
            todo = [(g, n, k) for g, (cc, n) in late.items() if cc == c for k in range(KT)][16 * n0:16 * n1]
            if todo and after is not None:
                wqu[c][after[0], 0] = pltpu.bitcast(after[1], u32)
            for (t, a), n, k in todo:
                y = pltpu.bitcast(pltpu.bitcast(vu[t][a, k], bf16).astype(f32), u32)
                wqu[c][late_at(n, k)] = y[8:16]
                vu[t][a, k] = y[0:8]

        def layer1(z):
            for u, mask in enumerate(masks()):
                cst[u] = jnp.where(mask, cexp, 0.0).astype(f32)
            wait(wq_cp())
            x = jnp.broadcast_to(x_buf[...].astype(f32), (8, D))
            _, xc, r = _stats(x)
            xn = xc * r

            def q_body(t, c):
                for i in range(3):
                    q = _tree(jnp.add, [_mm(xn[:, cols(j)], _wtile(wqu[j][:, 3 * t + i])) for j in range(DT)])
                    big[QP + 3 * t + i] = q * cst[i]
                return c
            lax.fori_loop(0, NP, q_body, 0)

            att = [jnp.zeros((8, 128), f32)] * DT
            for t in order1:
                def s_body(k, c, t=t, q=[big[QP + 3 * t + j] for j in range(3)]):
                    big[AL + k] = _tree(jnp.add, [_mm(q[j], _wtile(ku[t][rows(j), k])) for j in range(3)])
                    return c

                def o_body(k, o, t=t):
                    return [o[j] + _mm(big[AL + k], _wtile(vu[t][rows(j), k]), _NT) for j in range(3)]

                wait(kv_cp(0, t))
                lax.fori_loop(0, KT, s_body, 0, unroll=8)
                sc = big[AL:AL + KT]
                p = jnp.exp2(sc - jnp.max(jnp.max(sc, axis=0), axis=1, keepdims=True))
                big[AL:AL + KT] = p
                inv = 1.0 / jnp.sum(jnp.sum(p, axis=0), axis=1, keepdims=True)
                wait(kv_cp(1, t) + (wo_cp() if t == order1[0] else []))
                o = lax.fori_loop(0, KT, o_body, [jnp.zeros((8, 128), f32)] * 3, unroll=8)
                o = [jnp.where(mask, o[j] * inv, 0.0) for j, mask in enumerate(masks())]
                att = [att[c] + _tree(jnp.add, [_mm(o[j], _wtile(wou[rows(3 * t + j), c])) for j in range(3)])
                       for c in range(DT)]
                for j in [j for tt, j in xunits if tt == t]:
                    def t_body(k, c, t=t, j=j):
                        w = _wtile(vu[t][rows(j), k]).astype(f32).T.astype(bf16)
                        vu[t][rows(j), k] = pltpu.bitcast(w, u32).reshape(8, 8, 128)
                        return c
                    lax.fori_loop(0, nx[t, j], t_body, 0, unroll=4)
                for n, a in [(n, a) for n, (tt, a) in enumerate(wide) if tt == t]:
                    y = _wtile(vu[t][a]).astype(f32).reshape(KT, 16, 128)
                    big[WD + n * KT:WD + (n + 1) * KT] = y[:, 8:16]
                    vu[t][a] = pltpu.bitcast(y[:, 0:8], u32)
            att = jnp.concatenate(att, axis=1)
            x = x + (att + pltpu.roll(att, 1, 0))
            wait(w3_cp())
            y, hs = mlp_hidden(x, jnp.broadcast_to(jnp.mean(x, axis=-1, keepdims=True), (8, 128)))
            xres[...] = x + y
            for n in range(FT):
                hbuf[n] = hs[n]
            for c in range(DT - 1):
                wait(w4_cp(c))
                unpack_late(c - 1, 0, 7)
                xc = xres[:, cols(c)] + _tree(jnp.add, [_mm(hbuf[n], w4_tile(n, c)) for n in range(FT)])
                xres[:, cols(c)] = xc
                if c == DT - 2:
                    cst[3] = jnp.broadcast_to(jnp.mean(xres[:, :D - 128], axis=-1, keepdims=True), (8, 128))
                xc = jnp.where(top(128), xc, 1.0)
                unpack_late(c - 1, 7, 11, (z, xc))
                for n in range(3 * NP - (NQ if c == DT - 2 else 0)):
                    r = _mm(xc, _wtile(wqu[c][:, n]))
                    big[Q0 + n] = big[Q0 + n] + r if c else r
                    if n % 4 == 0:
                        unpack_late(c - 1, 11 + n // 4, 12 + n // 4, (z, r))

        def layer2(z):
            wait(w4_cp(DT - 1))
            if opts.get('skip2'):
                keep = big[Q0 + z] + sum(pltpu.bitcast(r[z, 1], f32) for r in wqu + vu)
                o_ref[...] = (xres[0:1, :] + jnp.concatenate([keep[0:1]] * DT, axis=1)).astype(o_ref.dtype)
                return
            xc = xres[:, cols(DT - 1)] + _tree(jnp.add, [_mm(hbuf[n], w4_tile(n, DT - 1)) for n in range(FT)])
            for n in range(3 * NP - NQ, 3 * NP):
                xp = jnp.where(top(128), xres[:, cols(DT - 2)], 1.0)
                big[Q0 + n] = big[Q0 + n] + _mm(xp, _wtile(wqu[DT - 2][:, n]))
            xres[:, cols(DT - 1)] = xc
            _, m, v = moments(xres[...], cst[3])
            big[XL] = xraw = jnp.where(top(128), xc, 1.0)
            big[XL + 1] = coef = jnp.where(top(128), 1.0, -m) * lax.rsqrt(v + _EPS)
            acc, val, fwd = {}, {}, []
            st = dict(pin=False, dirty=False, cnt=0, started=False, left=sum(e[0] == 'step' for e in events))

            def lhs(n):
                if st['pin']:
                    st['pin'] = False
                    return big[n + z]
                if n not in val:
                    val[n] = big[n]
                return val[n]

            def checkpoint():
                for (t, a), y in acc.items():
                    n = acc_at[t, a // 8] + 2 * (a % 8)
                    big[n:n + 2] = y.reshape(2, 8, 128)

            def two(n):
                return slice(2 * n, 2 * n + 2)

            def put(n, r, rs=slice(0, 8)):
                fwd.append((st['cnt'], n, r, rs))

            def flush(upto, pin=False):
                while fwd and fwd[0][0] <= upto:
                    _, n, r, rs = fwd.pop(0)
                    pbuf[z if pin else 0, rs, cols(n)] = r[rs]
                    pin = False

            def get(n, rs=slice(0, 8)):
                flush(max([f[0] for f in fwd if f[1] == n], default=-1))
                return pbuf[0, rs, cols(n)]

            def ptile(t, k):
                return cols(sp[t] * KP + k // SG)

            def prow(t, odd, k):
                r = 2 * (k % SG) + odd
                return pbuf[0, r:r + 1, ptile(t - (t + odd == 0), k)]

            def q_fin(t, i, y, coef):
                y = (y + big[Q0 + 3 * t + i]) * coef
                big[QP + 3 * t + i] = (y + pltpu.roll(y, 4, 0)) * cst[i]

            def t_qraw(t, i):
                q_fin(t, i, _mm(xraw, _wtile(wqu[DT - 1][:, 3 * t + i])), coef)

            def t_q(t, i):
                put(QR + sq[t] * 3 + i, _mm(lhs(XL), _wtile(wqu[DT - 1][:, 3 * t + i])))

            def t_qk(t, j, k):
                put(SP + (3 * ss[t] + j) * KP + k // SG, _mm(lhs(QP + 3 * t + j), _wtile(ku[t][rows(j), k])),
                    two(k % SG))

            def t_or(t, j):
                a = big[acc_at[t, j]:acc_at[t, j] + 16].reshape(128, 128)
                if j == 1:
                    r = _mm(jnp.concatenate([lhs(WB + 2 * t), lhs(WB + 2 * t + 1)], axis=0), a, _NT)
                    put(OR + 2 * so[t, j] + 1, r[8:16])
                else:
                    r = _mm(lhs(WB + 2 * t + j // 2), a, _NT)
                put(OR + 2 * so[t, j], r[0:8])

            def t_pvx(t, j, k):
                p = val.pop(('px', t, j, k)) * lhs(WB + 2 * t + j // 2)
                put(XP + sx[t, j] * KP + k // 4, _mm(p, _wtile(vu[t][rows(j), k])), two(k % 4))

            def t_wo(units, n, c):
                t, j = units[n]
                r = _mm(lhs(OB + 3 * t + j), _wtile(wou[rows(3 * t + j), c]))
                if units == list(sw)[-1]:
                    put(WR + (RM + n) * DT + c, r)
                else:
                    put(WR + sw[units] * DT + c, r, two(n))

            def p_qfin(t, i):
                q_fin(t, i, get(QR + sq[t] * 3 + i), big[XL + 1])

            def over_tiles(op, y):
                y = op(y, pltpu.roll(y, 2, 0))
                return op(y, pltpu.roll(y, 4, 0))

            def p_sma(t, k0):
                n = SP + 3 * ss[max(t, 0)] * KP + k0 // SG
                sc = get(n) + get(n + KP)
                sc = sc + get(n + 2 * KP) if t >= 0 else sc
                pbuf[0, :, ptile(t, k0)] = sc
                m = jnp.maximum(sc, val['m']) if k0 else sc
                big[MB + 2 + 2 * t] = val['m'] = over_tiles(jnp.maximum, m) if k0 + SG == KT else m

            def p_smb(t, k0):
                pbuf[0, :, ptile(t, k0)] = p = jnp.exp2(pbuf[0, :, ptile(t, k0)] - val['m'])
                if t >= 0:
                    big[MB + 3 + 2 * t] = val['l'] = p + val['l'] if k0 else p
                if t >= 0 and k0 + SG == KT:
                    n, rs = ML + 2 * sl[wgrp[t][-1]], two(wgrp[t].index(t))
                    pbuf[0, rs, cols(n)] = val['m'][rs]
                    pbuf[0, rs, cols(n + 1)] = over_tiles(jnp.add, val['l'])[rs]

            def p_wld(t):
                val['ml', t] = [pbuf[0, 0:2 * len(wgrp[t]), cols(ML + 2 * sl[t] + n)] for n in range(2)]

            def p_w(t):
                m, l = val['ml', t]
                e = jnp.exp2(m - jnp.max(m, axis=1, keepdims=True))
                w = e / jnp.sum(e * l, axis=1, keepdims=True)
                for h in range(2 * len(wgrp[t])):
                    big[WB + 2 * wgrp[t][0] + h] = jnp.broadcast_to(w[h:h + 1], (8, 128))
                if t == NP - 1:
                    pbuf[0, 0:2 * len(wgrp[t]), cols(WL)] = w
                    st['wl'] = True

            def p_ofin(t, j):
                r = get(OR + 2 * so[t, j])
                r = jnp.where(left(), r, get(OR + 2 * so[t, j] + 1)) if j == 1 else r
                big[OB + 3 * t + j] = r + big[OB + 3 * t + j] if (t, j) in nx else r

            def p_xsum(t, j):
                ys = [get(XP + sx[t, j] * KP + u) for u in range(nx[t, j] // 4)]
                big[OB + 3 * t + j] = over_tiles(jnp.add, _tree(jnp.add, ys))

            def p_wacc(units, c):
                if units == list(sw)[-1]:
                    rs = [get(WR + (RM + n) * DT + c) for n in range(len(units))]
                    big[XA + c] = _tree(jnp.add, rs + [over_tiles(jnp.add, big[XA + c])])
                elif units == list(sw)[0]:
                    assert len(units) == 4
                    big[XA + c] = get(WR + sw[units] * DT + c)
                else:
                    rs = slice(0, 2 * len(units))
                    big[XA + c, rs] = big[XA + c, rs] + get(WR + sw[units] * DT + c, rs)

            fns = {'qraw': t_qraw, 'q': t_q, 'qk': t_qk, 'or': t_or, 'pvx': t_pvx, 'wo': t_wo, 'qfin': p_qfin,
                   'sma': p_sma, 'smb': p_smb, 'wld': p_wld, 'w': p_w, 'ofin': p_ofin, 'xsum': p_xsum, 'wacc': p_wacc}
            tiles = [e for e in events if e[0] == 'tile' and e[1] != 'gap']
            for e in events:
                if e[0] == 'step':
                    _, t, a0, k = e
                    k0 = nx.get((t, a0 // 8), 0)
                    for a in range(a0, a0 + AB):
                        n = k + SKEW * (a - a0)
                        kk = k0 + (n - k0) % (KT - k0)
                        if ('p', t, a0, n) not in val:
                            val['p', t, a0, n] = prow(t, int(a0 >= AP // 2), kk)
                        if (t, a) in wide:
                            y = jnp.concatenate([pltpu.bitcast(vu[t][a, kk], f32),
                                                 big[WD + wide.index((t, a)) * KT + kk]])
                        elif (t, a) in late:
                            c, u = late[t, a]
                            y = pltpu.bitcast(jnp.concatenate([vu[t][a, kk], wqu[c][late_at(u, kk)]]), f32)
                        else:
                            y = pltpu.bitcast(vu[t][a, kk], bf16).astype(f32)
                        y = y * val['p', t, a0, n]
                        acc[t, a] = acc[t, a] + y if (t, a) in acc else y
                    st.update(dirty=True, started=True, left=st['left'] - 1)
                    if st['left'] == opts.get('vlead', 24) and vunits:
                        assert st['wl']
                        val['wl'] = [pbuf[0, h:h + 1, cols(WL)] for h in range(2 * len(wgrp[NP - 1]))]
                    if k == KT - 1:
                        checkpoint()
                        acc.clear()
                elif e[0] == 'piece':
                    fns[e[1]](*e[2:])
                elif e[1] == 'gap':
                    st['cnt'] += 4
                else:
                    pinned = st['cnt'] % 4 == opts.get('ph', 0) and st['left'] > 0
                    if pinned and st['dirty']:
                        checkpoint()
                    st.update(pin=pinned and st['started'], dirty=st['dirty'] and not pinned)
                    fns[e[1]](*e[2:])
                    st['pin'] = False
                    tiles.pop(0)
                    for u in tiles[:opts.get('pf', 4)]:
                        if u[1] == 'pvx' and ('px',) + u[2:] not in val:
                            val[('px',) + u[2:]] = prow(u[2], u[3] // 2, u[4])
                    if pinned:
                        flush(st['cnt'] - 4 * FD + 3, pin=st['started'])
                    st['cnt'] += 1
            assert not fwd
            att = [big[XA + c] for c in range(DT)]
            part = [None] * DT
            for t, a0 in [e[1:3] for e in events if e[0] == 'step' and e[3] == KT - 1 and (e[1], e[2] // 8) in vunits]:
                for a in range(a0, a0 + AB):
                    n = acc_at[t, a // 8] + 2 * (a % 8)
                    o = jnp.sum(big[n:n + 2].reshape(16, 128) * val['wl'][2 * wgrp[NP - 1].index(t) + (a >= AP // 2)],
                                axis=1, keepdims=True)
                    for c in range(DT):
                        u = pltpu.bitcast(wou[AP * t + a, c], bf16).astype(f32) * o
                        part[c] = u if part[c] is None else part[c] + u
            if vunits:
                att = [att[c] + jnp.sum(part[c], axis=0, keepdims=True) for c in range(DT)]
            x = xres[...] + jnp.concatenate(att, axis=1)
            y, hs = mlp_hidden(x, cst[3])
            out = [(x + y)[:, cols(c)] for c in range(DT)]
            part = [None] * DT
            hb = [jnp.concatenate([hs[n]] * 16, axis=0).T for n in range(NV)]
            for n0 in range(0, NV, 3):
                for a in range(8):
                    for n in range(n0, min(n0 + 3, NV)):
                        for c in range(DT):
                            u = pltpu.bitcast(w4u[c][rows(8 * n + a)], bf16).astype(f32) * hb[n][16 * a:16 * a + 16]
                            part[c] = u if part[c] is None else part[c] + u
            for n in range(NV, FT):
                out = [out[c] + _mm(hs[n], w4_tile(n, c)) for c in range(DT)]
            out = [out[c] + jnp.sum(part[c], axis=0, keepdims=True) for c in range(DT)]
            o_ref[...] = jnp.concatenate(out, axis=1)[0:1].astype(o_ref.dtype)

        def body(it, carry):
            pl.when(it == 0)(lambda: layer1(it >> 4) if not opts.get('skip1') else None)
            pl.when(it == 1)(lambda: layer2(it >> 4))
            return carry

        lax.fori_loop(0, 2, body, 0)

    def V(*s, dt=f32):
        return pltpu.VMEM(s, dt)

    out = pl.pallas_call(
        kernel,
        out_shape=jax.ShapeDtypeStruct((1, D), A_x.dtype),
        in_specs=[pl.BlockSpec(memory_space=pl.ANY)] * 7,
        out_specs=pl.BlockSpec(memory_space=pltpu.VMEM),
        scratch_shapes=(
            [V(AP, KT, 16, 128, dt=bf16)] * (2 * NP)
            + [V(F, 128, dt=bf16)] * DT + [V(8, 3 * NP, 16, 128, dt=bf16)] * DT
            + [V(AP * NP, DT, 16, 128, dt=bf16), V(D, F, dt=bf16),
               V(1, 8, -(-NPB // 4) * 512), V(4, 8, 128), V(-(-NBIG // 4) * 4, 8, 128),
               V(FT, 8, 128), V(8, D), V(1, D, dt=bf16),
               pltpu.SemaphoreType.DMA((2 * NP + 3 + DT,))]),
        compiler_params=pltpu.CompilerParams(
            vmem_limit_bytes=int(opts.get('vmem', 128) * 1024 * 1024),
            disable_semaphore_checks=True, disable_bounds_checks=True),
        name='fused_decode_layers',
    )(A_x.reshape(1, D), _cache_view(A_k_cache), _cache_view(A_v_cache),
      _weight_view(A_wq), _weight_view(A_wo), B_w3, B_w4)
    return out.reshape(B, S, D)


@jax.jit
def pallas_interleave_layers__sliding_block_cached__mixer_s_mlp__decode_kernel(
    A_x: jax.Array,
    A_k_cache: jax.Array,
    A_v_cache: jax.Array,
    A_wq: jax.Array,
    A_wo: jax.Array,
    B_x: jax.Array,
    B_w1: jax.Array,
    B_w2: jax.Array,
    B_w3: jax.Array,
    B_w4: jax.Array,
):
    return _run(_OPTS, A_x, A_k_cache, A_v_cache, A_wq, A_wo, B_w3, B_w4)
```

```python
import jax
import jax.numpy as jnp
from jax import lax
import jax.experimental.pallas as pl
import jax.experimental.pallas.tpu as pltpu

f32, bf16, u32, i32 = jnp.float32, jnp.bfloat16, jnp.uint32, jnp.int32
_EPS = 1e-5
_LOG2E = 1.4426950408889634
_NN = (((1,), (0,)), ((), ()))
_NT = (((1,), (1,)), ((), ()))

_OPTS = dict(
    xunits=[(5, 0, 32), (7, 2, 32), (9, 2, 32), (11, 0, 32), (13, 2, 8)],
    vunits=[(14, 2), (15, 0), (15, 1), (15, 2)], vlead=16,
    nwide=90, nlate=[10, 10, 9, 0],
    wlast=[3, 7, 11, 13, 15], qlead=2.0, keep=8, AD=60, LAT=205, LAT0=165, q2at=20)


def _stats(x):
    m = jnp.mean(x, axis=-1, keepdims=True)
    xc = x - m
    v = jnp.mean(xc * xc, axis=-1, keepdims=True)
    return m, xc, lax.rsqrt(v + _EPS)


def _tree(op, xs):
    xs = list(xs)
    while len(xs) > 1:
        nxt = [op(xs[i], xs[i + 1]) for i in range(0, len(xs) - 1, 2)]
        if len(xs) % 2:
            nxt.append(xs[-1])
        xs = nxt
    return xs[0]


def _wtile(u):
    return pltpu.bitcast(u.reshape(u.shape[0] * 8, 128), bf16)


def _mm(lhs, w, dims=_NN):
    return lax.dot_general(lhs, w, dims, preferred_element_type=f32)


def _cache_view(c):
    _, H, Sk, Dh = c.shape
    c = c.reshape(H, Sk // 128, 128, Dh // 16, 2, 8)
    c = jnp.transpose(c, (0, 3, 4, 1, 5, 2))
    return c.reshape(H * Dh // 16, 2, Sk // 128, 8, 128)


def _weight_view(w):
    R, N = w.shape
    w = w.reshape(R // 16, 2, 8, N // 128, 128)
    return jnp.transpose(w, (0, 1, 3, 2, 4))


def _schedule(NP, KT, DT, AP, AB, SG, xunits, qlead, keep, LAT=205, LAT0=165, LEAD=32, WD=140, WL=400, AD=160,
              vcost=5.95, pstride=2, nraw=8, q2at=40, ph=0, wide=(), wk=(8, 20), cmaj=4, wlast=(), vunits=(), **_):
    xs = {u[:2]: u[2] for u in xunits}
    grp = [(t, a) for t in range(NP) for a in range(0, AP, AB)]
    grp[-2:] = grp[:-3:-1]
    steps = [(t, a, k) for t, a in grp for k in range(xs.get((t, a // 8), 0), KT)]
    first_step = {}
    for i, s in enumerate(steps):
        first_step.setdefault(s[0], i)
    main = [('qraw', t, i) for t in range(nraw) for i in range(3)]
    for t in range(NP):
        qk = [('qk', t, j, k) for j in range(3) for k in range(KT)]
        main += qk[:q2at] + [('q', t + 1, i) for i in range(3) if nraw <= t + 1 < NP] + qk[q2at:]
    done = {('q', t): 3 for t in range(nraw)}
    or_left = [(t, j) for t in range(NP) for j in range(3) if xs.get((t, j), 0) < KT]
    or_left = [u for u in or_left if u not in vunits]
    wo_left = [(t, j) for t in range(NP) for j in range(3) if (t, j) not in vunits]
    px_left = list(xs)
    ev, pend, wait, cur, src = [], [], [], [], {}
    s = dict(tm=0.0, tv=0.0, i=0, mi=0, qk=0)

    def sm(t):
        return ([(('sma', t, k), 3 + 4 * (k == KT - SG), None, 0) for k in range(0, KT, SG)]
                + [(('smb', t, k), 3 + 4 * (k == KT - SG), ('p', t), SG) for k in range(0, KT, SG)])

    def has_w(u):
        return done.get(('w', min(t for t in wlast if t >= u[0])), 0)

    def g_wo(n):
        wo = tuple(u for u in wo_left if done.get(('o',) + u, 0) >= 1)[:4]
        if len(wo_left) > cmaj:
            wo = wo[:len(wo_left) - cmaj]
        if len(wo) < n:
            return None
        for u in wo:
            wo_left.remove(u)
        g = [(('wo', wo, n, c), 8, []) for n in range(len(wo)) for c in range(DT)]
        if not wo_left and cmaj:
            g.sort(key=lambda x: x[0][3])
        g[-1] = (g[-1][0], 8, [(('wacc', wo, c), 1, None, 0) for c in range(DT)])
        return g

    def g_or(n, last):
        rd = [u for u in or_left if done.get(('acc',) + u, 0) >= 8 // AB and has_w(u)
              and (last or done[('acct',) + u] + AD <= s['tv'])
              and done.get(('y',) + u, 0) >= xs.get(u, 0)][:4]
        if len(rd) < n:
            return None
        for u in rd:
            or_left.remove(u)
        return [(('gap',), 8 * len(rd), [])] + [(('or',) + u, 8, [(('ofin',) + u, 1, ('o',) + u, 1)]) for u in rd]

    def g_px():
        rd = [u for u in px_left if has_w(u)]
        if not rd:
            return None
        px_left.remove(rd[0])
        n = xs[rd[0]]
        g = [(('pvx',) + rd[0] + (k,), 8, []) for k in range(n)]
        g[-1] = (g[-1][0], 8, [(('xsum',) + rd[0], n // 4 + 3, ('o' if n == KT else 'y',) + rd[0], n)])
        return g

    def pick():
        last, endgame, nxt = s['i'] >= len(steps), s['mi'] >= len(main), s['qk']
        if last:
            return g_or(1, True) or g_px() or g_wo(len(wo_left) if 0 < len(wo_left) <= cmaj else 1)
        if endgame:
            return (g_or(min(4, len(or_left)) if vunits and or_left else 4, False) or g_px() or g_wo(4)
                    or (g_wo(1) if len(wo_left) > cmaj else None))
        rem = sum(8 for m in main[s['mi']:s['mi'] + 200] if m[0] != 'qk' or m[1] == nxt)
        if (first_step[nxt] - s['i']) * vcost - rem > qlead * 500:
            g = (g_wo(4) if len(wo_left) > keep else None) or g_or(4, False) or g_px()
            if g:
                return g
        m = main[s['mi']]
        if m[0] == 'qk' and done.get(('q', m[1]), 0) < 3:
            return None
        s['mi'] += 1
        pcs = []
        if m[0] == 'q':
            pcs = [(('qfin',) + m[1:], 5, ('q', m[1]), 1)]
        if m[0] == 'qk' and (m[2] == 2 or m[1:3] == (0, 1)) and m[3] % SG == SG - 1:
            t = m[1] if m[2] == 2 else -1
            pcs = [sm(t)[m[3] // SG]] + (sm(t)[KT // SG:] if m[3] == KT - 1 else [])
        return [(m, 8, pcs)]

    def later(t, pcs):
        wait.append((t, pcs))
        wait.sort(key=lambda w: w[0])

    def piece():
        a, cv, e, inc = pend.pop(0)
        if a[0] == 'wld' and s['i'] < len(steps) and not wk[0] <= steps[s['i']][2] <= wk[1]:
            return later(s['tv'] + 30, [(a, cv, e, inc)])
        ev.append(('piece',) + a)
        s['tv'] += cv / 4
        if e is not None:
            done[e] = done.get(e, 0) + inc
        if a[0] == 'smb' and a[2] == KT - SG and a[1] in wlast:
            later(s['tv'] + WD, [(('wld', a[1]), 0, ('wld', a[1]), 1)])
        if a[0] == 'wld':
            later(s['tv'] + WL, [(('w', a[1]), 26, ('w', a[1]), 1)])

    def urgent(p):
        return p[2] is not None and p[2][0] != 'p'

    while True:
        while wait and wait[0][0] <= s['tv']:
            pcs = wait.pop(0)[1]
            pend[:] = [p for p in pcs if urgent(p)] + pend + [p for p in pcs if not urgent(p)]
        i = s['i']
        more = i < len(steps)
        blocked = not more or done.get(('p', steps[i][0] - (i < AP // 2 // AB * KT)), 0) < min(KT, steps[i][2] + 6)
        if not more and or_left:
            cur = (g_or(1, True) or []) + cur
        if not cur and (s['tm'] + LEAD <= s['tv'] or blocked):
            cur = pick() or []
        if not more and not pend and not wait and not cur:
            break
        if cur and (s['tm'] + LEAD <= s['tv']
                    or (blocked and not pend and (not wait or s['tm'] + LEAD <= wait[0][0]))):
            a, cm, pcs = cur.pop(0)
            ev.append(('tile',) + a)
            s['tm'] = max(s['tm'], s['tv'] - LEAD - 8) + cm
            s['tv'] += 0.25 * (a[0] == 'pvx')
            s['qk'] += a[0] == 'qk' and a[2:] == (2, KT - 1)
            src.update({('piece',) + pc[0]: ev[-1] for pc in pcs})
            if pcs:
                later(s['tm'] + (LAT if 0 < i < len(steps) else LAT0), pcs)
        elif blocked and pend:
            piece()
        elif blocked:
            s['tv'] = max(s['tv'], wait[0][0])
        else:
            if pend and (i % pstride == 0 or urgent(pend[0])):
                piece()
            t, a, k = steps[i]
            ev.append(('step', t, a, k))
            if k == KT - 1:
                done['acc', t, a // 8] = done.get(('acc', t, a // 8), 0) + 1
                done['acct', t, a // 8] = s['tv']
            s['tv'] += vcost - 0.5 * sum((t, b) in wide for b in range(a, a + AB))
            s['i'] += 1
    assert not or_left and not wo_left and not px_left

    out, cur, cnt = [], [], 0
    for e in ev + [None]:
        if e is None or (e[0] == 'tile' and e[1] != 'gap' and cnt % 4 == ph):
            if any(x[0] == 'step' for x in cur) and len(cur) < 32 and not any(src.get(x) in cur for x in cur):
                cur = cur[:1] + [x for x in cur[1:] if x[0] == 'piece'] + [x for x in cur[1:] if x[0] != 'piece']
            out += cur
            cur = []
        if e is not None:
            cur.append(e)
            cnt += (4 if e[1] == 'gap' else 1) * (e[0] == 'tile')
    pos = {e: n for n, e in enumerate(out)}
    assert all(pos[a] < pos[b] for b, a in src.items())
    return out


def _slots(events, key):
    first, last = {}, {}
    for n, e in enumerate(events):
        k = key(e)
        if k is not None:
            first.setdefault(k, n)
            last[k] = n
    slot, busy = {}, []
    for k in first:
        free = [i for i, u in enumerate(busy) if u < first[k]]
        slot[k] = free[0] if free else len(busy)
        busy[slot[k]:slot[k] + 1] = [last[k]]
    return slot, len(busy)


def _run(opts, A_x, A_k_cache, A_v_cache, A_wq, A_wo, B_w3, B_w4):
    B, S, D = A_x.shape
    _, H, Sk, Dh = A_k_cache.shape
    F = B_w3.shape[1]
    W = min(4096, max(256, Sk // 4))
    assert (B, S, H, Dh, W) == (1, 1, 32, 192, 4096) and D % 128 == 0 and F % 128 == 0
    AP = Dh // 8
    KT = W // 128
    NP = H // 2
    DT, FT = D // 128, F // 128
    AB, SG, FD = 4, 4, opts.get('fd', 5)
    KP = KT // SG
    SKEW = opts.get('skew', 1)
    cexp = (Dh ** -0.5) * _LOG2E
    nx = {u[:2]: u[2] for u in opts['xunits']}
    xunits, vunits = list(nx), opts.get('vunits', [])
    wide = [(t, a) for t in range(NP) for a in range(0, AP, AB) if (t, a // 8) not in xunits + [(NP - 1, 2)]]
    drop = [g for n, g in enumerate(wide) if n % 3][:max(0, len(wide) - opts['nwide'])]
    wide = [g for g in wide if g not in drop] + [(t, a + 2) for t, a in wide[::-1]][:max(0, opts['nwide'] - len(wide))]
    late = [(t, a) for b in (0, 2) for t in range(NP - 1, 0, -1) for a in range(b, AP, AB)
            if (t, a // 8) not in xunits + [(NP - 1, 2)] and (t, a) not in wide]
    nlate = opts['nlate']
    late = {g: (c, n) for c in range(DT - 1) for n, g in enumerate(late[sum(nlate[:c]):sum(nlate[:c + 1])])}
    events = _schedule(NP, KT, DT, AP, AB, SG, wide=wide + list(late), **opts)
    sp, RP = _slots(events, lambda e: e[1] - (e[1] == 0 and e[2] < AP // 2) if e[0] == 'step'
                    else e[2] if e[1] in ('sma', 'smb', 'pvx') else None)
    ss, RS = _slots(events, lambda e: max(e[2], 0) if e[1] in ('qk', 'sma') else None)
    sq, RQ = _slots(events, lambda e: e[2] if e[1] in ('q', 'qfin') else None)
    sx, RX = _slots(events, lambda e: e[2:4] if e[1] in ('pvx', 'xsum') else None)
    sw, RM = _slots(events, lambda e: e[2] if e[1] in ('wo', 'wacc') else None)
    so, RO = _slots(events, lambda e: e[2:4] if e[1] in ('or', 'ofin') else None)
    wlast = opts['wlast']
    wgrp = {t: [u for u in range(NP) if max([-1] + [v for v in wlast if v < t]) < u <= min(v for v in wlast if v >= t)]
            for t in range(NP)}
    sl, RL = _slots(events, lambda e: wgrp[e[2]][-1] if e[1] in ('smb', 'wld') and e[2] >= 0 else None)
    assert _slots(events, lambda e: e[2] if e[1] in ('sma', 'smb') else None)[1] == 1
    sizes = [3 * NP, 3 * NP, 2 * NP, 2, DT, 2 * NP + 3, KT, KT * len(wide)]
    QP, Q0, WB, XL, XA, MB, AL, WD, NBIG = [sum(sizes[:n]) for n in range(len(sizes) + 1)]
    OB = Q0
    free, acc_at = [AL, AL + 16], {}
    for e in events:
        if e[0] == 'step' and (e[1], e[2] // 8) not in acc_at:
            acc_at[e[1], e[2] // 8] = free.pop(0)
        if e[0] == 'step' and e[3] == KT - 1:
            free += [WD + KT * wide.index((e[1], a)) + n for a in range(e[2], e[2] + AB) if (e[1], a) in wide
                     for n in (0, 16)]
    sizes = [RP * KP, 3 * RS * KP, RX * KP, 3 * RQ, DT * (RM + 4), 2 * RO, 2 * RL, 2]
    _, SP, XP, QR, WR, OR, ML, WL, NPB = [sum(sizes[:n]) for n in range(len(sizes) + 1)]
    NV, NQ = opts.get('nv', 6), opts.get('nq', 8)
    assert nlate[DT - 2] == 0 and 2 * nlate[DT - 3] <= 11 + (3 * NP - NQ) // 4
    if opts.get('verbose'):
        print('RP RS RQ RX RM', RP, RS, RQ, RX, RM, 'free tiles', (int(13.25 * 256) - NBIG - NPB))
    order1 = sorted(range(NP), key=lambda t: all(u[0] != t for u in xunits))

    def kernel(x_hbm, k_hbm, v_hbm, wq_hbm, wo_hbm, w3_hbm, w4_hbm, o_ref, *scratch):
        k_bufs, v_bufs, scratch = scratch[:NP], scratch[NP:2 * NP], scratch[2 * NP:]
        w4_bufs, wq_bufs, scratch = scratch[:DT], scratch[DT:2 * DT], scratch[2 * DT:]
        wo_buf, w3_buf, pbuf, cst, big, hbuf, xres, x_buf, sems = scratch
        t0 = (Sk - W) // 128

        def kv_cp(kind, t):
            src, dst = (k_hbm, k_bufs[t]) if kind == 0 else (v_hbm, v_bufs[t])
            return [pltpu.make_async_copy(src.at[pl.ds(AP * t, AP), a, pl.ds(t0, KT)],
                                          dst.at[:, :, pl.ds(8 * a, 8), :], sems.at[2 * t + kind])
                    for a in range(2)]

        def w_cp(src, dst, n, sem):
            rows = src.shape[0] // n
            return [pltpu.make_async_copy(src.at[pl.ds(i * rows, rows), a],
                                          dst.at[pl.ds(i * rows, rows), :, pl.ds(8 * a, 8), :], sem)
                    for i in range(n) for a in range(2)]

        def wq_cp():
            cps = [cp for j in range(DT) for cp in w_cp(wq_hbm.at[pl.ds(8 * j, 8)], wq_bufs[j], 1, sems.at[2 * NP])]
            return cps[:1] + [pltpu.make_async_copy(x_hbm, x_buf, sems.at[2 * NP])] + cps[1:]

        def wo_cp():
            return w_cp(wo_hbm, wo_buf, 8, sems.at[2 * NP + 1])

        def w3_cp():
            return [pltpu.make_async_copy(w3_hbm, w3_buf, sems.at[2 * NP + 2])]

        def w4_cp(c):
            return [pltpu.make_async_copy(w4_hbm.at[:, pl.ds(128 * c, 128)], w4_bufs[c], sems.at[2 * NP + 3 + c])]

        def wait(cps):
            for cp in cps:
                cp.wait()

        cps = wq_cp()
        for t in order1:
            cps += kv_cp(0, t) + kv_cp(1, t) + (wo_cp() if t == order1[0] else [])
        for cp in cps + w3_cp() + [cp for c in range(DT) for cp in w4_cp(c)]:
            cp.start()

        ku = [r.bitcast(u32) for r in k_bufs]
        vu = [r.bitcast(u32) for r in v_bufs]
        wqu = [r.bitcast(u32) for r in wq_bufs]
        wou = wo_buf.bitcast(u32)
        w4u = [r.bitcast(u32) for r in w4_bufs]

        def top(n):
            return lax.broadcasted_iota(i32, (8, n), 0) < 4

        def left():
            return lax.broadcasted_iota(i32, (8, 128), 1) < 64

        def cols(n):
            return slice(128 * n, 128 * (n + 1))

        def rows(j):
            return slice(8 * j, 8 * j + 8)

        def masks():
            even = lax.broadcasted_iota(i32, (8, 128), 0) % 2 == 0
            return [even, even == left(), jnp.logical_not(even)]

        def moments(x, c):
            d = x - jnp.concatenate([c] * DT, axis=1)
            md = jnp.mean(d, axis=-1, keepdims=True)
            return d - md, c + md, jnp.maximum(jnp.mean(d * d, axis=-1, keepdims=True) - md * md, 0.0)

        def mlp_hidden(x, c):
            lhs = jnp.where(top(D), x, 1.0)
            xc, m1, v1 = moments(x, c)
            r1 = lax.rsqrt(v1 + _EPS)
            y = xc * r1
            r2 = lax.rsqrt(v1 * r1 * r1 + _EPS)
            coef = jnp.where(top(128), 1.0, -m1) * (r1 * r2)
            hs, NF = [], opts.get('nf', 4)
            first = {(n, j): _mm(lhs[:, cols(j)], w3_buf[cols(j), cols(n)]) for j in range(DT) for n in range(NF)}
            for n in range(FT):
                u = _tree(jnp.add, [first[n, j] if n < NF else _mm(lhs[:, cols(j)], w3_buf[cols(j), cols(n)])
                                    for j in range(DT)]) * coef
                hs.append(jax.nn.gelu(u + pltpu.roll(u, 4, 0), approximate=True))
            return y, hs

        def w4_tile(n, c):
            return pltpu.bitcast(w4u[c][64 * n:64 * (n + 1)], bf16)

        def late_at(n, k):
            return ((n * KT + k + 2) % (24 * NP)) // (3 * NP), (n * KT + k + 2) % (3 * NP)

        def unpack_late(c, n0, n1, after=None):
            todo = [(g, n, k) for g, (cc, n) in late.items() if cc == c for k in range(KT)][16 * n0:16 * n1]
            if todo and after is not None:
                wqu[c][after[0], 0] = pltpu.bitcast(after[1], u32)
            for (t, a), n, k in todo:
                y = pltpu.bitcast(pltpu.bitcast(vu[t][a, k], bf16).astype(f32), u32)
                wqu[c][late_at(n, k)] = y[8:16]
                vu[t][a, k] = y[0:8]

        def layer1(z):
            for u, mask in enumerate(masks()):
                cst[u] = jnp.where(mask, cexp, 0.0).astype(f32)
            wait(wq_cp())
            x = jnp.broadcast_to(x_buf[...].astype(f32), (8, D))
            _, xc, r = _stats(x)
            xn = xc * r

            def q_body(t, c):
                for i in range(3):
                    q = _tree(jnp.add, [_mm(xn[:, cols(j)], _wtile(wqu[j][:, 3 * t + i])) for j in range(DT)])
                    big[QP + 3 * t + i] = q * cst[i]
                return c
            lax.fori_loop(0, NP, q_body, 0)

            att = [jnp.zeros((8, 128), f32)] * DT
            for t in order1:
                def s_body(k, c, t=t, q=[big[QP + 3 * t + j] for j in range(3)]):
                    big[AL + k] = _tree(jnp.add, [_mm(q[j], _wtile(ku[t][rows(j), k])) for j in range(3)])
                    return c

                def o_body(k, o, t=t):
                    return [o[j] + _mm(big[AL + k], _wtile(vu[t][rows(j), k]), _NT) for j in range(3)]

                wait(kv_cp(0, t))
                lax.fori_loop(0, KT, s_body, 0, unroll=8)
                sc = big[AL:AL + KT]
                p = jnp.exp2(sc - jnp.max(jnp.max(sc, axis=0), axis=1, keepdims=True))
                big[AL:AL + KT] = p
                inv = 1.0 / jnp.sum(jnp.sum(p, axis=0), axis=1, keepdims=True)
                wait(kv_cp(1, t) + (wo_cp() if t == order1[0] else []))
                o = lax.fori_loop(0, KT, o_body, [jnp.zeros((8, 128), f32)] * 3, unroll=8)
                o = [jnp.where(mask, o[j] * inv, 0.0) for j, mask in enumerate(masks())]
                att = [att[c] + _tree(jnp.add, [_mm(o[j], _wtile(wou[rows(3 * t + j), c])) for j in range(3)])
                       for c in range(DT)]
                for j in [j for tt, j in xunits if tt == t]:
                    def t_body(k, c, t=t, j=j):
                        w = _wtile(vu[t][rows(j), k]).astype(f32).T.astype(bf16)
                        vu[t][rows(j), k] = pltpu.bitcast(w, u32).reshape(8, 8, 128)
                        return c
                    lax.fori_loop(0, nx[t, j], t_body, 0, unroll=4)
                for n, a in [(n, a) for n, (tt, a) in enumerate(wide) if tt == t]:
                    y = _wtile(vu[t][a]).astype(f32).reshape(KT, 16, 128)
                    big[WD + n * KT:WD + (n + 1) * KT] = y[:, 8:16]
                    vu[t][a] = pltpu.bitcast(y[:, 0:8], u32)
            att = jnp.concatenate(att, axis=1)
            x = x + (att + pltpu.roll(att, 1, 0))
            wait(w3_cp())
            y, hs = mlp_hidden(x, jnp.broadcast_to(jnp.mean(x, axis=-1, keepdims=True), (8, 128)))
            xres[...] = x + y
            for n in range(FT):
                hbuf[n] = hs[n]
            for c in range(DT - 1):
                wait(w4_cp(c))
                unpack_late(c - 1, 0, 7)
                xc = xres[:, cols(c)] + _tree(jnp.add, [_mm(hbuf[n], w4_tile(n, c)) for n in range(FT)])
                xres[:, cols(c)] = xc
                if c == DT - 2:
                    cst[3] = jnp.broadcast_to(jnp.mean(xres[:, :D - 128], axis=-1, keepdims=True), (8, 128))
                xc = jnp.where(top(128), xc, 1.0)
                unpack_late(c - 1, 7, 11, (z, xc))
                for n in range(3 * NP - (NQ if c == DT - 2 else 0)):
                    r = _mm(xc, _wtile(wqu[c][:, n]))
                    big[Q0 + n] = big[Q0 + n] + r if c else r
                    if n % 4 == 0:
                        unpack_late(c - 1, 11 + n // 4, 12 + n // 4, (z, r))

        def layer2(z):
            wait(w4_cp(DT - 1))
            xc = xres[:, cols(DT - 1)] + _tree(jnp.add, [_mm(hbuf[n], w4_tile(n, DT - 1)) for n in range(FT)])
            for n in range(3 * NP - NQ, 3 * NP):
                xp = jnp.where(top(128), xres[:, cols(DT - 2)], 1.0)
                big[Q0 + n] = big[Q0 + n] + _mm(xp, _wtile(wqu[DT - 2][:, n]))
            xres[:, cols(DT - 1)] = xc
            _, m, v = moments(xres[...], cst[3])
            big[XL] = xraw = jnp.where(top(128), xc, 1.0)
            big[XL + 1] = coef = jnp.where(top(128), 1.0, -m) * lax.rsqrt(v + _EPS)
            acc, val, fwd = {}, {}, []
            st = dict(pin=False, dirty=False, cnt=0, started=False, left=sum(e[0] == 'step' for e in events))

            def lhs(n):
                if st['pin']:
                    st['pin'] = False
                    return big[n + z]
                if n not in val:
                    val[n] = big[n]
                return val[n]

            def checkpoint():
                for (t, a), y in acc.items():
                    n = acc_at[t, a // 8] + 2 * (a % 8)
                    big[n:n + 2] = y.reshape(2, 8, 128)

            def two(n):
                return slice(2 * n, 2 * n + 2)

            def put(n, r, rs=slice(0, 8)):
                fwd.append((st['cnt'], n, r, rs))

            def flush(upto, pin=False):
                while fwd and fwd[0][0] <= upto:
                    _, n, r, rs = fwd.pop(0)
                    pbuf[z if pin else 0, rs, cols(n)] = r[rs]
                    pin = False

            def get(n, rs=slice(0, 8)):
                flush(max([f[0] for f in fwd if f[1] == n], default=-1))
                return pbuf[0, rs, cols(n)]

            def ptile(t, k):
                return cols(sp[t] * KP + k // SG)

            def prow(t, odd, k):
                r = 2 * (k % SG) + odd
                return pbuf[0, r:r + 1, ptile(t - (t + odd == 0), k)]

            def q_fin(t, i, y, coef):
                y = (y + big[Q0 + 3 * t + i]) * coef
                big[QP + 3 * t + i] = (y + pltpu.roll(y, 4, 0)) * cst[i]

            def t_qraw(t, i):
                q_fin(t, i, _mm(xraw, _wtile(wqu[DT - 1][:, 3 * t + i])), coef)

            def t_q(t, i):
                put(QR + sq[t] * 3 + i, _mm(lhs(XL), _wtile(wqu[DT - 1][:, 3 * t + i])))

            def t_qk(t, j, k):
                put(SP + (3 * ss[t] + j) * KP + k // SG, _mm(lhs(QP + 3 * t + j), _wtile(ku[t][rows(j), k])),
                    two(k % SG))

            def t_or(t, j):
                a = big[acc_at[t, j]:acc_at[t, j] + 16].reshape(128, 128)
                if j == 1:
                    r = _mm(jnp.concatenate([lhs(WB + 2 * t), lhs(WB + 2 * t + 1)], axis=0), a, _NT)
                    put(OR + 2 * so[t, j] + 1, r[8:16])
                else:
                    r = _mm(lhs(WB + 2 * t + j // 2), a, _NT)
                put(OR + 2 * so[t, j], r[0:8])

            def t_pvx(t, j, k):
                p = val.pop(('px', t, j, k)) * lhs(WB + 2 * t + j // 2)
                put(XP + sx[t, j] * KP + k // 4, _mm(p, _wtile(vu[t][rows(j), k])), two(k % 4))

            def t_wo(units, n, c):
                t, j = units[n]
                r = _mm(lhs(OB + 3 * t + j), _wtile(wou[rows(3 * t + j), c]))
                if units == list(sw)[-1]:
                    put(WR + (RM + n) * DT + c, r)
                else:
                    put(WR + sw[units] * DT + c, r, two(n))

            def p_qfin(t, i):
                q_fin(t, i, get(QR + sq[t] * 3 + i), big[XL + 1])

            def over_tiles(op, y):
                y = op(y, pltpu.roll(y, 2, 0))
                return op(y, pltpu.roll(y, 4, 0))

            def p_sma(t, k0):
                n = SP + 3 * ss[max(t, 0)] * KP + k0 // SG
                sc = get(n) + get(n + KP)
                sc = sc + get(n + 2 * KP) if t >= 0 else sc
                pbuf[0, :, ptile(t, k0)] = sc
                m = jnp.maximum(sc, val['m']) if k0 else sc
                big[MB + 2 + 2 * t] = val['m'] = over_tiles(jnp.maximum, m) if k0 + SG == KT else m

            def p_smb(t, k0):
                pbuf[0, :, ptile(t, k0)] = p = jnp.exp2(pbuf[0, :, ptile(t, k0)] - val['m'])
                if t >= 0:
                    big[MB + 3 + 2 * t] = val['l'] = p + val['l'] if k0 else p
                if t >= 0 and k0 + SG == KT:
                    n, rs = ML + 2 * sl[wgrp[t][-1]], two(wgrp[t].index(t))
                    pbuf[0, rs, cols(n)] = val['m'][rs]
                    pbuf[0, rs, cols(n + 1)] = over_tiles(jnp.add, val['l'])[rs]

            def p_wld(t):
                val['ml', t] = [pbuf[0, 0:2 * len(wgrp[t]), cols(ML + 2 * sl[t] + n)] for n in range(2)]

            def p_w(t):
                m, l = val['ml', t]
                e = jnp.exp2(m - jnp.max(m, axis=1, keepdims=True))
                w = e / jnp.sum(e * l, axis=1, keepdims=True)
                for h in range(2 * len(wgrp[t])):
                    big[WB + 2 * wgrp[t][0] + h] = jnp.broadcast_to(w[h:h + 1], (8, 128))
                if t == NP - 1:
                    pbuf[0, 0:2 * len(wgrp[t]), cols(WL)] = w
                    st['wl'] = True

            def p_ofin(t, j):
                r = get(OR + 2 * so[t, j])
                r = jnp.where(left(), r, get(OR + 2 * so[t, j] + 1)) if j == 1 else r
                big[OB + 3 * t + j] = r + big[OB + 3 * t + j] if (t, j) in nx else r

            def p_xsum(t, j):
                ys = [get(XP + sx[t, j] * KP + u) for u in range(nx[t, j] // 4)]
                big[OB + 3 * t + j] = over_tiles(jnp.add, _tree(jnp.add, ys))

            def p_wacc(units, c):
                if units == list(sw)[-1]:
                    rs = [get(WR + (RM + n) * DT + c) for n in range(len(units))]
                    big[XA + c] = _tree(jnp.add, rs + [over_tiles(jnp.add, big[XA + c])])
                elif units == list(sw)[0]:
                    assert len(units) == 4
                    big[XA + c] = get(WR + sw[units] * DT + c)
                else:
                    rs = slice(0, 2 * len(units))
                    big[XA + c, rs] = big[XA + c, rs] + get(WR + sw[units] * DT + c, rs)

            fns = {'qraw': t_qraw, 'q': t_q, 'qk': t_qk, 'or': t_or, 'pvx': t_pvx, 'wo': t_wo, 'qfin': p_qfin,
                   'sma': p_sma, 'smb': p_smb, 'wld': p_wld, 'w': p_w, 'ofin': p_ofin, 'xsum': p_xsum, 'wacc': p_wacc}
            tiles = [e for e in events if e[0] == 'tile' and e[1] != 'gap']
            for e in events:
                if e[0] == 'step':
                    _, t, a0, k = e
                    k0 = nx.get((t, a0 // 8), 0)
                    for a in range(a0, a0 + AB):
                        n = k + SKEW * (a - a0)
                        kk = k0 + (n - k0) % (KT - k0)
                        if ('p', t, a0, n) not in val:
                            val['p', t, a0, n] = prow(t, int(a0 >= AP // 2), kk)
                        if (t, a) in wide:
                            y = jnp.concatenate([pltpu.bitcast(vu[t][a, kk], f32),
                                                 big[WD + wide.index((t, a)) * KT + kk]])
                        elif (t, a) in late:
                            c, u = late[t, a]
                            y = pltpu.bitcast(jnp.concatenate([vu[t][a, kk], wqu[c][late_at(u, kk)]]), f32)
                        else:
                            y = pltpu.bitcast(vu[t][a, kk], bf16).astype(f32)
                        y = y * val['p', t, a0, n]
                        acc[t, a] = acc[t, a] + y if (t, a) in acc else y
                    st.update(dirty=True, started=True, left=st['left'] - 1)
                    if st['left'] == opts.get('vlead', 24) and vunits:
                        assert st['wl']
                        val['wl'] = [pbuf[0, h:h + 1, cols(WL)] for h in range(2 * len(wgrp[NP - 1]))]
                    if k == KT - 1:
                        checkpoint()
                        acc.clear()
                elif e[0] == 'piece':
                    fns[e[1]](*e[2:])
                elif e[1] == 'gap':
                    st['cnt'] += 4
                else:
                    pinned = st['cnt'] % 4 == opts.get('ph', 0) and st['left'] > 0
                    if pinned and st['dirty']:
                        checkpoint()
                    st.update(pin=pinned and st['started'], dirty=st['dirty'] and not pinned)
                    fns[e[1]](*e[2:])
                    st['pin'] = False
                    tiles.pop(0)
                    for u in tiles[:opts.get('pf', 4)]:
                        if u[1] == 'pvx' and ('px',) + u[2:] not in val:
                            val[('px',) + u[2:]] = prow(u[2], u[3] // 2, u[4])
                    if pinned:
                        flush(st['cnt'] - 4 * FD + 3, pin=st['started'])
                    st['cnt'] += 1
            assert not fwd
            att = [big[XA + c] for c in range(DT)]
            part = [None] * DT
            for t, a0 in [e[1:3] for e in events if e[0] == 'step' and e[3] == KT - 1 and (e[1], e[2] // 8) in vunits]:
                for a in range(a0, a0 + AB):
                    n = acc_at[t, a // 8] + 2 * (a % 8)
                    o = jnp.sum(big[n:n + 2].reshape(16, 128) * val['wl'][2 * wgrp[NP - 1].index(t) + (a >= AP // 2)],
                                axis=1, keepdims=True)
                    for c in range(DT):
                        u = pltpu.bitcast(wou[AP * t + a, c], bf16).astype(f32) * o
                        part[c] = u if part[c] is None else part[c] + u
            if vunits:
                att = [att[c] + jnp.sum(part[c], axis=0, keepdims=True) for c in range(DT)]
            x = xres[...] + jnp.concatenate(att, axis=1)
            y, hs = mlp_hidden(x, cst[3])
            out = [(x + y)[:, cols(c)] for c in range(DT)]
            part = [None] * DT
            hb = [jnp.concatenate([hs[n]] * 16, axis=0).T for n in range(NV)]
            for n0 in range(0, NV, 3):
                for a in range(8):
                    for n in range(n0, min(n0 + 3, NV)):
                        for c in range(DT):
                            u = pltpu.bitcast(w4u[c][rows(8 * n + a)], bf16).astype(f32) * hb[n][16 * a:16 * a + 16]
                            part[c] = u if part[c] is None else part[c] + u
            for n in range(NV, FT):
                out = [out[c] + _mm(hs[n], w4_tile(n, c)) for c in range(DT)]
            out = [out[c] + jnp.sum(part[c], axis=0, keepdims=True) for c in range(DT)]
            o_ref[...] = jnp.concatenate(out, axis=1)[0:1].astype(o_ref.dtype)

        def body(it, carry):
            pl.when(it == 0)(lambda: layer1(it >> 4) if not opts.get('skip1') else None)
            pl.when(it == 1)(lambda: layer2(it >> 4))
            return carry

        lax.fori_loop(0, 2, body, 0)

    def V(*s, dt=f32):
        return pltpu.VMEM(s, dt)

    out = pl.pallas_call(
        kernel,
        out_shape=jax.ShapeDtypeStruct((1, D), A_x.dtype),
        in_specs=[pl.BlockSpec(memory_space=pl.ANY)] * 7,
        out_specs=pl.BlockSpec(memory_space=pltpu.VMEM),
        scratch_shapes=(
            [V(AP, KT, 16, 128, dt=bf16)] * (2 * NP)
            + [V(F, 128, dt=bf16)] * DT + [V(8, 3 * NP, 16, 128, dt=bf16)] * DT
            + [V(AP * NP, DT, 16, 128, dt=bf16), V(D, F, dt=bf16),
               V(1, 8, -(-NPB // 4) * 512), V(4, 8, 128), V(-(-NBIG // 4) * 4, 8, 128),
               V(FT, 8, 128), V(8, D), V(1, D, dt=bf16),
               pltpu.SemaphoreType.DMA((2 * NP + 3 + DT,))]),
        compiler_params=pltpu.CompilerParams(
            vmem_limit_bytes=int(opts.get('vmem', 128) * 1024 * 1024),
            disable_semaphore_checks=True, disable_bounds_checks=True),
        name='fused_decode_layers',
    )(A_x.reshape(1, D), _cache_view(A_k_cache), _cache_view(A_v_cache),
      _weight_view(A_wq), _weight_view(A_wo), B_w3, B_w4)
    return out.reshape(B, S, D)


@jax.jit
def pallas_interleave_layers__sliding_block_cached__mixer_s_mlp__decode_kernel(
    A_x: jax.Array,
    A_k_cache: jax.Array,
    A_v_cache: jax.Array,
    A_wq: jax.Array,
    A_wo: jax.Array,
    B_x: jax.Array,
    B_w1: jax.Array,
    B_w2: jax.Array,
    B_w3: jax.Array,
    B_w4: jax.Array,
):
    return _run(_OPTS, A_x, A_k_cache, A_v_cache, A_wq, A_wo, B_w3, B_w4)
```

```python
import jax
import jax.numpy as jnp
from jax import lax
import jax.experimental.pallas as pl
import jax.experimental.pallas.tpu as pltpu

f32, bf16, u32, i32 = jnp.float32, jnp.bfloat16, jnp.uint32, jnp.int32
_EPS = 1e-5
_LOG2E = 1.4426950408889634
_NN = (((1,), (0,)), ((), ()))
_NT = (((1,), (1,)), ((), ()))

_OPTS = dict(
    xunits=[(5, 0, 32), (7, 2, 32), (9, 2, 32), (11, 0, 32), (13, 2, 8)],
    vunits=[(14, 2), (15, 0), (15, 1), (15, 2)], vlead=16,
    nwide=90, nlate=[10, 10, 9, 0],
    wlast=[3, 7, 11, 13, 15], qlead=2.0, keep=8, AD=60, LAT=205, LAT0=165, q2at=20)


def _stats(x):
    m = jnp.mean(x, axis=-1, keepdims=True)
    xc = x - m
    v = jnp.mean(xc * xc, axis=-1, keepdims=True)
    return m, xc, lax.rsqrt(v + _EPS)


def _tree(op, xs):
    xs = list(xs)
    while len(xs) > 1:
        nxt = [op(xs[i], xs[i + 1]) for i in range(0, len(xs) - 1, 2)]
        if len(xs) % 2:
            nxt.append(xs[-1])
        xs = nxt
    return xs[0]


def _wtile(u):
    return pltpu.bitcast(u.reshape(u.shape[0] * 8, 128), bf16)


def _mm(lhs, w, dims=_NN):
    return lax.dot_general(lhs, w, dims, preferred_element_type=f32)


def _cache_view(c):
    _, H, Sk, Dh = c.shape
    c = c.reshape(H, Sk // 128, 128, Dh // 16, 2, 8)
    c = jnp.transpose(c, (0, 3, 4, 1, 5, 2))
    return c.reshape(H * Dh // 16, 2, Sk // 128, 8, 128)


def _weight_view(w):
    R, N = w.shape
    w = w.reshape(R // 16, 2, 8, N // 128, 128)
    return jnp.transpose(w, (0, 1, 3, 2, 4))


def _schedule(NP, KT, DT, AP, AB, SG, xunits, qlead, keep, LAT=205, LAT0=165, LEAD=32, WD=140, WL=400, AD=160,
              vcost=5.95, pstride=2, nraw=8, q2at=40, ph=0, wide=(), wk=(8, 20), cmaj=4, wlast=(), vunits=(), **_):
    xs = {u[:2]: u[2] for u in xunits}
    grp = [(t, a) for t in range(NP) for a in range(0, AP, AB)]
    grp[-2:] = grp[:-3:-1]
    steps = [(t, a, k) for t, a in grp for k in range(xs.get((t, a // 8), 0), KT)]
    first_step = {}
    for i, s in enumerate(steps):
        first_step.setdefault(s[0], i)
    main = [('qraw', t, i) for t in range(nraw) for i in range(3)]
    for t in range(NP):
        qk = [('qk', t, j, k) for j in range(3) for k in range(KT)]
        main += qk[:q2at] + [('q', t + 1, i) for i in range(3) if nraw <= t + 1 < NP] + qk[q2at:]
    done = {('q', t): 3 for t in range(nraw)}
    or_left = [(t, j) for t in range(NP) for j in range(3) if xs.get((t, j), 0) < KT]
    or_left = [u for u in or_left if u not in vunits]
    wo_left = [(t, j) for t in range(NP) for j in range(3) if (t, j) not in vunits]
    px_left = list(xs)
    ev, pend, wait, cur, src = [], [], [], [], {}
    s = dict(tm=0.0, tv=0.0, i=0, mi=0, qk=0)

    def sm(t):
        return ([(('sma', t, k), 3 + 4 * (k == KT - SG), None, 0) for k in range(0, KT, SG)]
                + [(('smb', t, k), 3 + 4 * (k == KT - SG), ('p', t), SG) for k in range(0, KT, SG)])

    def has_w(u):
        return done.get(('w', min(t for t in wlast if t >= u[0])), 0)

    def g_wo(n):
        wo = tuple(u for u in wo_left if done.get(('o',) + u, 0) >= 1)[:4]
        if len(wo_left) > cmaj:
            wo = wo[:len(wo_left) - cmaj]
        if len(wo) < n:
            return None
        for u in wo:
            wo_left.remove(u)
        g = [(('wo', wo, n, c), 8, []) for n in range(len(wo)) for c in range(DT)]
        if not wo_left and cmaj:
            g.sort(key=lambda x: x[0][3])
        g[-1] = (g[-1][0], 8, [(('wacc', wo, c), 1, None, 0) for c in range(DT)])
        return g

    def g_or(n, last):
        rd = [u for u in or_left if done.get(('acc',) + u, 0) >= 8 // AB and has_w(u)
              and (last or done[('acct',) + u] + AD <= s['tv'])
              and done.get(('y',) + u, 0) >= xs.get(u, 0)][:4]
        if len(rd) < n:
            return None
        for u in rd:
            or_left.remove(u)
        return [(('gap',), 8 * len(rd), [])] + [(('or',) + u, 8, [(('ofin',) + u, 1, ('o',) + u, 1)]) for u in rd]

    def g_px():
        rd = [u for u in px_left if has_w(u)]
        if not rd:
            return None
        px_left.remove(rd[0])
        n = xs[rd[0]]
        g = [(('pvx',) + rd[0] + (k,), 8, []) for k in range(n)]
        g[-1] = (g[-1][0], 8, [(('xsum',) + rd[0], n // 4 + 3, ('o' if n == KT else 'y',) + rd[0], n)])
        return g

    def pick():
        last, endgame, nxt = s['i'] >= len(steps), s['mi'] >= len(main), s['qk']
        if last:
            return g_or(1, True) or g_px() or g_wo(len(wo_left) if 0 < len(wo_left) <= cmaj else 1)
        if endgame:
            return (g_or(min(4, len(or_left)) if vunits and or_left else 4, False) or g_px() or g_wo(4)
                    or (g_wo(1) if len(wo_left) > cmaj else None))
        rem = sum(8 for m in main[s['mi']:s['mi'] + 200] if m[0] != 'qk' or m[1] == nxt)
        if (first_step[nxt] - s['i']) * vcost - rem > qlead * 500:
            g = (g_wo(4) if len(wo_left) > keep else None) or g_or(4, False) or g_px()
            if g:
                return g
        m = main[s['mi']]
        if m[0] == 'qk' and done.get(('q', m[1]), 0) < 3:
            return None
        s['mi'] += 1
        pcs = []
        if m[0] == 'q':
            pcs = [(('qfin',) + m[1:], 5, ('q', m[1]), 1)]
        if m[0] == 'qk' and (m[2] == 2 or m[1:3] == (0, 1)) and m[3] % SG == SG - 1:
            t = m[1] if m[2] == 2 else -1
            pcs = [sm(t)[m[3] // SG]] + (sm(t)[KT // SG:] if m[3] == KT - 1 else [])
        return [(m, 8, pcs)]

    def later(t, pcs):
        wait.append((t, pcs))
        wait.sort(key=lambda w: w[0])

    def piece():
        a, cv, e, inc = pend.pop(0)
        if a[0] == 'wld' and s['i'] < len(steps) and not wk[0] <= steps[s['i']][2] <= wk[1]:
            return later(s['tv'] + 30, [(a, cv, e, inc)])
        ev.append(('piece',) + a)
        s['tv'] += cv / 4
        if e is not None:
            done[e] = done.get(e, 0) + inc
        if a[0] == 'smb' and a[2] == KT - SG and a[1] in wlast:
            later(s['tv'] + WD, [(('wld', a[1]), 0, ('wld', a[1]), 1)])
        if a[0] == 'wld':
            later(s['tv'] + WL, [(('w', a[1]), 26, ('w', a[1]), 1)])

    def urgent(p):
        return p[2] is not None and p[2][0] != 'p'

    while True:
        while wait and wait[0][0] <= s['tv']:
            pcs = wait.pop(0)[1]
            pend[:] = [p for p in pcs if urgent(p)] + pend + [p for p in pcs if not urgent(p)]
        i = s['i']
        more = i < len(steps)
        blocked = not more or done.get(('p', steps[i][0] - (i < AP // 2 // AB * KT)), 0) < min(KT, steps[i][2] + 6)
        if not more and or_left:
            cur = (g_or(1, True) or []) + cur
        if not cur and (s['tm'] + LEAD <= s['tv'] or blocked):
            cur = pick() or []
        if not more and not pend and not wait and not cur:
            break
        if cur and (s['tm'] + LEAD <= s['tv']
                    or (blocked and not pend and (not wait or s['tm'] + LEAD <= wait[0][0]))):
            a, cm, pcs = cur.pop(0)
            ev.append(('tile',) + a)
            s['tm'] = max(s['tm'], s['tv'] - LEAD - 8) + cm
            s['tv'] += 0.25 * (a[0] == 'pvx')
            s['qk'] += a[0] == 'qk' and a[2:] == (2, KT - 1)
            src.update({('piece',) + pc[0]: ev[-1] for pc in pcs})
            if pcs:
                later(s['tm'] + (LAT if 0 < i < len(steps) else LAT0), pcs)
        elif blocked and pend:
            piece()
        elif blocked:
            s['tv'] = max(s['tv'], wait[0][0])
        else:
            if pend and (i % pstride == 0 or urgent(pend[0])):
                piece()
            t, a, k = steps[i]
            ev.append(('step', t, a, k))
            if k == KT - 1:
                done['acc', t, a // 8] = done.get(('acc', t, a // 8), 0) + 1
                done['acct', t, a // 8] = s['tv']
            s['tv'] += vcost - 0.5 * sum((t, b) in wide for b in range(a, a + AB))
            s['i'] += 1
    assert not or_left and not wo_left and not px_left

    out, cur, cnt = [], [], 0
    for e in ev + [None]:
        if e is None or (e[0] == 'tile' and e[1] != 'gap' and cnt % 4 == ph):
            if any(x[0] == 'step' for x in cur) and len(cur) < 32 and not any(src.get(x) in cur for x in cur):
                cur = cur[:1] + [x for x in cur[1:] if x[0] == 'piece'] + [x for x in cur[1:] if x[0] != 'piece']
            out += cur
            cur = []
        if e is not None:
            cur.append(e)
            cnt += (4 if e[1] == 'gap' else 1) * (e[0] == 'tile')
    pos = {e: n for n, e in enumerate(out)}
    assert all(pos[a] < pos[b] for b, a in src.items())
    return out


def _slots(events, key):
    first, last = {}, {}
    for n, e in enumerate(events):
        k = key(e)
        if k is not None:
            first.setdefault(k, n)
            last[k] = n
    slot, busy = {}, []
    for k in first:
        free = [i for i, u in enumerate(busy) if u < first[k]]
        slot[k] = free[0] if free else len(busy)
        busy[slot[k]:slot[k] + 1] = [last[k]]
    return slot, len(busy)


def _run(opts, A_x, A_k_cache, A_v_cache, A_wq, A_wo, B_w3, B_w4):
    B, S, D = A_x.shape
    _, H, Sk, Dh = A_k_cache.shape
    F = B_w3.shape[1]
    W = min(4096, max(256, Sk // 4))
    assert (B, S, H, Dh, W) == (1, 1, 32, 192, 4096) and D % 128 == 0 and F % 128 == 0
    AP = Dh // 8
    KT = W // 128
    NP = H // 2
    DT, FT = D // 128, F // 128
    AB, SG, FD = 4, 4, opts.get('fd', 5)
    KP = KT // SG
    SKEW = opts.get('skew', 1)
    cexp = (Dh ** -0.5) * _LOG2E
    nx = {u[:2]: u[2] for u in opts['xunits']}
    xunits, vunits = list(nx), opts.get('vunits', [])
    wide = [(t, a) for t in range(NP) for a in range(0, AP, AB) if (t, a // 8) not in xunits + [(NP - 1, 2)]]
    drop = [g for n, g in enumerate(wide) if n % 3][:max(0, len(wide) - opts['nwide'])]
    wide = [g for g in wide if g not in drop] + [(t, a + 2) for t, a in wide[::-1]][:max(0, opts['nwide'] - len(wide))]
    late = [(t, a) for b in (0, 2) for t in range(NP - 1, 0, -1) for a in range(b, AP, AB)
            if (t, a // 8) not in xunits + [(NP - 1, 2)] and (t, a) not in wide]
    nlate = opts['nlate']
    late = {g: (c, n) for c in range(DT - 1) for n, g in enumerate(late[sum(nlate[:c]):sum(nlate[:c + 1])])}
    events = _schedule(NP, KT, DT, AP, AB, SG, wide=wide + list(late), **opts)
    sp, RP = _slots(events, lambda e: e[1] - (e[1] == 0 and e[2] < AP // 2) if e[0] == 'step'
                    else e[2] if e[1] in ('sma', 'smb', 'pvx') else None)
    ss, RS = _slots(events, lambda e: max(e[2], 0) if e[1] in ('qk', 'sma') else None)
    sq, RQ = _slots(events, lambda e: e[2] if e[1] in ('q', 'qfin') else None)
    sx, RX = _slots(events, lambda e: e[2:4] if e[1] in ('pvx', 'xsum') else None)
    sw, RM = _slots(events, lambda e: e[2] if e[1] in ('wo', 'wacc') else None)
    so, RO = _slots(events, lambda e: e[2:4] if e[1] in ('or', 'ofin') else None)
    wlast = opts['wlast']
    wgrp = {t: [u for u in range(NP) if max([-1] + [v for v in wlast if v < t]) < u <= min(v for v in wlast if v >= t)]
            for t in range(NP)}
    sl, RL = _slots(events, lambda e: wgrp[e[2]][-1] if e[1] in ('smb', 'wld') and e[2] >= 0 else None)
    assert _slots(events, lambda e: e[2] if e[1] in ('sma', 'smb') else None)[1] == 1
    sizes = [3 * NP, 2, DT, 3, 4 * 16, KT * len(wide)]
    QP, XL, XA, _, AL, WD, NBIG = [sum(sizes[:n]) for n in range(len(sizes) + 1)]
    free, acc_at, at = [AL + 16 * n for n in range(4)], {}, {}
    for e in events:
        if e[0] == 'step' and (e[1], e[2] // 8) not in acc_at:
            acc_at[e[1], e[2] // 8] = free.pop(0)
        if e[1] == 'sma' and e[2] not in at:
            at[e[2]], at[e[2] + 1] = free[0], free.pop(0) + 8
        if e[0] == 'step' and e[3] == KT - 1:
            free += [WD + KT * wide.index((e[1], a)) + n for a in range(e[2], e[2] + AB) if (e[1], a) in wide
                     for n in (0, 16)]
    sizes = [RP * KP, 3 * RS * KP, RX * KP, 3 * RQ, DT * (RM + 4), 2 * RO, 2 * RL, 2]
    _, SP, XP, QR, WR, OR, ML, WL, NPB = [sum(sizes[:n]) for n in range(len(sizes) + 1)]
    NV, NQ = opts.get('nv', 6), opts.get('nq', 8)
    assert nlate[DT - 2] == 0 and 2 * nlate[DT - 3] <= 11 + (3 * NP - NQ) // 4
    if opts.get('verbose'):
        print('RP RS RQ RX RM', RP, RS, RQ, RX, RM, 'free tiles', (int(13.25 * 256) - NBIG - NPB))
    order1 = sorted(range(NP), key=lambda t: all(u[0] != t for u in xunits))

    def kernel(x_hbm, k_hbm, v_hbm, wq_hbm, wo_hbm, w3_hbm, w4_hbm, o_ref, *scratch):
        k_bufs, v_bufs, scratch = scratch[:NP], scratch[NP:2 * NP], scratch[2 * NP:]
        w4_bufs, wq_bufs, scratch = scratch[:DT], scratch[DT:2 * DT], scratch[2 * DT:]
        wo_buf, w3_buf, pbuf, cst, big, hbuf, xres, x_buf, sems = scratch
        t0 = (Sk - W) // 128

        def kv_cp(kind, t):
            src, dst = (k_hbm, k_bufs[t]) if kind == 0 else (v_hbm, v_bufs[t])
            return [pltpu.make_async_copy(src.at[pl.ds(AP * t, AP), a, pl.ds(t0, KT)],
                                          dst.at[:, :, pl.ds(8 * a, 8), :], sems.at[2 * t + kind])
                    for a in range(2)]

        def w_cp(src, dst, n, sem):
            rows = src.shape[0] // n
            return [pltpu.make_async_copy(src.at[pl.ds(i * rows, rows), a],
                                          dst.at[pl.ds(i * rows, rows), :, pl.ds(8 * a, 8), :], sem)
                    for i in range(n) for a in range(2)]

        def wq_cp():
            cps = [cp for j in range(DT) for cp in w_cp(wq_hbm.at[pl.ds(8 * j, 8)], wq_bufs[j], 1, sems.at[2 * NP])]
            return cps[:1] + [pltpu.make_async_copy(x_hbm, x_buf, sems.at[2 * NP])] + cps[1:]

        def wo_cp():
            return w_cp(wo_hbm, wo_buf, 8, sems.at[2 * NP + 1])

        def w3_cp():
            return [pltpu.make_async_copy(w3_hbm, w3_buf, sems.at[2 * NP + 2])]

        def w4_cp(c):
            return [pltpu.make_async_copy(w4_hbm.at[:, pl.ds(128 * c, 128)], w4_bufs[c], sems.at[2 * NP + 3 + c])]

        def wait(cps):
            for cp in cps:
                cp.wait()

        cps = wq_cp()
        for t in order1:
            cps += kv_cp(0, t) + kv_cp(1, t) + (wo_cp() if t == order1[0] else [])
        for cp in cps + w3_cp() + [cp for c in range(DT) for cp in w4_cp(c)]:
            cp.start()

        ku = [r.bitcast(u32) for r in k_bufs]
        vu = [r.bitcast(u32) for r in v_bufs]
        wqu = [r.bitcast(u32) for r in wq_bufs]
        wou = wo_buf.bitcast(u32)
        w4u = [r.bitcast(u32) for r in w4_bufs]

        def top(n):
            return lax.broadcasted_iota(i32, (8, n), 0) < 4

        def left():
            return lax.broadcasted_iota(i32, (8, 128), 1) < 64

        def cols(n):
            return slice(128 * n, 128 * (n + 1))

        def rows(j):
            return slice(8 * j, 8 * j + 8)

        def masks():
            even = lax.broadcasted_iota(i32, (8, 128), 0) % 2 == 0
            return [even, even == left(), jnp.logical_not(even)]

        def moments(x, c):
            d = x - jnp.concatenate([c] * DT, axis=1)
            md = jnp.mean(d, axis=-1, keepdims=True)
            return d - md, c + md, jnp.maximum(jnp.mean(d * d, axis=-1, keepdims=True) - md * md, 0.0)

        def mlp_hidden(x, c):
            lhs = jnp.where(top(D), x, 1.0)
            xc, m1, v1 = moments(x, c)
            r1 = lax.rsqrt(v1 + _EPS)
            y = xc * r1
            r2 = lax.rsqrt(v1 * r1 * r1 + _EPS)
            coef = jnp.where(top(128), 1.0, -m1) * (r1 * r2)
            hs, NF = [], opts.get('nf', 4)
            first = {(n, j): _mm(lhs[:, cols(j)], w3_buf[cols(j), cols(n)]) for j in range(DT) for n in range(NF)}
            for n in range(FT):
                u = _tree(jnp.add, [first[n, j] if n < NF else _mm(lhs[:, cols(j)], w3_buf[cols(j), cols(n)])
                                    for j in range(DT)]) * coef
                hs.append(jax.nn.gelu(u + pltpu.roll(u, 4, 0), approximate=True))
            return y, hs

        def w4_tile(n, c):
            return pltpu.bitcast(w4u[c][64 * n:64 * (n + 1)], bf16)

        def late_at(n, k):
            return ((n * KT + k + 2) % (24 * NP)) // (3 * NP), (n * KT + k + 2) % (3 * NP)

        def unpack_late(c, n0, n1, after=None):
            todo = [(g, n, k) for g, (cc, n) in late.items() if cc == c for k in range(KT)][16 * n0:16 * n1]
            if todo and after is not None:
                wqu[c][after[0], 0] = pltpu.bitcast(after[1], u32)
            for (t, a), n, k in todo:
                y = pltpu.bitcast(pltpu.bitcast(vu[t][a, k], bf16).astype(f32), u32)
                wqu[c][late_at(n, k)] = y[8:16]
                vu[t][a, k] = y[0:8]

        def layer1(z):
            for u, mask in enumerate(masks()):
                cst[u] = jnp.where(mask, cexp, 0.0).astype(f32)
            wait(wq_cp())
            x = jnp.broadcast_to(x_buf[...].astype(f32), (8, D))
            _, xc, r = _stats(x)
            xn = xc * r

            def q_body(t, c):
                for i in range(3):
                    q = _tree(jnp.add, [_mm(xn[:, cols(j)], _wtile(wqu[j][:, 3 * t + i])) for j in range(DT)])
                    big[QP + 3 * t + i] = q * cst[i]
                return c
            lax.fori_loop(0, NP, q_body, 0)

            att = [jnp.zeros((8, 128), f32)] * DT
            for t in order1:
                def s_body(k, c, t=t, q=[big[QP + 3 * t + j] for j in range(3)]):
                    big[AL + k] = _tree(jnp.add, [_mm(q[j], _wtile(ku[t][rows(j), k])) for j in range(3)])
                    return c

                def o_body(k, o, t=t):
                    return [o[j] + _mm(big[AL + k], _wtile(vu[t][rows(j), k]), _NT) for j in range(3)]

                wait(kv_cp(0, t))
                lax.fori_loop(0, KT, s_body, 0, unroll=8)
                sc = big[AL:AL + KT]
                p = jnp.exp2(sc - jnp.max(jnp.max(sc, axis=0), axis=1, keepdims=True))
                big[AL:AL + KT] = p
                inv = 1.0 / jnp.sum(jnp.sum(p, axis=0), axis=1, keepdims=True)
                wait(kv_cp(1, t) + (wo_cp() if t == order1[0] else []))
                o = lax.fori_loop(0, KT, o_body, [jnp.zeros((8, 128), f32)] * 3, unroll=8)
                o = [jnp.where(mask, o[j] * inv, 0.0) for j, mask in enumerate(masks())]
                att = [att[c] + _tree(jnp.add, [_mm(o[j], _wtile(wou[rows(3 * t + j), c])) for j in range(3)])
                       for c in range(DT)]
                for j in [j for tt, j in xunits if tt == t]:
                    def t_body(k, c, t=t, j=j):
                        w = _wtile(vu[t][rows(j), k]).astype(f32).T.astype(bf16)
                        vu[t][rows(j), k] = pltpu.bitcast(w, u32).reshape(8, 8, 128)
                        return c
                    lax.fori_loop(0, nx[t, j], t_body, 0, unroll=4)
                for n, a in [(n, a) for n, (tt, a) in enumerate(wide) if tt == t]:
                    y = _wtile(vu[t][a]).astype(f32).reshape(KT, 16, 128)
                    big[WD + n * KT:WD + (n + 1) * KT] = y[:, 8:16]
                    vu[t][a] = pltpu.bitcast(y[:, 0:8], u32)
            att = jnp.concatenate(att, axis=1)
            x = x + (att + pltpu.roll(att, 1, 0))
            wait(w3_cp())
            y, hs = mlp_hidden(x, jnp.broadcast_to(jnp.mean(x, axis=-1, keepdims=True), (8, 128)))
            xres[...] = x + y
            for n in range(FT):
                hbuf[n] = hs[n]
            for c in range(DT - 1):
                wait(w4_cp(c))
                unpack_late(c - 1, 0, 7)
                xc = xres[:, cols(c)] + _tree(jnp.add, [_mm(hbuf[n], w4_tile(n, c)) for n in range(FT)])
                xres[:, cols(c)] = xc
                if c == DT - 2:
                    cst[3] = jnp.broadcast_to(jnp.mean(xres[:, :D - 128], axis=-1, keepdims=True), (8, 128))
                xc = jnp.where(top(128), xc, 1.0)
                unpack_late(c - 1, 7, 11, (z, xc))
                for n in range(3 * NP - (NQ if c == DT - 2 else 0)):
                    r = _mm(xc, _wtile(wqu[c][:, n]))
                    big[QP + n] = big[QP + n] + r if c else r
                    if n % 4 == 0:
                        unpack_late(c - 1, 11 + n // 4, 12 + n // 4, (z, r))

        def layer2(z):
            wait(w4_cp(DT - 1))
            xc = xres[:, cols(DT - 1)] + _tree(jnp.add, [_mm(hbuf[n], w4_tile(n, DT - 1)) for n in range(FT)])
            for n in range(3 * NP - NQ, 3 * NP):
                xp = jnp.where(top(128), xres[:, cols(DT - 2)], 1.0)
                big[QP + n] = big[QP + n] + _mm(xp, _wtile(wqu[DT - 2][:, n]))
            xres[:, cols(DT - 1)] = xc
            _, m, v = moments(xres[...], cst[3])
            big[XL] = xraw = jnp.where(top(128), xc, 1.0)
            big[XL + 1] = coef = jnp.where(top(128), 1.0, -m) * lax.rsqrt(v + _EPS)
            acc, val, fwd = {}, {}, []
            st = dict(pin=False, dirty=False, cnt=0, started=False, left=sum(e[0] == 'step' for e in events))

            def lhs(n):
                if st['pin']:
                    st['pin'] = False
                    return big[n + z]
                if n not in val:
                    val[n] = big[n]
                return val[n]

            def checkpoint():
                for (t, a), y in acc.items():
                    n = acc_at[t, a // 8] + 2 * (a % 8)
                    big[n:n + 2] = y.reshape(2, 8, 128)

            def two(n):
                return slice(2 * n, 2 * n + 2)

            def put(n, r, rs=slice(0, 8)):
                fwd.append((st['cnt'], n, r, rs))

            def flush(upto, pin=False):
                while fwd and fwd[0][0] <= upto:
                    _, n, r, rs = fwd.pop(0)
                    pbuf[z if pin else 0, rs, cols(n)] = r[rs]
                    pin = False

            def get(n, rs=slice(0, 8)):
                flush(max([f[0] for f in fwd if f[1] == n], default=-1))
                return pbuf[0, rs, cols(n)]

            def ptile(t, k):
                return cols(sp[t] * KP + k // SG)

            def prow(t, odd, k):
                r = 2 * (k % SG) + odd
                return pbuf[0, r:r + 1, ptile(t - (t + odd == 0), k)]

            def q_fin(t, i, y, coef):
                y = (y + big[QP + 3 * t + i]) * coef
                big[QP + 3 * t + i] = (y + pltpu.roll(y, 4, 0)) * cst[i]

            def t_qraw(t, i):
                q_fin(t, i, _mm(xraw, _wtile(wqu[DT - 1][:, 3 * t + i])), coef)

            def t_q(t, i):
                put(QR + sq[t] * 3 + i, _mm(lhs(XL), _wtile(wqu[DT - 1][:, 3 * t + i])))

            def t_qk(t, j, k):
                put(SP + (3 * ss[t] + j) * KP + k // SG, _mm(lhs(QP + 3 * t + j), _wtile(ku[t][rows(j), k])),
                    two(k % SG))

            def t_or(t, j):
                a = big[acc_at[t, j]:acc_at[t, j] + 16].reshape(128, 128)
                if j == 1:
                    r = _mm(jnp.concatenate([lhs(at[t] + 2), lhs(at[t] + 3)], axis=0), a, _NT)
                    put(OR + 2 * so[t, j] + 1, r[8:16])
                else:
                    r = _mm(lhs(at[t] + 2 + j // 2), a, _NT)
                put(OR + 2 * so[t, j], r[0:8])

            def t_pvx(t, j, k):
                p = val.pop(('px', t, j, k)) * lhs(at[t] + 2 + j // 2)
                put(XP + sx[t, j] * KP + k // 4, _mm(p, _wtile(vu[t][rows(j), k])), two(k % 4))

            def t_wo(units, n, c):
                t, j = units[n]
                r = _mm(lhs(at[t] + 4 + j), _wtile(wou[rows(3 * t + j), c]))
                if units == list(sw)[-1]:
                    put(WR + (RM + n) * DT + c, r)
                else:
                    put(WR + sw[units] * DT + c, r, two(n))

            def p_qfin(t, i):
                q_fin(t, i, get(QR + sq[t] * 3 + i), big[XL + 1])

            def over_tiles(op, y):
                y = op(y, pltpu.roll(y, 2, 0))
                return op(y, pltpu.roll(y, 4, 0))

            def p_sma(t, k0):
                n = SP + 3 * ss[max(t, 0)] * KP + k0 // SG
                sc = get(n) + get(n + KP)
                sc = sc + get(n + 2 * KP) if t >= 0 else sc
                pbuf[0, :, ptile(t, k0)] = sc
                m = jnp.maximum(sc, val['m']) if k0 else sc
                big[at[t]] = val['m'] = over_tiles(jnp.maximum, m) if k0 + SG == KT else m

            def p_smb(t, k0):
                pbuf[0, :, ptile(t, k0)] = p = jnp.exp2(pbuf[0, :, ptile(t, k0)] - val['m'])
                if t >= 0:
                    big[at[t] + 1] = val['l'] = p + val['l'] if k0 else p
                if t >= 0 and k0 + SG == KT:
                    n, rs = ML + 2 * sl[wgrp[t][-1]], two(wgrp[t].index(t))
                    pbuf[0, rs, cols(n)] = val['m'][rs]
                    pbuf[0, rs, cols(n + 1)] = over_tiles(jnp.add, val['l'])[rs]

            def p_wld(t):
                val['ml', t] = [pbuf[0, 0:2 * len(wgrp[t]), cols(ML + 2 * sl[t] + n)] for n in range(2)]

            def p_w(t):
                m, l = val['ml', t]
                e = jnp.exp2(m - jnp.max(m, axis=1, keepdims=True))
                w = e / jnp.sum(e * l, axis=1, keepdims=True)
                for h in range(2 * len(wgrp[t])):
                    big[at[wgrp[t][h // 2]] + 2 + h % 2] = jnp.broadcast_to(w[h:h + 1], (8, 128))
                if t == NP - 1:
                    pbuf[0, 0:2 * len(wgrp[t]), cols(WL)] = w
                    st['wl'] = True

            def p_ofin(t, j):
                r = get(OR + 2 * so[t, j])
                r = jnp.where(left(), r, get(OR + 2 * so[t, j] + 1)) if j == 1 else r
                big[at[t] + 4 + j] = r + big[at[t] + 4 + j] if (t, j) in nx else r

            def p_xsum(t, j):
                ys = [get(XP + sx[t, j] * KP + u) for u in range(nx[t, j] // 4)]
                big[at[t] + 4 + j] = over_tiles(jnp.add, _tree(jnp.add, ys))

            def p_wacc(units, c):
                if units == list(sw)[-1]:
                    rs = [get(WR + (RM + n) * DT + c) for n in range(len(units))]
                    big[XA + c] = _tree(jnp.add, rs + [over_tiles(jnp.add, big[XA + c])])
                elif units == list(sw)[0]:
                    assert len(units) == 4
                    big[XA + c] = get(WR + sw[units] * DT + c)
                else:
                    rs = slice(0, 2 * len(units))
                    big[XA + c, rs] = big[XA + c, rs] + get(WR + sw[units] * DT + c, rs)

            fns = {'qraw': t_qraw, 'q': t_q, 'qk': t_qk, 'or': t_or, 'pvx': t_pvx, 'wo': t_wo, 'qfin': p_qfin,
                   'sma': p_sma, 'smb': p_smb, 'wld': p_wld, 'w': p_w, 'ofin': p_ofin, 'xsum': p_xsum, 'wacc': p_wacc}
            tiles = [e for e in events if e[0] == 'tile' and e[1] != 'gap']
            for e in events:
                if e[0] == 'step':
                    _, t, a0, k = e
                    k0 = nx.get((t, a0 // 8), 0)
                    for a in range(a0, a0 + AB):
                        n = k + SKEW * (a - a0)
                        kk = k0 + (n - k0) % (KT - k0)
                        if ('p', t, a0, n) not in val:
                            val['p', t, a0, n] = prow(t, int(a0 >= AP // 2), kk)
                        if (t, a) in wide:
                            y = jnp.concatenate([pltpu.bitcast(vu[t][a, kk], f32),
                                                 big[WD + wide.index((t, a)) * KT + kk]])
                        elif (t, a) in late:
                            c, u = late[t, a]
                            y = pltpu.bitcast(jnp.concatenate([vu[t][a, kk], wqu[c][late_at(u, kk)]]), f32)
                        else:
                            y = pltpu.bitcast(vu[t][a, kk], bf16).astype(f32)
                        y = y * val['p', t, a0, n]
                        acc[t, a] = acc[t, a] + y if (t, a) in acc else y
                    st.update(dirty=True, started=True, left=st['left'] - 1)
                    if st['left'] == opts.get('vlead', 24) and vunits:
                        assert st['wl']
                        val['wl'] = [pbuf[0, h:h + 1, cols(WL)] for h in range(2 * len(wgrp[NP - 1]))]
                    if k == KT - 1:
                        checkpoint()
                        acc.clear()
                elif e[0] == 'piece':
                    fns[e[1]](*e[2:])
                elif e[1] == 'gap':
                    st['cnt'] += 4
                else:
                    pinned = st['cnt'] % 4 == opts.get('ph', 0) and st['left'] > 0
                    if pinned and st['dirty']:
                        checkpoint()
                    st.update(pin=pinned and st['started'], dirty=st['dirty'] and not pinned)
                    fns[e[1]](*e[2:])
                    st['pin'] = False
                    tiles.pop(0)
                    for u in tiles[:opts.get('pf', 4)]:
                        if u[1] == 'pvx' and ('px',) + u[2:] not in val:
                            val[('px',) + u[2:]] = prow(u[2], u[3] // 2, u[4])
                    if pinned:
                        flush(st['cnt'] - 4 * FD + 3, pin=st['started'])
                    st['cnt'] += 1
            assert not fwd
            att = [big[XA + c] for c in range(DT)]
            part = [None] * DT
            for t, a0 in [e[1:3] for e in events if e[0] == 'step' and e[3] == KT - 1 and (e[1], e[2] // 8) in vunits]:
                for a in range(a0, a0 + AB):
                    n = acc_at[t, a // 8] + 2 * (a % 8)
                    o = jnp.sum(big[n:n + 2].reshape(16, 128) * val['wl'][2 * wgrp[NP - 1].index(t) + (a >= AP // 2)],
                                axis=1, keepdims=True)
                    for c in range(DT):
                        u = pltpu.bitcast(wou[AP * t + a, c], bf16).astype(f32) * o
                        part[c] = u if part[c] is None else part[c] + u
            if vunits:
                att = [att[c] + jnp.sum(part[c], axis=0, keepdims=True) for c in range(DT)]
            x = xres[...] + jnp.concatenate(att, axis=1)
            y, hs = mlp_hidden(x, cst[3])
            out = [(x + y)[:, cols(c)] for c in range(DT)]
            part = [None] * DT
            hb = [jnp.concatenate([hs[n]] * 16, axis=0).T for n in range(NV)]
            for n0 in range(0, NV, 3):
                for a in range(8):
                    for n in range(n0, min(n0 + 3, NV)):
                        for c in range(DT):
                            u = pltpu.bitcast(w4u[c][rows(8 * n + a)], bf16).astype(f32) * hb[n][16 * a:16 * a + 16]
                            part[c] = u if part[c] is None else part[c] + u
            for n in range(NV, FT):
                out = [out[c] + _mm(hs[n], w4_tile(n, c)) for c in range(DT)]
            out = [out[c] + jnp.sum(part[c], axis=0, keepdims=True) for c in range(DT)]
            o_ref[...] = jnp.concatenate(out, axis=1)[0:1].astype(o_ref.dtype)

        def body(it, carry):
            pl.when(it == 0)(lambda: layer1(it >> 4) if not opts.get('skip1') else None)
            pl.when(it == 1)(lambda: layer2(it >> 4))
            return carry

        lax.fori_loop(0, 2, body, 0)

    def V(*s, dt=f32):
        return pltpu.VMEM(s, dt)

    out = pl.pallas_call(
        kernel,
        out_shape=jax.ShapeDtypeStruct((1, D), A_x.dtype),
        in_specs=[pl.BlockSpec(memory_space=pl.ANY)] * 7,
        out_specs=pl.BlockSpec(memory_space=pltpu.VMEM),
        scratch_shapes=(
            [V(AP, KT, 16, 128, dt=bf16)] * (2 * NP)
            + [V(F, 128, dt=bf16)] * DT + [V(8, 3 * NP, 16, 128, dt=bf16)] * DT
            + [V(AP * NP, DT, 16, 128, dt=bf16), V(D, F, dt=bf16),
               V(1, 8, -(-NPB // 4) * 512), V(4, 8, 128), V(-(-NBIG // 4) * 4, 8, 128),
               V(FT, 8, 128), V(8, D), V(1, D, dt=bf16),
               pltpu.SemaphoreType.DMA((2 * NP + 3 + DT,))]),
        compiler_params=pltpu.CompilerParams(
            vmem_limit_bytes=int(opts.get('vmem', 128) * 1024 * 1024),
            disable_semaphore_checks=True, disable_bounds_checks=True),
        name='fused_decode_layers',
    )(A_x.reshape(1, D), _cache_view(A_k_cache), _cache_view(A_v_cache),
      _weight_view(A_wq), _weight_view(A_wo), B_w3, B_w4)
    return out.reshape(B, S, D)


@jax.jit
def pallas_interleave_layers__sliding_block_cached__mixer_s_mlp__decode_kernel(
    A_x: jax.Array,
    A_k_cache: jax.Array,
    A_v_cache: jax.Array,
    A_wq: jax.Array,
    A_wo: jax.Array,
    B_x: jax.Array,
    B_w1: jax.Array,
    B_w2: jax.Array,
    B_w3: jax.Array,
    B_w4: jax.Array,
):
    return _run(_OPTS, A_x, A_k_cache, A_v_cache, A_wq, A_wo, B_w3, B_w4)
```
